```python
import jax
import jax.numpy as jnp

def _softmax(x, axis=-1):
    return jax.nn.softmax(x, axis=axis)

def _gelu(x):
    return jax.nn.gelu(x, approximate=True)

def _silu(x):
    return jax.nn.silu(x)

def _sigmoid(x):
    return jax.nn.sigmoid(x)

def _layernorm(x, axis=-1, eps=1e-05):
    m = jnp.mean(x, axis=axis, keepdims=True)
    v = jnp.var(x, axis=axis, keepdims=True)
    return (x - m) / jnp.sqrt(v + eps)

def _scatter_add(tgt, idx, src, axis=0):
    return tgt.at[idx].add(src)

def _segment_sum(src, seg, n):
    return jax.ops.segment_sum(src, seg, n)

class _Rng:

    def __init__(self, key):
        self._k = key

    def _next(self):
        self._k, sub = jax.random.split(self._k)
        return sub

    def normal(self, shape):
        return jax.random.normal(self._next(), shape, dtype=jnp.bfloat16)

    def randint(self, lo, hi, shape):
        return jax.random.randint(self._next(), shape, lo, hi, dtype=jnp.int32)

    def uniform(self, shape, lo=0.0, hi=1.0):
        return jax.random.uniform(self._next(), shape, jnp.bfloat16, lo, hi)

    def permutation(self, n):
        return jax.random.permutation(self._next(), n)
kernel_name = 'gated_mix__ssm_conv_h3__memory_aug_recurrent_mem_tr__prompt'

def setup_inputs():
    _rng = _Rng(jax.random.key(int.from_bytes(__import__("os").urandom(4), "little")))
    _w = lambda a: (lambda t: t.astype(jnp.bfloat16) if jnp.issubdtype(t.dtype, jnp.floating) else t)(jnp.asarray(a))

    def _A_setup():
        B, S, D = (1, 2048, 1024)
        ks = 4
        return {'q': _w((lambda *s: _rng.normal(s) * 0.05)(B, S, D)), 'k': _w((lambda *s: _rng.normal(s) * 0.05)(B, S, D)), 'v': _w((lambda *s: _rng.normal(s) * 0.05)(B, S, D)), 'shift_k': _w((lambda *s: _rng.normal(s) * 0.05)(D, ks) * 0.5), 'ssm_k': _w((lambda *s: _rng.normal(s) * 0.05)(D, S) * (1.0 / S ** 0.5)), 'ssm_D': _w((lambda *s: _rng.normal(s) * 0.05)(D))}
    _A_in = _A_setup()

    def _B_setup():
        B, S, Dm = (1, 2048, 1024)
        H, Dh = (32, 128)
        M, seg = (8, 32)
        seg = min(seg, S)
        S = S // seg * seg
        return {'x': _w((lambda *s: _rng.normal(s) * 0.05)(B, S, Dm)), 'mem0': _w((lambda *s: _rng.normal(s) * 0.05)(B, M, Dm)), 'Wq': _w((lambda *s: _rng.normal(s) * 0.05)(Dm, H, Dh) * Dm ** (-0.5)), 'Wk': _w((lambda *s: _rng.normal(s) * 0.05)(Dm, H, Dh) * Dm ** (-0.5)), 'Wv': _w((lambda *s: _rng.normal(s) * 0.05)(Dm, H, Dh) * Dm ** (-0.5)), 'Wo': _w((lambda *s: _rng.normal(s) * 0.05)(H, Dh, Dm) * (H * Dh) ** (-0.5)), 'seg_len': seg}
    _B_in = _B_setup()
    return {'A_q': _A_in['q'], 'A_k': _A_in['k'], 'A_v': _A_in['v'], 'A_shift_k': _A_in['shift_k'], 'A_ssm_k': _A_in['ssm_k'], 'A_ssm_D': _A_in['ssm_D'], 'B_x': _B_in['x'], 'B_mem0': _B_in['mem0'], 'B_Wq': _B_in['Wq'], 'B_Wk': _B_in['Wk'], 'B_Wv': _B_in['Wv'], 'B_Wo': _B_in['Wo'], 'B_seg_len': _B_in['seg_len'], 'gate_w': _w((lambda *s: _rng.normal(s) * 0.05)(1024))}

def reference(A_q, A_k, A_v, A_shift_k, A_ssm_k, A_ssm_D, B_x, B_mem0, B_Wq, B_Wk, B_Wv, B_Wo, B_seg_len, gate_w):

    def _A_ref(q, k, v, shift_k, ssm_k, ssm_D):
        B, S, D = q.shape
        ks = shift_k.shape[-1]
        k_pad = jnp.pad(k, ((0, 0), (ks - 1, 0), (0, 0)))
        k_shift = jnp.zeros_like(k)
        for t in range(ks):
            k_shift = k_shift + k_pad[:, t:t + S, :] * shift_k[:, ks - 1 - t][None, None, :]
        kv = k_shift * v
        L = 2 * S
        kv_pad = jnp.pad(kv, ((0, 0), (0, S), (0, 0)))
        kf_pad = jnp.pad(ssm_k, ((0, 0), (0, S)))
        kv_f = (lambda x, axes=(-2, -1): jnp.fft.rfft2(x.astype(jnp.float32), axes=axes))(kv_pad[:, None, :, :], axes=(1, 2))
        kf_f = (lambda x, axes=(-2, -1): jnp.fft.rfft2(x.astype(jnp.float32), axes=axes))(kf_pad[:, None, :], axes=(1, 2))
        kf_f = (lambda x, *d: x.transpose(*d))(kf_f, 1, 2, 0)
        y_f = kv_f * kf_f[None, :, :, :]
        y = (lambda x, s, axes=(-2, -1): jnp.fft.irfft2(x, s=s, axes=axes).astype(jnp.bfloat16))(y_f, (1, L), axes=(1, 2))[:, 0, :S, :]
        y = y + kv * ssm_D[None, None, :]
        return q * y

    def _B_ref(x, mem0, Wq, Wk, Wv, Wo, seg_len):
        B, S, Dm = x.shape
        H, Dh = (Wq.shape[1], Wq.shape[2])
        M = mem0.shape[1]
        scale = Dh ** (-0.5)
        n_seg = S // seg_len
        L = M + seg_len
        idx = jnp.arange(L)
        mask = (idx[:, None] < M) | (idx[:, None] >= idx[None, :])
        mem = mem0
        outs = []
        for s in range(n_seg):
            xs = x[:, s * seg_len:(s + 1) * seg_len, :].copy()
            h = jnp.concatenate([mem, xs], axis=1)
            q = jnp.einsum('btd,dhe->bhte', h, Wq)
            k = jnp.einsum('btd,dhe->bhte', h, Wk)
            v = jnp.einsum('btd,dhe->bhte', h, Wv)
            scores = jnp.einsum('bhqe,bhke->bhqk', q, k) * scale
            scores = jnp.where(mask[None, None], scores, -1000000000.0)
            p = _softmax(scores, axis=-1)
            o = jnp.einsum('bhqk,bhke->bhqe', p, v)
            o = jnp.einsum('bhte,hed->btd', o, Wo)
            mem = o[:, :M, :].copy()
            outs.append(o[:, M:, :])
        return jnp.concatenate(outs, axis=1)
    x = A_q
    g = _sigmoid((x * gate_w).sum(-1, keepdims=True))
    a = _A_ref(x, A_k, A_v, A_shift_k, A_ssm_k, A_ssm_D)
    b = _B_ref(x, B_mem0, B_Wq, B_Wk, B_Wv, B_Wo, B_seg_len)
    return g * a + (1 - g) * b
```

```python
import functools
import math

import jax
import jax.numpy as jnp
import numpy as np
import jax.experimental.pallas as pl
import jax.experimental.pallas.tpu as pltpu

F32 = jnp.float32
BF16 = jnp.bfloat16
U32 = jnp.uint32

S = 2048
D = 1024
H = 32
E = 128
M = 8
SEG = 32
NSEG = S // SEG
RX = 24
PRO = S - RX * NSEG
QCAP = 576
QOFF = QCAP - PRO
C = 128
NCH = S // C
NB = D // 128
KS = 4
NEG = -1000000000.0


def _dft_tables():
    n = np.arange(C, dtype=np.float64)
    th = np.pi * (2.0 * np.arange(C, dtype=np.float64) + 1.0) / (2 * C)
    fwd = np.concatenate([np.cos(th[:, None] * n[None, :]), -np.sin(th[:, None] * n[None, :])], axis=0)
    inv = np.concatenate([np.cos(n[:, None] * th[None, :]), -np.sin(n[:, None] * th[None, :])], axis=1) / C
    return fwd.astype(np.float32), inv.astype(np.float32)


def _attn_fill():
    n = 2 * (SEG + M)
    head = np.array([0] * SEG + [1] * SEG + [0] * M + [1] * M)
    pos = np.concatenate([M + np.arange(SEG), M + np.arange(SEG), np.arange(M), np.arange(M)])
    fill = np.full((n, 128), -np.inf, np.float32)
    for i in range(n):
        for j in range(n):
            if head[i] == head[j]:
                ok = pos[i] < M or pos[i] >= pos[j]
                fill[i, j] = 0.0 if ok else NEG
    return fill


def _dot(a, b):
    return jnp.dot(a, b, preferred_element_type=F32)


def _dot_nt(a, b):
    return jax.lax.dot_general(a, b, (((1,), (1,)), ((), ())), preferred_element_type=F32)


def _kernel(x_hbm, k_hbm, v_hbm, h_hbm, wq_hbm, wk_hbm, wv_hbm, wo_hbm,
            sk_ref, dd_ref, gw_ref, mem0_ref, fwd_ref, inv_ref, fill_ref,
            out_ref,
            x_v, k_v, v_v, h_v, wqkv, wo_v, y_v, qkv_b, o_b, omem, mem_v,
            kf, kvb, u_s, h_s, yf_s, sems, wsems):
    scale = E ** (-0.5)

    in_cp = [pltpu.make_async_copy(src, dst, sems.at[i])
             for i, (src, dst) in enumerate(((k_hbm, k_v), (v_hbm, v_v), (h_hbm, h_v), (x_hbm, x_v)))]
    for cp in in_cp:
        cp.start()
    w32 = [w.bitcast(U32) for w in (wq_hbm, wk_hbm, wv_hbm)]

    def w_copy(mat, hp, par):
        return pltpu.make_async_copy(w32[mat].at[:, par, hp, :], wqkv.at[mat, hp, par], wsems.at[hp])

    for hp in range(H // 2):
        for mat in range(3):
            for par in range(2):
                w_copy(mat, hp, par).start()
    wo32 = wo_hbm.bitcast(U32)
    wo_cp = [pltpu.make_async_copy(wo32.at[:, pl.ds(j * 128, 128)], wo_v.at[j], sems.at[4])
             for j in range(NB)]
    for cp in wo_cp:
        cp.start()

    for cp in in_cp[:3]:
        cp.wait()
    eye = (jax.lax.broadcasted_iota(jnp.int32, (8, KS), 0)
           == jax.lax.broadcasted_iota(jnp.int32, (8, KS), 1)).astype(BF16)
    sgn = (1 - 2 * (jax.lax.broadcasted_iota(jnp.int32, (C, 128), 0) % 2)).astype(F32)
    kf[0:8, :] = jnp.zeros((8, 128), F32)

    def conv_block(c, carry):
        col = pl.ds(pl.multiple_of(c * 128, 128), 128)
        skt = _dot_nt(eye, sk_ref[col, :])
        dd = dd_ref[:, col].astype(F32)
        kf[8:, :] = k_v[:, col].astype(F32)
        fwd = fwd_ref[...]
        inv = inv_ref[...]
        hprev = None
        for a in range(NCH):
            ks_ = kf[pl.ds(8 + a * C, C), :] * skt[0:1, :]
            for j in range(1, KS):
                ks_ = ks_ + kf[pl.ds(8 + a * C - j, C), :] * skt[j:j + 1, :]
            kv = (ks_ * v_v[pl.ds(a * C, C), col].astype(F32)).astype(BF16)
            kvb[pl.ds(a * C, C), :] = kv
            u_s[a] = _dot(fwd, kv)
            hf = _dot_nt(fwd, h_v[col, pl.ds(a * C, C)])
            if hprev is None:
                h_s[a] = hf
            else:
                h_s[a, 0:C, :] = hf[0:C] - sgn * hprev[C:]
                h_s[a, C:, :] = hf[C:] + sgn * hprev[0:C]
            hprev = hf

        def mac(p, carry2):
            re = pl.ds(pl.multiple_of(p * 8, 8), 8)
            im = pl.ds(pl.multiple_of(C + p * 8, 8), 8)
            ur = [u_s[a, re, :] for a in range(NCH)]
            ui = [u_s[a, im, :] for a in range(NCH)]
            for a in range(NCH):
                yr = None
                yi = None
                for m in range(a + 1):
                    hr = h_s[m, re, :]
                    hi = h_s[m, im, :]
                    tr = hr * ur[a - m] - hi * ui[a - m]
                    ti = hr * ui[a - m] + hi * ur[a - m]
                    yr = tr if yr is None else yr + tr
                    yi = ti if yi is None else yi + ti
                yf_s[a, re, :] = yr
                yf_s[a, im, :] = yi
            return carry2

        jax.lax.fori_loop(0, C // 8, mac, 0)
        for a in range(NCH):
            y = _dot(inv, yf_s[a].astype(BF16))
            y = y + kvb[pl.ds(a * C, C), :].astype(F32) * dd
            y_v[pl.ds(a * C, C), col] = y.astype(BF16)
        return carry

    jax.lax.fori_loop(0, NB, conv_block, 0)

    in_cp[3].wait()
    for hp in range(H // 2):
        for mat in range(3):
            for par in range(2):
                w_copy(mat, hp, par).wait()

    def pro(hp, carry):
        for mat in range(3):
            a = wqkv[mat, hp, 0]
            b = wqkv[mat, hp, 1]
            wqkv[mat, hp, 0] = (a & U32(0xFFFF)) | (b << 16)
            wqkv[mat, hp, 1] = (a >> 16) | (b & U32(0xFFFF0000))
        for mat in range(3):
            for j in range(2):
                w = pltpu.bitcast(wqkv[mat, hp, j], BF16)
                for r in range(PRO // 128):
                    res = _dot(x_v[pl.ds(r * 128, 128), :], w)
                    qkv_b[mat, hp, j, pl.ds(QOFF + r * 128, 128), :] = res.astype(BF16)
        return carry

    jax.lax.fori_loop(0, H // 2, pro, 0)
    for cp in wo_cp:
        cp.wait()

    mem_v[...] = mem0_ref[...]
    gw = gw_ref[...].astype(F32)

    def finalize(rows, b):
        xr = x_v[rows, :].astype(F32)
        g = jax.nn.sigmoid(jnp.sum(xr * gw, axis=-1, keepdims=True))
        a = xr * y_v[rows, :].astype(F32)
        out_ref[rows, :] = (g * a + (1.0 - g) * b).astype(BF16)

    def step(s, carry):
        xo = pl.multiple_of(PRO + RX * s, 8)
        wpos = pl.multiple_of((RX * s) % QCAP, 8)
        rpos = pl.multiple_of((SEG * s + QOFF) % QCAP, SEG)
        opos = pl.multiple_of(SEG * s, SEG)
        lhs = jnp.concatenate([mem_v[...], x_v[pl.ds(xo, RX), :]], axis=0)
        zpad = jnp.zeros((128 - 2 * (SEG + M), E), BF16)
        for hp in range(H // 2):
            cat = []
            for mat in range(3):
                mm = []
                for j in range(2):
                    w = pltpu.bitcast(wqkv[mat, hp, j], BF16)
                    res = _dot(lhs, w)
                    qkv_b[mat, hp, j, pl.ds(wpos, RX), :] = res[M:].astype(BF16)
                    mm.append(res[:M])
                parts = [qkv_b[mat, hp, 0, pl.ds(rpos, SEG), :], qkv_b[mat, hp, 1, pl.ds(rpos, SEG), :],
                         jnp.concatenate(mm, axis=0).astype(BF16)]
                if mat > 0:
                    parts.append(zpad)
                cat.append(jnp.concatenate(parts, axis=0))
            sc = _dot_nt(cat[0], cat[1]) * scale
            fill = fill_ref[...]
            sc = jnp.where(fill == 0.0, sc, fill)
            mx = jnp.max(sc, axis=-1, keepdims=True)
            p = jnp.exp(sc - mx)
            l = jnp.sum(p, axis=-1, keepdims=True)
            o = (_dot(p.astype(BF16), cat[2]) * (1.0 / l)).astype(BF16)
            for j in range(2):
                h = 2 * hp + j
                o_b[pl.ds(opos, SEG), h * E:(h + 1) * E] = o[j * SEG:(j + 1) * SEG]
                omem[:, h * E:(h + 1) * E] = o[2 * SEG + j * M:2 * SEG + (j + 1) * M]
        frows = pl.ds(pl.multiple_of(RX * s, 8), RX)
        outs = []
        for j in range(NB):
            lo = jnp.concatenate([omem[...], o_b[frows, :]], axis=0)
            outs.append(_dot(lo, pltpu.bitcast(wo_v[j], BF16)))
        res = jnp.concatenate(outs, axis=1)
        mem_v[...] = res[:M].astype(BF16)
        finalize(frows, res[M:])
        return carry

    jax.lax.fori_loop(0, NSEG, step, 0)

    def epi(r, carry):
        rows = pl.ds(pl.multiple_of(S - PRO + r * 64, 64), 64)
        lo = o_b[rows, :]
        outs = [_dot(lo, pltpu.bitcast(wo_v[j], BF16)) for j in range(NB)]
        finalize(rows, jnp.concatenate(outs, axis=1))
        return carry

    jax.lax.fori_loop(0, PRO // 64, epi, 0)


@jax.jit
def _run(A_q, A_k, A_v, A_shift_k, A_ssm_k, A_ssm_D, B_mem0, B_Wq, B_Wk, B_Wv, B_Wo, gate_w):
    fwd, inv = _dft_tables()
    any_spec = pl.BlockSpec(memory_space=pl.ANY)
    vmem = pl.BlockSpec(memory_space=pltpu.VMEM)
    out = pl.pallas_call(
        _kernel,
        out_shape=jax.ShapeDtypeStruct((S, D), BF16),
        in_specs=[any_spec] * 8 + [vmem] * 7,
        out_specs=vmem,
        scratch_shapes=[
            pltpu.VMEM((S, D), BF16),
            pltpu.VMEM((S, D), BF16),
            pltpu.VMEM((S, D), BF16),
            pltpu.VMEM((D, S), BF16),
            pltpu.VMEM((3, H // 2, 2, D // 2, E), U32),
            pltpu.VMEM((NB, H * E // 2, 128), U32),
            pltpu.VMEM((S, D), BF16),
            pltpu.VMEM((3, H // 2, 2, QCAP, E), BF16),
            pltpu.VMEM((S, H * E), BF16),
            pltpu.VMEM((M, H * E), BF16),
            pltpu.VMEM((M, D), BF16),
            pltpu.VMEM((S + 8, 128), F32),
            pltpu.VMEM((S, 128), BF16),
            pltpu.VMEM((NCH, 2 * C, 128), F32),
            pltpu.VMEM((NCH, 2 * C, 128), F32),
            pltpu.VMEM((NCH, 2 * C, 128), F32),
            pltpu.SemaphoreType.DMA((5,)),
            pltpu.SemaphoreType.DMA((H // 2,)),
        ],
        compiler_params=pltpu.CompilerParams(vmem_limit_bytes=120 * 2 ** 20),
    )(
        A_q.reshape(S, D), A_k.reshape(S, D), A_v.reshape(S, D), A_ssm_k,
        B_Wq.reshape(D // 2, 2, H, E), B_Wk.reshape(D // 2, 2, H, E), B_Wv.reshape(D // 2, 2, H, E),
        B_Wo.reshape(H * E, D),
        A_shift_k, A_ssm_D.reshape(1, D), gate_w.reshape(1, D), B_mem0.reshape(M, D),
        jnp.asarray(fwd, BF16), jnp.asarray(inv, BF16), jnp.asarray(_attn_fill()),
    )
    return out.reshape(1, S, D)


def pallas_gated_mix__ssm_conv_h3__memory_aug_recurrent_mem_tr__prompt_kernel(
    A_q, A_k, A_v, A_shift_k, A_ssm_k, A_ssm_D, B_x, B_mem0, B_Wq, B_Wk, B_Wv, B_Wo, B_seg_len, gate_w,
):
    del B_x
    if isinstance(B_seg_len, int):
        assert B_seg_len == SEG
    return _run(A_q, A_k, A_v, A_shift_k, A_ssm_k, A_ssm_D, B_mem0, B_Wq, B_Wk, B_Wv, B_Wo, gate_w)
```

```python
import functools
import math

import jax
import jax.numpy as jnp
import numpy as np
import jax.experimental.pallas as pl
import jax.experimental.pallas.tpu as pltpu

F32 = jnp.float32
BF16 = jnp.bfloat16
U32 = jnp.uint32

S = 2048
D = 1024
H = 32
E = 128
M = 8
SEG = 32
NSEG = S // SEG
RX = 24
PRO = S - RX * (NSEG - 1)
PRO16 = 544
QCAP = 672
QOFF = 64
C = 128
NCH = S // C
NB = D // 128
KS = 4
NEG = -1000000000.0


def _dft_tables():
    n = np.arange(C, dtype=np.float64)
    th = np.pi * (2.0 * np.arange(C, dtype=np.float64) + 1.0) / (2 * C)
    fwd = np.concatenate([np.cos(th[:, None] * n[None, :]), -np.sin(th[:, None] * n[None, :])], axis=0)
    inv = np.concatenate([np.cos(n[:, None] * th[None, :]), -np.sin(n[:, None] * th[None, :])], axis=1) / C
    return fwd.astype(np.float32), inv.astype(np.float32)


def _attn_fill():
    n = 2 * (SEG + M)
    head = np.array([0] * SEG + [1] * SEG + [0] * M + [1] * M)
    pos = np.concatenate([M + np.arange(SEG), M + np.arange(SEG), np.arange(M), np.arange(M)])
    fill = np.full((n, 128), -np.inf, np.float32)
    for i in range(n):
        for j in range(n):
            if head[i] == head[j]:
                ok = pos[i] < M or pos[i] >= pos[j]
                fill[i, j] = 0.0 if ok else NEG
    return fill


def _dot(a, b):
    return jnp.dot(a, b, preferred_element_type=F32)


def _dot_nt(a, b):
    return jax.lax.dot_general(a, b, (((1,), (1,)), ((), ())), preferred_element_type=F32)


def _kernel(x_hbm, k_hbm, v_hbm, h_hbm, wq_hbm, wk_hbm, wv_hbm, wo_hbm,
            sk_ref, dd_ref, gw_ref, mem0_ref, fwd_ref, inv_ref, fill_ref,
            out_ref,
            x_v, k_v, v_v, h_v, wqkv, wo_v, y_v, qkv_b, o_b, omem, mem_v, st_q, st_o,
            kf, kvb, u_s, h_s, yf_s, sems, wsems):
    scale = E ** (-0.5)

    in_cp = [pltpu.make_async_copy(src, dst, sems.at[i])
             for i, (src, dst) in enumerate(((k_hbm, k_v), (v_hbm, v_v), (h_hbm, h_v), (x_hbm, x_v)))]
    for cp in in_cp:
        cp.start()
    w32 = [w.bitcast(U32) for w in (wq_hbm, wk_hbm, wv_hbm)]

    def w_copy(mat, hp, par):
        return pltpu.make_async_copy(w32[mat].at[:, par, hp, :], wqkv.at[mat, hp, par], wsems.at[hp])

    for hp in range(H // 2):
        for mat in range(3):
            for par in range(2):
                w_copy(mat, hp, par).start()
    wo32 = wo_hbm.bitcast(U32)
    wo_cp = [pltpu.make_async_copy(wo32.at[:, pl.ds(j * 128, 128)], wo_v.at[j], sems.at[4])
             for j in range(NB)]
    for cp in wo_cp:
        cp.start()

    with jax.named_scope("wait_in"):
        for cp in in_cp[:3]:
            cp.wait()
    eye = (jax.lax.broadcasted_iota(jnp.int32, (8, KS), 0)
           == jax.lax.broadcasted_iota(jnp.int32, (8, KS), 1)).astype(BF16)
    sgn = (1 - 2 * (jax.lax.broadcasted_iota(jnp.int32, (C, 128), 0) % 2)).astype(F32)
    kf[0:8, :] = jnp.zeros((8, 128), F32)

    def conv_block(c, carry):
        col = pl.ds(pl.multiple_of(c * 128, 128), 128)
        skt = _dot_nt(eye, sk_ref[col, :])
        dd = dd_ref[:, col].astype(F32)
        kf[8:, :] = k_v[:, col].astype(F32)
        fwd = fwd_ref[...]
        inv = inv_ref[...]
        hprev = None
        for a in range(NCH):
            ks_ = kf[pl.ds(8 + a * C, C), :] * skt[0:1, :]
            for j in range(1, KS):
                ks_ = ks_ + kf[pl.ds(8 + a * C - j, C), :] * skt[j:j + 1, :]
            kv = (ks_ * v_v[pl.ds(a * C, C), col].astype(F32)).astype(BF16)
            kvb[pl.ds(a * C, C), :] = kv
            u_s[a] = _dot(fwd, kv)
            hf = _dot_nt(fwd, h_v[col, pl.ds(a * C, C)])
            if hprev is None:
                h_s[a] = hf
            else:
                h_s[a, 0:C, :] = hf[0:C] - sgn * hprev[C:]
                h_s[a, C:, :] = hf[C:] + sgn * hprev[0:C]
            hprev = hf

        def mac(p, carry2):
            re = pl.ds(pl.multiple_of(p * 8, 8), 8)
            im = pl.ds(pl.multiple_of(C + p * 8, 8), 8)
            ur = [u_s[a, re, :] for a in range(NCH)]
            ui = [u_s[a, im, :] for a in range(NCH)]
            for a in range(NCH):
                yr = None
                yi = None
                for m in range(a + 1):
                    hr = h_s[m, re, :]
                    hi = h_s[m, im, :]
                    tr = hr * ur[a - m] - hi * ui[a - m]
                    ti = hr * ui[a - m] + hi * ur[a - m]
                    yr = tr if yr is None else yr + tr
                    yi = ti if yi is None else yi + ti
                yf_s[a, re, :] = yr
                yf_s[a, im, :] = yi
            return carry2

        jax.lax.fori_loop(0, C // 8, mac, 0)
        for a in range(NCH):
            y = _dot(inv, yf_s[a].astype(BF16))
            y = y + kvb[pl.ds(a * C, C), :].astype(F32) * dd
            y_v[pl.ds(a * C, C), col] = y.astype(BF16)
        return carry

    with jax.named_scope("conv"):
        jax.lax.fori_loop(0, NB, conv_block, 0)

    with jax.named_scope("wait_w"):
        in_cp[3].wait()
        for hp in range(H // 2):
            for mat in range(3):
                for par in range(2):
                    w_copy(mat, hp, par).wait()

    def pro(hp, carry):
        for mat in range(3):
            a = wqkv[mat, hp, 0]
            b = wqkv[mat, hp, 1]
            wqkv[mat, hp, 0] = (a & U32(0xFFFF)) | (b << 16)
            wqkv[mat, hp, 1] = (a >> 16) | (b & U32(0xFFFF0000))
        for mat in range(3):
            for j in range(2):
                w = pltpu.bitcast(wqkv[mat, hp, j], BF16)
                for r0, n in ((0, 128), (128, 128), (256, 128), (384, 160)):
                    res = _dot(x_v[pl.ds(r0, n), :], w)
                    qkv_b[mat, hp, j, pl.ds(QOFF + r0, n), :] = res.astype(BF16)
        return carry

    with jax.named_scope("pro"):
        jax.lax.fori_loop(0, H // 2, pro, 0)
    for cp in wo_cp:
        cp.wait()

    mem_v[...] = mem0_ref[...]
    o_b[0:SEG, :] = jnp.zeros((SEG, H * E), BF16)
    gw = gw_ref[...].astype(F32)

    def finalize(rows, b):
        xr = x_v[rows, :].astype(F32)
        g = jax.nn.sigmoid(jnp.sum(xr * gw, axis=-1, keepdims=True))
        a = xr * y_v[rows, :].astype(F32)
        out_ref[rows, :] = (g * a + (1.0 - g) * b).astype(BF16)

    def step(s, carry):
        xo = pl.multiple_of(jnp.minimum(PRO + RX * s, S - RX), 8)
        wpos = pl.multiple_of((PRO + QOFF + RX * s) % QCAP, 8)
        rpos = pl.multiple_of((SEG * s + QOFF) % QCAP, SEG)
        opos = pl.multiple_of(SEG * s, SEG)
        lhs = jnp.concatenate([mem_v[...], x_v[pl.ds(xo, RX), :]], axis=0)
        zpad = jnp.zeros((128 - 2 * (SEG + M), E), BF16)
        frows = pl.ds(pl.multiple_of(jnp.maximum(RX * (s - 1), 0), 8), RX)
        NP = H // 2
        mem_qkv = {}
        probs = {}

        def cat(mat, hp):
            parts = [qkv_b[mat, hp, 0, pl.ds(rpos, SEG), :], qkv_b[mat, hp, 1, pl.ds(rpos, SEG), :],
                     mem_qkv[(hp, mat)]]
            if mat > 0:
                parts.append(zpad)
            return jnp.concatenate(parts, axis=0)

        def stage_a(hp):
            for mat in range(3):
                mm = []
                for j in range(2):
                    w = pltpu.bitcast(wqkv[mat, hp, j], BF16)
                    res = _dot(lhs, w)
                    st_q[mat, hp, j] = res[M:].astype(BF16)
                    mm.append(res[:M])
                mem_qkv[(hp, mat)] = jnp.concatenate(mm, axis=0).astype(BF16)

        def stage_b(hp):
            sc = _dot_nt(cat(0, hp), cat(1, hp)) * scale
            fill = fill_ref[...]
            sc = jnp.where(fill == 0.0, sc, fill)
            mx = jnp.max(sc, axis=-1, keepdims=True)
            p = jnp.exp(sc - mx)
            l = jnp.sum(p, axis=-1, keepdims=True)
            r = pl.reciprocal(l, approx=True)
            r = r * (2.0 - l * r)
            probs[hp] = (p * r).astype(BF16)

        def stage_c(hp):
            o = _dot(probs[hp], cat(2, hp)).astype(BF16)
            for j in range(2):
                h = 2 * hp + j
                st_o[:, h * E:(h + 1) * E] = o[j * SEG:(j + 1) * SEG]
                omem[:, h * E:(h + 1) * E] = o[2 * SEG + j * M:2 * SEG + (j + 1) * M]

        def oproj(j, h0, h1):
            lo = jnp.concatenate([omem[:, h0 * E:h1 * E], o_b[frows, h0 * E:h1 * E]], axis=0)
            return _dot(lo, pltpu.bitcast(wo_v[j, h0 * E // 2:h1 * E // 2, :], BF16))

        DB, DC = 2, 4
        for hp in range(NP):
            stage_a(hp)
            if hp >= DB:
                stage_b(hp - DB)
            if hp >= DC:
                stage_c(hp - DC)
        HS = H - 2 * (DC + 2)
        outs = [None] * NB
        for j in range(NB):
            outs[j] = oproj(j, 0, HS)
            t = NP + j // 2
            if j % 2 == 1:
                if t - DB < NP:
                    stage_b(t - DB)
                if t - DC < NP:
                    stage_c(t - DC)
        for mat in range(3):
            for hp in range(NP):
                for j in range(2):
                    qkv_b[mat, hp, j, pl.ds(wpos, RX), :] = st_q[mat, hp, j]
        for j in range(NB):
            outs[j] = outs[j] + oproj(j, HS, H - 4)
        for j in range(NB):
            outs[j] = outs[j] + oproj(j, H - 4, H)
        res = jnp.concatenate(outs, axis=1)
        mem_v[...] = res[:M].astype(BF16)
        finalize(frows, res[M:])
        o_b[pl.ds(opos, SEG), :] = st_o[...]
        return carry

    with jax.named_scope("main"):
        jax.lax.fori_loop(0, NSEG, step, 0)

    def epi_rows(rows):
        lo = o_b[rows, :]
        outs = [_dot(lo, pltpu.bitcast(wo_v[j], BF16)) for j in range(NB)]
        finalize(rows, jnp.concatenate(outs, axis=1))

    def epi(r, carry):
        epi_rows(pl.ds(pl.multiple_of(S - 512 + r * 64, 64), 64))
        return carry

    with jax.named_scope("epi"):
        epi_rows(pl.ds(S - PRO16, PRO16 - 512))
        jax.lax.fori_loop(0, 512 // 64, epi, 0)


@jax.jit
def _run(A_q, A_k, A_v, A_shift_k, A_ssm_k, A_ssm_D, B_mem0, B_Wq, B_Wk, B_Wv, B_Wo, gate_w):
    fwd, inv = _dft_tables()
    any_spec = pl.BlockSpec(memory_space=pl.ANY)
    vmem = pl.BlockSpec(memory_space=pltpu.VMEM)
    out = pl.pallas_call(
        _kernel,
        out_shape=jax.ShapeDtypeStruct((S, D), BF16),
        in_specs=[any_spec] * 8 + [vmem] * 7,
        out_specs=vmem,
        scratch_shapes=[
            pltpu.VMEM((S, D), BF16),
            pltpu.VMEM((S, D), BF16),
            pltpu.VMEM((S, D), BF16),
            pltpu.VMEM((D, S), BF16),
            pltpu.VMEM((3, H // 2, 2, D // 2, E), U32),
            pltpu.VMEM((NB, H * E // 2, 128), U32),
            pltpu.VMEM((S, D), BF16),
            pltpu.VMEM((3, H // 2, 2, QCAP, E), BF16),
            pltpu.VMEM((S, H * E), BF16),
            pltpu.VMEM((M, H * E), BF16),
            pltpu.VMEM((M, D), BF16),
            pltpu.VMEM((3, H // 2, 2, RX, E), BF16),
            pltpu.VMEM((SEG, H * E), BF16),
            pltpu.VMEM((S + 8, 128), F32),
            pltpu.VMEM((S, 128), BF16),
            pltpu.VMEM((NCH, 2 * C, 128), F32),
            pltpu.VMEM((NCH, 2 * C, 128), F32),
            pltpu.VMEM((NCH, 2 * C, 128), F32),
            pltpu.SemaphoreType.DMA((5,)),
            pltpu.SemaphoreType.DMA((H // 2,)),
        ],
        compiler_params=pltpu.CompilerParams(vmem_limit_bytes=120 * 2 ** 20),
    )(
        A_q.reshape(S, D), A_k.reshape(S, D), A_v.reshape(S, D), A_ssm_k,
        B_Wq.reshape(D // 2, 2, H, E), B_Wk.reshape(D // 2, 2, H, E), B_Wv.reshape(D // 2, 2, H, E),
        B_Wo.reshape(H * E, D),
        A_shift_k, A_ssm_D.reshape(1, D), gate_w.reshape(1, D), B_mem0.reshape(M, D),
        jnp.asarray(fwd, BF16), jnp.asarray(inv, BF16), jnp.asarray(_attn_fill()),
    )
    return out.reshape(1, S, D)


def pallas_gated_mix__ssm_conv_h3__memory_aug_recurrent_mem_tr__prompt_kernel(
    A_q, A_k, A_v, A_shift_k, A_ssm_k, A_ssm_D, B_x, B_mem0, B_Wq, B_Wk, B_Wv, B_Wo, B_seg_len, gate_w,
):
    del B_x
    if isinstance(B_seg_len, int):
        assert B_seg_len == SEG
    return _run(A_q, A_k, A_v, A_shift_k, A_ssm_k, A_ssm_D, B_mem0, B_Wq, B_Wk, B_Wv, B_Wo, gate_w)
```

```python
import functools
import math

import jax
import jax.numpy as jnp
import numpy as np
import jax.experimental.pallas as pl
import jax.experimental.pallas.tpu as pltpu

F32 = jnp.float32
BF16 = jnp.bfloat16
U32 = jnp.uint32

S = 2048
D = 1024
H = 32
E = 128
M = 8
SEG = 32
NSEG = S // SEG
RX = 24
PRO = S - RX * NSEG
QCAP = 576
QOFF = QCAP - PRO
HL = 8
HS = H - HL
C = 128
NCH = S // C
NB = D // 128
KS = 4
NEG = -1000000000.0


def _dft_tables():
    n = np.arange(C, dtype=np.float64)
    th = np.pi * (2.0 * np.arange(C, dtype=np.float64) + 1.0) / (2 * C)
    fwd = np.concatenate([np.cos(th[:, None] * n[None, :]), -np.sin(th[:, None] * n[None, :])], axis=0)
    inv = np.concatenate([np.cos(n[:, None] * th[None, :]), -np.sin(n[:, None] * th[None, :])], axis=1) / C
    return fwd.astype(np.float32), inv.astype(np.float32)


def _attn_fill():
    n = 2 * (SEG + M)
    head = np.array([0] * SEG + [1] * SEG + [0] * M + [1] * M)
    pos = np.concatenate([M + np.arange(SEG), M + np.arange(SEG), np.arange(M), np.arange(M)])
    fill = np.full((n, 128), -np.inf, np.float32)
    for i in range(n):
        for j in range(n):
            if head[i] == head[j]:
                ok = pos[i] < M or pos[i] >= pos[j]
                fill[i, j] = 0.0 if ok else NEG
    return fill


def _dot(a, b):
    return jnp.dot(a, b, preferred_element_type=F32)


def _dot_nt(a, b):
    return jax.lax.dot_general(a, b, (((1,), (1,)), ((), ())), preferred_element_type=F32)


def _kernel(x_hbm, k_hbm, v_hbm, h_hbm, wq_hbm, wk_hbm, wv_hbm, wo_hbm,
            sk_ref, dd_ref, gw_ref, mem0_ref, fwd_ref, inv_ref, fill_ref,
            out_ref,
            x_v, k_v, v_v, h_v, wqkv, wo_v, y_v, qkv_b, o_b, o_l, omem, mem_v, oacc,
            kf, kvb, u_s, h_s, yf_s, sems, wsems):
    scale = E ** (-0.5)

    in_cp = [pltpu.make_async_copy(src, dst, sems.at[i])
             for i, (src, dst) in enumerate(((k_hbm, k_v), (v_hbm, v_v), (h_hbm, h_v), (x_hbm, x_v)))]
    for cp in in_cp:
        cp.start()
    w32 = [w.bitcast(U32) for w in (wq_hbm, wk_hbm, wv_hbm)]

    def w_copy(mat, hp, par):
        return pltpu.make_async_copy(w32[mat].at[:, par, hp, :], wqkv.at[mat, hp, par], wsems.at[hp])

    for hp in range(H // 2):
        for mat in range(3):
            for par in range(2):
                w_copy(mat, hp, par).start()
    wo32 = wo_hbm.bitcast(U32)
    wo_cp = [pltpu.make_async_copy(wo32.at[:, pl.ds(j * 128, 128)], wo_v.at[j], sems.at[4])
             for j in range(NB)]
    for cp in wo_cp:
        cp.start()

    with jax.named_scope("wait_in"):
        for cp in in_cp[:3]:
            cp.wait()
    eye = (jax.lax.broadcasted_iota(jnp.int32, (8, KS), 0)
           == jax.lax.broadcasted_iota(jnp.int32, (8, KS), 1)).astype(BF16)
    sgn = (1 - 2 * (jax.lax.broadcasted_iota(jnp.int32, (C, 128), 0) % 2)).astype(F32)
    kf[0:8, :] = jnp.zeros((8, 128), F32)

    def conv_block(c, carry):
        col = pl.ds(pl.multiple_of(c * 128, 128), 128)
        skt = _dot_nt(eye, sk_ref[col, :])
        dd = dd_ref[:, col].astype(F32)
        kf[8:, :] = k_v[:, col].astype(F32)
        fwd = fwd_ref[...]
        inv = inv_ref[...]
        hprev = None
        for a in range(NCH):
            ks_ = kf[pl.ds(8 + a * C, C), :] * skt[0:1, :]
            for j in range(1, KS):
                ks_ = ks_ + kf[pl.ds(8 + a * C - j, C), :] * skt[j:j + 1, :]
            kv = (ks_ * v_v[pl.ds(a * C, C), col].astype(F32)).astype(BF16)
            kvb[pl.ds(a * C, C), :] = kv
            u_s[a] = _dot(fwd, kv)
            hf = _dot_nt(fwd, h_v[col, pl.ds(a * C, C)])
            if hprev is None:
                h_s[a] = hf
            else:
                h_s[a, 0:C, :] = hf[0:C] - sgn * hprev[C:]
                h_s[a, C:, :] = hf[C:] + sgn * hprev[0:C]
            hprev = hf

        def mac(p, carry2):
            re = pl.ds(pl.multiple_of(p * 8, 8), 8)
            im = pl.ds(pl.multiple_of(C + p * 8, 8), 8)
            ur = [u_s[a, re, :] for a in range(NCH)]
            ui = [u_s[a, im, :] for a in range(NCH)]
            for a in range(NCH):
                yr = None
                yi = None
                for m in range(a + 1):
                    hr = h_s[m, re, :]
                    hi = h_s[m, im, :]
                    tr = hr * ur[a - m] - hi * ui[a - m]
                    ti = hr * ui[a - m] + hi * ur[a - m]
                    yr = tr if yr is None else yr + tr
                    yi = ti if yi is None else yi + ti
                yf_s[a, re, :] = yr
                yf_s[a, im, :] = yi
            return carry2

        jax.lax.fori_loop(0, C // 8, mac, 0)
        for a in range(NCH):
            y = _dot(inv, yf_s[a].astype(BF16))
            y = y + kvb[pl.ds(a * C, C), :].astype(F32) * dd
            y_v[pl.ds(a * C, C), col] = y.astype(BF16)
        return carry

    with jax.named_scope("conv"):
        jax.lax.fori_loop(0, NB, conv_block, 0)

    with jax.named_scope("wait_w"):
        in_cp[3].wait()
        for hp in range(H // 2):
            for mat in range(3):
                for par in range(2):
                    w_copy(mat, hp, par).wait()

    def pro(hp, carry):
        for mat in range(3):
            a = wqkv[mat, hp, 0]
            b = wqkv[mat, hp, 1]
            wqkv[mat, hp, 0] = (a & U32(0xFFFF)) | (b << 16)
            wqkv[mat, hp, 1] = (a >> 16) | (b & U32(0xFFFF0000))
        for mat in range(3):
            for j in range(2):
                w = pltpu.bitcast(wqkv[mat, hp, j], BF16)
                for r0, n in ((0, 128), (128, 128), (256, 128), (384, 128)):
                    res = _dot(x_v[pl.ds(r0, n), :], w)
                    qkv_b[mat, hp, j, pl.ds(QOFF + r0, n), :] = res.astype(BF16)
        return carry

    with jax.named_scope("pro"):
        jax.lax.fori_loop(0, H // 2, pro, 0)
    for cp in wo_cp:
        cp.wait()

    mem_v[...] = mem0_ref[...]
    gw = gw_ref[...].astype(F32)

    def finalize(rows, b):
        xr = x_v[rows, :].astype(F32)
        g = jax.nn.sigmoid(jnp.sum(xr * gw, axis=-1, keepdims=True))
        a = xr * y_v[rows, :].astype(F32)
        out_ref[rows, :] = (g * a + (1.0 - g) * b).astype(BF16)

    def step(s, carry):
        xo = pl.multiple_of(PRO + RX * s, 8)
        wpos = pl.multiple_of((RX * s) % QCAP, 8)
        rpos = pl.multiple_of((SEG * s + QOFF) % QCAP, SEG)
        opos = pl.multiple_of(SEG * s, SEG)
        lhs = jnp.concatenate([mem_v[...], x_v[pl.ds(xo, RX), :]], axis=0)
        zpad = jnp.zeros((128 - 2 * (SEG + M), E), BF16)
        frows = pl.ds(pl.multiple_of(RX * s, 8), RX)
        NP = H // 2
        mem_qkv = {}
        probs = {}
        cats = {}

        def load(mat, hp):
            if not 0 <= hp < NP:
                return
            parts = [qkv_b[mat, hp, 0, pl.ds(rpos, SEG), :], qkv_b[mat, hp, 1, pl.ds(rpos, SEG), :],
                     mem_qkv[(hp, mat)]]
            if mat > 0:
                parts.append(zpad)
            cats[(mat, hp)] = jnp.concatenate(parts, axis=0)

        def stage_a(hp):
            for mat in range(3):
                mm = []
                for j in range(2):
                    w = pltpu.bitcast(wqkv[mat, hp, j], BF16)
                    res = _dot(lhs, w)
                    qkv_b[mat, hp, j, pl.ds(wpos, RX), :] = res[M:].astype(BF16)
                    mm.append(res[:M])
                mem_qkv[(hp, mat)] = jnp.concatenate(mm, axis=0).astype(BF16)

        def stage_b(hp):
            if not 0 <= hp < NP:
                return
            sc = _dot_nt(cats[(0, hp)], cats[(1, hp)]) * scale
            fill = fill_ref[...]
            sc = jnp.where(fill == 0.0, sc, fill)
            mx = jnp.max(sc, axis=-1, keepdims=True)
            p = jnp.exp(sc - mx)
            l = jnp.sum(p, axis=-1, keepdims=True)
            r = pl.reciprocal(l, approx=True)
            r = r * (2.0 - l * r)
            probs[hp] = (p * r).astype(BF16)

        def stage_c(hp):
            if not 0 <= hp < NP:
                return
            o = _dot(probs[hp], cats[(2, hp)]).astype(BF16)
            for j in range(2):
                h = 2 * hp + j
                if h < HS:
                    o_b[pl.ds(opos, SEG), h * E:(h + 1) * E] = o[j * SEG:(j + 1) * SEG]
                else:
                    o_l[pl.ds(opos, SEG), (h - HS) * E:(h - HS + 1) * E] = o[j * SEG:(j + 1) * SEG]
                omem[:, h * E:(h + 1) * E] = o[2 * SEG + j * M:2 * SEG + (j + 1) * M]

        def oproj(j, late):
            if late:
                lo = jnp.concatenate([omem[:, HS * E:], o_l[frows, :]], axis=0)
                return _dot(lo, pltpu.bitcast(wo_v[j, HS * E // 2:, :], BF16))
            lo = jnp.concatenate([omem[:, :HS * E], o_b[frows, :]], axis=0)
            return _dot(lo, pltpu.bitcast(wo_v[j, :HS * E // 2, :], BF16))

        DB, DC = 1, 3
        outs = [None] * NB
        for t in range(NP + DC):
            load(0, t - DB)
            load(1, t - DB)
            load(2, t - DC)
            if t < NP:
                stage_a(t)
            else:
                for j in range(2 * (t - NP), 2 * (t - NP) + 2):
                    oacc[:, j * 128:(j + 1) * 128] = oproj(j, False)
            stage_b(t - DB)
            stage_c(t - DC)
        for j in range(2 * DC, NB):
            oacc[:, j * 128:(j + 1) * 128] = oproj(j, False)
        for j in range(NB):
            outs[j] = oacc[:, j * 128:(j + 1) * 128] + oproj(j, True)
        res = jnp.concatenate(outs, axis=1)
        mem_v[...] = res[:M].astype(BF16)
        finalize(frows, res[M:])
        return carry

    with jax.named_scope("main"):
        jax.lax.fori_loop(0, NSEG, step, 0)

    def epi_rows(rows):
        lo = jnp.concatenate([o_b[rows, :], o_l[rows, :]], axis=1)
        outs = [_dot(lo, pltpu.bitcast(wo_v[j], BF16)) for j in range(NB)]
        finalize(rows, jnp.concatenate(outs, axis=1))

    def epi(r, carry):
        epi_rows(pl.ds(pl.multiple_of(S - 512 + r * 64, 64), 64))
        return carry

    with jax.named_scope("epi"):
        jax.lax.fori_loop(0, 512 // 64, epi, 0)


@jax.jit
def _run(A_q, A_k, A_v, A_shift_k, A_ssm_k, A_ssm_D, B_mem0, B_Wq, B_Wk, B_Wv, B_Wo, gate_w):
    fwd, inv = _dft_tables()
    any_spec = pl.BlockSpec(memory_space=pl.ANY)
    vmem = pl.BlockSpec(memory_space=pltpu.VMEM)
    out = pl.pallas_call(
        _kernel,
        out_shape=jax.ShapeDtypeStruct((S, D), BF16),
        in_specs=[any_spec] * 8 + [vmem] * 7,
        out_specs=vmem,
        scratch_shapes=[
            pltpu.VMEM((S, D), BF16),
            pltpu.VMEM((S, D), BF16),
            pltpu.VMEM((S, D), BF16),
            pltpu.VMEM((D, S), BF16),
            pltpu.VMEM((3, H // 2, 2, D // 2, E), U32),
            pltpu.VMEM((NB, H * E // 2, 128), U32),
            pltpu.VMEM((S, D), BF16),
            pltpu.VMEM((3, H // 2, 2, QCAP, E), BF16),
            pltpu.VMEM((S, HS * E), BF16),
            pltpu.VMEM((S, HL * E), BF16),
            pltpu.VMEM((M, H * E), BF16),
            pltpu.VMEM((M, D), BF16),
            pltpu.VMEM((M + RX, D), F32),
            pltpu.VMEM((S + 8, 128), F32),
            pltpu.VMEM((S, 128), BF16),
            pltpu.VMEM((NCH, 2 * C, 128), F32),
            pltpu.VMEM((NCH, 2 * C, 128), F32),
            pltpu.VMEM((NCH, 2 * C, 128), F32),
            pltpu.SemaphoreType.DMA((5,)),
            pltpu.SemaphoreType.DMA((H // 2,)),
        ],
        compiler_params=pltpu.CompilerParams(vmem_limit_bytes=120 * 2 ** 20),
    )(
        A_q.reshape(S, D), A_k.reshape(S, D), A_v.reshape(S, D), A_ssm_k,
        B_Wq.reshape(D // 2, 2, H, E), B_Wk.reshape(D // 2, 2, H, E), B_Wv.reshape(D // 2, 2, H, E),
        B_Wo.reshape(H * E, D),
        A_shift_k, A_ssm_D.reshape(1, D), gate_w.reshape(1, D), B_mem0.reshape(M, D),
        jnp.asarray(fwd, BF16), jnp.asarray(inv, BF16), jnp.asarray(_attn_fill()),
    )
    return out.reshape(1, S, D)


def pallas_gated_mix__ssm_conv_h3__memory_aug_recurrent_mem_tr__prompt_kernel(
    A_q, A_k, A_v, A_shift_k, A_ssm_k, A_ssm_D, B_x, B_mem0, B_Wq, B_Wk, B_Wv, B_Wo, B_seg_len, gate_w,
):
    del B_x
    if isinstance(B_seg_len, int):
        assert B_seg_len == SEG
    return _run(A_q, A_k, A_v, A_shift_k, A_ssm_k, A_ssm_D, B_mem0, B_Wq, B_Wk, B_Wv, B_Wo, gate_w)
```

```python
import functools
import math

import jax
import jax.numpy as jnp
import numpy as np
import jax.experimental.pallas as pl
import jax.experimental.pallas.tpu as pltpu

F32 = jnp.float32
BF16 = jnp.bfloat16
U32 = jnp.uint32

S = 2048
D = 1024
H = 32
E = 128
M = 8
SEG = 32
NSEG = S // SEG
RX = 24
PRO = S - RX * NSEG
QCAP = 576
QOFF = QCAP - PRO
HL = 8
HS = H - HL
C = 128
NCH = S // C
NB = D // 128
KS = 4
NEG = -1000000000.0


def _dft_tables():
    n = np.arange(C, dtype=np.float64)
    th = np.pi * (2.0 * np.arange(C, dtype=np.float64) + 1.0) / (2 * C)
    fwd = np.concatenate([np.cos(th[:, None] * n[None, :]), -np.sin(th[:, None] * n[None, :])], axis=0)
    inv = np.concatenate([np.cos(n[:, None] * th[None, :]), -np.sin(n[:, None] * th[None, :])], axis=1) / C
    return fwd.astype(np.float32), inv.astype(np.float32)


def _attn_fill():
    n = 2 * (SEG + M)
    head = np.array([0] * SEG + [1] * SEG + [0] * M + [1] * M)
    pos = np.concatenate([M + np.arange(SEG), M + np.arange(SEG), np.arange(M), np.arange(M)])
    fill = np.full((n, 128), -np.inf, np.float32)
    for i in range(n):
        for j in range(n):
            if head[i] == head[j]:
                ok = pos[i] < M or pos[i] >= pos[j]
                fill[i, j] = 0.0 if ok else NEG
    return fill


def _dot(a, b):
    return jnp.dot(a, b, preferred_element_type=F32)


def _dot_nt(a, b):
    return jax.lax.dot_general(a, b, (((1,), (1,)), ((), ())), preferred_element_type=F32)


def _kernel(x_hbm, k_hbm, v_hbm, h_hbm, wq_hbm, wk_hbm, wv_hbm, wo_hbm,
            sk_ref, dd_ref, gw_ref, mem0_ref, fwd_ref, inv_ref, fill_ref,
            out_ref,
            x_v, xp, k_v, v_v, h_v, w_even, w_odd, wo_v, y_v, qkv_b, o_b, o_l, omem, mem_v, oacc,
            kf, kvb, u_s, h_s, yf_s, zs, sems):
    scale = E ** (-0.5)
    wbuf = (w_even, w_odd)

    w32 = [w.bitcast(U32) for w in (wq_hbm, wk_hbm, wv_hbm)]
    wo32 = wo_hbm.bitcast(U32)
    x32 = x_hbm.bitcast(U32)

    def lanes(c):
        return pl.ds(pl.multiple_of(c * 128, 128), 128)

    def w_copies(c):
        return [pltpu.make_async_copy(w32[mat].at[:, par, 2 * c + e, :], wbuf[e].at[mat, c, par], sems.at[0])
                for e in range(2) for mat in range(3) for par in range(2)]

    def kv_copies(c):
        return [pltpu.make_async_copy(k_hbm.at[:, lanes(c)], k_v.at[c], sems.at[1]),
                pltpu.make_async_copy(v_hbm.at[:, lanes(c)], v_v.at[c], sems.at[1])]

    def h_copy(c):
        return pltpu.make_async_copy(h_hbm.at[lanes(c), :], h_v.at[c], sems.at[2])

    def rest_copies(c):
        rows = pl.ds(pl.multiple_of(c * (S // NB), S // NB), S // NB)
        return [pltpu.make_async_copy(wo32.at[:, lanes(c)], wo_v.at[c], sems.at[3]),
                pltpu.make_async_copy(x_hbm.at[rows, :], x_v.at[rows, :], sems.at[3])]

    xp_copy = pltpu.make_async_copy(x32.at[pl.ds(0, PRO // 2), :], xp, sems.at[4])

    eye = (jax.lax.broadcasted_iota(jnp.int32, (8, KS), 0)
           == jax.lax.broadcasted_iota(jnp.int32, (8, KS), 1)).astype(BF16)

    def kv_prep(c):
        skt = _dot_nt(eye, sk_ref[lanes(c), :])
        kf[8:, :] = k_v[c].astype(F32)
        for a in range(NCH):
            ks_ = kf[pl.ds(8 + a * C, C), :] * skt[0:1, :]
            for j in range(1, KS):
                ks_ = ks_ + kf[pl.ds(8 + a * C - j, C), :] * skt[j:j + 1, :]
            kvb[pl.ds(a * C, C), :] = (ks_ * v_v[c, pl.ds(a * C, C), :].astype(F32)).astype(BF16)

    def fwd_dft(c, zw):
        sgn = (1 - 2 * (jax.lax.broadcasted_iota(jnp.int32, (C, 128), 0) % 2)).astype(F32)
        hprev = None
        for a in range(NCH):
            u_s[zw, a] = _dot(fwd_ref[...], kvb[pl.ds(a * C, C), :])
            hf = _dot_nt(fwd_ref[...], h_v[c, :, pl.ds(a * C, C)])
            if hprev is None:
                h_s[zw, a, 0:C, :] = hf[0:C] + dd_ref[:, lanes(c)].astype(F32)
                h_s[zw, a, C:, :] = hf[C:]
            else:
                h_s[zw, a, 0:C, :] = hf[0:C] - sgn * hprev[C:]
                h_s[zw, a, C:, :] = hf[C:] + sgn * hprev[0:C]
            hprev = hf

    def mac(p, zw, zr):
        re = pl.ds(p * 8, 8)
        im = pl.ds(C + p * 8, 8)
        AB = 4
        for a0 in range(0, NCH, AB):
            yr = [None] * AB
            yi = [None] * AB
            for m in range(a0 + AB):
                hr = h_s[zr, m, re, :]
                hi = h_s[zr, m, im, :]
                for i in range(AB):
                    t = a0 + i - m
                    if t < 0:
                        continue
                    ur = u_s[zr, t, re, :]
                    ui = u_s[zr, t, im, :]
                    tr = hr * ur - hi * ui
                    ti = hr * ui + hi * ur
                    yr[i] = tr if yr[i] is None else yr[i] + tr
                    yi[i] = ti if yi[i] is None else yi[i] + ti
            for i in range(AB):
                yf_s[zw, a0 + i, re, :] = yr[i]
                yf_s[zw, a0 + i, im, :] = yi[i]

    def inv_dft(c, zr):
        for a in range(NCH):
            y_v[pl.ds(a * C, C), lanes(c)] = _dot(inv_ref[...], yf_s[zr, a].astype(BF16)).astype(BF16)

    def fixup(e, c):
        for mat in range(3):
            a = wbuf[e][mat, c, 0]
            b = wbuf[e][mat, c, 1]
            wbuf[e][mat, c, 0] = (a & U32(0xFFFF)) | (b << 16)
            wbuf[e][mat, c, 1] = (a >> 16) | (b & U32(0xFFFF0000))

    RB = 128

    def qkv_tile(e, c, n):
        mat, j = n // 2, n % 2
        for r in range(PRO // RB):
            w = pltpu.bitcast(wbuf[e][mat, c, j], BF16)
            xr = pltpu.bitcast(xp[pl.ds(r * RB // 2, RB // 2), :], BF16)
            qkv_b[mat, 2 * c + e, j, pl.ds(QOFF + r * RB, RB), :] = _dot(xr, w).astype(BF16)

    for cp in kv_copies(0):
        cp.start()
    h_copy(0).start()
    xp_copy.start()
    for cp in w_copies(0):
        cp.start()
    kf[0:8, :] = jnp.zeros((8, 128), F32)
    zs[0] = 0
    zs[1] = 0
    for cp in kv_copies(0):
        cp.wait()
    for cp in kv_copies(1):
        cp.start()
    kv_prep(0)
    xp_copy.wait()

    def pro(c, carry):
        nxt = jnp.minimum(c + 1, NB - 1)
        h_copy(c).wait()
        for cp in w_copies(c):
            cp.wait()

        @pl.when(c + 1 < NB)
        def _():
            for cp in kv_copies(c + 1):
                cp.wait()
            h_copy(c + 1).start()
            for cp in w_copies(c + 1):
                cp.start()

        @pl.when(c + 2 < NB)
        def _():
            for cp in kv_copies(c + 2):
                cp.start()

        for cp in rest_copies(c):
            cp.start()

        zw = zs[0]
        zr = zs[1]
        fixup(0, c)
        fwd_dft(c, zw)
        fixup(1, c)
        for n in range(6):
            qkv_tile(0, c, n)
            for p in range(n * 2, n * 2 + 2):
                mac(p, zw, zr)
        for n in range(4):
            qkv_tile(1, c, n)
            mac(12 + n, zw, zr)
        kv_prep(nxt)
        inv_dft(c, zr)
        for n in range(4, 6):
            qkv_tile(1, c, n)
        return carry

    with jax.named_scope("pro"):
        jax.lax.fori_loop(0, NB, pro, 0)
    for c in range(NB):
        for cp in rest_copies(c):
            cp.wait()

    mem_v[...] = mem0_ref[...]
    gw = gw_ref[...].astype(F32)

    def finalize(rows, b):
        xr = x_v[rows, :].astype(F32)
        g = jax.nn.sigmoid(jnp.sum(xr * gw, axis=-1, keepdims=True))
        a = xr * y_v[rows, :].astype(F32)
        out_ref[rows, :] = (g * a + (1.0 - g) * b).astype(BF16)

    def step(s, carry):
        xo = pl.multiple_of(PRO + RX * s, 8)
        wpos = pl.multiple_of((RX * s) % QCAP, 8)
        rpos = pl.multiple_of((SEG * s + QOFF) % QCAP, SEG)
        opos = pl.multiple_of(SEG * s, SEG)
        lhs = jnp.concatenate([mem_v[...], x_v[pl.ds(xo, RX), :]], axis=0)
        zpad = jnp.zeros((128 - 2 * (SEG + M), E), BF16)
        frows = pl.ds(pl.multiple_of(RX * s, 8), RX)
        NP = H // 2
        mem_qkv = {}
        probs = {}
        cats = {}

        def load(mat, hp):
            if not 0 <= hp < NP:
                return
            parts = [qkv_b[mat, hp, 0, pl.ds(rpos, SEG), :], qkv_b[mat, hp, 1, pl.ds(rpos, SEG), :],
                     mem_qkv[(hp, mat)]]
            if mat > 0:
                parts.append(zpad)
            cats[(mat, hp)] = jnp.concatenate(parts, axis=0)

        def stage_a(hp):
            for mat in range(3):
                mm = []
                for j in range(2):
                    w = pltpu.bitcast(wbuf[hp % 2][mat, hp // 2, j], BF16)
                    res = _dot(lhs, w)
                    qkv_b[mat, hp, j, pl.ds(wpos, RX), :] = res[M:].astype(BF16)
                    mm.append(res[:M])
                mem_qkv[(hp, mat)] = jnp.concatenate(mm, axis=0).astype(BF16)

        def stage_b(hp):
            if not 0 <= hp < NP:
                return
            sc = _dot_nt(cats[(0, hp)], cats[(1, hp)]) * scale
            fill = fill_ref[...]
            sc = jnp.where(fill == 0.0, sc, fill)
            mx = jnp.max(sc, axis=-1, keepdims=True)
            p = jnp.exp(sc - mx)
            l = jnp.sum(p, axis=-1, keepdims=True)
            r = pl.reciprocal(l, approx=True)
            r = r * (2.0 - l * r)
            probs[hp] = (p * r).astype(BF16)

        def stage_c(hp):
            if not 0 <= hp < NP:
                return
            o = _dot(probs[hp], cats[(2, hp)]).astype(BF16)
            for j in range(2):
                h = 2 * hp + j
                if h < HS:
                    o_b[pl.ds(opos, SEG), h * E:(h + 1) * E] = o[j * SEG:(j + 1) * SEG]
                else:
                    o_l[pl.ds(opos, SEG), (h - HS) * E:(h - HS + 1) * E] = o[j * SEG:(j + 1) * SEG]
                omem[:, h * E:(h + 1) * E] = o[2 * SEG + j * M:2 * SEG + (j + 1) * M]

        def oproj(j, late):
            if late:
                lo = jnp.concatenate([omem[:, HS * E:], o_l[frows, :]], axis=0)
                return _dot(lo, pltpu.bitcast(wo_v[j, HS * E // 2:, :], BF16))
            lo = jnp.concatenate([omem[:, :HS * E], o_b[frows, :]], axis=0)
            return _dot(lo, pltpu.bitcast(wo_v[j, :HS * E // 2, :], BF16))

        DB, DC = 1, 3
        outs = [None] * NB
        for t in range(NP + DC):
            load(0, t - DB)
            load(1, t - DB)
            load(2, t - DC)
            if t < NP:
                stage_a(t)
            else:
                for j in range(2 * (t - NP), 2 * (t - NP) + 2):
                    oacc[:, j * 128:(j + 1) * 128] = oproj(j, False)
            stage_b(t - DB)
            stage_c(t - DC)
        for j in range(2 * DC, NB):
            oacc[:, j * 128:(j + 1) * 128] = oproj(j, False)
        for j in range(NB):
            outs[j] = oacc[:, j * 128:(j + 1) * 128] + oproj(j, True)
        res = jnp.concatenate(outs, axis=1)
        mem_v[...] = res[:M].astype(BF16)
        finalize(frows, res[M:])
        return carry

    with jax.named_scope("main"):
        jax.lax.fori_loop(0, NSEG, step, 0)

    def epi_rows(rows):
        lo = jnp.concatenate([o_b[rows, :], o_l[rows, :]], axis=1)
        outs = [_dot(lo, pltpu.bitcast(wo_v[j], BF16)) for j in range(NB)]
        finalize(rows, jnp.concatenate(outs, axis=1))

    def epi(r, carry):
        epi_rows(pl.ds(pl.multiple_of(S - 512 + r * 64, 64), 64))
        return carry

    with jax.named_scope("epi"):
        jax.lax.fori_loop(0, 512 // 64, epi, 0)


@jax.jit
def _run(A_q, A_k, A_v, A_shift_k, A_ssm_k, A_ssm_D, B_mem0, B_Wq, B_Wk, B_Wv, B_Wo, gate_w):
    fwd, inv = _dft_tables()
    any_spec = pl.BlockSpec(memory_space=pl.ANY)
    vmem = pl.BlockSpec(memory_space=pltpu.VMEM)
    out = pl.pallas_call(
        _kernel,
        out_shape=jax.ShapeDtypeStruct((S, D), BF16),
        in_specs=[any_spec] * 8 + [vmem] * 7,
        out_specs=vmem,
        scratch_shapes=[
            pltpu.VMEM((S, D), BF16),
            pltpu.VMEM((PRO // 2, D), U32),
            pltpu.VMEM((NB, S, 128), BF16),
            pltpu.VMEM((NB, S, 128), BF16),
            pltpu.VMEM((NB, 128, S), BF16),
            pltpu.VMEM((3, H // 4, 2, D // 2, E), U32),
            pltpu.VMEM((3, H // 4, 2, D // 2, E), U32),
            pltpu.VMEM((NB, H * E // 2, 128), U32),
            pltpu.VMEM((S, D), BF16),
            pltpu.VMEM((3, H // 2, 2, QCAP, E), BF16),
            pltpu.VMEM((S, HS * E), BF16),
            pltpu.VMEM((S, HL * E), BF16),
            pltpu.VMEM((M, H * E), BF16),
            pltpu.VMEM((M, D), BF16),
            pltpu.VMEM((M + RX, D), F32),
            pltpu.VMEM((S + 8, 128), F32),
            pltpu.VMEM((S, 128), BF16),
            pltpu.VMEM((1, NCH, 2 * C, 128), F32),
            pltpu.VMEM((1, NCH, 2 * C, 128), F32),
            pltpu.VMEM((1, NCH, 2 * C, 128), F32),
            pltpu.SMEM((2,), jnp.int32),
            pltpu.SemaphoreType.DMA((5,)),
        ],
        compiler_params=pltpu.CompilerParams(vmem_limit_bytes=120 * 2 ** 20),
    )(
        A_q.reshape(S, D), A_k.reshape(S, D), A_v.reshape(S, D), A_ssm_k,
        B_Wq.reshape(D // 2, 2, H, E), B_Wk.reshape(D // 2, 2, H, E), B_Wv.reshape(D // 2, 2, H, E),
        B_Wo.reshape(H * E, D),
        A_shift_k, A_ssm_D.reshape(1, D), gate_w.reshape(1, D), B_mem0.reshape(M, D),
        jnp.asarray(fwd, BF16), jnp.asarray(inv, BF16), jnp.asarray(_attn_fill()),
    )
    return out.reshape(1, S, D)


def pallas_gated_mix__ssm_conv_h3__memory_aug_recurrent_mem_tr__prompt_kernel(
    A_q, A_k, A_v, A_shift_k, A_ssm_k, A_ssm_D, B_x, B_mem0, B_Wq, B_Wk, B_Wv, B_Wo, B_seg_len, gate_w,
):
    del B_x
    if isinstance(B_seg_len, int):
        assert B_seg_len == SEG
    return _run(A_q, A_k, A_v, A_shift_k, A_ssm_k, A_ssm_D, B_mem0, B_Wq, B_Wk, B_Wv, B_Wo, gate_w)
```

```python
import functools
import math

import jax
import jax.numpy as jnp
import numpy as np
import jax.experimental.pallas as pl
import jax.experimental.pallas.tpu as pltpu

F32 = jnp.float32
BF16 = jnp.bfloat16
U32 = jnp.uint32

S = 2048
D = 1024
H = 32
E = 128
M = 8
SEG = 32
NSEG = S // SEG
RX = 24
PRO = S - RX * NSEG
QCAP = 576
QOFF = QCAP - PRO
HL = 8
HS = H - HL
C = 128
NCH = S // C
NB = D // 128
KS = 4
NEG = -1000000000.0


def _dft_tables():
    n = np.arange(C, dtype=np.float64)
    th = np.pi * (2.0 * np.arange(C, dtype=np.float64) + 1.0) / (2 * C)
    fwd = np.concatenate([np.cos(th[:, None] * n[None, :]), -np.sin(th[:, None] * n[None, :])], axis=0)
    inv = np.concatenate([np.cos(n[:, None] * th[None, :]), -np.sin(n[:, None] * th[None, :])], axis=1) / C
    return fwd.astype(np.float32), inv.astype(np.float32)


def _attn_fill():
    n = 2 * (SEG + M)
    head = np.array([0] * SEG + [1] * SEG + [0] * M + [1] * M)
    pos = np.concatenate([M + np.arange(SEG), M + np.arange(SEG), np.arange(M), np.arange(M)])
    fill = np.full((n, 128), -np.inf, np.float32)
    for i in range(n):
        for j in range(n):
            if head[i] == head[j]:
                ok = pos[i] < M or pos[i] >= pos[j]
                fill[i, j] = 0.0 if ok else NEG
    return fill


def _dot(a, b):
    return jnp.dot(a, b, preferred_element_type=F32)


def _dot_nt(a, b):
    return jax.lax.dot_general(a, b, (((1,), (1,)), ((), ())), preferred_element_type=F32)


def _kernel(x_hbm, k_hbm, v_hbm, h_hbm, wq_hbm, wk_hbm, wv_hbm, wo_hbm,
            sk_ref, dd_ref, gw_ref, mem0_ref, fwd_ref, inv_ref, fill_ref,
            out_ref,
            x_v, xp, k_v, v_v, h_v, w_even, w_odd, wo_v, y_v, qkv_b, o_b, o_l, omem, mem_v, oacc,
            skt_v, kf, kvb, u_s, h_s, yf_s, zs, sems):
    scale = E ** (-0.5)
    wbuf = (w_even, w_odd)

    w32 = [w.bitcast(U32) for w in (wq_hbm, wk_hbm, wv_hbm)]
    wo32 = wo_hbm.bitcast(U32)
    x32 = x_hbm.bitcast(U32)

    def lanes(c):
        return pl.ds(pl.multiple_of(c * 128, 128), 128)

    def w_copies(c):
        return [pltpu.make_async_copy(w32[mat].at[:, par, 2 * c + e, :], wbuf[e].at[mat, c, par], sems.at[0])
                for e in range(2) for mat in range(3) for par in range(2)]

    def kv_copies(c):
        return [pltpu.make_async_copy(k_hbm.at[:, lanes(c)], k_v.at[c], sems.at[1]),
                pltpu.make_async_copy(v_hbm.at[:, lanes(c)], v_v.at[c], sems.at[1])]

    def h_copy(c):
        return pltpu.make_async_copy(h_hbm.at[lanes(c), :], h_v.at[c], sems.at[2])

    def rest_copies(c):
        rows = pl.ds(pl.multiple_of(c * (S // NB), S // NB), S // NB)
        return [pltpu.make_async_copy(wo32.at[:, lanes(c)], wo_v.at[c], sems.at[3]),
                pltpu.make_async_copy(x_hbm.at[rows, :], x_v.at[rows, :], sems.at[3])]

    xp_copy = pltpu.make_async_copy(x32.at[pl.ds(0, PRO // 2), :], xp, sems.at[4])

    eye = (jax.lax.broadcasted_iota(jnp.int32, (8, KS), 0)
           == jax.lax.broadcasted_iota(jnp.int32, (8, KS), 1)).astype(BF16)

    def kv_prep(c):
        skt = skt_v[:, lanes(c)]
        kf[8:, :] = k_v[c].astype(F32)
        for a in range(NCH):
            ks_ = kf[pl.ds(8 + a * C, C), :] * skt[0:1, :]
            for j in range(1, KS):
                ks_ = ks_ + kf[pl.ds(8 + a * C - j, C), :] * skt[j:j + 1, :]
            kvb[pl.ds(a * C, C), :] = (ks_ * v_v[c, pl.ds(a * C, C), :].astype(F32)).astype(BF16)

    def fwd_dft(c, zw):
        sgn = (1 - 2 * (jax.lax.broadcasted_iota(jnp.int32, (C, 128), 0) % 2)).astype(F32)
        hprev = None
        for a in range(NCH):
            u_s[zw, a] = _dot(fwd_ref[...], kvb[pl.ds(a * C, C), :])
            hf = _dot_nt(fwd_ref[...], h_v[c, :, pl.ds(a * C, C)])
            if hprev is None:
                h_s[zw, a, 0:C, :] = hf[0:C] + dd_ref[:, lanes(c)].astype(F32)
                h_s[zw, a, C:, :] = hf[C:]
            else:
                h_s[zw, a, 0:C, :] = hf[0:C] - sgn * hprev[C:]
                h_s[zw, a, C:, :] = hf[C:] + sgn * hprev[0:C]
            hprev = hf

    def mac(p, zw, zr):
        re = pl.ds(p * 8, 8)
        im = pl.ds(C + p * 8, 8)
        AB = 4
        for a0 in range(0, NCH, AB):
            yr = [None] * AB
            yi = [None] * AB
            for m in range(a0 + AB):
                hr = h_s[zr, m, re, :]
                hi = h_s[zr, m, im, :]
                for i in range(AB):
                    t = a0 + i - m
                    if t < 0:
                        continue
                    ur = u_s[zr, t, re, :]
                    ui = u_s[zr, t, im, :]
                    tr = hr * ur - hi * ui
                    ti = hr * ui + hi * ur
                    yr[i] = tr if yr[i] is None else yr[i] + tr
                    yi[i] = ti if yi[i] is None else yi[i] + ti
            for i in range(AB):
                yf_s[zw, a0 + i, re, :] = yr[i]
                yf_s[zw, a0 + i, im, :] = yi[i]

    def inv_dft(c, zr):
        for a in range(NCH):
            y_v[pl.ds(a * C, C), lanes(c)] = _dot(inv_ref[...], yf_s[zr, a].astype(BF16)).astype(BF16)

    def fixup(e, c):
        for mat in range(3):
            a = wbuf[e][mat, c, 0]
            b = wbuf[e][mat, c, 1]
            wbuf[e][mat, c, 0] = (a & U32(0xFFFF)) | (b << 16)
            wbuf[e][mat, c, 1] = (a >> 16) | (b & U32(0xFFFF0000))

    RB = 128

    def qkv_tile(e, c, n):
        mat, j = n // 2, n % 2
        for r in range(PRO // RB):
            w = pltpu.bitcast(wbuf[e][mat, c, j], BF16)
            xr = pltpu.bitcast(xp[pl.ds(r * RB // 2, RB // 2), :], BF16)
            qkv_b[mat, 2 * c + e, j, pl.ds(QOFF + r * RB, RB), :] = _dot(xr, w).astype(BF16)

    for cp in kv_copies(0):
        cp.start()
    h_copy(0).start()
    xp_copy.start()
    for cp in w_copies(0):
        cp.start()
    kf[0:8, :] = jnp.zeros((8, 128), F32)
    skt_v[...] = _dot_nt(eye, sk_ref[...])
    zs[0] = 0
    zs[1] = 0
    zs[2] = 1
    for cp in kv_copies(0):
        cp.wait()
    for cp in kv_copies(1):
        cp.start()
    kv_prep(0)
    xp_copy.wait()

    def pro(c, carry):
        nxt = jnp.minimum(c + 1, NB - 1)

        def dma_block(_, carry2):
            h_copy(c).wait()
            for cp in w_copies(c):
                cp.wait()

            @pl.when(c + 1 < NB)
            def _():
                for cp in kv_copies(c + 1):
                    cp.wait()
                h_copy(c + 1).start()
                for cp in w_copies(c + 1):
                    cp.start()

            @pl.when(c + 2 < NB)
            def _():
                for cp in kv_copies(c + 2):
                    cp.start()

            for cp in rest_copies(c):
                cp.start()
            return carry2

        jax.lax.fori_loop(0, zs[2], dma_block, 0)
        zw = zs[0]
        zr = zs[1]
        fixup(0, c)
        fwd_dft(c, zw)
        fixup(1, c)
        for n in range(6):
            qkv_tile(0, c, n)
            for p in range(n * 2, n * 2 + 2):
                mac(p, zw, zr)
        for n in range(4):
            qkv_tile(1, c, n)
            mac(12 + n, zw, zr)
        kv_prep(nxt)
        inv_dft(c, zr)
        for n in range(4, 6):
            qkv_tile(1, c, n)
        return carry

    with jax.named_scope("pro"):
        jax.lax.fori_loop(0, NB, pro, 0)
    for c in range(NB):
        for cp in rest_copies(c):
            cp.wait()

    mem_v[...] = mem0_ref[...]
    gw = gw_ref[...].astype(F32)

    def finalize(rows, b):
        xr = x_v[rows, :].astype(F32)
        g = jax.nn.sigmoid(jnp.sum(xr * gw, axis=-1, keepdims=True))
        a = xr * y_v[rows, :].astype(F32)
        out_ref[rows, :] = (g * a + (1.0 - g) * b).astype(BF16)

    def step(s, carry):
        xo = pl.multiple_of(PRO + RX * s, 8)
        wpos = pl.multiple_of((RX * s) % QCAP, 8)
        rpos = pl.multiple_of((SEG * s + QOFF) % QCAP, SEG)
        opos = pl.multiple_of(SEG * s, SEG)
        lhs = jnp.concatenate([mem_v[...], x_v[pl.ds(xo, RX), :]], axis=0)
        zpad = jnp.zeros((128 - 2 * (SEG + M), E), BF16)
        frows = pl.ds(pl.multiple_of(RX * s, 8), RX)
        NP = H // 2
        mem_qkv = {}
        probs = {}
        cats = {}

        def load(mat, hp):
            if not 0 <= hp < NP:
                return
            parts = [qkv_b[mat, hp, 0, pl.ds(rpos, SEG), :], qkv_b[mat, hp, 1, pl.ds(rpos, SEG), :],
                     mem_qkv[(hp, mat)]]
            if mat > 0:
                parts.append(zpad)
            cats[(mat, hp)] = jnp.concatenate(parts, axis=0)

        def stage_a(hp):
            for mat in range(3):
                mm = []
                for j in range(2):
                    w = pltpu.bitcast(wbuf[hp % 2][mat, hp // 2, j], BF16)
                    res = _dot(lhs, w)
                    qkv_b[mat, hp, j, pl.ds(wpos, RX), :] = res[M:].astype(BF16)
                    mm.append(res[:M])
                mem_qkv[(hp, mat)] = jnp.concatenate(mm, axis=0).astype(BF16)

        def stage_b(hp):
            if not 0 <= hp < NP:
                return
            sc = _dot_nt(cats[(0, hp)], cats[(1, hp)]) * scale
            fill = fill_ref[...]
            sc = jnp.where(fill == 0.0, sc, fill)
            mx = jnp.max(sc, axis=-1, keepdims=True)
            p = jnp.exp(sc - mx)
            l = jnp.sum(p, axis=-1, keepdims=True)
            r = pl.reciprocal(l, approx=True)
            r = r * (2.0 - l * r)
            probs[hp] = (p * r).astype(BF16)

        def stage_c(hp):
            if not 0 <= hp < NP:
                return
            o = _dot(probs[hp], cats[(2, hp)]).astype(BF16)
            for j in range(2):
                h = 2 * hp + j
                if h < HS:
                    o_b[pl.ds(opos, SEG), h * E:(h + 1) * E] = o[j * SEG:(j + 1) * SEG]
                else:
                    o_l[pl.ds(opos, SEG), (h - HS) * E:(h - HS + 1) * E] = o[j * SEG:(j + 1) * SEG]
                omem[:, h * E:(h + 1) * E] = o[2 * SEG + j * M:2 * SEG + (j + 1) * M]

        def oproj(j, late):
            if late:
                lo = jnp.concatenate([omem[:, HS * E:], o_l[frows, :]], axis=0)
                return _dot(lo, pltpu.bitcast(wo_v[j, HS * E // 2:, :], BF16))
            lo = jnp.concatenate([omem[:, :HS * E], o_b[frows, :]], axis=0)
            return _dot(lo, pltpu.bitcast(wo_v[j, :HS * E // 2, :], BF16))

        DB, DC = 1, 3
        outs = [None] * NB
        for t in range(NP + DC):
            load(0, t - DB)
            load(1, t - DB)
            load(2, t - DC)
            if t < NP:
                stage_a(t)
            else:
                for j in range(2 * (t - NP), 2 * (t - NP) + 2):
                    oacc[:, j * 128:(j + 1) * 128] = oproj(j, False)
            stage_b(t - DB)
            stage_c(t - DC)
        for j in range(2 * DC, NB):
            oacc[:, j * 128:(j + 1) * 128] = oproj(j, False)
        for j in range(NB):
            outs[j] = oacc[:, j * 128:(j + 1) * 128] + oproj(j, True)
        res = jnp.concatenate(outs, axis=1)
        mem_v[...] = res[:M].astype(BF16)
        finalize(frows, res[M:])
        return carry

    with jax.named_scope("main"):
        jax.lax.fori_loop(0, NSEG, step, 0)

    def epi_rows(rows):
        lo = jnp.concatenate([o_b[rows, :], o_l[rows, :]], axis=1)
        outs = [_dot(lo, pltpu.bitcast(wo_v[j], BF16)) for j in range(NB)]
        finalize(rows, jnp.concatenate(outs, axis=1))

    def epi(r, carry):
        epi_rows(pl.ds(pl.multiple_of(S - 512 + r * 64, 64), 64))
        return carry

    with jax.named_scope("epi"):
        jax.lax.fori_loop(0, 512 // 64, epi, 0)


@jax.jit
def _run(A_q, A_k, A_v, A_shift_k, A_ssm_k, A_ssm_D, B_mem0, B_Wq, B_Wk, B_Wv, B_Wo, gate_w):
    fwd, inv = _dft_tables()
    any_spec = pl.BlockSpec(memory_space=pl.ANY)
    vmem = pl.BlockSpec(memory_space=pltpu.VMEM)
    out = pl.pallas_call(
        _kernel,
        out_shape=jax.ShapeDtypeStruct((S, D), BF16),
        in_specs=[any_spec] * 8 + [vmem] * 7,
        out_specs=vmem,
        scratch_shapes=[
            pltpu.VMEM((S, D), BF16),
            pltpu.VMEM((PRO // 2, D), U32),
            pltpu.VMEM((NB, S, 128), BF16),
            pltpu.VMEM((NB, S, 128), BF16),
            pltpu.VMEM((NB, 128, S), BF16),
            pltpu.VMEM((3, H // 4, 2, D // 2, E), U32),
            pltpu.VMEM((3, H // 4, 2, D // 2, E), U32),
            pltpu.VMEM((NB, H * E // 2, 128), U32),
            pltpu.VMEM((S, D), BF16),
            pltpu.VMEM((3, H // 2, 2, QCAP, E), BF16),
            pltpu.VMEM((S, HS * E), BF16),
            pltpu.VMEM((S, HL * E), BF16),
            pltpu.VMEM((M, H * E), BF16),
            pltpu.VMEM((M, D), BF16),
            pltpu.VMEM((M + RX, D), F32),
            pltpu.VMEM((8, D), F32),
            pltpu.VMEM((S + 8, 128), F32),
            pltpu.VMEM((S, 128), BF16),
            pltpu.VMEM((1, NCH, 2 * C, 128), F32),
            pltpu.VMEM((1, NCH, 2 * C, 128), F32),
            pltpu.VMEM((1, NCH, 2 * C, 128), F32),
            pltpu.SMEM((3,), jnp.int32),
            pltpu.SemaphoreType.DMA((5,)),
        ],
        compiler_params=pltpu.CompilerParams(vmem_limit_bytes=120 * 2 ** 20, disable_bounds_checks=True),
    )(
        A_q.reshape(S, D), A_k.reshape(S, D), A_v.reshape(S, D), A_ssm_k,
        B_Wq.reshape(D // 2, 2, H, E), B_Wk.reshape(D // 2, 2, H, E), B_Wv.reshape(D // 2, 2, H, E),
        B_Wo.reshape(H * E, D),
        A_shift_k, A_ssm_D.reshape(1, D), gate_w.reshape(1, D), B_mem0.reshape(M, D),
        jnp.asarray(fwd, BF16), jnp.asarray(inv, BF16), jnp.asarray(_attn_fill()),
    )
    return out.reshape(1, S, D)


def pallas_gated_mix__ssm_conv_h3__memory_aug_recurrent_mem_tr__prompt_kernel(
    A_q, A_k, A_v, A_shift_k, A_ssm_k, A_ssm_D, B_x, B_mem0, B_Wq, B_Wk, B_Wv, B_Wo, B_seg_len, gate_w,
):
    del B_x
    if isinstance(B_seg_len, int):
        assert B_seg_len == SEG
    return _run(A_q, A_k, A_v, A_shift_k, A_ssm_k, A_ssm_D, B_mem0, B_Wq, B_Wk, B_Wv, B_Wo, gate_w)
```

```python
import functools
import math

import jax
import jax.numpy as jnp
import numpy as np
import jax.experimental.pallas as pl
import jax.experimental.pallas.tpu as pltpu

F32 = jnp.float32
BF16 = jnp.bfloat16
U32 = jnp.uint32

S = 2048
D = 1024
H = 32
E = 128
M = 8
SEG = 32
NSEG = S // SEG
RX = 24
PRO = S - RX * NSEG
QCAP = 576
QOFF = QCAP - PRO
HL = 8
HS = H - HL
C = 128
NCH = S // C
NB = D // 128
KS = 4
NEG = -1000000000.0


def _dft_tables():
    n = np.arange(C, dtype=np.float64)
    th = np.pi * (2.0 * np.arange(C, dtype=np.float64) + 1.0) / (2 * C)
    fwd = np.concatenate([np.cos(th[:, None] * n[None, :]), -np.sin(th[:, None] * n[None, :])], axis=0)
    inv = np.concatenate([np.cos(n[:, None] * th[None, :]), -np.sin(n[:, None] * th[None, :])], axis=1) / C
    return fwd.astype(np.float32), inv.astype(np.float32)


def _attn_fill():
    n = 2 * (SEG + M)
    head = np.array([0] * SEG + [1] * SEG + [0] * M + [1] * M)
    pos = np.concatenate([M + np.arange(SEG), M + np.arange(SEG), np.arange(M), np.arange(M)])
    fill = np.full((n, 128), -np.inf, np.float32)
    for i in range(n):
        for j in range(n):
            if head[i] == head[j]:
                ok = pos[i] < M or pos[i] >= pos[j]
                fill[i, j] = 0.0 if ok else NEG
    return fill


def _dot(a, b):
    return jnp.dot(a, b, preferred_element_type=F32)


def _dot_nt(a, b):
    return jax.lax.dot_general(a, b, (((1,), (1,)), ((), ())), preferred_element_type=F32)


def _kernel(x_hbm, k_hbm, v_hbm, h_hbm, wq_hbm, wk_hbm, wv_hbm, wo_hbm,
            sk_hbm, dd_hbm, gw_hbm, mem0_hbm, fwd_hbm, inv_hbm, fill_hbm,
            out_hbm,
            x_v, xp, k_v, v_v, h_v, w_even, w_odd, wo_v, y_v, qkv_b, o_b, o_l, omem, mem_v, oacc,
            kf, kvb, u_s, h_s, yf_s,
            out_v, fwd_ref, inv_ref, fill_ref, sk_ref, dd_ref, gw_ref, zs, sems, wsems):
    scale = E ** (-0.5)
    wbuf = (w_even, w_odd)

    w32 = [w.bitcast(U32) for w in (wq_hbm, wk_hbm, wv_hbm)]
    wo32 = wo_hbm.bitcast(U32)
    x32 = x_hbm.bitcast(U32)

    def lanes(c):
        return pl.ds(pl.multiple_of(c * 128, 128), 128)

    def w_copies(c, e, mat):
        return [pltpu.make_async_copy(w32[mat].at[:, par, 2 * c + e, :], wbuf[e].at[mat, c, par],
                                      wsems.at[(c % 2) * 6 + e * 3 + mat])
                for par in range(2)]

    def kv_copies(c):
        return [pltpu.make_async_copy(k_hbm.at[:, lanes(c)], k_v.at[c], sems.at[c % 2]),
                pltpu.make_async_copy(v_hbm.at[:, lanes(c)], v_v.at[c], sems.at[c % 2])]

    def h_copy(c):
        return pltpu.make_async_copy(h_hbm.at[lanes(c), :], h_v.at[c], sems.at[2 + c % 2])

    def rest_copies(c):
        rows = pl.ds(pl.multiple_of(c * (S // NB), S // NB), S // NB)
        return [pltpu.make_async_copy(wo32.at[:, lanes(c)], wo_v.at[c], sems.at[4]),
                pltpu.make_async_copy(x_hbm.at[rows, :], x_v.at[rows, :], sems.at[4])]

    xp_copy = pltpu.make_async_copy(x32.at[pl.ds(0, PRO // 2), :], xp, sems.at[5])
    small_copies = [pltpu.make_async_copy(src, dst, sems.at[6]) for src, dst in (
        (sk_hbm, sk_ref), (fwd_hbm, fwd_ref), (dd_hbm, dd_ref), (inv_hbm, inv_ref),
        (gw_hbm, gw_ref), (mem0_hbm, mem_v), (fill_hbm, fill_ref))]

    def out_copy(start, n):
        rows = pl.ds(start, n)
        return pltpu.make_async_copy(out_v.at[rows, :], out_hbm.at[rows, :], sems.at[7])

    def kv_prep(c):
        skt = sk_ref[:, lanes(c)].astype(F32)
        kf[8:8 + S, :] = k_v[c].astype(F32)
        for a in range(NCH):
            ks_ = kf[pl.ds(8 + a * C, C), :] * skt[0:1, :]
            for j in range(1, KS):
                ks_ = ks_ + kf[pl.ds(8 + a * C - j, C), :] * skt[j:j + 1, :]
            kvb[pl.ds(a * C, C), :] = (ks_ * v_v[c, pl.ds(a * C, C), :].astype(F32)).astype(BF16)

    def row_of(ref, c):
        t = ref[...].astype(F32)
        sel = jax.lax.broadcasted_iota(jnp.int32, (NB, 128), 0) == c
        return jnp.sum(jnp.where(sel, t, 0.0), axis=0, keepdims=True)

    def fwd_dft(c, zw):
        sgn = (1 - 2 * (jax.lax.broadcasted_iota(jnp.int32, (C, 128), 0) % 2)).astype(F32)
        hprev = None
        for a in range(NCH):
            u_s[zw, a] = _dot(fwd_ref[...], kvb[pl.ds(a * C, C), :])
            hf = _dot_nt(fwd_ref[...], h_v[c, :, pl.ds(a * C, C)])
            if hprev is None:
                h_s[zw, a, 0:C, :] = hf[0:C] + row_of(dd_ref, c)
                h_s[zw, a, C:, :] = hf[C:]
            else:
                h_s[zw, a, 0:C, :] = hf[0:C] - sgn * hprev[C:]
                h_s[zw, a, C:, :] = hf[C:] + sgn * hprev[0:C]
            hprev = hf

    def mac(p, zw, zr):
        re = pl.ds(p * 8, 8)
        im = pl.ds(C + p * 8, 8)
        AB = 4
        for a0 in range(0, NCH, AB):
            yr = [None] * AB
            yi = [None] * AB
            for m in range(a0 + AB):
                hr = h_s[zr, m, re, :]
                hi = h_s[zr, m, im, :]
                for i in range(AB):
                    t = a0 + i - m
                    if t < 0:
                        continue
                    ur = u_s[zr, t, re, :]
                    ui = u_s[zr, t, im, :]
                    tr = hr * ur - hi * ui
                    ti = hr * ui + hi * ur
                    yr[i] = tr if yr[i] is None else yr[i] + tr
                    yi[i] = ti if yi[i] is None else yi[i] + ti
            for i in range(AB):
                yf_s[zw, a0 + i, re, :] = yr[i]
                yf_s[zw, a0 + i, im, :] = yi[i]

    def inv_dft(c, zr):
        for a in range(NCH):
            y_v[pl.ds(a * C, C), lanes(c)] = _dot(inv_ref[...], yf_s[zr, a].astype(BF16)).astype(BF16)

    def fixup(e, c, mat):
        a = wbuf[e][mat, c, 0]
        b = wbuf[e][mat, c, 1]
        wbuf[e][mat, c, 0] = (a & U32(0xFFFF)) | (b << 16)
        wbuf[e][mat, c, 1] = (a >> 16) | (b & U32(0xFFFF0000))

    RB = 128

    def qkv_tile(e, c, n):
        mat, j = n // 2, n % 2
        for r in range(PRO // RB):
            w = pltpu.bitcast(wbuf[e][mat, c, j], BF16)
            xr = pltpu.bitcast(xp[pl.ds(r * RB // 2, RB // 2), :], BF16)
            qkv_b[mat, 2 * c + e, j, pl.ds(QOFF + r * RB, RB), :] = _dot(xr, w).astype(BF16)

    def start_w(c):
        for e in range(2):
            for mat in range(3):
                for cp in w_copies(c, e, mat):
                    cp.start()

    for cp in kv_copies(0) + small_copies:
        cp.start()
    h_copy(0).start()
    xp_copy.start()
    start_w(0)
    for cp in kv_copies(1):
        cp.start()
    kf[0:8, :] = jnp.zeros((8, 128), F32)
    zs[0] = 0
    zs[1] = 0
    zs[2] = 1
    for cp in kv_copies(0) + small_copies:
        cp.wait()
    kv_prep(0)
    xp_copy.wait()

    def pro(c, carry):
        nxt = jnp.minimum(c + 1, NB - 1)

        def dma_block(_, carry2):
            h_copy(c).wait()
            for e in range(2):
                for mat in range(3):
                    for cp in w_copies(c, e, mat):
                        cp.wait()

            @pl.when(c + 1 < NB)
            def _():
                for cp in kv_copies(c + 1):
                    cp.wait()
                h_copy(c + 1).start()
                start_w(c + 1)

            @pl.when(c + 2 < NB)
            def _():
                for cp in kv_copies(c + 2):
                    cp.start()

            for cp in rest_copies(c):
                cp.start()
            return carry2

        jax.lax.fori_loop(0, zs[2], dma_block, 0)
        zw = zs[0]
        zr = zs[1]
        fwd_dft(c, zw)

        for n in range(6):
            if n % 2 == 0:
                fixup(0, c, n // 2)
            qkv_tile(0, c, n)
            for p in range(n * 2, n * 2 + 2):
                mac(p, zw, zr)
        for n in range(4):
            if n % 2 == 0:
                fixup(1, c, n // 2)
            qkv_tile(1, c, n)
            mac(12 + n, zw, zr)

        kv_prep(nxt)
        fixup(1, c, 2)
        inv_dft(c, zr)
        for n in range(4, 6):
            qkv_tile(1, c, n)
        return carry

    with jax.named_scope("pro"):
        jax.lax.fori_loop(0, NB, pro, 0)
    for c in range(NB):
        for cp in rest_copies(c):
            cp.wait()

    gwt = gw_ref[...].astype(F32)
    gw = jnp.concatenate([gwt[j:j + 1, :] for j in range(NB)], axis=1)

    def finalize(rows, b):
        xr = x_v[rows, :].astype(F32)
        g = jax.nn.sigmoid(jnp.sum(xr * gw, axis=-1, keepdims=True))
        a = xr * y_v[rows, :].astype(F32)
        out_v[rows, :] = (g * a + (1.0 - g) * b).astype(BF16)

    def step(s, carry):
        xo = pl.multiple_of(PRO + RX * s, 8)
        wpos = pl.multiple_of((RX * s) % QCAP, 8)
        rpos = pl.multiple_of((SEG * s + QOFF) % QCAP, SEG)
        opos = pl.multiple_of(SEG * s, SEG)
        lhs = jnp.concatenate([mem_v[...], x_v[pl.ds(xo, RX), :]], axis=0)
        zpad = jnp.zeros((128 - 2 * (SEG + M), E), BF16)
        frows = pl.ds(pl.multiple_of(RX * s, 8), RX)
        NP = H // 2


        mem_qkv = {}
        probs = {}
        cats = {}

        def load(mat, hp):
            if not 0 <= hp < NP:
                return
            parts = [qkv_b[mat, hp, 0, pl.ds(rpos, SEG), :], qkv_b[mat, hp, 1, pl.ds(rpos, SEG), :],
                     mem_qkv[(hp, mat)]]
            if mat > 0:
                parts.append(zpad)
            cats[(mat, hp)] = jnp.concatenate(parts, axis=0)

        def stage_a(hp):
            for mat in range(3):
                mm = []
                for j in range(2):
                    w = pltpu.bitcast(wbuf[hp % 2][mat, hp // 2, j], BF16)
                    res = _dot(lhs, w)
                    qkv_b[mat, hp, j, pl.ds(wpos, RX), :] = res[M:].astype(BF16)
                    mm.append(res[:M])
                mem_qkv[(hp, mat)] = jnp.concatenate(mm, axis=0).astype(BF16)

        def stage_b(hp):
            if not 0 <= hp < NP:
                return
            sc = _dot_nt(cats[(0, hp)], cats[(1, hp)]) * scale
            fill = fill_ref[...]
            sc = jnp.where(fill == 0.0, sc, fill)
            mx = jnp.max(sc, axis=-1, keepdims=True)
            p = jnp.exp(sc - mx)
            l = jnp.sum(p, axis=-1, keepdims=True)
            r = pl.reciprocal(l, approx=True)
            r = r * (2.0 - l * r)
            probs[hp] = (p * r).astype(BF16)

        def stage_c(hp):
            if not 0 <= hp < NP:
                return
            o = _dot(probs[hp], cats[(2, hp)]).astype(BF16)
            for j in range(2):
                h = 2 * hp + j
                if h < HS:
                    o_b[pl.ds(opos, SEG), h * E:(h + 1) * E] = o[j * SEG:(j + 1) * SEG]
                else:
                    o_l[pl.ds(opos, SEG), (h - HS) * E:(h - HS + 1) * E] = o[j * SEG:(j + 1) * SEG]
                omem[:, h * E:(h + 1) * E] = o[2 * SEG + j * M:2 * SEG + (j + 1) * M]

        def oproj(j, late):
            if late:
                lo = jnp.concatenate([omem[:, HS * E:], o_l[frows, :]], axis=0)
                return _dot(lo, pltpu.bitcast(wo_v[j, HS * E // 2:, :], BF16))
            lo = jnp.concatenate([omem[:, :HS * E], o_b[frows, :]], axis=0)
            return _dot(lo, pltpu.bitcast(wo_v[j, :HS * E // 2, :], BF16))

        DB, DC = 1, 3
        outs = [None] * NB
        for t in range(NP + DC):
            load(0, t - DB)
            load(1, t - DB)
            load(2, t - DC)
            if t < NP:
                stage_a(t)
            else:
                for j in range(2 * (t - NP), 2 * (t - NP) + 2):
                    oacc[:, j * 128:(j + 1) * 128] = oproj(j, False)
            stage_b(t - DB)
            stage_c(t - DC)
        for j in range(2 * DC, NB):
            oacc[:, j * 128:(j + 1) * 128] = oproj(j, False)
        for j in range(NB):
            outs[j] = oacc[:, j * 128:(j + 1) * 128] + oproj(j, True)
        res = jnp.concatenate(outs, axis=1)
        mem_v[...] = res[:M].astype(BF16)
        finalize(frows, res[M:])
        return carry

    with jax.named_scope("main"):
        jax.lax.fori_loop(0, NSEG, step, 0)

    def epi_rows(rows):
        lo = jnp.concatenate([o_b[rows, :], o_l[rows, :]], axis=1)
        outs = [_dot(lo, pltpu.bitcast(wo_v[j], BF16)) for j in range(NB)]
        finalize(rows, jnp.concatenate(outs, axis=1))

    EB = 64

    def epi(r, carry):
        r0 = pl.multiple_of(S - PRO + r * EB, EB)

        @pl.when(r == PRO // EB - 1)
        def _():
            out_copy(S - PRO, PRO - EB).start()

        epi_rows(pl.ds(r0, EB))
        return carry

    with jax.named_scope("epi"):
        out_copy(0, S - PRO).start()
        jax.lax.fori_loop(0, PRO // EB, epi, 0)
    out_copy(S - EB, EB).start()
    out_copy(0, S).wait()


@jax.jit
def _run(A_q, A_k, A_v, A_shift_k, A_ssm_k, A_ssm_D, B_mem0, B_Wq, B_Wk, B_Wv, B_Wo, gate_w):
    fwd, inv = _dft_tables()
    any_spec = pl.BlockSpec(memory_space=pl.ANY)
    out = pl.pallas_call(
        _kernel,
        out_shape=jax.ShapeDtypeStruct((S, D), BF16),
        in_specs=[any_spec] * 15,
        out_specs=any_spec,
        scratch_shapes=[
            pltpu.VMEM((S, D), BF16),
            pltpu.VMEM((PRO // 2, D), U32),
            pltpu.VMEM((NB, S, 128), BF16),
            pltpu.VMEM((NB, S, 128), BF16),
            pltpu.VMEM((NB, 128, S), BF16),
            pltpu.VMEM((3, H // 4, 2, D // 2, E), U32),
            pltpu.VMEM((3, H // 4, 2, D // 2, E), U32),
            pltpu.VMEM((NB, H * E // 2, 128), U32),
            pltpu.VMEM((S, D), BF16),
            pltpu.VMEM((3, H // 2, 2, QCAP, E), BF16),
            pltpu.VMEM((S, HS * E), BF16),
            pltpu.VMEM((S, HL * E), BF16),
            pltpu.VMEM((M, H * E), BF16),
            pltpu.VMEM((M, D), BF16),
            pltpu.VMEM((M + RX, D), F32),
            pltpu.VMEM((S + 32, 128), F32),
            pltpu.VMEM((S, 128), BF16),
            pltpu.VMEM((1, NCH, 2 * C, 128), F32),
            pltpu.VMEM((1, NCH, 2 * C, 128), F32),
            pltpu.VMEM((1, NCH, 2 * C, 128), F32),
            pltpu.VMEM((S, D), BF16),
            pltpu.VMEM((2 * C, C), BF16),
            pltpu.VMEM((C, 2 * C), BF16),
            pltpu.VMEM((2 * (SEG + M), 128), F32),
            pltpu.VMEM((KS, D), BF16),
            pltpu.VMEM((NB, 128), BF16),
            pltpu.VMEM((NB, 128), BF16),
            pltpu.SMEM((3,), jnp.int32),
            pltpu.SemaphoreType.DMA((8,)),
            pltpu.SemaphoreType.DMA((12,)),
        ],
        compiler_params=pltpu.CompilerParams(vmem_limit_bytes=120 * 2 ** 20, disable_bounds_checks=True),
    )(
        A_q.reshape(S, D), A_k.reshape(S, D), A_v.reshape(S, D), A_ssm_k,
        B_Wq.reshape(D // 2, 2, H, E), B_Wk.reshape(D // 2, 2, H, E), B_Wv.reshape(D // 2, 2, H, E),
        B_Wo.reshape(H * E, D),
        A_shift_k.T, A_ssm_D.reshape(NB, 128), gate_w.reshape(NB, 128), B_mem0.reshape(M, D),
        jnp.asarray(fwd, BF16), jnp.asarray(inv, BF16), jnp.asarray(_attn_fill()),
    )
    return out.reshape(1, S, D)


def pallas_gated_mix__ssm_conv_h3__memory_aug_recurrent_mem_tr__prompt_kernel(
    A_q, A_k, A_v, A_shift_k, A_ssm_k, A_ssm_D, B_x, B_mem0, B_Wq, B_Wk, B_Wv, B_Wo, B_seg_len, gate_w,
):
    del B_x
    if isinstance(B_seg_len, int):
        assert B_seg_len == SEG
    return _run(A_q, A_k, A_v, A_shift_k, A_ssm_k, A_ssm_D, B_mem0, B_Wq, B_Wk, B_Wv, B_Wo, gate_w)
```

```python
import functools
import math

import jax
import jax.numpy as jnp
import numpy as np
import jax.experimental.pallas as pl
import jax.experimental.pallas.tpu as pltpu

F32 = jnp.float32
BF16 = jnp.bfloat16
U32 = jnp.uint32

S = 2048
D = 1024
H = 32
E = 128
M = 8
SEG = 32
NSEG = S // SEG
RX = 24
PRO = S - RX * NSEG
QCAP = 576
QOFF = QCAP - PRO
HL = 8
HS = H - HL
UNROLL = 4
C = 128
NCH = S // C
NB = D // 128
KS = 4
NEG = -1000000000.0


def _dft_tables():
    n = np.arange(C, dtype=np.float64)
    th = np.pi * (2.0 * np.arange(C, dtype=np.float64) + 1.0) / (2 * C)
    fwd = np.concatenate([np.cos(th[:, None] * n[None, :]), -np.sin(th[:, None] * n[None, :])], axis=0)
    inv = np.concatenate([np.cos(n[:, None] * th[None, :]), -np.sin(n[:, None] * th[None, :])], axis=1) / C
    return fwd.astype(np.float32), inv.astype(np.float32)


def _attn_fill():
    n = 2 * (SEG + M)
    head = np.array([0] * SEG + [1] * SEG + [0] * M + [1] * M)
    pos = np.concatenate([M + np.arange(SEG), M + np.arange(SEG), np.arange(M), np.arange(M)])
    fill = np.full((n, 128), -np.inf, np.float32)
    for i in range(n):
        for j in range(n):
            if head[i] == head[j]:
                ok = pos[i] < M or pos[i] >= pos[j]
                fill[i, j] = 0.0 if ok else NEG
    return fill


def _dot(a, b):
    return jnp.dot(a, b, preferred_element_type=F32)


def _dot_nt(a, b):
    return jax.lax.dot_general(a, b, (((1,), (1,)), ((), ())), preferred_element_type=F32)


def _kernel(x_hbm, k_hbm, v_hbm, h_hbm, wq_hbm, wk_hbm, wv_hbm, wo_hbm,
            sk_hbm, dd_hbm, gw_hbm, mem0_hbm, fwd_hbm, inv_hbm, fill_hbm,
            out_hbm,
            x_v, xp, k_v, v_v, h_v, w_even, w_odd, wo_v, y_v, qkv_b, o_b, o_l, omem, mem_v, oacc, qacc,
            kf, kvb, u_s, h_s, yf_s,
            out_v, fwd_ref, inv_ref, fill_ref, sk_ref, dd_ref, gw_ref, zs, sems, wsems):
    scale = E ** (-0.5)
    wbuf = (w_even, w_odd)

    w32 = [w.bitcast(U32) for w in (wq_hbm, wk_hbm, wv_hbm)]
    wo32 = wo_hbm.bitcast(U32)
    x32 = x_hbm.bitcast(U32)

    def lanes(c):
        return pl.ds(pl.multiple_of(c * 128, 128), 128)

    def w_copies(c, e, mat):
        return [pltpu.make_async_copy(w32[mat].at[:, par, 2 * c + e, :], wbuf[e].at[mat, c, par],
                                      wsems.at[(c % 2) * 6 + e * 3 + mat])
                for par in range(2)]

    def kv_copies(c):
        return [pltpu.make_async_copy(k_hbm.at[:, lanes(c)], k_v.at[c], sems.at[c % 2]),
                pltpu.make_async_copy(v_hbm.at[:, lanes(c)], v_v.at[c], sems.at[c % 2])]

    def h_copy(c):
        return pltpu.make_async_copy(h_hbm.at[lanes(c), :], h_v.at[c], sems.at[2 + c % 2])

    def rest_copies(c):
        rows = pl.ds(pl.multiple_of(c * (S // NB), S // NB), S // NB)
        return [pltpu.make_async_copy(wo32.at[:, lanes(c)], wo_v.at[c], sems.at[4]),
                pltpu.make_async_copy(x_hbm.at[rows, :], x_v.at[rows, :], sems.at[4])]

    xp_copy = pltpu.make_async_copy(x32.at[pl.ds(0, PRO // 2), :], xp, sems.at[5])
    small_copies = [pltpu.make_async_copy(src, dst, sems.at[6]) for src, dst in (
        (sk_hbm, sk_ref), (fwd_hbm, fwd_ref), (dd_hbm, dd_ref), (inv_hbm, inv_ref),
        (gw_hbm, gw_ref), (mem0_hbm, mem_v), (fill_hbm, fill_ref))]

    def out_copy(start, n):
        rows = pl.ds(start, n)
        return pltpu.make_async_copy(out_v.at[rows, :], out_hbm.at[rows, :], sems.at[7])

    def kv_prep(c):
        skt = sk_ref[:, lanes(c)].astype(F32)
        kf[8:8 + S, :] = k_v[c].astype(F32)
        for a in range(NCH):
            ks_ = kf[pl.ds(8 + a * C, C), :] * skt[0:1, :]
            for j in range(1, KS):
                ks_ = ks_ + kf[pl.ds(8 + a * C - j, C), :] * skt[j:j + 1, :]
            kvb[pl.ds(a * C, C), :] = (ks_ * v_v[c, pl.ds(a * C, C), :].astype(F32)).astype(BF16)

    def row_of(ref, c):
        t = ref[...].astype(F32)
        sel = jax.lax.broadcasted_iota(jnp.int32, (NB, 128), 0) == c
        return jnp.sum(jnp.where(sel, t, 0.0), axis=0, keepdims=True)

    def fwd_dft(c, zw):
        sgn = (1 - 2 * (jax.lax.broadcasted_iota(jnp.int32, (C, 128), 0) % 2)).astype(F32)
        hprev = None
        for a in range(NCH):
            u_s[zw, a] = _dot(fwd_ref[...], kvb[pl.ds(a * C, C), :])
            hf = _dot_nt(fwd_ref[...], h_v[c, :, pl.ds(a * C, C)])
            if hprev is None:
                h_s[zw, a, 0:C, :] = hf[0:C] + row_of(dd_ref, c)
                h_s[zw, a, C:, :] = hf[C:]
            else:
                h_s[zw, a, 0:C, :] = hf[0:C] - sgn * hprev[C:]
                h_s[zw, a, C:, :] = hf[C:] + sgn * hprev[0:C]
            hprev = hf

    def mac(p, zw, zr):
        re = pl.ds(p * 8, 8)
        im = pl.ds(C + p * 8, 8)
        AB = 4
        for a0 in range(0, NCH, AB):
            yr = [None] * AB
            yi = [None] * AB
            for m in range(a0 + AB):
                hr = h_s[zr, m, re, :]
                hi = h_s[zr, m, im, :]
                for i in range(AB):
                    t = a0 + i - m
                    if t < 0:
                        continue
                    ur = u_s[zr, t, re, :]
                    ui = u_s[zr, t, im, :]
                    tr = hr * ur - hi * ui
                    ti = hr * ui + hi * ur
                    yr[i] = tr if yr[i] is None else yr[i] + tr
                    yi[i] = ti if yi[i] is None else yi[i] + ti
            for i in range(AB):
                yf_s[zw, a0 + i, re, :] = yr[i]
                yf_s[zw, a0 + i, im, :] = yi[i]

    def inv_dft(c, zr):
        for a in range(NCH):
            y_v[pl.ds(a * C, C), lanes(c)] = _dot(inv_ref[...], yf_s[zr, a].astype(BF16)).astype(BF16)

    def fixup(e, c, mat):
        a = wbuf[e][mat, c, 0]
        b = wbuf[e][mat, c, 1]
        wbuf[e][mat, c, 0] = (a & U32(0xFFFF)) | (b << 16)
        wbuf[e][mat, c, 1] = (a >> 16) | (b & U32(0xFFFF0000))

    RB = 128

    def qkv_tile(e, c, n):
        mat, j = n // 2, n % 2
        for r in range(PRO // RB):
            w = pltpu.bitcast(wbuf[e][mat, c, j], BF16)
            xr = pltpu.bitcast(xp[pl.ds(r * RB // 2, RB // 2), :], BF16)
            qkv_b[mat, 2 * c + e, j, pl.ds(QOFF + r * RB, RB), :] = _dot(xr, w).astype(BF16)

    def start_w(c):
        for e in range(2):
            for mat in range(3):
                for cp in w_copies(c, e, mat):
                    cp.start()

    for cp in kv_copies(0) + small_copies:
        cp.start()
    h_copy(0).start()
    xp_copy.start()
    start_w(0)
    for cp in kv_copies(1):
        cp.start()
    kf[0:8, :] = jnp.zeros((8, 128), F32)
    zs[0] = 0
    zs[1] = 0
    zs[2] = 1
    for cp in kv_copies(0) + small_copies:
        cp.wait()
    kv_prep(0)
    xp_copy.wait()

    def pro(c, carry):
        nxt = jnp.minimum(c + 1, NB - 1)

        def dma_block(_, carry2):
            h_copy(c).wait()
            for e in range(2):
                for mat in range(3):
                    for cp in w_copies(c, e, mat):
                        cp.wait()

            @pl.when(c + 1 < NB)
            def _():
                for cp in kv_copies(c + 1):
                    cp.wait()
                h_copy(c + 1).start()
                start_w(c + 1)

            @pl.when(c + 2 < NB)
            def _():
                for cp in kv_copies(c + 2):
                    cp.start()

            for cp in rest_copies(c):
                cp.start()
            return carry2

        jax.lax.fori_loop(0, zs[2], dma_block, 0)
        zw = zs[0]
        zr = zs[1]
        fwd_dft(c, zw)

        for n in range(6):
            if n % 2 == 0:
                fixup(0, c, n // 2)
            qkv_tile(0, c, n)
            for p in range(n * 2, n * 2 + 2):
                mac(p, zw, zr)
        for n in range(4):
            if n % 2 == 0:
                fixup(1, c, n // 2)
            qkv_tile(1, c, n)
            mac(12 + n, zw, zr)

        kv_prep(nxt)
        fixup(1, c, 2)
        inv_dft(c, zr)
        for n in range(4, 6):
            qkv_tile(1, c, n)
        return carry

    with jax.named_scope("pro"):
        jax.lax.fori_loop(0, NB, pro, 0)
    for c in range(NB):
        for cp in rest_copies(c):
            cp.wait()

    gwt = gw_ref[...].astype(F32)
    gw = jnp.concatenate([gwt[j:j + 1, :] for j in range(NB)], axis=1)

    def finalize(rows, b):
        xr = x_v[rows, :].astype(F32)
        g = jax.nn.sigmoid(jnp.sum(xr * gw, axis=-1, keepdims=True))
        a = xr * y_v[rows, :].astype(F32)
        out_v[rows, :] = (g * a + (1.0 - g) * b).astype(BF16)

    def step(s, mem, split_first):
        xo = pl.multiple_of(PRO + RX * s, 8)
        wpos = pl.multiple_of((RX * s) % QCAP, 8)
        rpos = pl.multiple_of((SEG * s + QOFF) % QCAP, SEG)
        opos = pl.multiple_of(SEG * s, SEG)
        lhs = jnp.concatenate([mem, x_v[pl.ds(xo, RX), :]], axis=0)
        zpad = jnp.zeros((128 - 2 * (SEG + M), E), BF16)
        frows = pl.ds(pl.multiple_of(RX * s, 8), RX)
        NP = H // 2


        mem_qkv = {}
        probs = {}
        cats = {}

        def load(mat, hp):
            if not 0 <= hp < NP:
                return
            parts = [qkv_b[mat, hp, 0, pl.ds(rpos, SEG), :], qkv_b[mat, hp, 1, pl.ds(rpos, SEG), :],
                     mem_qkv[(hp, mat)]]
            if mat > 0:
                parts.append(zpad)
            cats[(mat, hp)] = jnp.concatenate(parts, axis=0)

        def stage_a(hp):
            KH = D // 2
            split = split_first and hp == 0
            if split:
                for mat in range(3):
                    for j in range(2):
                        w = pltpu.bitcast(wbuf[hp % 2][mat, hp // 2, j, :KH // 2, :], BF16)
                        qacc[2 * mat + j] = _dot(lhs[:, :KH], w)
            for mat in range(3):
                mm = []
                for j in range(2):
                    if split:
                        w = pltpu.bitcast(wbuf[hp % 2][mat, hp // 2, j, KH // 2:, :], BF16)
                        res = qacc[2 * mat + j] + _dot(lhs[:, KH:], w)
                    else:
                        res = _dot(lhs, pltpu.bitcast(wbuf[hp % 2][mat, hp // 2, j], BF16))
                    qkv_b[mat, hp, j, pl.ds(wpos, RX), :] = res[M:].astype(BF16)
                    mm.append(res[:M])
                mem_qkv[(hp, mat)] = jnp.concatenate(mm, axis=0).astype(BF16)

        def stage_b(hp):
            if not 0 <= hp < NP:
                return
            sc = _dot_nt(cats[(0, hp)], cats[(1, hp)]) * scale
            fill = fill_ref[...]
            sc = jnp.where(fill == 0.0, sc, fill)
            mx = jnp.max(sc, axis=-1, keepdims=True)
            p = jnp.exp(sc - mx)
            l = jnp.sum(p, axis=-1, keepdims=True)
            r = pl.reciprocal(l, approx=True)
            r = r * (2.0 - l * r)
            probs[hp] = (p.astype(BF16), r)

        def stage_c(hp):
            if not 0 <= hp < NP:
                return
            o = (_dot(probs[hp][0], cats[(2, hp)]) * probs[hp][1]).astype(BF16)
            for j in range(2):
                h = 2 * hp + j
                if h < HS:
                    o_b[pl.ds(opos, SEG), h * E:(h + 1) * E] = o[j * SEG:(j + 1) * SEG]
                else:
                    o_l[pl.ds(opos, SEG), (h - HS) * E:(h - HS + 1) * E] = o[j * SEG:(j + 1) * SEG]
                omem[:, h * E:(h + 1) * E] = o[2 * SEG + j * M:2 * SEG + (j + 1) * M]

        def oproj(j, late):
            if late:
                lo = jnp.concatenate([omem[:, HS * E:], o_l[frows, :]], axis=0)
                return _dot(lo, pltpu.bitcast(wo_v[j, HS * E // 2:, :], BF16))
            lo = jnp.concatenate([omem[:, :HS * E], o_b[frows, :]], axis=0)
            return _dot(lo, pltpu.bitcast(wo_v[j, :HS * E // 2, :], BF16))

        DB, DC = 1, 2
        outs = [None] * NB
        for t in range(NP + DC):
            load(0, t - DB)
            load(1, t - DB)
            load(2, t - DC)
            if t < NP:
                stage_a(t)
            else:
                for j in range(2 * (t - NP), 2 * (t - NP) + 2):
                    oacc[:, j * 128:(j + 1) * 128] = oproj(j, False)
            stage_b(t - DB)
            stage_c(t - DC)
        for j in range(2 * DC, NB):
            oacc[:, j * 128:(j + 1) * 128] = oproj(j, False)
        for j in range(NB):
            outs[j] = oacc[:, j * 128:(j + 1) * 128] + oproj(j, True)
        res = jnp.concatenate(outs, axis=1)
        finalize(frows, res[M:])
        return res[:M].astype(BF16)

    def steps(i, carry):
        mem = mem_v[...]
        for u in range(UNROLL):
            mem = step(i * UNROLL + u, mem, u > 0)
        mem_v[...] = mem
        return carry

    with jax.named_scope("main"):
        jax.lax.fori_loop(0, NSEG // UNROLL, steps, 0)

    def epi_rows(rows):
        lo = jnp.concatenate([o_b[rows, :], o_l[rows, :]], axis=1)
        outs = [_dot(lo, pltpu.bitcast(wo_v[j], BF16)) for j in range(NB)]
        finalize(rows, jnp.concatenate(outs, axis=1))

    EB = 128

    def epi(r, carry):
        r0 = pl.multiple_of(S - PRO + r * EB, EB)

        @pl.when(r == PRO // EB - 1)
        def _():
            out_copy(S - PRO, PRO - EB).start()

        epi_rows(pl.ds(r0, EB))
        return carry

    with jax.named_scope("epi"):
        out_copy(0, S - PRO).start()
        jax.lax.fori_loop(0, PRO // EB, epi, 0)
    out_copy(S - EB, EB).start()
    out_copy(0, S).wait()


@jax.jit
def _run(A_q, A_k, A_v, A_shift_k, A_ssm_k, A_ssm_D, B_mem0, B_Wq, B_Wk, B_Wv, B_Wo, gate_w):
    fwd, inv = _dft_tables()
    any_spec = pl.BlockSpec(memory_space=pl.ANY)
    out = pl.pallas_call(
        _kernel,
        out_shape=jax.ShapeDtypeStruct((S, D), BF16),
        in_specs=[any_spec] * 15,
        out_specs=any_spec,
        scratch_shapes=[
            pltpu.VMEM((S, D), BF16),
            pltpu.VMEM((PRO // 2, D), U32),
            pltpu.VMEM((NB, S, 128), BF16),
            pltpu.VMEM((NB, S, 128), BF16),
            pltpu.VMEM((NB, 128, S), BF16),
            pltpu.VMEM((3, H // 4, 2, D // 2, E), U32),
            pltpu.VMEM((3, H // 4, 2, D // 2, E), U32),
            pltpu.VMEM((NB, H * E // 2, 128), U32),
            pltpu.VMEM((S, D), BF16),
            pltpu.VMEM((3, H // 2, 2, QCAP, E), BF16),
            pltpu.VMEM((S, HS * E), BF16),
            pltpu.VMEM((S, HL * E), BF16),
            pltpu.VMEM((M, H * E), BF16),
            pltpu.VMEM((M, D), BF16),
            pltpu.VMEM((M + RX, D), F32),
            pltpu.VMEM((6, M + RX, E), F32),
            pltpu.VMEM((S + 32, 128), F32),
            pltpu.VMEM((S, 128), BF16),
            pltpu.VMEM((1, NCH, 2 * C, 128), F32),
            pltpu.VMEM((1, NCH, 2 * C, 128), F32),
            pltpu.VMEM((1, NCH, 2 * C, 128), F32),
            pltpu.VMEM((S, D), BF16),
            pltpu.VMEM((2 * C, C), BF16),
            pltpu.VMEM((C, 2 * C), BF16),
            pltpu.VMEM((2 * (SEG + M), 128), F32),
            pltpu.VMEM((KS, D), BF16),
            pltpu.VMEM((NB, 128), BF16),
            pltpu.VMEM((NB, 128), BF16),
            pltpu.SMEM((3,), jnp.int32),
            pltpu.SemaphoreType.DMA((8,)),
            pltpu.SemaphoreType.DMA((12,)),
        ],
        compiler_params=pltpu.CompilerParams(vmem_limit_bytes=120 * 2 ** 20, disable_bounds_checks=True),
    )(
        A_q.reshape(S, D), A_k.reshape(S, D), A_v.reshape(S, D), A_ssm_k,
        B_Wq.reshape(D // 2, 2, H, E), B_Wk.reshape(D // 2, 2, H, E), B_Wv.reshape(D // 2, 2, H, E),
        B_Wo.reshape(H * E, D),
        A_shift_k.T, A_ssm_D.reshape(NB, 128), gate_w.reshape(NB, 128), B_mem0.reshape(M, D),
        jnp.asarray(fwd, BF16), jnp.asarray(inv, BF16), jnp.asarray(_attn_fill()),
    )
    return out.reshape(1, S, D)


def pallas_gated_mix__ssm_conv_h3__memory_aug_recurrent_mem_tr__prompt_kernel(
    A_q, A_k, A_v, A_shift_k, A_ssm_k, A_ssm_D, B_x, B_mem0, B_Wq, B_Wk, B_Wv, B_Wo, B_seg_len, gate_w,
):
    del B_x
    if isinstance(B_seg_len, int):
        assert B_seg_len == SEG
    return _run(A_q, A_k, A_v, A_shift_k, A_ssm_k, A_ssm_D, B_mem0, B_Wq, B_Wk, B_Wv, B_Wo, gate_w)
```

```python
import functools
import math

import jax
import jax.numpy as jnp
import numpy as np
import jax.experimental.pallas as pl
import jax.experimental.pallas.tpu as pltpu

F32 = jnp.float32
BF16 = jnp.bfloat16
U32 = jnp.uint32

S = 2048
D = 1024
H = 32
E = 128
M = 8
SEG = 32
NSEG = S // SEG
RX = 24
PRO = S - RX * NSEG
QCAP = 576
QOFF = QCAP - PRO
HL = 8
HS = H - HL
UNROLL = 4
C = 128
NCH = S // C
NB = D // 128
KS = 4
NEG = -1000000000.0


def _dft_tables():
    n = np.arange(C, dtype=np.float64)
    th = np.pi * (2.0 * np.arange(C, dtype=np.float64) + 1.0) / (2 * C)
    fwd = np.concatenate([np.cos(th[:, None] * n[None, :]), -np.sin(th[:, None] * n[None, :])], axis=0)
    inv = np.concatenate([np.cos(n[:, None] * th[None, :]), -np.sin(n[:, None] * th[None, :])], axis=1) / C
    return fwd.astype(np.float32), inv.astype(np.float32)


def _attn_fill():
    n = 2 * (SEG + M)
    head = np.array([0] * SEG + [1] * SEG + [0] * M + [1] * M)
    pos = np.concatenate([M + np.arange(SEG), M + np.arange(SEG), np.arange(M), np.arange(M)])
    fill = np.full((n, 128), -np.inf, np.float32)
    for i in range(n):
        for j in range(n):
            if head[i] == head[j]:
                ok = pos[i] < M or pos[i] >= pos[j]
                fill[i, j] = 0.0 if ok else NEG
    return fill


def _dot(a, b):
    return jnp.dot(a, b, preferred_element_type=F32)


def _dot_nt(a, b):
    return jax.lax.dot_general(a, b, (((1,), (1,)), ((), ())), preferred_element_type=F32)


def _kernel(x_hbm, k_hbm, v_hbm, h_hbm, wq_hbm, wk_hbm, wv_hbm, wo_hbm,
            sk_hbm, dd_hbm, gw_hbm, mem0_hbm, fwd_hbm, inv_hbm, fill_hbm,
            out_hbm,
            x_v, xp, k_v, v_v, h_v, w_even, w_odd, wo_v, y_v, qkv_b, o_b, o_l, omem, mem_v, oacc, qacc,
            kf, kvb, u_s, h_s, yf_s,
            out_v, fwd_ref, inv_ref, fill_ref, sk_ref, dd_ref, gw_ref, zs, sems, qsems):
    scale = E ** (-0.5)
    wbuf = (w_even, w_odd)

    w32 = [w.bitcast(U32) for w in (wq_hbm, wk_hbm, wv_hbm)]
    wo32 = wo_hbm.bitcast(U32)
    x32 = x_hbm.bitcast(U32)

    def lanes(c):
        return pl.ds(pl.multiple_of(c * 128, 128), 128)

    def w_copies(c, e, mat, sem):
        return [pltpu.make_async_copy(w32[mat].at[:, par, 2 * c + e, :], wbuf[e].at[mat, c, par], sem)
                for par in range(2)]

    def wq0_copies(c):
        return w_copies(c, 0, 0, qsems.at[c])

    def block_copies(c):
        sem = sems.at[c % 2]
        return ([[pltpu.make_async_copy(h_hbm.at[lanes(c), :], h_v.at[c], sem)],
                 [pltpu.make_async_copy(k_hbm.at[:, lanes(c)], k_v.at[c], sem)],
                 [pltpu.make_async_copy(v_hbm.at[:, lanes(c)], v_v.at[c], sem)]]
                + [w_copies(c, e, mat, sem) for e in range(2) for mat in range(3) if (e, mat) != (0, 0)])

    def rest_copies(c):
        rows = pl.ds(pl.multiple_of(c * (S // NB), S // NB), S // NB)
        return [pltpu.make_async_copy(wo32.at[:, lanes(c)], wo_v.at[c], sems.at[2]),
                pltpu.make_async_copy(x_hbm.at[rows, :], x_v.at[rows, :], sems.at[2])]

    xp_copy = pltpu.make_async_copy(x32.at[pl.ds(0, PRO // 2), :], xp, sems.at[3])
    small_copies = [pltpu.make_async_copy(src, dst, sems.at[4]) for src, dst in (
        (sk_hbm, sk_ref), (fwd_hbm, fwd_ref), (dd_hbm, dd_ref), (inv_hbm, inv_ref),
        (gw_hbm, gw_ref), (mem0_hbm, mem_v), (fill_hbm, fill_ref))]

    def out_copy(start, n):
        rows = pl.ds(start, n)
        return pltpu.make_async_copy(out_v.at[rows, :], out_hbm.at[rows, :], sems.at[5])

    def kv_prep(c, zw):
        skt = sk_ref[:, lanes(c)].astype(F32)
        kf[8:8 + S, :] = k_v[c].astype(F32)
        for a in range(NCH):
            ks_ = kf[pl.ds(8 + a * C, C), :] * skt[0:1, :]
            for j in range(1, KS):
                ks_ = ks_ + kf[pl.ds(8 + a * C - j, C), :] * skt[j:j + 1, :]
            kvb[zw, pl.ds(a * C, C), :] = (ks_ * v_v[c, pl.ds(a * C, C), :].astype(F32)).astype(BF16)

    def row_of(ref, c):
        t = ref[...].astype(F32)
        sel = jax.lax.broadcasted_iota(jnp.int32, (NB, 128), 0) == c
        return jnp.sum(jnp.where(sel, t, 0.0), axis=0, keepdims=True)

    def fwd_u(zw, zr):
        for a in range(NCH):
            u_s[zw, a] = _dot(fwd_ref[...], kvb[zr, pl.ds(a * C, C), :])

    def fwd_h(c, zw):
        sgn = (1 - 2 * (jax.lax.broadcasted_iota(jnp.int32, (C, 128), 0) % 2)).astype(F32)
        hprev = None
        for a in range(NCH):
            hf = _dot_nt(fwd_ref[...], h_v[c, :, pl.ds(a * C, C)])
            if hprev is None:
                h_s[zw, a, 0:C, :] = hf[0:C] + row_of(dd_ref, c)
                h_s[zw, a, C:, :] = hf[C:]
            else:
                h_s[zw, a, 0:C, :] = hf[0:C] - sgn * hprev[C:]
                h_s[zw, a, C:, :] = hf[C:] + sgn * hprev[0:C]
            hprev = hf

    def mac(p, zw, zr):
        re = pl.ds(p * 8, 8)
        im = pl.ds(C + p * 8, 8)
        AB = 4
        for a0 in range(0, NCH, AB):
            yr = [None] * AB
            yi = [None] * AB
            for m in range(a0 + AB):
                hr = h_s[zr, m, re, :]
                hi = h_s[zr, m, im, :]
                for i in range(AB):
                    t = a0 + i - m
                    if t < 0:
                        continue
                    ur = u_s[zr, t, re, :]
                    ui = u_s[zr, t, im, :]
                    tr = hr * ur - hi * ui
                    ti = hr * ui + hi * ur
                    yr[i] = tr if yr[i] is None else yr[i] + tr
                    yi[i] = ti if yi[i] is None else yi[i] + ti
            for i in range(AB):
                yf_s[zw, a0 + i, re, :] = yr[i]
                yf_s[zw, a0 + i, im, :] = yi[i]

    def inv_dft(c, zr):
        for a in range(NCH):
            y_v[pl.ds(a * C, C), lanes(c)] = _dot(inv_ref[...], yf_s[zr, a].astype(BF16)).astype(BF16)

    def fixup(e, c, mat):
        a = wbuf[e][mat, c, 0]
        b = wbuf[e][mat, c, 1]
        wbuf[e][mat, c, 0] = (a & U32(0xFFFF)) | (b << 16)
        wbuf[e][mat, c, 1] = (a >> 16) | (b & U32(0xFFFF0000))

    RB = 128

    def qkv_tile(e, c, n):
        mat, j = n // 2, n % 2
        for r in range(PRO // RB):
            w = pltpu.bitcast(wbuf[e][mat, c, j], BF16)
            xr = pltpu.bitcast(xp[pl.ds(r * RB // 2, RB // 2), :], BF16)
            qkv_b[mat, 2 * c + e, j, pl.ds(QOFF + r * RB, RB), :] = _dot(xr, w).astype(BF16)

    xp_copy.start()
    for cp in wq0_copies(0) + wq0_copies(1) + small_copies:
        cp.start()
    kf[0:8, :] = jnp.zeros((8, 128), F32)
    zs[0] = 0
    zs[1] = 0
    xp_copy.wait()

    def pro0(c, carry):
        @pl.when(c + 2 < NB)
        def _():
            for cp in wq0_copies(c + 2):
                cp.start()

        for i, piece in enumerate(block_copies(0)):
            @pl.when(c == i)
            def _():
                for cp in piece:
                    cp.start()

        for cp in wq0_copies(c):
            cp.wait()
        fixup(0, c, 0)
        qkv_tile(0, c, 0)
        qkv_tile(0, c, 1)
        return carry

    with jax.named_scope("pro0"):
        jax.lax.fori_loop(0, NB, pro0, 0)
    for cp in small_copies:
        cp.wait()

    def pro(c, carry):
        @pl.when(c + 1 < NB)
        def _():
            for piece in block_copies(c + 1):
                for cp in piece:
                    cp.start()

        for cp in rest_copies(c):
            cp.start()
        for piece in block_copies(c):
            for cp in piece:
                cp.wait()

        zw = zs[0]
        zr = zs[1]
        tiles = [(0, n) for n in range(2, 6)] + [(1, n) for n in range(6)]

        def tile(i):
            e, n = tiles[i]
            if n % 2 == 0:
                fixup(e, c, n // 2)
            qkv_tile(e, c, n)

        kv_prep(c, zw)
        fwd_h(c, zw)
        tile(0)
        fwd_u(zw, zr)
        p = 0
        for i in range(1, 8):
            tile(i)
            for _ in range(3 if i < 3 else 2):
                mac(p, zw, zr)
                p += 1
        inv_dft(c, zr)
        tile(8)
        tile(9)
        return carry

    with jax.named_scope("pro"):
        jax.lax.fori_loop(0, NB, pro, 0)
    for c in range(NB):
        for cp in rest_copies(c):
            cp.wait()

    gwt = gw_ref[...].astype(F32)
    gw = jnp.concatenate([gwt[j:j + 1, :] for j in range(NB)], axis=1)

    def finalize(rows, b):
        xr = x_v[rows, :].astype(F32)
        g = jax.nn.sigmoid(jnp.sum(xr * gw, axis=-1, keepdims=True))
        a = xr * y_v[rows, :].astype(F32)
        out_v[rows, :] = (g * a + (1.0 - g) * b).astype(BF16)

    def step(s, mem, split_first):
        xo = pl.multiple_of(PRO + RX * s, 8)
        wpos = pl.multiple_of((RX * s) % QCAP, 8)
        rpos = pl.multiple_of((SEG * s + QOFF) % QCAP, SEG)
        opos = pl.multiple_of(SEG * s, SEG)
        lhs = jnp.concatenate([mem, x_v[pl.ds(xo, RX), :]], axis=0)
        zpad = jnp.zeros((128 - 2 * (SEG + M), E), BF16)
        frows = pl.ds(pl.multiple_of(RX * s, 8), RX)
        NP = H // 2


        mem_qkv = {}
        probs = {}
        cats = {}

        def load(mat, hp):
            if not 0 <= hp < NP:
                return
            parts = [qkv_b[mat, hp, 0, pl.ds(rpos, SEG), :], qkv_b[mat, hp, 1, pl.ds(rpos, SEG), :],
                     mem_qkv[(hp, mat)]]
            if mat > 0:
                parts.append(zpad)
            cats[(mat, hp)] = jnp.concatenate(parts, axis=0)

        def stage_a(hp):
            KH = D // 2
            split = split_first and hp == 0
            if split:
                for mat in range(3):
                    for j in range(2):
                        w = pltpu.bitcast(wbuf[hp % 2][mat, hp // 2, j, :KH // 2, :], BF16)
                        qacc[2 * mat + j] = _dot(lhs[:, :KH], w)
            for mat in range(3):
                mm = []
                for j in range(2):
                    if split:
                        w = pltpu.bitcast(wbuf[hp % 2][mat, hp // 2, j, KH // 2:, :], BF16)
                        res = qacc[2 * mat + j] + _dot(lhs[:, KH:], w)
                    else:
                        res = _dot(lhs, pltpu.bitcast(wbuf[hp % 2][mat, hp // 2, j], BF16))
                    qkv_b[mat, hp, j, pl.ds(wpos, RX), :] = res[M:].astype(BF16)
                    mm.append(res[:M])
                mem_qkv[(hp, mat)] = jnp.concatenate(mm, axis=0).astype(BF16)

        def stage_b(hp):
            if not 0 <= hp < NP:
                return
            sc = _dot_nt(cats[(0, hp)], cats[(1, hp)]) * scale
            fill = fill_ref[...]
            sc = jnp.where(fill == 0.0, sc, fill)
            mx = jnp.max(sc, axis=-1, keepdims=True)
            p = jnp.exp(sc - mx)
            l = jnp.sum(p, axis=-1, keepdims=True)
            r = pl.reciprocal(l, approx=True)
            r = r * (2.0 - l * r)
            probs[hp] = (p.astype(BF16), r)

        def stage_c(hp):
            if not 0 <= hp < NP:
                return
            o = (_dot(probs[hp][0], cats[(2, hp)]) * probs[hp][1]).astype(BF16)
            for j in range(2):
                h = 2 * hp + j
                if h < HS:
                    o_b[pl.ds(opos, SEG), h * E:(h + 1) * E] = o[j * SEG:(j + 1) * SEG]
                else:
                    o_l[pl.ds(opos, SEG), (h - HS) * E:(h - HS + 1) * E] = o[j * SEG:(j + 1) * SEG]
                omem[:, h * E:(h + 1) * E] = o[2 * SEG + j * M:2 * SEG + (j + 1) * M]

        def oproj(j, late):
            if late:
                lo = jnp.concatenate([omem[:, HS * E:], o_l[frows, :]], axis=0)
                return _dot(lo, pltpu.bitcast(wo_v[j, HS * E // 2:, :], BF16))
            lo = jnp.concatenate([omem[:, :HS * E], o_b[frows, :]], axis=0)
            return _dot(lo, pltpu.bitcast(wo_v[j, :HS * E // 2, :], BF16))

        DB, DC = 1, 2
        outs = [None] * NB
        for t in range(NP + DC):
            load(0, t - DB)
            load(1, t - DB)
            load(2, t - DC)
            if t < NP:
                stage_a(t)
            else:
                for j in range(2 * (t - NP), 2 * (t - NP) + 2):
                    oacc[:, j * 128:(j + 1) * 128] = oproj(j, False)
            stage_b(t - DB)
            stage_c(t - DC)
        for j in range(2 * DC, NB):
            oacc[:, j * 128:(j + 1) * 128] = oproj(j, False)
        for j in range(NB):
            outs[j] = oacc[:, j * 128:(j + 1) * 128] + oproj(j, True)
        res = jnp.concatenate(outs, axis=1)
        finalize(frows, res[M:])
        return res[:M].astype(BF16)

    def steps(i, carry):
        mem = mem_v[...]
        for u in range(UNROLL):
            mem = step(i * UNROLL + u, mem, u > 0)
        mem_v[...] = mem
        return carry

    with jax.named_scope("main"):
        jax.lax.fori_loop(0, NSEG // UNROLL, steps, 0)

    def epi_rows(rows):
        lo = jnp.concatenate([o_b[rows, :], o_l[rows, :]], axis=1)
        outs = [_dot(lo, pltpu.bitcast(wo_v[j], BF16)) for j in range(NB)]
        finalize(rows, jnp.concatenate(outs, axis=1))

    EB = 128

    def epi(r, carry):
        r0 = pl.multiple_of(S - PRO + r * EB, EB)

        @pl.when(r == PRO // EB - 1)
        def _():
            out_copy(S - PRO, PRO - EB).start()

        epi_rows(pl.ds(r0, EB))
        return carry

    with jax.named_scope("epi"):
        out_copy(0, S - PRO).start()
        jax.lax.fori_loop(0, PRO // EB, epi, 0)
    out_copy(S - EB, EB).start()
    out_copy(0, S).wait()


@jax.jit
def _run(A_q, A_k, A_v, A_shift_k, A_ssm_k, A_ssm_D, B_mem0, B_Wq, B_Wk, B_Wv, B_Wo, gate_w):
    fwd, inv = _dft_tables()
    any_spec = pl.BlockSpec(memory_space=pl.ANY)
    out = pl.pallas_call(
        _kernel,
        out_shape=jax.ShapeDtypeStruct((S, D), BF16),
        in_specs=[any_spec] * 15,
        out_specs=any_spec,
        scratch_shapes=[
            pltpu.VMEM((S, D), BF16),
            pltpu.VMEM((PRO // 2, D), U32),
            pltpu.VMEM((NB, S, 128), BF16),
            pltpu.VMEM((NB, S, 128), BF16),
            pltpu.VMEM((NB, 128, S), BF16),
            pltpu.VMEM((3, H // 4, 2, D // 2, E), U32),
            pltpu.VMEM((3, H // 4, 2, D // 2, E), U32),
            pltpu.VMEM((NB, H * E // 2, 128), U32),
            pltpu.VMEM((S, D), BF16),
            pltpu.VMEM((3, H // 2, 2, QCAP, E), BF16),
            pltpu.VMEM((S, HS * E), BF16),
            pltpu.VMEM((S, HL * E), BF16),
            pltpu.VMEM((M, H * E), BF16),
            pltpu.VMEM((M, D), BF16),
            pltpu.VMEM((M + RX, D), F32),
            pltpu.VMEM((6, M + RX, E), F32),
            pltpu.VMEM((S + 32, 128), F32),
            pltpu.VMEM((1, S, 128), BF16),
            pltpu.VMEM((1, NCH, 2 * C, 128), F32),
            pltpu.VMEM((1, NCH, 2 * C, 128), F32),
            pltpu.VMEM((1, NCH, 2 * C, 128), F32),
            pltpu.VMEM((S, D), BF16),
            pltpu.VMEM((2 * C, C), BF16),
            pltpu.VMEM((C, 2 * C), BF16),
            pltpu.VMEM((2 * (SEG + M), 128), F32),
            pltpu.VMEM((KS, D), BF16),
            pltpu.VMEM((NB, 128), BF16),
            pltpu.VMEM((NB, 128), BF16),
            pltpu.SMEM((2,), jnp.int32),
            pltpu.SemaphoreType.DMA((6,)),
            pltpu.SemaphoreType.DMA((NB,)),
        ],
        compiler_params=pltpu.CompilerParams(vmem_limit_bytes=120 * 2 ** 20, disable_bounds_checks=True),
    )(
        A_q.reshape(S, D), A_k.reshape(S, D), A_v.reshape(S, D), A_ssm_k,
        B_Wq.reshape(D // 2, 2, H, E), B_Wk.reshape(D // 2, 2, H, E), B_Wv.reshape(D // 2, 2, H, E),
        B_Wo.reshape(H * E, D),
        A_shift_k.T, A_ssm_D.reshape(NB, 128), gate_w.reshape(NB, 128), B_mem0.reshape(M, D),
        jnp.asarray(fwd, BF16), jnp.asarray(inv, BF16), jnp.asarray(_attn_fill()),
    )
    return out.reshape(1, S, D)


def pallas_gated_mix__ssm_conv_h3__memory_aug_recurrent_mem_tr__prompt_kernel(
    A_q, A_k, A_v, A_shift_k, A_ssm_k, A_ssm_D, B_x, B_mem0, B_Wq, B_Wk, B_Wv, B_Wo, B_seg_len, gate_w,
):
    del B_x
    if isinstance(B_seg_len, int):
        assert B_seg_len == SEG
    return _run(A_q, A_k, A_v, A_shift_k, A_ssm_k, A_ssm_D, B_mem0, B_Wq, B_Wk, B_Wv, B_Wo, gate_w)
```

```python
import functools
import math

import jax
import jax.numpy as jnp
import numpy as np
import jax.experimental.pallas as pl
import jax.experimental.pallas.tpu as pltpu

F32 = jnp.float32
BF16 = jnp.bfloat16
U32 = jnp.uint32

S = 2048
D = 1024
H = 32
E = 128
M = 8
SEG = 32
NSEG = S // SEG
RX = 24
PRO = S - RX * NSEG
QCAP = 576
QOFF = QCAP - PRO
HL = 8
HS = H - HL
UNROLL = 4
C = 128
NCH = S // C
NB = D // 128
KS = 4
NEG = -1000000000.0


def _dft_tables():
    n = np.arange(C, dtype=np.float64)
    th = np.pi * (2.0 * np.arange(C, dtype=np.float64) + 1.0) / (2 * C)
    fwd = np.concatenate([np.cos(th[:, None] * n[None, :]), -np.sin(th[:, None] * n[None, :])], axis=0)
    inv = np.concatenate([np.cos(n[:, None] * th[None, :]), -np.sin(n[:, None] * th[None, :])], axis=1) / C
    return fwd.astype(np.float32), inv.astype(np.float32)


def _attn_fill():
    n = 2 * (SEG + M)
    head = np.array([0] * SEG + [1] * SEG + [0] * M + [1] * M)
    pos = np.concatenate([M + np.arange(SEG), M + np.arange(SEG), np.arange(M), np.arange(M)])
    fill = np.full((n, 128), -np.inf, np.float32)
    for i in range(n):
        for j in range(n):
            if head[i] == head[j]:
                ok = pos[i] < M or pos[i] >= pos[j]
                fill[i, j] = 0.0 if ok else NEG
    return fill


def _dot(a, b):
    return jnp.dot(a, b, preferred_element_type=F32)


def _dot_nt(a, b):
    return jax.lax.dot_general(a, b, (((1,), (1,)), ((), ())), preferred_element_type=F32)


def _kernel(x_hbm, k_hbm, v_hbm, h_hbm, wq_hbm, wk_hbm, wv_hbm, wo_hbm,
            sk_hbm, dd_hbm, gw_hbm, mem0_hbm, fwd_hbm, inv_hbm, fill_hbm,
            out_hbm,
            x_v, xp, k_v, v_v, h_v, w_even, w_odd, wo_v, y_v, qkv_b, o_b, o_l, omem, mem_v, oacc, qacc,
            kf, u_s, h_s, yf_s,
            out_v, fwd_ref, inv_ref, fill_ref, sk_ref, dd_ref, gw_ref, zs, sems, qsems):
    scale = E ** (-0.5)
    wbuf = (w_even, w_odd)

    w32 = [w.bitcast(U32) for w in (wq_hbm, wk_hbm, wv_hbm)]
    wo32 = wo_hbm.bitcast(U32)
    x32 = x_hbm.bitcast(U32)

    def lanes(c):
        return pl.ds(pl.multiple_of(c * 128, 128), 128)

    def w_copies(c, e, mat, sem):
        return [pltpu.make_async_copy(w32[mat].at[:, par, 2 * c + e, :], wbuf[e].at[mat, c, par], sem)
                for par in range(2)]

    def wq0_copies(c):
        return w_copies(c, 0, 0, qsems.at[c])

    def block_copies(c):
        sem = sems.at[c % 2]
        return ([[pltpu.make_async_copy(h_hbm.at[lanes(c), :], h_v.at[c], sem)],
                 [pltpu.make_async_copy(k_hbm.at[:, lanes(c)], k_v.at[c], sem)],
                 [pltpu.make_async_copy(v_hbm.at[:, lanes(c)], v_v.at[c], sem)]]
                + [w_copies(c, e, mat, sem) for e in range(2) for mat in range(3) if (e, mat) != (0, 0)])

    def rest_copies(c):
        rows = pl.ds(pl.multiple_of(c * (S // NB), S // NB), S // NB)
        return [pltpu.make_async_copy(wo32.at[:, lanes(c)], wo_v.at[c], sems.at[2]),
                pltpu.make_async_copy(x_hbm.at[rows, :], x_v.at[rows, :], sems.at[2])]

    xp_copy = pltpu.make_async_copy(x32.at[pl.ds(0, PRO // 2), :], xp, sems.at[3])
    small_copies = [pltpu.make_async_copy(src, dst, sems.at[4]) for src, dst in (
        (sk_hbm, sk_ref), (fwd_hbm, fwd_ref), (dd_hbm, dd_ref), (inv_hbm, inv_ref),
        (gw_hbm, gw_ref), (mem0_hbm, mem_v), (fill_hbm, fill_ref))]

    def out_copy(start, n):
        rows = pl.ds(start, n)
        return pltpu.make_async_copy(out_v.at[rows, :], out_hbm.at[rows, :], sems.at[5])

    def row_of(ref, c):
        t = ref[...].astype(F32)
        sel = jax.lax.broadcasted_iota(jnp.int32, (NB, 128), 0) == c
        return jnp.sum(jnp.where(sel, t, 0.0), axis=0, keepdims=True)

    def fwd_dft(c, zw):
        skt = sk_ref[:, lanes(c)].astype(F32)
        for a in range(NCH):
            hf = _dot_nt(fwd_ref[...], h_v[c, :, pl.ds(a * C, C)])
            if a == 0:
                h_s[zw, a, 0:C, :] = hf[0:C] + row_of(dd_ref, c)
                h_s[zw, a, C:, :] = hf[C:]
            else:
                h_s[zw, a] = hf
            kf[pl.ds(8 + a * C, C), :] = k_v[c, pl.ds(a * C, C), :].astype(F32)
            ks_ = kf[pl.ds(8 + a * C, C), :] * skt[0:1, :]
            for j in range(1, KS):
                ks_ = ks_ + kf[pl.ds(8 + a * C - j, C), :] * skt[j:j + 1, :]
            kv = (ks_ * v_v[c, pl.ds(a * C, C), :].astype(F32)).astype(BF16)
            u_s[zw, a] = _dot(fwd_ref[...], kv)

    def mac(p, zw, zr):
        re = pl.ds(p * 8, 8)
        im = pl.ds(C + p * 8, 8)
        sgn = (1 - 2 * (jax.lax.broadcasted_iota(jnp.int32, (8, 128), 0) % 2)).astype(F32)
        AB = 4
        prev = None
        for a0 in range(0, NCH, AB):
            zre = [None] * AB
            zim = [None] * AB
            for m in range(a0 + AB):
                hr = h_s[zr, m, re, :]
                hi = h_s[zr, m, im, :]
                for i in range(AB):
                    t = a0 + i - m
                    if t < 0:
                        continue
                    ur = u_s[zr, t, re, :]
                    ui = u_s[zr, t, im, :]
                    tr = hr * ur - hi * ui
                    ti = hr * ui + hi * ur
                    zre[i] = tr if zre[i] is None else zre[i] + tr
                    zim[i] = ti if zim[i] is None else zim[i] + ti
            for i in range(AB):
                if prev is None:
                    yf_s[zw, a0 + i, re, :] = zre[i]
                    yf_s[zw, a0 + i, im, :] = zim[i]
                else:
                    yf_s[zw, a0 + i, re, :] = zre[i] - sgn * prev[1]
                    yf_s[zw, a0 + i, im, :] = zim[i] + sgn * prev[0]
                prev = (zre[i], zim[i])

    def inv_dft(c, zr):
        for a in range(NCH):
            y_v[pl.ds(a * C, C), lanes(c)] = _dot(inv_ref[...], yf_s[zr, a].astype(BF16)).astype(BF16)

    def fixup(e, c, mat):
        a = wbuf[e][mat, c, 0]
        b = wbuf[e][mat, c, 1]
        wbuf[e][mat, c, 0] = (a & U32(0xFFFF)) | (b << 16)
        wbuf[e][mat, c, 1] = (a >> 16) | (b & U32(0xFFFF0000))

    RB = 128

    def qkv_tile(e, c, n):
        mat, j = n // 2, n % 2
        for r in range(PRO // RB):
            w = pltpu.bitcast(wbuf[e][mat, c, j], BF16)
            xr = pltpu.bitcast(xp[pl.ds(r * RB // 2, RB // 2), :], BF16)
            qkv_b[mat, 2 * c + e, j, pl.ds(QOFF + r * RB, RB), :] = _dot(xr, w).astype(BF16)

    xp_copy.start()
    for cp in wq0_copies(0) + wq0_copies(1) + small_copies:
        cp.start()
    kf[0:8, :] = jnp.zeros((8, 128), F32)
    zs[0] = 0
    zs[1] = 0
    xp_copy.wait()

    def pro0(c, carry):
        @pl.when(c + 2 < NB)
        def _():
            for cp in wq0_copies(c + 2):
                cp.start()

        for i, piece in enumerate(block_copies(0)):
            @pl.when(c == i)
            def _():
                for cp in piece:
                    cp.start()

        for cp in wq0_copies(c):
            cp.wait()
        fixup(0, c, 0)
        qkv_tile(0, c, 0)
        qkv_tile(0, c, 1)
        return carry

    with jax.named_scope("pro0"):
        jax.lax.fori_loop(0, NB, pro0, 0)
    for cp in small_copies:
        cp.wait()

    zw = zs[0]
    zr = zs[1]

    def pro(c, carry):
        @pl.when(c + 1 < NB)
        def _():
            for piece in block_copies(c + 1):
                for cp in piece:
                    cp.start()

        for cp in rest_copies(c):
            cp.start()
        for piece in block_copies(c):
            for cp in piece:
                cp.wait()

        tiles = [(0, n) for n in range(2, 6)] + [(1, n) for n in range(6)]

        def tile(i):
            e, n = tiles[i]
            if n % 2 == 0:
                fixup(e, c, n // 2)
            qkv_tile(e, c, n)

        tile(0)
        fwd_dft(c, zw)
        p = 0
        for i in range(1, 8):
            tile(i)
            for _ in range(3 if i < 3 else 2):
                mac(p, zw, zr)
                p += 1
        inv_dft(c, zr)
        tile(8)
        tile(9)
        return carry

    with jax.named_scope("pro"):
        jax.lax.fori_loop(0, NB, pro, 0)
    for c in range(NB):
        for cp in rest_copies(c):
            cp.wait()

    gwt = gw_ref[...].astype(F32)
    gw = jnp.concatenate([gwt[j:j + 1, :] for j in range(NB)], axis=1)

    def finalize(rows, b):
        xr = x_v[rows, :].astype(F32)
        g = jax.nn.sigmoid(jnp.sum(xr * gw, axis=-1, keepdims=True))
        a = xr * y_v[rows, :].astype(F32)
        out_v[rows, :] = (g * a + (1.0 - g) * b).astype(BF16)

    def step(s, mem, split_first):
        xo = pl.multiple_of(PRO + RX * s, 8)
        wpos = pl.multiple_of((RX * s) % QCAP, 8)
        rpos = pl.multiple_of((SEG * s + QOFF) % QCAP, SEG)
        opos = pl.multiple_of(SEG * s, SEG)
        lhs = jnp.concatenate([mem, x_v[pl.ds(xo, RX), :]], axis=0)
        zpad = jnp.zeros((128 - 2 * (SEG + M), E), BF16)
        frows = pl.ds(pl.multiple_of(RX * s, 8), RX)
        NP = H // 2


        mem_qkv = {}
        probs = {}
        cats = {}

        def load(mat, hp):
            if not 0 <= hp < NP:
                return
            parts = [qkv_b[mat, hp, 0, pl.ds(rpos, SEG), :], qkv_b[mat, hp, 1, pl.ds(rpos, SEG), :],
                     mem_qkv[(hp, mat)]]
            if mat > 0:
                parts.append(zpad)
            cats[(mat, hp)] = jnp.concatenate(parts, axis=0)

        def stage_a(hp):
            KH = D // 2
            split = split_first and hp == 0
            if split:
                for mat in range(3):
                    for j in range(2):
                        w = pltpu.bitcast(wbuf[hp % 2][mat, hp // 2, j, :KH // 2, :], BF16)
                        qacc[2 * mat + j] = _dot(lhs[:, :KH], w)
            for mat in range(3):
                mm = []
                for j in range(2):
                    if split:
                        w = pltpu.bitcast(wbuf[hp % 2][mat, hp // 2, j, KH // 2:, :], BF16)
                        res = qacc[2 * mat + j] + _dot(lhs[:, KH:], w)
                    else:
                        res = _dot(lhs, pltpu.bitcast(wbuf[hp % 2][mat, hp // 2, j], BF16))
                    qkv_b[mat, hp, j, pl.ds(wpos, RX), :] = res[M:].astype(BF16)
                    mm.append(res[:M])
                mem_qkv[(hp, mat)] = jnp.concatenate(mm, axis=0).astype(BF16)

        def stage_b(hp):
            if not 0 <= hp < NP:
                return
            sc = _dot_nt(cats[(0, hp)], cats[(1, hp)]) * scale
            fill = fill_ref[...]
            sc = jnp.where(fill == 0.0, sc, fill)
            mx = jnp.max(sc, axis=-1, keepdims=True)
            p = jnp.exp(sc - mx)
            l = jnp.sum(p, axis=-1, keepdims=True)
            r = pl.reciprocal(l, approx=True)
            r = r * (2.0 - l * r)
            probs[hp] = (p.astype(BF16), r)

        def stage_c(hp):
            if not 0 <= hp < NP:
                return
            o = (_dot(probs[hp][0], cats[(2, hp)]) * probs[hp][1]).astype(BF16)
            for j in range(2):
                h = 2 * hp + j
                if h < HS:
                    o_b[pl.ds(opos, SEG), h * E:(h + 1) * E] = o[j * SEG:(j + 1) * SEG]
                else:
                    o_l[pl.ds(opos, SEG), (h - HS) * E:(h - HS + 1) * E] = o[j * SEG:(j + 1) * SEG]
                omem[:, h * E:(h + 1) * E] = o[2 * SEG + j * M:2 * SEG + (j + 1) * M]

        def oproj(j, late):
            if late:
                lo = jnp.concatenate([omem[:, HS * E:], o_l[frows, :]], axis=0)
                return _dot(lo, pltpu.bitcast(wo_v[j, HS * E // 2:, :], BF16))
            lo = jnp.concatenate([omem[:, :HS * E], o_b[frows, :]], axis=0)
            return _dot(lo, pltpu.bitcast(wo_v[j, :HS * E // 2, :], BF16))

        DB, DC = 1, 2
        outs = [None] * NB
        for t in range(NP + DC):
            load(0, t - DB)
            load(1, t - DB)
            load(2, t - DC)
            if t < NP:
                stage_a(t)
            else:
                for j in range(2 * (t - NP), 2 * (t - NP) + 2):
                    oacc[:, j * 128:(j + 1) * 128] = oproj(j, False)
            stage_b(t - DB)
            stage_c(t - DC)
        for j in range(2 * DC, NB):
            oacc[:, j * 128:(j + 1) * 128] = oproj(j, False)
        for j in range(NB):
            outs[j] = oacc[:, j * 128:(j + 1) * 128] + oproj(j, True)
        res = jnp.concatenate(outs, axis=1)
        finalize(frows, res[M:])
        return res[:M].astype(BF16)

    def steps(i, carry):
        mem = mem_v[...]
        for u in range(UNROLL):
            mem = step(i * UNROLL + u, mem, u > 0)
        mem_v[...] = mem
        return carry

    with jax.named_scope("main"):
        jax.lax.fori_loop(0, NSEG // UNROLL, steps, 0)

    def epi_rows(rows):
        lo = jnp.concatenate([o_b[rows, :], o_l[rows, :]], axis=1)
        outs = [_dot(lo, pltpu.bitcast(wo_v[j], BF16)) for j in range(NB)]
        finalize(rows, jnp.concatenate(outs, axis=1))

    EB = 128

    def epi(r, carry):
        r0 = pl.multiple_of(S - PRO + r * EB, EB)

        @pl.when(r == PRO // EB - 1)
        def _():
            out_copy(S - PRO, PRO - EB).start()

        epi_rows(pl.ds(r0, EB))
        return carry

    with jax.named_scope("epi"):
        out_copy(0, S - PRO).start()
        jax.lax.fori_loop(0, PRO // EB, epi, 0)
    out_copy(S - EB, EB).start()
    out_copy(0, S).wait()


@jax.jit
def _run(A_q, A_k, A_v, A_shift_k, A_ssm_k, A_ssm_D, B_mem0, B_Wq, B_Wk, B_Wv, B_Wo, gate_w):
    fwd, inv = _dft_tables()
    any_spec = pl.BlockSpec(memory_space=pl.ANY)
    out = pl.pallas_call(
        _kernel,
        out_shape=jax.ShapeDtypeStruct((S, D), BF16),
        in_specs=[any_spec] * 15,
        out_specs=any_spec,
        scratch_shapes=[
            pltpu.VMEM((S, D), BF16),
            pltpu.VMEM((PRO // 2, D), U32),
            pltpu.VMEM((NB, S, 128), BF16),
            pltpu.VMEM((NB, S, 128), BF16),
            pltpu.VMEM((NB, 128, S), BF16),
            pltpu.VMEM((3, H // 4, 2, D // 2, E), U32),
            pltpu.VMEM((3, H // 4, 2, D // 2, E), U32),
            pltpu.VMEM((NB, H * E // 2, 128), U32),
            pltpu.VMEM((S, D), BF16),
            pltpu.VMEM((3, H // 2, 2, QCAP, E), BF16),
            pltpu.VMEM((S, HS * E), BF16),
            pltpu.VMEM((S, HL * E), BF16),
            pltpu.VMEM((M, H * E), BF16),
            pltpu.VMEM((M, D), BF16),
            pltpu.VMEM((M + RX, D), F32),
            pltpu.VMEM((6, M + RX, E), F32),
            pltpu.VMEM((S + 32, 128), F32),
            pltpu.VMEM((1, NCH, 2 * C, 128), F32),
            pltpu.VMEM((1, NCH, 2 * C, 128), F32),
            pltpu.VMEM((1, NCH, 2 * C, 128), F32),
            pltpu.VMEM((S, D), BF16),
            pltpu.VMEM((2 * C, C), BF16),
            pltpu.VMEM((C, 2 * C), BF16),
            pltpu.VMEM((2 * (SEG + M), 128), F32),
            pltpu.VMEM((KS, D), BF16),
            pltpu.VMEM((NB, 128), BF16),
            pltpu.VMEM((NB, 128), BF16),
            pltpu.SMEM((2,), jnp.int32),
            pltpu.SemaphoreType.DMA((6,)),
            pltpu.SemaphoreType.DMA((NB,)),
        ],
        compiler_params=pltpu.CompilerParams(vmem_limit_bytes=120 * 2 ** 20, disable_bounds_checks=True),
    )(
        A_q.reshape(S, D), A_k.reshape(S, D), A_v.reshape(S, D), A_ssm_k,
        B_Wq.reshape(D // 2, 2, H, E), B_Wk.reshape(D // 2, 2, H, E), B_Wv.reshape(D // 2, 2, H, E),
        B_Wo.reshape(H * E, D),
        A_shift_k.T, A_ssm_D.reshape(NB, 128), gate_w.reshape(NB, 128), B_mem0.reshape(M, D),
        jnp.asarray(fwd, BF16), jnp.asarray(inv, BF16), jnp.asarray(_attn_fill()),
    )
    return out.reshape(1, S, D)


def pallas_gated_mix__ssm_conv_h3__memory_aug_recurrent_mem_tr__prompt_kernel(
    A_q, A_k, A_v, A_shift_k, A_ssm_k, A_ssm_D, B_x, B_mem0, B_Wq, B_Wk, B_Wv, B_Wo, B_seg_len, gate_w,
):
    del B_x
    if isinstance(B_seg_len, int):
        assert B_seg_len == SEG
    return _run(A_q, A_k, A_v, A_shift_k, A_ssm_k, A_ssm_D, B_mem0, B_Wq, B_Wk, B_Wv, B_Wo, gate_w)
```

```python
import functools
import math

import jax
import jax.numpy as jnp
import numpy as np
import jax.experimental.pallas as pl
import jax.experimental.pallas.tpu as pltpu

F32 = jnp.float32
BF16 = jnp.bfloat16
U32 = jnp.uint32

S = 2048
D = 1024
H = 32
E = 128
M = 8
SEG = 32
NSEG = S // SEG
RX = 24
PRO = S - RX * NSEG
QCAP = 576
QOFF = QCAP - PRO
HL = 8
HS = H - HL
UNROLL = 4
C = 128
NCH = S // C
NB = D // 128
KS = 4
NEG = -1000000000.0


def _dft_tables():
    n = np.arange(C, dtype=np.float64)
    th = np.pi * (2.0 * np.arange(C, dtype=np.float64) + 1.0) / (2 * C)
    fwd = np.concatenate([np.cos(th[:, None] * n[None, :]), -np.sin(th[:, None] * n[None, :])], axis=0)
    inv = np.concatenate([np.cos(n[:, None] * th[None, :]), -np.sin(n[:, None] * th[None, :])], axis=1) / C
    return fwd.astype(np.float32), inv.astype(np.float32)


def _attn_fill():
    n = 2 * (SEG + M)
    head = np.array([0] * SEG + [1] * SEG + [0] * M + [1] * M)
    pos = np.concatenate([M + np.arange(SEG), M + np.arange(SEG), np.arange(M), np.arange(M)])
    fill = np.full((n, 128), -np.inf, np.float32)
    for i in range(n):
        for j in range(n):
            if head[i] == head[j]:
                ok = pos[i] < M or pos[i] >= pos[j]
                fill[i, j] = 0.0 if ok else NEG
    return fill


def _dot(a, b):
    return jnp.dot(a, b, preferred_element_type=F32)


def _dot_nt(a, b):
    return jax.lax.dot_general(a, b, (((1,), (1,)), ((), ())), preferred_element_type=F32)


def _pack(a):
    return pltpu.bitcast(a.astype(BF16), U32)


def _unpack(a):
    return pltpu.bitcast(a, BF16)


def _kernel(x_hbm, k_hbm, v_hbm, h_hbm, wq_hbm, wk_hbm, wv_hbm, wo_hbm,
            sk_hbm, dd_hbm, gw_hbm, mem0_hbm, fwd_hbm, inv_hbm, fill_hbm,
            out_hbm,
            x_v, xp, k_v, v_v, h_v, w_even, w_odd, wo_v, y_v, qkv_b, o_b, lo_s, mem_v, oacc, qacc,
            kf, u_s, h_s, yf_s,
            out_v, fwd_ref, inv_ref, fill_ref, sk_ref, dd_ref, gw_ref, zs, sems, qsems):
    scale = E ** (-0.5)
    wbuf = (w_even, w_odd)

    w32 = [w.bitcast(U32) for w in (wq_hbm, wk_hbm, wv_hbm)]
    wo32 = wo_hbm.bitcast(U32)
    x32 = x_hbm.bitcast(U32)

    def lanes(c):
        return pl.ds(pl.multiple_of(c * 128, 128), 128)

    def w_copies(c, e, mat, sem):
        return [pltpu.make_async_copy(w32[mat].at[:, par, 2 * c + e, :], wbuf[e].at[mat, c, par], sem)
                for par in range(2)]

    def wq0_copies(c):
        return w_copies(c, 0, 0, qsems.at[c])

    def block_copies(c):
        sem = sems.at[c % 2]
        return ([[pltpu.make_async_copy(h_hbm.at[lanes(c), :], h_v.at[c], sem)],
                 [pltpu.make_async_copy(k_hbm.at[:, lanes(c)], k_v.at[c], sem)],
                 [pltpu.make_async_copy(v_hbm.at[:, lanes(c)], v_v.at[c], sem)]]
                + [w_copies(c, e, mat, sem) for e in range(2) for mat in range(3) if (e, mat) != (0, 0)])

    def rest_copies(c):
        rows = pl.ds(pl.multiple_of(c * (S // NB), S // NB), S // NB)
        return [pltpu.make_async_copy(wo32.at[:, lanes(c)], wo_v.at[c], sems.at[2]),
                pltpu.make_async_copy(x_hbm.at[rows, :], x_v.at[rows, :], sems.at[2])]

    xp_copy = pltpu.make_async_copy(x32.at[pl.ds(0, PRO // 2), :], xp, sems.at[3])
    small_copies = [pltpu.make_async_copy(src, dst, sems.at[4]) for src, dst in (
        (sk_hbm, sk_ref), (fwd_hbm, fwd_ref), (dd_hbm, dd_ref), (inv_hbm, inv_ref),
        (gw_hbm, gw_ref), (mem0_hbm, mem_v), (fill_hbm, fill_ref))]

    def out_copy(start, n):
        rows = pl.ds(start, n)
        return pltpu.make_async_copy(out_v.at[rows, :], out_hbm.at[rows, :], sems.at[5])

    def row_of(ref, c):
        t = ref[...].astype(F32)
        sel = jax.lax.broadcasted_iota(jnp.int32, (NB, 128), 0) == c
        return jnp.sum(jnp.where(sel, t, 0.0), axis=0, keepdims=True)

    def fwd_dft(c, zw):
        skt = sk_ref[:, lanes(c)].astype(F32)
        for a in range(NCH):
            hf = _dot_nt(fwd_ref[...], h_v[c, :, pl.ds(a * C, C)])
            if a == 0:
                h_s[zw, a, 0:C, :] = hf[0:C] + row_of(dd_ref, c)
                h_s[zw, a, C:, :] = hf[C:]
            else:
                h_s[zw, a] = hf
            kf[pl.ds(8 + a * C, C), :] = k_v[c, pl.ds(a * C, C), :].astype(F32)
            ks_ = kf[pl.ds(8 + a * C, C), :] * skt[0:1, :]
            for j in range(1, KS):
                ks_ = ks_ + kf[pl.ds(8 + a * C - j, C), :] * skt[j:j + 1, :]
            kv = (ks_ * v_v[c, pl.ds(a * C, C), :].astype(F32)).astype(BF16)
            u_s[zw, a] = _dot(fwd_ref[...], kv)

    def mac(p, zw, zr):
        re = pl.ds(p * 8, 8)
        im = pl.ds(C + p * 8, 8)
        sgn = (1 - 2 * (jax.lax.broadcasted_iota(jnp.int32, (8, 128), 0) % 2)).astype(F32)
        AB = 4
        prev = None
        for a0 in range(0, NCH, AB):
            zre = [None] * AB
            zim = [None] * AB
            for m in range(a0 + AB):
                hr = h_s[zr, m, re, :]
                hi = h_s[zr, m, im, :]
                for i in range(AB):
                    t = a0 + i - m
                    if t < 0:
                        continue
                    ur = u_s[zr, t, re, :]
                    ui = u_s[zr, t, im, :]
                    tr = hr * ur - hi * ui
                    ti = hr * ui + hi * ur
                    zre[i] = tr if zre[i] is None else zre[i] + tr
                    zim[i] = ti if zim[i] is None else zim[i] + ti
            for i in range(AB):
                if prev is None:
                    yf_s[zw, a0 + i, re, :] = zre[i]
                    yf_s[zw, a0 + i, im, :] = zim[i]
                else:
                    yf_s[zw, a0 + i, re, :] = zre[i] - sgn * prev[1]
                    yf_s[zw, a0 + i, im, :] = zim[i] + sgn * prev[0]
                prev = (zre[i], zim[i])

    def inv_dft(c, zr):
        for a in range(NCH):
            y_v[pl.ds(a * C, C), lanes(c)] = _dot(inv_ref[...], yf_s[zr, a].astype(BF16)).astype(BF16)

    def fixup(e, c, mat):
        a = wbuf[e][mat, c, 0]
        b = wbuf[e][mat, c, 1]
        wbuf[e][mat, c, 0] = (a & U32(0xFFFF)) | (b << 16)
        wbuf[e][mat, c, 1] = (a >> 16) | (b & U32(0xFFFF0000))

    RB = 128

    def qkv_tile(e, c, n):
        mat, j = n // 2, n % 2
        for r in range(PRO // RB):
            w = _unpack(wbuf[e][mat, c, j])
            xr = _unpack(xp[pl.ds(r * RB // 2, RB // 2), :])
            qkv_b[mat, 2 * c + e, j, pl.ds((QOFF + r * RB) // 2, RB // 2), :] = _pack(_dot(xr, w))

    xp_copy.start()
    for cp in wq0_copies(0) + wq0_copies(1) + small_copies:
        cp.start()
    kf[0:8, :] = jnp.zeros((8, 128), F32)
    zs[0] = 0
    zs[1] = 0
    xp_copy.wait()

    def pro0(c, carry):
        @pl.when(c + 2 < NB)
        def _():
            for cp in wq0_copies(c + 2):
                cp.start()

        for i, piece in enumerate(block_copies(0)):
            @pl.when(c == i)
            def _():
                for cp in piece:
                    cp.start()

        for cp in wq0_copies(c):
            cp.wait()
        fixup(0, c, 0)
        qkv_tile(0, c, 0)
        qkv_tile(0, c, 1)
        return carry

    with jax.named_scope("pro0"):
        jax.lax.fori_loop(0, NB, pro0, 0)
    for cp in small_copies:
        cp.wait()

    zw = zs[0]
    zr = zs[1]

    def pro(c, carry):
        @pl.when(c + 1 < NB)
        def _():
            for piece in block_copies(c + 1):
                for cp in piece:
                    cp.start()

        for cp in rest_copies(c):
            cp.start()
        for piece in block_copies(c):
            for cp in piece:
                cp.wait()

        tiles = [(0, n) for n in range(2, 6)] + [(1, n) for n in range(6)]

        def tile(i):
            e, n = tiles[i]
            if n % 2 == 0:
                fixup(e, c, n // 2)
            qkv_tile(e, c, n)

        tile(0)
        fwd_dft(c, zw)
        p = 0
        for i in range(1, 8):
            tile(i)
            for _ in range(3 if i < 3 else 2):
                mac(p, zw, zr)
                p += 1
        inv_dft(c, zr)
        tile(8)
        tile(9)
        return carry

    with jax.named_scope("pro"):
        jax.lax.fori_loop(0, NB, pro, 0)
    for c in range(NB):
        for cp in rest_copies(c):
            cp.wait()

    gwt = gw_ref[...].astype(F32)
    gw = jnp.concatenate([gwt[j:j + 1, :] for j in range(NB)], axis=1)

    def finalize(rows, b):
        xr = x_v[rows, :].astype(F32)
        g = jax.nn.sigmoid(jnp.sum(xr * gw, axis=-1, keepdims=True))
        a = xr * y_v[rows, :].astype(F32)
        out_v[rows, :] = (g * a + (1.0 - g) * b).astype(BF16)

    def step(s, mem, split_first, odd):
        xrows = slice(M, M + RX) if odd else slice(0, RX)
        mrows = slice(0, M) if odd else slice(RX, RX + M)
        sh = 4 if odd else 0
        xo = pl.multiple_of(PRO + RX * s, 8)
        wbase = pl.multiple_of((RX // 2 * s) % (QCAP // 2) - sh, 8)
        rpos = pl.multiple_of((SEG // 2 * s + QOFF // 2) % (QCAP // 2), SEG // 2)
        opos = pl.multiple_of(SEG // 2 * s, SEG // 2)
        fbase = pl.multiple_of(RX // 2 * s - sh, 8)
        xs = x_v[pl.ds(xo, RX), :]
        lhs = jnp.concatenate([mem, xs] if odd else [xs, mem], axis=0)
        zpad = jnp.zeros((128 - 2 * (SEG + M), E), BF16)
        frows = pl.ds(pl.multiple_of(RX * s, 8), RX)
        low = jax.lax.broadcasted_iota(jnp.int32, (8, E), 0) < 4
        NP = H // 2

        mem_qkv = {}
        probs = {}
        cats = {}

        def load(mat, hp):
            if not 0 <= hp < NP:
                return
            parts = [_unpack(qkv_b[mat, hp, 0, pl.ds(rpos, SEG // 2), :]),
                     _unpack(qkv_b[mat, hp, 1, pl.ds(rpos, SEG // 2), :]), mem_qkv[(hp, mat)]]
            if mat > 0:
                parts.append(zpad)
            cats[(mat, hp)] = jnp.concatenate(parts, axis=0)

        def stage_a(hp):
            KH = D // 2
            split = split_first and hp == 0
            if split:
                for mat in range(3):
                    for j in range(2):
                        w = _unpack(wbuf[hp % 2][mat, hp // 2, j, :KH // 2, :])
                        qacc[2 * mat + j] = _dot(lhs[:, :KH], w)
            for mat in range(3):
                mm = []
                for j in range(2):
                    if split:
                        w = _unpack(wbuf[hp % 2][mat, hp // 2, j, KH // 2:, :])
                        res = qacc[2 * mat + j] + _dot(lhs[:, KH:], w)
                    else:
                        res = _dot(lhs, _unpack(wbuf[hp % 2][mat, hp // 2, j]))
                    pk = _pack(res)
                    if odd:
                        qkv_b[mat, hp, j, pl.ds(wbase + 4, 4), :] = pk[4:8]
                        qkv_b[mat, hp, j, pl.ds(wbase + 8, 8), :] = pk[8:16]
                    else:
                        qkv_b[mat, hp, j, pl.ds(wbase, 8), :] = pk[0:8]
                        qkv_b[mat, hp, j, pl.ds(wbase + 8, 4), :] = pk[8:12]
                    mm.append(res[mrows])
                mem_qkv[(hp, mat)] = jnp.concatenate(mm, axis=0).astype(BF16)

        def stage_b(hp):
            if not 0 <= hp < NP:
                return
            sc = _dot_nt(cats[(0, hp)], cats[(1, hp)]) * scale
            fill = fill_ref[...]
            sc = jnp.where(fill == 0.0, sc, fill)
            mx = jnp.max(sc, axis=-1, keepdims=True)
            p = jnp.exp(sc - mx)
            l = jnp.sum(p, axis=-1, keepdims=True)
            r = pl.reciprocal(l, approx=True)
            r = r * (2.0 - l * r)
            probs[hp] = (p.astype(BF16), r)

        def stage_c(hp):
            if not 0 <= hp < NP:
                return
            o = _dot(probs[hp][0], cats[(2, hp)]) * probs[hp][1]
            for j in range(2):
                h = 2 * hp + j
                cols = slice(h * E, (h + 1) * E)
                o_b[pl.ds(opos, SEG // 2), cols] = _pack(o[j * SEG:(j + 1) * SEG])
                om = o[2 * SEG + j * M:2 * SEG + (j + 1) * M]
                om = _pack(jnp.concatenate([om, om], axis=0))
                w0 = o_b[pl.ds(fbase, 8), cols]
                w1 = o_b[pl.ds(fbase + 8, 8), cols]
                lo_s[0:8, cols] = jnp.where(low, om, w0) if odd else w0
                lo_s[8:16, cols] = w1 if odd else jnp.where(low, w1, om)

        def oproj(j, late):
            ks = slice(HS * E, H * E) if late else slice(0, HS * E)
            kw = slice(ks.start // 2, ks.stop // 2)
            return _dot(_unpack(lo_s[:, ks]), _unpack(wo_v[j, kw, :]))

        DB, DC = 1, 3
        outs = [None] * NB
        for t in range(NP + DC):
            load(0, t - DB)
            load(1, t - DB)
            load(2, t - DC)
            if t < NP:
                stage_a(t)
            else:
                for j in range(2 * (t - NP), 2 * (t - NP) + 2):
                    oacc[:, j * 128:(j + 1) * 128] = oproj(j, False)
            stage_c(t - DC)
            stage_b(t - DB)
        for j in range(2 * DC, NB):
            oacc[:, j * 128:(j + 1) * 128] = oproj(j, False)
        for j in range(NB):
            outs[j] = oacc[:, j * 128:(j + 1) * 128] + oproj(j, True)
        res = jnp.concatenate(outs, axis=1)
        finalize(frows, res[xrows])
        return res[mrows].astype(BF16)

    def steps(i, carry):
        mem = mem_v[...]
        for u in range(UNROLL):
            mem = step(i * UNROLL + u, mem, u > 0, u % 2 == 1)
        mem_v[...] = mem
        return carry

    with jax.named_scope("main"):
        jax.lax.fori_loop(0, NSEG // UNROLL, steps, 0)

    def epi_rows(r0, n):
        lo = _unpack(o_b[pl.ds(pl.multiple_of(r0 // 2, 8), n // 2), :])
        outs = [_dot(lo, _unpack(wo_v[j])) for j in range(NB)]
        finalize(pl.ds(r0, n), jnp.concatenate(outs, axis=1))

    EB = 128

    def epi(r, carry):
        r0 = pl.multiple_of(S - PRO + r * EB, EB)

        @pl.when(r == PRO // EB - 1)
        def _():
            out_copy(S - PRO, PRO - EB).start()

        epi_rows(r0, EB)
        return carry

    with jax.named_scope("epi"):
        out_copy(0, S - PRO).start()
        jax.lax.fori_loop(0, PRO // EB, epi, 0)
    out_copy(S - EB, EB).start()
    out_copy(0, S).wait()


@jax.jit
def _run(A_q, A_k, A_v, A_shift_k, A_ssm_k, A_ssm_D, B_mem0, B_Wq, B_Wk, B_Wv, B_Wo, gate_w):
    fwd, inv = _dft_tables()
    any_spec = pl.BlockSpec(memory_space=pl.ANY)
    out = pl.pallas_call(
        _kernel,
        out_shape=jax.ShapeDtypeStruct((S, D), BF16),
        in_specs=[any_spec] * 15,
        out_specs=any_spec,
        scratch_shapes=[
            pltpu.VMEM((S, D), BF16),
            pltpu.VMEM((PRO // 2, D), U32),
            pltpu.VMEM((NB, S, 128), BF16),
            pltpu.VMEM((NB, S, 128), BF16),
            pltpu.VMEM((NB, 128, S), BF16),
            pltpu.VMEM((3, H // 4, 2, D // 2, E), U32),
            pltpu.VMEM((3, H // 4, 2, D // 2, E), U32),
            pltpu.VMEM((NB, H * E // 2, 128), U32),
            pltpu.VMEM((S, D), BF16),
            pltpu.VMEM((3, H // 2, 2, QCAP // 2, E), U32),
            pltpu.VMEM((S // 2, H * E), U32),
            pltpu.VMEM(((M + RX) // 2, H * E), U32),
            pltpu.VMEM((M, D), BF16),
            pltpu.VMEM((M + RX, D), F32),
            pltpu.VMEM((6, M + RX, E), F32),
            pltpu.VMEM((S + 32, 128), F32),
            pltpu.VMEM((1, NCH, 2 * C, 128), F32),
            pltpu.VMEM((1, NCH, 2 * C, 128), F32),
            pltpu.VMEM((1, NCH, 2 * C, 128), F32),
            pltpu.VMEM((S, D), BF16),
            pltpu.VMEM((2 * C, C), BF16),
            pltpu.VMEM((C, 2 * C), BF16),
            pltpu.VMEM((2 * (SEG + M), 128), F32),
            pltpu.VMEM((KS, D), BF16),
            pltpu.VMEM((NB, 128), BF16),
            pltpu.VMEM((NB, 128), BF16),
            pltpu.SMEM((2,), jnp.int32),
            pltpu.SemaphoreType.DMA((6,)),
            pltpu.SemaphoreType.DMA((NB,)),
        ],
        compiler_params=pltpu.CompilerParams(vmem_limit_bytes=120 * 2 ** 20, disable_bounds_checks=True),
    )(
        A_q.reshape(S, D), A_k.reshape(S, D), A_v.reshape(S, D), A_ssm_k,
        B_Wq.reshape(D // 2, 2, H, E), B_Wk.reshape(D // 2, 2, H, E), B_Wv.reshape(D // 2, 2, H, E),
        B_Wo.reshape(H * E, D),
        A_shift_k.T, A_ssm_D.reshape(NB, 128), gate_w.reshape(NB, 128), B_mem0.reshape(M, D),
        jnp.asarray(fwd, BF16), jnp.asarray(inv, BF16), jnp.asarray(_attn_fill()),
    )
    return out.reshape(1, S, D)


def pallas_gated_mix__ssm_conv_h3__memory_aug_recurrent_mem_tr__prompt_kernel(
    A_q, A_k, A_v, A_shift_k, A_ssm_k, A_ssm_D, B_x, B_mem0, B_Wq, B_Wk, B_Wv, B_Wo, B_seg_len, gate_w,
):
    del B_x
    if isinstance(B_seg_len, int):
        assert B_seg_len == SEG
    return _run(A_q, A_k, A_v, A_shift_k, A_ssm_k, A_ssm_D, B_mem0, B_Wq, B_Wk, B_Wv, B_Wo, gate_w)
```

```python
import functools
import math

import jax
import jax.numpy as jnp
import numpy as np
import jax.experimental.pallas as pl
import jax.experimental.pallas.tpu as pltpu

F32 = jnp.float32
BF16 = jnp.bfloat16
U32 = jnp.uint32

S = 2048
D = 1024
H = 32
E = 128
M = 8
SEG = 32
NSEG = S // SEG
RX = 24
PRO = S - RX * NSEG
QCAP = 576
QOFF = QCAP - PRO
HL = 8
HS = H - HL
UNROLL = 4
C = 128
NCH = S // C
NB = D // 128
KS = 4
NEG = -1000000000.0


def _dft_tables():
    n = np.arange(C, dtype=np.float64)
    th = np.pi * (2.0 * np.arange(C, dtype=np.float64) + 1.0) / (2 * C)
    fwd = np.concatenate([np.cos(th[:, None] * n[None, :]), -np.sin(th[:, None] * n[None, :])], axis=0)
    inv = np.concatenate([np.cos(n[:, None] * th[None, :]), -np.sin(n[:, None] * th[None, :])], axis=1) / C
    return fwd.astype(np.float32), inv.astype(np.float32)


def _attn_fill():
    n = 2 * (SEG + M)
    head = np.array([0] * SEG + [1] * SEG + [0] * M + [1] * M)
    pos = np.concatenate([M + np.arange(SEG), M + np.arange(SEG), np.arange(M), np.arange(M)])
    fill = np.full((n, 128), -np.inf, np.float32)
    for i in range(n):
        for j in range(n):
            if head[i] == head[j]:
                ok = pos[i] < M or pos[i] >= pos[j]
                fill[i, j] = 0.0 if ok else NEG
    return fill


def _dot(a, b):
    return jnp.dot(a, b, preferred_element_type=F32)


def _dot_nt(a, b):
    return jax.lax.dot_general(a, b, (((1,), (1,)), ((), ())), preferred_element_type=F32)


def _pack(a):
    return pltpu.bitcast(a.astype(BF16), U32)


def _unpack(a):
    return pltpu.bitcast(a, BF16)


def _kernel(x_hbm, k_hbm, v_hbm, h_hbm, wq_hbm, wk_hbm, wv_hbm, wo_hbm,
            sk_hbm, dd_hbm, gw_hbm, mem0_hbm, fwd_hbm, inv_hbm, fill_hbm,
            out_hbm,
            x_v, xp, k_v, v_v, h_v, w_even, w_odd, wo_v, y_v, qkv_b, o_b, lo_s, mem_v, oacc, qacc,
            kf, u_s, h_s, yf_s,
            out_v, fwd_ref, inv_ref, fill_ref, sk_ref, dd_ref, gw_ref, zs, sems, qsems):
    scale = E ** (-0.5)
    wbuf = (w_even, w_odd)

    w32 = [w.bitcast(U32) for w in (wq_hbm, wk_hbm, wv_hbm)]
    wo32 = wo_hbm.bitcast(U32)
    x32 = x_hbm.bitcast(U32)

    def lanes(c):
        return pl.ds(pl.multiple_of(c * 128, 128), 128)

    def w_copies(c, e, mat, sem):
        return [pltpu.make_async_copy(w32[mat].at[:, par, 2 * c + e, :], wbuf[e].at[mat, c, par], sem)
                for par in range(2)]

    def wq0_copies(c):
        return w_copies(c, 0, 0, qsems.at[c])

    def block_copies(c):
        sem = sems.at[c % 2]
        return ([[pltpu.make_async_copy(h_hbm.at[lanes(c), :], h_v.at[c], sem)],
                 [pltpu.make_async_copy(k_hbm.at[:, lanes(c)], k_v.at[c], sem)],
                 [pltpu.make_async_copy(v_hbm.at[:, lanes(c)], v_v.at[c], sem)]]
                + [w_copies(c, e, mat, sem) for e in range(2) for mat in range(3) if (e, mat) != (0, 0)])

    def rest_copies(c):
        rows = pl.ds(pl.multiple_of(c * (S // NB), S // NB), S // NB)
        return [pltpu.make_async_copy(wo32.at[:, lanes(c)], wo_v.at[c], sems.at[2]),
                pltpu.make_async_copy(x_hbm.at[rows, :], x_v.at[rows, :], sems.at[2])]

    xp_copy = pltpu.make_async_copy(x32.at[pl.ds(0, PRO // 2), :], xp, sems.at[3])
    small_copies = [pltpu.make_async_copy(src, dst, sems.at[4]) for src, dst in (
        (sk_hbm, sk_ref), (fwd_hbm, fwd_ref), (dd_hbm, dd_ref), (inv_hbm, inv_ref),
        (gw_hbm, gw_ref), (mem0_hbm, mem_v), (fill_hbm, fill_ref))]

    def out_copy(start, n):
        rows = pl.ds(start, n)
        return pltpu.make_async_copy(out_v.at[rows, :], out_hbm.at[rows, :], sems.at[5])

    def row_of(ref, c):
        t = ref[...].astype(F32)
        sel = jax.lax.broadcasted_iota(jnp.int32, (NB, 128), 0) == c
        return jnp.sum(jnp.where(sel, t, 0.0), axis=0, keepdims=True)

    def fwd_dft(c, zw):
        skt = sk_ref[:, lanes(c)].astype(F32)
        for a in range(NCH):
            hf = _dot_nt(fwd_ref[...], h_v[c, :, pl.ds(a * C, C)])
            if a == 0:
                h_s[zw, a, 0:C, :] = hf[0:C] + row_of(dd_ref, c)
                h_s[zw, a, C:, :] = hf[C:]
            else:
                h_s[zw, a] = hf
            kf[pl.ds(8 + a * C, C), :] = k_v[c, pl.ds(a * C, C), :].astype(F32)
            ks_ = kf[pl.ds(8 + a * C, C), :] * skt[0:1, :]
            for j in range(1, KS):
                ks_ = ks_ + kf[pl.ds(8 + a * C - j, C), :] * skt[j:j + 1, :]
            kv = (ks_ * v_v[c, pl.ds(a * C, C), :].astype(F32)).astype(BF16)
            u_s[zw, a] = _dot(fwd_ref[...], kv)

    def mac(p, zw, zr):
        re = pl.ds(p * 8, 8)
        im = pl.ds(C + p * 8, 8)
        sgn = (1 - 2 * (jax.lax.broadcasted_iota(jnp.int32, (8, 128), 0) % 2)).astype(F32)
        AB = 4
        prev = None
        for a0 in range(0, NCH, AB):
            zre = [None] * AB
            zim = [None] * AB
            for m in range(a0 + AB):
                hr = h_s[zr, m, re, :]
                hi = h_s[zr, m, im, :]
                for i in range(AB):
                    t = a0 + i - m
                    if t < 0:
                        continue
                    ur = u_s[zr, t, re, :]
                    ui = u_s[zr, t, im, :]
                    tr = hr * ur - hi * ui
                    ti = hr * ui + hi * ur
                    zre[i] = tr if zre[i] is None else zre[i] + tr
                    zim[i] = ti if zim[i] is None else zim[i] + ti
            for i in range(AB):
                if prev is None:
                    yf_s[zw, a0 + i, re, :] = zre[i]
                    yf_s[zw, a0 + i, im, :] = zim[i]
                else:
                    yf_s[zw, a0 + i, re, :] = zre[i] - sgn * prev[1]
                    yf_s[zw, a0 + i, im, :] = zim[i] + sgn * prev[0]
                prev = (zre[i], zim[i])

    def inv_dft(c, zr):
        for a in range(NCH):
            y_v[pl.ds(a * C, C), lanes(c)] = _dot(inv_ref[...], yf_s[zr, a].astype(BF16)).astype(BF16)

    def fixup(e, c, mat):
        a = wbuf[e][mat, c, 0]
        b = wbuf[e][mat, c, 1]
        wbuf[e][mat, c, 0] = (a & U32(0xFFFF)) | (b << 16)
        wbuf[e][mat, c, 1] = (a >> 16) | (b & U32(0xFFFF0000))

    RB = 128

    def qkv_tile(e, c, n):
        mat, j = n // 2, n % 2
        for r in range(PRO // RB):
            w = _unpack(wbuf[e][mat, c, j])
            xr = _unpack(xp[pl.ds(r * RB // 2, RB // 2), :])
            qkv_b[mat, 2 * c + e, j, pl.ds((QOFF + r * RB) // 2, RB // 2), :] = _pack(_dot(xr, w))

    xp_copy.start()
    for cp in wq0_copies(0) + wq0_copies(1) + small_copies:
        cp.start()
    kf[0:8, :] = jnp.zeros((8, 128), F32)
    zs[0] = 0
    zs[1] = 0
    xp_copy.wait()

    def pro0(c, carry):
        @pl.when(c + 2 < NB)
        def _():
            for cp in wq0_copies(c + 2):
                cp.start()

        for i, piece in enumerate(block_copies(0)):
            @pl.when(c == i)
            def _():
                for cp in piece:
                    cp.start()

        for cp in wq0_copies(c):
            cp.wait()
        fixup(0, c, 0)
        qkv_tile(0, c, 0)
        qkv_tile(0, c, 1)
        return carry

    with jax.named_scope("pro0"):
        jax.lax.fori_loop(0, NB, pro0, 0)
    for cp in small_copies:
        cp.wait()

    zw = zs[0]
    zr = zs[1]

    def pro(c, carry):
        @pl.when(c + 1 < NB)
        def _():
            for piece in block_copies(c + 1):
                for cp in piece:
                    cp.start()

        for cp in rest_copies(c):
            cp.start()
        for piece in block_copies(c):
            for cp in piece:
                cp.wait()

        tiles = [(0, n) for n in range(2, 6)] + [(1, n) for n in range(6)]

        def tile(i):
            e, n = tiles[i]
            if n % 2 == 0:
                fixup(e, c, n // 2)
            qkv_tile(e, c, n)

        tile(0)
        fwd_dft(c, zw)
        p = 0
        for i in range(1, 8):
            tile(i)
            for _ in range(3 if i < 3 else 2):
                mac(p, zw, zr)
                p += 1
        inv_dft(c, zr)
        tile(8)
        tile(9)
        return carry

    with jax.named_scope("pro"):
        jax.lax.fori_loop(0, NB, pro, 0)
    for c in range(NB):
        for cp in rest_copies(c):
            cp.wait()

    gwt = gw_ref[...].astype(F32)
    gw = jnp.concatenate([gwt[j:j + 1, :] for j in range(NB)], axis=1)

    def finalize(rows, b):
        xr = x_v[rows, :].astype(F32)
        g = jax.nn.sigmoid(jnp.sum(xr * gw, axis=-1, keepdims=True))
        a = xr * y_v[rows, :].astype(F32)
        out_v[rows, :] = (g * a + (1.0 - g) * b).astype(BF16)

    def step(s, mem, split_first, odd):
        xrows = slice(M, M + RX) if odd else slice(0, RX)
        mrows = slice(0, M) if odd else slice(RX, RX + M)
        sh = 4 if odd else 0
        xo = pl.multiple_of(PRO + RX * s, 8)
        wbase = pl.multiple_of((RX // 2 * s) % (QCAP // 2) - sh, 8)
        rpos = pl.multiple_of((SEG // 2 * s + QOFF // 2) % (QCAP // 2), SEG // 2)
        opos = pl.multiple_of(SEG // 2 * s, SEG // 2)
        fbase = pl.multiple_of(RX // 2 * s - sh, 8)
        xs = x_v[pl.ds(xo, RX), :]
        lhs = jnp.concatenate([mem, xs] if odd else [xs, mem], axis=0)
        zpad = jnp.zeros((128 - 2 * (SEG + M), E), BF16)
        frows = pl.ds(pl.multiple_of(RX * s, 8), RX)
        low = jax.lax.broadcasted_iota(jnp.int32, (8, E), 0) < 4
        NP = H // 2

        mem_qkv = {}
        probs = {}
        cats = {}

        def load(mat, hp):
            if not 0 <= hp < NP:
                return
            parts = [_unpack(qkv_b[mat, hp, 0, pl.ds(rpos, SEG // 2), :]),
                     _unpack(qkv_b[mat, hp, 1, pl.ds(rpos, SEG // 2), :]), mem_qkv[(hp, mat)]]
            if mat > 0:
                parts.append(zpad)
            cats[(mat, hp)] = jnp.concatenate(parts, axis=0)

        def stage_a(hp, midfn):
            KH = D // 2
            split = split_first and hp == 0
            if split:
                for mat in range(3):
                    for j in range(2):
                        w = _unpack(wbuf[hp % 2][mat, hp // 2, j, :KH // 2, :])
                        qacc[2 * mat + j] = _dot(lhs[:, :KH], w)
            for mat in range(3):
                mm = []
                for j in range(2):
                    if split:
                        w = _unpack(wbuf[hp % 2][mat, hp // 2, j, KH // 2:, :])
                        res = qacc[2 * mat + j] + _dot(lhs[:, KH:], w)
                    else:
                        res = _dot(lhs, _unpack(wbuf[hp % 2][mat, hp // 2, j]))
                    pk = _pack(res)
                    if odd:
                        qkv_b[mat, hp, j, pl.ds(wbase + 4, 4), :] = pk[4:8]
                        qkv_b[mat, hp, j, pl.ds(wbase + 8, 8), :] = pk[8:16]
                    else:
                        qkv_b[mat, hp, j, pl.ds(wbase, 8), :] = pk[0:8]
                        qkv_b[mat, hp, j, pl.ds(wbase + 8, 4), :] = pk[8:12]
                    mm.append(res[mrows])
                    if (mat, j) == (1, 0):
                        midfn()
                mem_qkv[(hp, mat)] = jnp.concatenate(mm, axis=0).astype(BF16)

        def stage_b(hp):
            if not 0 <= hp < NP:
                return
            sc = _dot_nt(cats[(0, hp)], cats[(1, hp)]) * scale
            fill = fill_ref[...]
            sc = jnp.where(fill == 0.0, sc, fill)
            mx = jnp.max(sc, axis=-1, keepdims=True)
            p = jnp.exp(sc - mx)
            l = jnp.sum(p, axis=-1, keepdims=True)
            r = pl.reciprocal(l, approx=True)
            r = r * (2.0 - l * r)
            probs[hp] = (p.astype(BF16), r)

        def stage_c(hp):
            if not 0 <= hp < NP:
                return
            o = _dot(probs[hp][0], cats[(2, hp)]) * probs[hp][1]
            for j in range(2):
                h = 2 * hp + j
                cols = slice(h * E, (h + 1) * E)
                o_b[pl.ds(opos, SEG // 2), cols] = _pack(o[j * SEG:(j + 1) * SEG])
                om = o[2 * SEG + j * M:2 * SEG + (j + 1) * M]
                om = _pack(jnp.concatenate([om, om], axis=0))
                w0 = o_b[pl.ds(fbase, 8), cols]
                w1 = o_b[pl.ds(fbase + 8, 8), cols]
                lo_s[0:8, cols] = jnp.where(low, om, w0) if odd else w0
                lo_s[8:16, cols] = w1 if odd else jnp.where(low, w1, om)

        def oproj(j, late):
            ks = slice(HS * E, H * E) if late else slice(0, HS * E)
            kw = slice(ks.start // 2, ks.stop // 2)
            return _dot(_unpack(lo_s[:, ks]), _unpack(wo_v[j, kw, :]))

        DB, DC = 1, 3
        outs = [None] * NB
        for t in range(NP + DC):
            load(0, t - DB)
            load(1, t - DB)
            load(2, t - DC)
            if t < NP:
                stage_a(t, lambda: stage_c(t - DC))
            else:
                for j in range(2 * (t - NP), 2 * (t - NP) + 2):
                    oacc[:, j * 128:(j + 1) * 128] = oproj(j, False)
            if t >= NP:
                stage_c(t - DC)
            stage_b(t - DB)
        for j in range(2 * DC, NB):
            oacc[:, j * 128:(j + 1) * 128] = oproj(j, False)
        for j in range(NB):
            outs[j] = oacc[:, j * 128:(j + 1) * 128] + oproj(j, True)
        res = jnp.concatenate(outs, axis=1)
        finalize(frows, res[xrows])
        return res[mrows].astype(BF16)

    def steps(i, carry):
        mem = mem_v[...]
        for u in range(UNROLL):
            mem = step(i * UNROLL + u, mem, u > 0, u % 2 == 1)
        mem_v[...] = mem
        return carry

    with jax.named_scope("main"):
        jax.lax.fori_loop(0, NSEG // UNROLL, steps, 0)

    def epi_rows(r0, n):
        lo = _unpack(o_b[pl.ds(pl.multiple_of(r0 // 2, 8), n // 2), :])
        outs = [_dot(lo, _unpack(wo_v[j])) for j in range(NB)]
        finalize(pl.ds(r0, n), jnp.concatenate(outs, axis=1))

    EB = 128

    def epi(r, carry):
        r0 = pl.multiple_of(S - PRO + r * EB, EB)

        @pl.when(r == PRO // EB - 1)
        def _():
            out_copy(S - PRO, PRO - EB).start()

        epi_rows(r0, EB)
        return carry

    with jax.named_scope("epi"):
        out_copy(0, S - PRO).start()
        jax.lax.fori_loop(0, PRO // EB, epi, 0)
    out_copy(S - EB, EB).start()
    out_copy(0, S).wait()


@jax.jit
def _run(A_q, A_k, A_v, A_shift_k, A_ssm_k, A_ssm_D, B_mem0, B_Wq, B_Wk, B_Wv, B_Wo, gate_w):
    fwd, inv = _dft_tables()
    any_spec = pl.BlockSpec(memory_space=pl.ANY)
    out = pl.pallas_call(
        _kernel,
        out_shape=jax.ShapeDtypeStruct((S, D), BF16),
        in_specs=[any_spec] * 15,
        out_specs=any_spec,
        scratch_shapes=[
            pltpu.VMEM((S, D), BF16),
            pltpu.VMEM((PRO // 2, D), U32),
            pltpu.VMEM((NB, S, 128), BF16),
            pltpu.VMEM((NB, S, 128), BF16),
            pltpu.VMEM((NB, 128, S), BF16),
            pltpu.VMEM((3, H // 4, 2, D // 2, E), U32),
            pltpu.VMEM((3, H // 4, 2, D // 2, E), U32),
            pltpu.VMEM((NB, H * E // 2, 128), U32),
            pltpu.VMEM((S, D), BF16),
            pltpu.VMEM((3, H // 2, 2, QCAP // 2, E), U32),
            pltpu.VMEM((S // 2, H * E), U32),
            pltpu.VMEM(((M + RX) // 2, H * E), U32),
            pltpu.VMEM((M, D), BF16),
            pltpu.VMEM((M + RX, D), F32),
            pltpu.VMEM((6, M + RX, E), F32),
            pltpu.VMEM((S + 32, 128), F32),
            pltpu.VMEM((1, NCH, 2 * C, 128), F32),
            pltpu.VMEM((1, NCH, 2 * C, 128), F32),
            pltpu.VMEM((1, NCH, 2 * C, 128), F32),
            pltpu.VMEM((S, D), BF16),
            pltpu.VMEM((2 * C, C), BF16),
            pltpu.VMEM((C, 2 * C), BF16),
            pltpu.VMEM((2 * (SEG + M), 128), F32),
            pltpu.VMEM((KS, D), BF16),
            pltpu.VMEM((NB, 128), BF16),
            pltpu.VMEM((NB, 128), BF16),
            pltpu.SMEM((2,), jnp.int32),
            pltpu.SemaphoreType.DMA((6,)),
            pltpu.SemaphoreType.DMA((NB,)),
        ],
        compiler_params=pltpu.CompilerParams(vmem_limit_bytes=120 * 2 ** 20, disable_bounds_checks=True),
    )(
        A_q.reshape(S, D), A_k.reshape(S, D), A_v.reshape(S, D), A_ssm_k,
        B_Wq.reshape(D // 2, 2, H, E), B_Wk.reshape(D // 2, 2, H, E), B_Wv.reshape(D // 2, 2, H, E),
        B_Wo.reshape(H * E, D),
        A_shift_k.T, A_ssm_D.reshape(NB, 128), gate_w.reshape(NB, 128), B_mem0.reshape(M, D),
        jnp.asarray(fwd, BF16), jnp.asarray(inv, BF16), jnp.asarray(_attn_fill()),
    )
    return out.reshape(1, S, D)


def pallas_gated_mix__ssm_conv_h3__memory_aug_recurrent_mem_tr__prompt_kernel(
    A_q, A_k, A_v, A_shift_k, A_ssm_k, A_ssm_D, B_x, B_mem0, B_Wq, B_Wk, B_Wv, B_Wo, B_seg_len, gate_w,
):
    del B_x
    if isinstance(B_seg_len, int):
        assert B_seg_len == SEG
    return _run(A_q, A_k, A_v, A_shift_k, A_ssm_k, A_ssm_D, B_mem0, B_Wq, B_Wk, B_Wv, B_Wo, gate_w)
```

```python
import functools
import math

import jax
import jax.numpy as jnp
import numpy as np
import jax.experimental.pallas as pl
import jax.experimental.pallas.tpu as pltpu

F32 = jnp.float32
BF16 = jnp.bfloat16
U32 = jnp.uint32

S = 2048
D = 1024
H = 32
E = 128
M = 8
SEG = 32
NSEG = S // SEG
RX = 24
PRO = S - RX * NSEG
QCAP = 576
QOFF = QCAP - PRO
HL = 8
HS = H - HL
MAT_ORDER = (0, 1, 2)
OFF_LQK, OFF_S, OFF_LV, OFF_PV = 4, 9, 15, 18
UNROLL = 4
C = 128
NCH = S // C
NB = D // 128
KS = 4
NEG = -1000000000.0


def _dft_tables():
    n = np.arange(C, dtype=np.float64)
    k = np.concatenate([np.arange(C // 2), C - 1 - np.arange(C // 2)]).astype(np.float64)
    th = np.pi * (2.0 * k + 1.0) / (2 * C)
    fwd = np.concatenate([np.cos(th[:, None] * n[None, :]), -np.sin(th[:, None] * n[None, :])], axis=0)
    no = np.concatenate([n[0::2], n[1::2]])
    tl = th[:C // 2]
    inv = np.concatenate([np.cos(no[:, None] * tl[None, :]), -np.sin(no[:, None] * tl[None, :])], axis=1) / C
    return fwd.astype(np.float32), inv.astype(np.float32)


def _attn_fill():
    n = 2 * (SEG + M)
    head = np.array([0] * SEG + [1] * SEG + [0] * M + [1] * M)
    pos = np.concatenate([M + np.arange(SEG), M + np.arange(SEG), np.arange(M), np.arange(M)])
    fill = np.full((n, 128), -np.inf, np.float32)
    for i in range(n):
        for j in range(n):
            if head[i] == head[j]:
                ok = pos[i] < M or pos[i] >= pos[j]
                fill[i, j] = 0.0 if ok else NEG
    return fill


def _dot(a, b):
    return jnp.dot(a, b, preferred_element_type=F32)


def _dot_nt(a, b):
    return jax.lax.dot_general(a, b, (((1,), (1,)), ((), ())), preferred_element_type=F32)


def _pack(a):
    return pltpu.bitcast(a.astype(BF16), U32)


def _unpack(a):
    return pltpu.bitcast(a, BF16)


def _kernel(x_hbm, k_hbm, v_hbm, h_hbm, wq_hbm, wk_hbm, wv_hbm, wo_hbm,
            sk_hbm, dd_hbm, gw_hbm, mem0_hbm, fwd_hbm, inv_hbm, fill_hbm,
            out_hbm,
            x_v, xp, k_v, v_v, h_v, w_even, w_odd, wo_v, y_v, qkv_b, o_b, lo_s, mem_v, oacc, qacc,
            kf, u_s, h_s, yf_s,
            out_v, fwd_ref, inv_ref, fill_ref, sk_ref, dd_ref, gw_ref, zs, sems, qsems):
    scale = E ** (-0.5)
    wbuf = (w_even, w_odd)

    w32 = [w.bitcast(U32) for w in (wq_hbm, wk_hbm, wv_hbm)]
    wo32 = wo_hbm.bitcast(U32)
    x32 = x_hbm.bitcast(U32)

    def lanes(c):
        return pl.ds(pl.multiple_of(c * 128, 128), 128)

    def w_copies(c, e, mat, sem):
        return [pltpu.make_async_copy(w32[mat].at[:, par, 2 * c + e, :], wbuf[e].at[mat, c, par], sem)
                for par in range(2)]

    def wq0_copies(c):
        return w_copies(c, 0, 0, qsems.at[c])

    def block_copies(c):
        sem = sems.at[c % 2]
        return ([[pltpu.make_async_copy(h_hbm.at[lanes(c), :], h_v.at[c], sem)],
                 [pltpu.make_async_copy(k_hbm.at[:, lanes(c)], k_v.at[c], sem)],
                 [pltpu.make_async_copy(v_hbm.at[:, lanes(c)], v_v.at[c], sem)]]
                + [w_copies(c, e, mat, sem) for e in range(2) for mat in range(3) if (e, mat) != (0, 0)])

    def rest_copies(c):
        rows = pl.ds(pl.multiple_of(c * (S // NB), S // NB), S // NB)
        return [pltpu.make_async_copy(wo32.at[:, lanes(c)], wo_v.at[c], sems.at[2]),
                pltpu.make_async_copy(x_hbm.at[rows, :], x_v.at[rows, :], sems.at[2])]

    xp_copy = pltpu.make_async_copy(x32.at[pl.ds(0, PRO // 2), :], xp, sems.at[3])
    small_copies = [pltpu.make_async_copy(src, dst, sems.at[4]) for src, dst in (
        (sk_hbm, sk_ref), (fwd_hbm, fwd_ref), (dd_hbm, dd_ref), (inv_hbm, inv_ref),
        (gw_hbm, gw_ref), (mem0_hbm, mem_v), (fill_hbm, fill_ref))]

    def out_copy(start, n):
        rows = pl.ds(start, n)
        return pltpu.make_async_copy(out_v.at[rows, :], out_hbm.at[rows, :], sems.at[5])

    def row_of(ref, c):
        t = ref[...].astype(F32)
        sel = jax.lax.broadcasted_iota(jnp.int32, (NB, 128), 0) == c
        return jnp.sum(jnp.where(sel, t, 0.0), axis=0, keepdims=True)

    def fwd_dft(c, zw):
        skt = sk_ref[:, lanes(c)].astype(F32)
        for a in range(NCH):
            hf = _dot_nt(fwd_ref[...], h_v[c, :, pl.ds(a * C, C)])
            if a == 0:
                h_s[zw, a, 0:C, :] = hf[0:C] + row_of(dd_ref, c)
                h_s[zw, a, C:, :] = hf[C:]
            else:
                h_s[zw, a] = hf
            kf[pl.ds(8 + a * C, C), :] = k_v[c, pl.ds(a * C, C), :].astype(F32)
            ks_ = kf[pl.ds(8 + a * C, C), :] * skt[0:1, :]
            for j in range(1, KS):
                ks_ = ks_ + kf[pl.ds(8 + a * C - j, C), :] * skt[j:j + 1, :]
            kv = (ks_ * v_v[c, pl.ds(a * C, C), :].astype(F32)).astype(BF16)
            u_s[zw, a] = _dot(fwd_ref[...], kv)

    def mac(p, zw, zr):
        re = pl.ds(p * 8, 8)
        im = pl.ds(C + p * 8, 8)
        sgn = (1 - 2 * (jax.lax.broadcasted_iota(jnp.int32, (8, 128), 0) % 2)).astype(F32)
        if p >= C // 16:
            sgn = -sgn
        AB = 4
        prev = None
        for a0 in range(0, NCH, AB):
            zre = [None] * AB
            zim = [None] * AB
            for m in range(a0 + AB):
                hr = h_s[zr, m, re, :]
                hi = h_s[zr, m, im, :]
                for i in range(AB):
                    t = a0 + i - m
                    if t < 0:
                        continue
                    ur = u_s[zr, t, re, :]
                    ui = u_s[zr, t, im, :]
                    tr = hr * ur - hi * ui
                    ti = hr * ui + hi * ur
                    zre[i] = tr if zre[i] is None else zre[i] + tr
                    zim[i] = ti if zim[i] is None else zim[i] + ti
            for i in range(AB):
                if prev is None:
                    yf_s[zw, a0 + i, re, :] = zre[i]
                    yf_s[zw, a0 + i, im, :] = zim[i]
                else:
                    yf_s[zw, a0 + i, re, :] = zre[i] - sgn * prev[1]
                    yf_s[zw, a0 + i, im, :] = zim[i] + sgn * prev[0]
                prev = (zre[i], zim[i])

    def inv_dft(c, zr):
        hc = C // 2
        for a in range(NCH):
            yr, yrm = yf_s[zr, a, 0:hc, :], yf_s[zr, a, hc:C, :]
            yi, yim = yf_s[zr, a, C:C + hc, :], yf_s[zr, a, C + hc:, :]
            fe = jnp.concatenate([yr + yrm, yi - yim], axis=0).astype(BF16)
            fo = jnp.concatenate([yr - yrm, yi + yim], axis=0).astype(BF16)
            y_v[c, pl.ds(a * C, hc, stride=2), :] = _dot(inv_ref[0:hc, :], fe)
            y_v[c, pl.ds(a * C + 1, hc, stride=2), :] = _dot(inv_ref[hc:, :], fo)

    def fixup(e, c, mat):
        a = wbuf[e][mat, c, 0]
        b = wbuf[e][mat, c, 1]
        wbuf[e][mat, c, 0] = (a & U32(0xFFFF)) | (b << 16)
        wbuf[e][mat, c, 1] = (a >> 16) | (b & U32(0xFFFF0000))

    RB = 128

    def qkv_tile(e, c, n):
        mat, j = n // 2, n % 2
        for r in range(PRO // RB):
            w = _unpack(wbuf[e][mat, c, j])
            xr = _unpack(xp[pl.ds(r * RB // 2, RB // 2), :])
            qkv_b[mat, 2 * c + e, j, pl.ds((QOFF + r * RB) // 2, RB // 2), :] = _pack(_dot(xr, w))

    xp_copy.start()
    for cp in wq0_copies(0) + wq0_copies(1) + small_copies:
        cp.start()
    kf[0:8, :] = jnp.zeros((8, 128), F32)
    zs[0] = 0
    zs[1] = 0
    xp_copy.wait()

    def pro0(c, carry):
        @pl.when(c + 2 < NB)
        def _():
            for cp in wq0_copies(c + 2):
                cp.start()

        for i, piece in enumerate(block_copies(0)):
            @pl.when(c == i)
            def _():
                for cp in piece:
                    cp.start()

        for cp in wq0_copies(c):
            cp.wait()
        fixup(0, c, 0)
        qkv_tile(0, c, 0)
        qkv_tile(0, c, 1)
        return carry

    with jax.named_scope("pro0"):
        jax.lax.fori_loop(0, NB, pro0, 0)
    for cp in small_copies:
        cp.wait()

    zw = zs[0]
    zr = zs[1]

    def pro(c, carry):
        @pl.when(c + 1 < NB)
        def _():
            for piece in block_copies(c + 1):
                for cp in piece:
                    cp.start()

        for cp in rest_copies(c):
            cp.start()
        for piece in block_copies(c):
            for cp in piece:
                cp.wait()

        tiles = [(0, n) for n in range(2, 6)] + [(1, n) for n in range(6)]

        def tile(i):
            e, n = tiles[i]
            if n % 2 == 0:
                fixup(e, c, n // 2)
            qkv_tile(e, c, n)

        tile(0)
        fwd_dft(c, zw)
        p = 0
        for i in range(1, 8):
            tile(i)
            for _ in range(3 if i < 3 else 2):
                mac(p, zw, zr)
                p += 1
        inv_dft(c, zr)
        tile(8)
        tile(9)
        return carry

    with jax.named_scope("pro"):
        jax.lax.fori_loop(0, NB, pro, 0)
    for c in range(NB):
        for cp in rest_copies(c):
            cp.wait()

    gwt = gw_ref[...].astype(F32)
    gw = jnp.concatenate([gwt[j:j + 1, :] for j in range(NB)], axis=1)

    def finalize(rows, b):
        xr = x_v[rows, :].astype(F32)
        g = jax.nn.sigmoid(jnp.sum(xr * gw, axis=-1, keepdims=True))
        a = xr * jnp.concatenate([y_v[j, rows, :] for j in range(NB)], axis=1)
        out_v[rows, :] = (g * a + (1.0 - g) * b).astype(BF16)

    def step(s, mem, split_first, odd):
        xrows = slice(M, M + RX) if odd else slice(0, RX)
        mrows = slice(0, M) if odd else slice(RX, RX + M)
        sh = 4 if odd else 0
        xo = pl.multiple_of(PRO + RX * s, 8)
        wbase = pl.multiple_of((RX // 2 * s) % (QCAP // 2) - sh, 8)
        rpos = pl.multiple_of((SEG // 2 * s + QOFF // 2) % (QCAP // 2), SEG // 2)
        opos = pl.multiple_of(SEG // 2 * s, SEG // 2)
        fbase = pl.multiple_of(RX // 2 * s - sh, 8)
        xs = x_v[pl.ds(xo, RX), :]
        lhs = jnp.concatenate([mem, xs] if odd else [xs, mem], axis=0)
        zpad = jnp.zeros((128 - 2 * (SEG + M), E), BF16)
        frows = pl.ds(pl.multiple_of(RX * s, 8), RX)
        low = jax.lax.broadcasted_iota(jnp.int32, (8, E), 0) < 4
        NP = H // 2

        mem_qkv = {}
        probs = {}
        cats = {}

        def load(mat, hp):
            parts = [_unpack(qkv_b[mat, hp, 0, pl.ds(rpos, SEG // 2), :]),
                     _unpack(qkv_b[mat, hp, 1, pl.ds(rpos, SEG // 2), :]), mem_qkv[(hp, mat)]]
            if mat > 0:
                parts.append(zpad)
            cats[(mat, hp)] = jnp.concatenate(parts, axis=0)

        def stage_a(hp):
            KH = D // 2
            split = split_first and hp == 0
            if split:
                for mat in range(3):
                    for j in range(2):
                        w = _unpack(wbuf[hp % 2][mat, hp // 2, j, :KH // 2, :])
                        qacc[2 * mat + j] = _dot(lhs[:, :KH], w)
            for mi, mat in enumerate(MAT_ORDER):
                mm = []
                for j in range(2):
                    if split:
                        w = _unpack(wbuf[hp % 2][mat, hp // 2, j, KH // 2:, :])
                        res = qacc[2 * mat + j] + _dot(lhs[:, KH:], w)
                    else:
                        res = _dot(lhs, _unpack(wbuf[hp % 2][mat, hp // 2, j]))
                    pk = _pack(res)
                    if odd:
                        qkv_b[mat, hp, j, pl.ds(wbase + 4, 4), :] = pk[4:8]
                        qkv_b[mat, hp, j, pl.ds(wbase + 8, 8), :] = pk[8:16]
                    else:
                        qkv_b[mat, hp, j, pl.ds(wbase, 8), :] = pk[0:8]
                        qkv_b[mat, hp, j, pl.ds(wbase + 8, 4), :] = pk[8:12]
                    mm.append(res[mrows])
                    if j == 1:
                        mem_qkv[(hp, mat)] = jnp.concatenate(mm, axis=0).astype(BF16)
                    advance(6 * hp + 2 * mi + j + 1)

        def stage_b(hp):
            sc = _dot_nt(cats[(0, hp)], cats[(1, hp)]) * scale
            fill = fill_ref[...]
            sc = jnp.where(fill == 0.0, sc, fill)
            mx = jnp.max(sc, axis=-1, keepdims=True)
            p = jnp.exp(sc - mx)
            l = jnp.sum(p, axis=-1, keepdims=True)
            r = pl.reciprocal(l, approx=True)
            r = r * (2.0 - l * r)
            probs[hp] = (p.astype(BF16), r)

        def stage_c(hp):
            o = _dot(probs[hp][0], cats[(2, hp)]) * probs[hp][1]
            for j in range(2):
                h = 2 * hp + j
                cols = slice(h * E, (h + 1) * E)
                o_b[pl.ds(opos, SEG // 2), cols] = _pack(o[j * SEG:(j + 1) * SEG])
                om = o[2 * SEG + j * M:2 * SEG + (j + 1) * M]
                om = _pack(jnp.concatenate([om, om], axis=0))
                w0 = o_b[pl.ds(fbase, 8), cols]
                w1 = o_b[pl.ds(fbase + 8, 8), cols]
                lo_s[0:8, cols] = jnp.where(low, om, w0) if odd else w0
                lo_s[8:16, cols] = w1 if odd else jnp.where(low, w1, om)

        def oproj(j, late):
            ks = slice(HS * E, H * E) if late else slice(0, HS * E)
            kw = slice(ks.start // 2, ks.stop // 2)
            return _dot(_unpack(lo_s[:, ks]), _unpack(wo_v[j, kw, :]))

        events = []
        for hp in range(NP):
            events.append((6 * hp + OFF_LQK, 0, functools.partial(load, 0, hp)))
            events.append((6 * hp + OFF_LQK, 1, functools.partial(load, 1, hp)))
            events.append((6 * hp + OFF_LV, 2, functools.partial(load, 2, hp)))
            events.append((6 * hp + OFF_PV, 3, functools.partial(stage_c, hp)))
            events.append((6 * hp + OFF_S, 4, functools.partial(stage_b, hp)))
        events.sort(key=lambda ev: ev[:2])

        def advance(slot):
            while events and events[0][0] <= slot:
                events.pop(0)[2]()

        outs = [None] * NB
        for hp in range(NP):
            stage_a(hp)
        for j in range(NB):
            oacc[:, j * 128:(j + 1) * 128] = oproj(j, False)
            advance(6 * NP + (j + 1) * HS // 8)
        assert not events
        for j in range(NB):
            outs[j] = oacc[:, j * 128:(j + 1) * 128] + oproj(j, True)
        res = jnp.concatenate(outs, axis=1)
        finalize(frows, res[xrows])
        return res[mrows].astype(BF16)

    def steps(i, carry):
        mem = mem_v[...]
        for u in range(UNROLL):
            mem = step(i * UNROLL + u, mem, u > 0, u % 2 == 1)
        mem_v[...] = mem
        return carry

    with jax.named_scope("main"):
        jax.lax.fori_loop(0, NSEG // UNROLL, steps, 0)

    def epi_rows(r0, n):
        lo = _unpack(o_b[pl.ds(pl.multiple_of(r0 // 2, 8), n // 2), :])
        outs = [_dot(lo, _unpack(wo_v[j])) for j in range(NB)]
        finalize(pl.ds(r0, n), jnp.concatenate(outs, axis=1))

    EB = 128

    def epi(r, carry):
        r0 = pl.multiple_of(S - PRO + r * EB, EB)

        @pl.when(r == PRO // EB - 1)
        def _():
            out_copy(S - PRO, PRO - EB).start()

        epi_rows(r0, EB)
        return carry

    with jax.named_scope("epi"):
        out_copy(0, S - PRO).start()
        jax.lax.fori_loop(0, PRO // EB, epi, 0)
    out_copy(S - EB, EB).start()
    out_copy(0, S).wait()


@jax.jit
def _run(A_q, A_k, A_v, A_shift_k, A_ssm_k, A_ssm_D, B_mem0, B_Wq, B_Wk, B_Wv, B_Wo, gate_w):
    fwd, inv = _dft_tables()
    any_spec = pl.BlockSpec(memory_space=pl.ANY)
    out = pl.pallas_call(
        _kernel,
        out_shape=jax.ShapeDtypeStruct((S, D), BF16),
        in_specs=[any_spec] * 15,
        out_specs=any_spec,
        scratch_shapes=[
            pltpu.VMEM((S, D), BF16),
            pltpu.VMEM((PRO // 2, D), U32),
            pltpu.VMEM((NB, S, 128), BF16),
            pltpu.VMEM((NB, S, 128), BF16),
            pltpu.VMEM((NB, 128, S), BF16),
            pltpu.VMEM((3, H // 4, 2, D // 2, E), U32),
            pltpu.VMEM((3, H // 4, 2, D // 2, E), U32),
            pltpu.VMEM((NB, H * E // 2, 128), U32),
            pltpu.VMEM((NB, S, 128), F32),
            pltpu.VMEM((3, H // 2, 2, QCAP // 2, E), U32),
            pltpu.VMEM((S // 2, H * E), U32),
            pltpu.VMEM(((M + RX) // 2, H * E), U32),
            pltpu.VMEM((M, D), BF16),
            pltpu.VMEM((M + RX, D), F32),
            pltpu.VMEM((6, M + RX, E), F32),
            pltpu.VMEM((S + 32, 128), F32),
            pltpu.VMEM((1, NCH, 2 * C, 128), F32),
            pltpu.VMEM((1, NCH, 2 * C, 128), F32),
            pltpu.VMEM((1, NCH, 2 * C, 128), F32),
            pltpu.VMEM((S, D), BF16),
            pltpu.VMEM((2 * C, C), BF16),
            pltpu.VMEM((C, C), BF16),
            pltpu.VMEM((2 * (SEG + M), 128), F32),
            pltpu.VMEM((KS, D), BF16),
            pltpu.VMEM((NB, 128), BF16),
            pltpu.VMEM((NB, 128), BF16),
            pltpu.SMEM((2,), jnp.int32),
            pltpu.SemaphoreType.DMA((6,)),
            pltpu.SemaphoreType.DMA((NB,)),
        ],
        compiler_params=pltpu.CompilerParams(vmem_limit_bytes=120 * 2 ** 20, disable_bounds_checks=True),
    )(
        A_q.reshape(S, D), A_k.reshape(S, D), A_v.reshape(S, D), A_ssm_k,
        B_Wq.reshape(D // 2, 2, H, E), B_Wk.reshape(D // 2, 2, H, E), B_Wv.reshape(D // 2, 2, H, E),
        B_Wo.reshape(H * E, D),
        A_shift_k.T, A_ssm_D.reshape(NB, 128), gate_w.reshape(NB, 128), B_mem0.reshape(M, D),
        jnp.asarray(fwd, BF16), jnp.asarray(inv, BF16), jnp.asarray(_attn_fill()),
    )
    return out.reshape(1, S, D)


def pallas_gated_mix__ssm_conv_h3__memory_aug_recurrent_mem_tr__prompt_kernel(
    A_q, A_k, A_v, A_shift_k, A_ssm_k, A_ssm_D, B_x, B_mem0, B_Wq, B_Wk, B_Wv, B_Wo, B_seg_len, gate_w,
):
    del B_x
    if isinstance(B_seg_len, int):
        assert B_seg_len == SEG
    return _run(A_q, A_k, A_v, A_shift_k, A_ssm_k, A_ssm_D, B_mem0, B_Wq, B_Wk, B_Wv, B_Wo, gate_w)
```

```python
import functools
import math

import jax
import jax.numpy as jnp
import numpy as np
import jax.experimental.pallas as pl
import jax.experimental.pallas.tpu as pltpu

F32 = jnp.float32
BF16 = jnp.bfloat16
U32 = jnp.uint32

S = 2048
D = 1024
H = 32
E = 128
M = 8
SEG = 32
NSEG = S // SEG
RX = 24
PRO = S - RX * NSEG
QCAP = 576
QOFF = QCAP - PRO
HL = 8
HS = H - HL
MAT_ORDER = (0, 1, 2)
OFF_LQK, OFF_S, OFF_LV, OFF_PV = 4, 9, 15, 18
UNROLL = 4
C = 128
NCH = S // C
NB = D // 128
KS = 4
NEG = -1000000000.0


def _dft_tables():
    n = np.arange(C, dtype=np.float64)
    k = np.concatenate([np.arange(C // 2), C - 1 - np.arange(C // 2)]).astype(np.float64)
    th = np.pi * (2.0 * k + 1.0) / (2 * C)
    fwd = np.concatenate([np.cos(th[:, None] * n[None, :]), -np.sin(th[:, None] * n[None, :])], axis=0)
    no = np.concatenate([n[0::2], n[1::2]])
    tl = th[:C // 2]
    inv = np.concatenate([np.cos(no[:, None] * tl[None, :]), -np.sin(no[:, None] * tl[None, :])], axis=1) / C
    return fwd.astype(np.float32), inv.astype(np.float32)


def _attn_fill():
    n = 2 * (SEG + M)
    head = np.array([0] * SEG + [1] * SEG + [0] * M + [1] * M)
    pos = np.concatenate([M + np.arange(SEG), M + np.arange(SEG), np.arange(M), np.arange(M)])
    fill = np.full((n, 128), -np.inf, np.float32)
    for i in range(n):
        for j in range(n):
            if head[i] == head[j]:
                ok = pos[i] < M or pos[i] >= pos[j]
                fill[i, j] = 0.0 if ok else NEG
    return fill


def _dot(a, b):
    return jnp.dot(a, b, preferred_element_type=F32)


def _dot_nt(a, b):
    return jax.lax.dot_general(a, b, (((1,), (1,)), ((), ())), preferred_element_type=F32)


def _pack(a):
    return pltpu.bitcast(a.astype(BF16), U32)


def _unpack(a):
    return pltpu.bitcast(a, BF16)


def _kernel(x_hbm, k_hbm, v_hbm, h_hbm, wq_hbm, wk_hbm, wv_hbm, wo_hbm,
            sk_hbm, dd_hbm, gw_hbm, mem0_hbm, fwd_hbm, inv_hbm, fill_hbm,
            out_hbm,
            x_v, xp, k_v, v_v, h_v, w_even, w_odd, wo_v, y_v, qkv_b, o_b, lo_s, mem_v, oacc, qacc,
            kf, u_s, h_s, yf_s,
            out_v, fwd_ref, inv_ref, fill_ref, sk_ref, dd_ref, gw_ref, zs, sems, qsems):
    scale = E ** (-0.5)
    wbuf = (w_even, w_odd)

    w32 = [w.bitcast(U32) for w in (wq_hbm, wk_hbm, wv_hbm)]
    wo32 = wo_hbm.bitcast(U32)
    x32 = x_hbm.bitcast(U32)

    def lanes(c):
        return pl.ds(pl.multiple_of(c * 128, 128), 128)

    def w_copies(c, e, mat, sem):
        return [pltpu.make_async_copy(w32[mat].at[:, par, 2 * c + e, :], wbuf[e].at[mat, c, par], sem)
                for par in range(2)]

    def wq0_copies(c):
        return w_copies(c, 0, 0, qsems.at[c])

    def block_copies(c):
        sem = sems.at[c % 2]
        return ([[pltpu.make_async_copy(h_hbm.at[lanes(c), :], h_v.at[c], sem)],
                 [pltpu.make_async_copy(k_hbm.at[:, lanes(c)], k_v.at[c], sem)],
                 [pltpu.make_async_copy(v_hbm.at[:, lanes(c)], v_v.at[c], sem)]]
                + [w_copies(c, e, mat, sem) for e in range(2) for mat in range(3) if (e, mat) != (0, 0)])

    def rest_copies(c):
        rows = pl.ds(pl.multiple_of(c * (S // NB), S // NB), S // NB)
        return [pltpu.make_async_copy(wo32.at[:, lanes(c)], wo_v.at[c], sems.at[2]),
                pltpu.make_async_copy(x_hbm.at[rows, :], x_v.at[rows, :], sems.at[2])]

    xp_copy = pltpu.make_async_copy(x32.at[pl.ds(0, PRO // 2), :], xp, sems.at[3])
    small_copies = [pltpu.make_async_copy(src, dst, sems.at[4]) for src, dst in (
        (sk_hbm, sk_ref), (fwd_hbm, fwd_ref), (dd_hbm, dd_ref), (inv_hbm, inv_ref),
        (gw_hbm, gw_ref), (mem0_hbm, mem_v), (fill_hbm, fill_ref))]

    def out_copy(start, n):
        rows = pl.ds(start, n)
        return pltpu.make_async_copy(out_v.at[rows, :], out_hbm.at[rows, :], sems.at[5])

    def row_of(ref, c):
        t = ref[...].astype(F32)
        sel = jax.lax.broadcasted_iota(jnp.int32, (NB, 128), 0) == c
        return jnp.sum(jnp.where(sel, t, 0.0), axis=0, keepdims=True)

    def fwd_dft(c, zw):
        skt = sk_ref[:, lanes(c)].astype(F32)
        for a in range(NCH):
            hf = _dot_nt(fwd_ref[...], h_v[c, :, pl.ds(a * C, C)])
            if a == 0:
                h_s[zw, a, 0:C, :] = hf[0:C] + row_of(dd_ref, c)
                h_s[zw, a, C:, :] = hf[C:]
            else:
                h_s[zw, a] = hf
            kf[pl.ds(8 + a * C, C), :] = k_v[c, pl.ds(a * C, C), :].astype(F32)
            ks_ = kf[pl.ds(8 + a * C, C), :] * skt[0:1, :]
            for j in range(1, KS):
                ks_ = ks_ + kf[pl.ds(8 + a * C - j, C), :] * skt[j:j + 1, :]
            kv = (ks_ * v_v[c, pl.ds(a * C, C), :].astype(F32)).astype(BF16)
            u_s[zw, a] = _dot(fwd_ref[...], kv)

    def mac(p, zw, zr):
        re = pl.ds(p * 8, 8)
        im = pl.ds(C + p * 8, 8)
        sgn = (1 - 2 * (jax.lax.broadcasted_iota(jnp.int32, (8, 128), 0) % 2)).astype(F32)
        if p >= C // 16:
            sgn = -sgn
        AB = 4
        prev = None
        for a0 in range(0, NCH, AB):
            zre = [None] * AB
            zim = [None] * AB
            for m in range(a0 + AB):
                hr = h_s[zr, m, re, :]
                hi = h_s[zr, m, im, :]
                for i in range(AB):
                    t = a0 + i - m
                    if t < 0:
                        continue
                    ur = u_s[zr, t, re, :]
                    ui = u_s[zr, t, im, :]
                    tr = hr * ur - hi * ui
                    ti = hr * ui + hi * ur
                    zre[i] = tr if zre[i] is None else zre[i] + tr
                    zim[i] = ti if zim[i] is None else zim[i] + ti
            for i in range(AB):
                if prev is None:
                    yf_s[zw, a0 + i, re, :] = zre[i]
                    yf_s[zw, a0 + i, im, :] = zim[i]
                else:
                    yf_s[zw, a0 + i, re, :] = zre[i] - sgn * prev[1]
                    yf_s[zw, a0 + i, im, :] = zim[i] + sgn * prev[0]
                prev = (zre[i], zim[i])

    def inv_dft(c, zr):
        hc = C // 2
        for a in range(NCH):
            yr, yrm = yf_s[zr, a, 0:hc, :], yf_s[zr, a, hc:C, :]
            yi, yim = yf_s[zr, a, C:C + hc, :], yf_s[zr, a, C + hc:, :]
            fe = jnp.concatenate([yr + yrm, yi - yim], axis=0).astype(BF16)
            fo = jnp.concatenate([yr - yrm, yi + yim], axis=0).astype(BF16)
            y_v[c, pl.ds(a * C, hc, stride=2), :] = _dot(inv_ref[0:hc, :], fe)
            y_v[c, pl.ds(a * C + 1, hc, stride=2), :] = _dot(inv_ref[hc:, :], fo)

    def fixup(e, c, mat):
        a = wbuf[e][mat, c, 0]
        b = wbuf[e][mat, c, 1]
        wbuf[e][mat, c, 0] = (a & U32(0xFFFF)) | (b << 16)
        wbuf[e][mat, c, 1] = (a >> 16) | (b & U32(0xFFFF0000))

    RB = 128

    def qkv_tile(e, c, n):
        mat, j = n // 2, n % 2
        for r in range(PRO // RB):
            w = _unpack(wbuf[e][mat, c, j])
            xr = _unpack(xp[pl.ds(r * RB // 2, RB // 2), :])
            qkv_b[mat, 2 * c + e, j, pl.ds((QOFF + r * RB) // 2, RB // 2), :] = _pack(_dot(xr, w))

    xp_copy.start()
    for cp in wq0_copies(0) + wq0_copies(1) + small_copies:
        cp.start()
    kf[0:8, :] = jnp.zeros((8, 128), F32)
    zs[0] = 0
    zs[1] = 0
    xp_copy.wait()

    def start_when(cond, copies):
        @pl.when(cond)
        def _():
            for cp in copies:
                cp.start()

    def pro0(c, carry):
        for cp in wq0_copies(c):
            cp.wait()
        fixup(0, c, 0)
        qkv_tile(0, c, 0)
        qkv_tile(0, c, 1)
        start_when(c + 2 < NB, wq0_copies(c + 2))
        for i, piece in enumerate(block_copies(0)):
            start_when(c == min(i, NB - 2), piece)
        return carry

    with jax.named_scope("pro0"):
        jax.lax.fori_loop(0, NB, pro0, 0)
    for piece in block_copies(1):
        for cp in piece:
            cp.start()
    for cp in small_copies:
        cp.wait()

    zw = zs[0]
    zr = zs[1]

    def pro(c, carry):
        for piece in block_copies(c):
            for cp in piece:
                cp.wait()

        tiles = [(0, n) for n in range(2, 6)] + [(1, n) for n in range(6)]

        def tile(i):
            e, n = tiles[i]
            if n % 2 == 0:
                fixup(e, c, n // 2)
            qkv_tile(e, c, n)

        tile(0)
        fwd_dft(c, zw)
        p = 0
        for i in range(1, 8):
            tile(i)
            for _ in range(3 if i < 3 else 2):
                mac(p, zw, zr)
                p += 1
        inv_dft(c, zr)
        tile(8)
        tile(9)
        for piece in block_copies(c + 2):
            start_when(c + 2 < NB, piece)
        start_when(c + 1 < NB, rest_copies(c))
        start_when(c + 2 == NB, rest_copies(NB - 1))
        return carry

    with jax.named_scope("pro"):
        jax.lax.fori_loop(0, NB, pro, 0)
    for c in range(NB):
        for cp in rest_copies(c):
            cp.wait()

    gwt = gw_ref[...].astype(F32)
    gw = jnp.concatenate([gwt[j:j + 1, :] for j in range(NB)], axis=1)

    def finalize(rows, b):
        xr = x_v[rows, :].astype(F32)
        g = jax.nn.sigmoid(jnp.sum(xr * gw, axis=-1, keepdims=True))
        a = xr * jnp.concatenate([y_v[j, rows, :] for j in range(NB)], axis=1)
        out_v[rows, :] = (g * a + (1.0 - g) * b).astype(BF16)

    def step(s, mem, split_first, odd):
        xrows = slice(M, M + RX) if odd else slice(0, RX)
        mrows = slice(0, M) if odd else slice(RX, RX + M)
        sh = 4 if odd else 0
        xo = pl.multiple_of(PRO + RX * s, 8)
        wbase = pl.multiple_of((RX // 2 * s) % (QCAP // 2) - sh, 8)
        rpos = pl.multiple_of((SEG // 2 * s + QOFF // 2) % (QCAP // 2), SEG // 2)
        opos = pl.multiple_of(SEG // 2 * s, SEG // 2)
        fbase = pl.multiple_of(RX // 2 * s - sh, 8)
        xs = x_v[pl.ds(xo, RX), :]
        lhs = jnp.concatenate([mem, xs] if odd else [xs, mem], axis=0)
        zpad = jnp.zeros((128 - 2 * (SEG + M), E), BF16)
        frows = pl.ds(pl.multiple_of(RX * s, 8), RX)
        low = jax.lax.broadcasted_iota(jnp.int32, (8, E), 0) < 4
        NP = H // 2

        mem_qkv = {}
        probs = {}
        cats = {}

        def load(mat, hp):
            parts = [_unpack(qkv_b[mat, hp, 0, pl.ds(rpos, SEG // 2), :]),
                     _unpack(qkv_b[mat, hp, 1, pl.ds(rpos, SEG // 2), :]), mem_qkv[(hp, mat)]]
            if mat > 0:
                parts.append(zpad)
            cats[(mat, hp)] = jnp.concatenate(parts, axis=0)

        def stage_a(hp):
            KH = D // 2
            split = split_first and hp == 0
            if split:
                for mat in range(3):
                    for j in range(2):
                        w = _unpack(wbuf[hp % 2][mat, hp // 2, j, :KH // 2, :])
                        qacc[2 * mat + j] = _dot(lhs[:, :KH], w)
            for mi, mat in enumerate(MAT_ORDER):
                mm = []
                for j in range(2):
                    if split:
                        w = _unpack(wbuf[hp % 2][mat, hp // 2, j, KH // 2:, :])
                        res = qacc[2 * mat + j] + _dot(lhs[:, KH:], w)
                    else:
                        res = _dot(lhs, _unpack(wbuf[hp % 2][mat, hp // 2, j]))
                    pk = _pack(res)
                    if odd:
                        qkv_b[mat, hp, j, pl.ds(wbase + 4, 4), :] = pk[4:8]
                        qkv_b[mat, hp, j, pl.ds(wbase + 8, 8), :] = pk[8:16]
                    else:
                        qkv_b[mat, hp, j, pl.ds(wbase, 8), :] = pk[0:8]
                        qkv_b[mat, hp, j, pl.ds(wbase + 8, 4), :] = pk[8:12]
                    mm.append(res[mrows])
                    if j == 1:
                        mem_qkv[(hp, mat)] = jnp.concatenate(mm, axis=0).astype(BF16)
                    advance(6 * hp + 2 * mi + j + 1)

        def stage_b(hp):
            sc = _dot_nt(cats[(0, hp)], cats[(1, hp)]) * scale
            fill = fill_ref[...]
            sc = jnp.where(fill == 0.0, sc, fill)
            mx = jnp.max(sc, axis=-1, keepdims=True)
            p = jnp.exp(sc - mx)
            l = jnp.sum(p, axis=-1, keepdims=True)
            r = pl.reciprocal(l, approx=True)
            r = r * (2.0 - l * r)
            probs[hp] = (p.astype(BF16), r)

        def stage_c(hp):
            o = _dot(probs[hp][0], cats[(2, hp)]) * probs[hp][1]
            for j in range(2):
                h = 2 * hp + j
                cols = slice(h * E, (h + 1) * E)
                o_b[pl.ds(opos, SEG // 2), cols] = _pack(o[j * SEG:(j + 1) * SEG])
                om = o[2 * SEG + j * M:2 * SEG + (j + 1) * M]
                om = _pack(jnp.concatenate([om, om], axis=0))
                w0 = o_b[pl.ds(fbase, 8), cols]
                w1 = o_b[pl.ds(fbase + 8, 8), cols]
                lo_s[0:8, cols] = jnp.where(low, om, w0) if odd else w0
                lo_s[8:16, cols] = w1 if odd else jnp.where(low, w1, om)

        def oproj(j, late):
            ks = slice(HS * E, H * E) if late else slice(0, HS * E)
            kw = slice(ks.start // 2, ks.stop // 2)
            return _dot(_unpack(lo_s[:, ks]), _unpack(wo_v[j, kw, :]))

        events = []
        for hp in range(NP):
            events.append((6 * hp + OFF_LQK, 0, functools.partial(load, 0, hp)))
            events.append((6 * hp + OFF_LQK, 1, functools.partial(load, 1, hp)))
            events.append((6 * hp + OFF_LV, 2, functools.partial(load, 2, hp)))
            events.append((6 * hp + OFF_PV, 3, functools.partial(stage_c, hp)))
            events.append((6 * hp + OFF_S, 4, functools.partial(stage_b, hp)))
        events.sort(key=lambda ev: ev[:2])

        def advance(slot):
            while events and events[0][0] <= slot:
                events.pop(0)[2]()

        outs = [None] * NB
        for hp in range(NP):
            stage_a(hp)
        for j in range(NB):
            oacc[:, j * 128:(j + 1) * 128] = oproj(j, False)
            advance(6 * NP + (j + 1) * HS // 8)
        assert not events
        for j in range(NB):
            outs[j] = oacc[:, j * 128:(j + 1) * 128] + oproj(j, True)
        res = jnp.concatenate(outs, axis=1)
        finalize(frows, res[xrows])
        return res[mrows].astype(BF16)

    def steps(i, carry):
        mem = mem_v[...]
        for u in range(UNROLL):
            mem = step(i * UNROLL + u, mem, u > 0, u % 2 == 1)
        mem_v[...] = mem
        return carry

    with jax.named_scope("main"):
        jax.lax.fori_loop(0, NSEG // UNROLL, steps, 0)

    def epi_rows(r0, n):
        lo = _unpack(o_b[pl.ds(pl.multiple_of(r0 // 2, 8), n // 2), :])
        outs = [_dot(lo, _unpack(wo_v[j])) for j in range(NB)]
        finalize(pl.ds(r0, n), jnp.concatenate(outs, axis=1))

    EB = 128

    def epi(r, carry):
        r0 = pl.multiple_of(S - PRO + r * EB, EB)

        @pl.when(r == PRO // EB - 1)
        def _():
            out_copy(S - PRO, PRO - EB).start()

        epi_rows(r0, EB)
        return carry

    with jax.named_scope("epi"):
        out_copy(0, S - PRO).start()
        jax.lax.fori_loop(0, PRO // EB, epi, 0)
    out_copy(S - EB, EB).start()
    out_copy(0, S).wait()


@jax.jit
def _run(A_q, A_k, A_v, A_shift_k, A_ssm_k, A_ssm_D, B_mem0, B_Wq, B_Wk, B_Wv, B_Wo, gate_w):
    fwd, inv = _dft_tables()
    any_spec = pl.BlockSpec(memory_space=pl.ANY)
    out = pl.pallas_call(
        _kernel,
        out_shape=jax.ShapeDtypeStruct((S, D), BF16),
        in_specs=[any_spec] * 15,
        out_specs=any_spec,
        scratch_shapes=[
            pltpu.VMEM((S, D), BF16),
            pltpu.VMEM((PRO // 2, D), U32),
            pltpu.VMEM((NB, S, 128), BF16),
            pltpu.VMEM((NB, S, 128), BF16),
            pltpu.VMEM((NB, 128, S), BF16),
            pltpu.VMEM((3, H // 4, 2, D // 2, E), U32),
            pltpu.VMEM((3, H // 4, 2, D // 2, E), U32),
            pltpu.VMEM((NB, H * E // 2, 128), U32),
            pltpu.VMEM((NB, S, 128), F32),
            pltpu.VMEM((3, H // 2, 2, QCAP // 2, E), U32),
            pltpu.VMEM((S // 2, H * E), U32),
            pltpu.VMEM(((M + RX) // 2, H * E), U32),
            pltpu.VMEM((M, D), BF16),
            pltpu.VMEM((M + RX, D), F32),
            pltpu.VMEM((6, M + RX, E), F32),
            pltpu.VMEM((S + 32, 128), F32),
            pltpu.VMEM((1, NCH, 2 * C, 128), F32),
            pltpu.VMEM((1, NCH, 2 * C, 128), F32),
            pltpu.VMEM((1, NCH, 2 * C, 128), F32),
            pltpu.VMEM((S, D), BF16),
            pltpu.VMEM((2 * C, C), BF16),
            pltpu.VMEM((C, C), BF16),
            pltpu.VMEM((2 * (SEG + M), 128), F32),
            pltpu.VMEM((KS, D), BF16),
            pltpu.VMEM((NB, 128), BF16),
            pltpu.VMEM((NB, 128), BF16),
            pltpu.SMEM((2,), jnp.int32),
            pltpu.SemaphoreType.DMA((6,)),
            pltpu.SemaphoreType.DMA((NB,)),
        ],
        compiler_params=pltpu.CompilerParams(vmem_limit_bytes=120 * 2 ** 20, disable_bounds_checks=True),
    )(
        A_q.reshape(S, D), A_k.reshape(S, D), A_v.reshape(S, D), A_ssm_k,
        B_Wq.reshape(D // 2, 2, H, E), B_Wk.reshape(D // 2, 2, H, E), B_Wv.reshape(D // 2, 2, H, E),
        B_Wo.reshape(H * E, D),
        A_shift_k.T, A_ssm_D.reshape(NB, 128), gate_w.reshape(NB, 128), B_mem0.reshape(M, D),
        jnp.asarray(fwd, BF16), jnp.asarray(inv, BF16), jnp.asarray(_attn_fill()),
    )
    return out.reshape(1, S, D)


def pallas_gated_mix__ssm_conv_h3__memory_aug_recurrent_mem_tr__prompt_kernel(
    A_q, A_k, A_v, A_shift_k, A_ssm_k, A_ssm_D, B_x, B_mem0, B_Wq, B_Wk, B_Wv, B_Wo, B_seg_len, gate_w,
):
    del B_x
    if isinstance(B_seg_len, int):
        assert B_seg_len == SEG
    return _run(A_q, A_k, A_v, A_shift_k, A_ssm_k, A_ssm_D, B_mem0, B_Wq, B_Wk, B_Wv, B_Wo, gate_w)
```

```python
import functools
import math

import jax
import jax.numpy as jnp
import numpy as np
import jax.experimental.pallas as pl
import jax.experimental.pallas.tpu as pltpu

F32 = jnp.float32
BF16 = jnp.bfloat16
U32 = jnp.uint32

S = 2048
D = 1024
H = 32
E = 128
M = 8
SEG = 32
NSEG = S // SEG
RX = 24
PRO = S - RX * NSEG
QCAP = 576
QOFF = QCAP - PRO
HL = 4
HS = H - HL
MAT_ORDER = (0, 1, 2)
OFF_LQK, OFF_S, OFF_LV, OFF_PV = 4, 9, 15, 18
UNROLL = 4
C = 128
NCH = S // C
NB = D // 128
KS = 4
NEG = -1000000000.0


def _dft_tables():
    n = np.arange(C, dtype=np.float64)
    k = np.concatenate([np.arange(C // 2), C - 1 - np.arange(C // 2)]).astype(np.float64)
    th = np.pi * (2.0 * k + 1.0) / (2 * C)
    fwd = np.concatenate([np.cos(th[:, None] * n[None, :]), -np.sin(th[:, None] * n[None, :])], axis=0)
    no = np.concatenate([n[0::2], n[1::2]])
    tl = th[:C // 2]
    inv = np.concatenate([np.cos(no[:, None] * tl[None, :]), -np.sin(no[:, None] * tl[None, :])], axis=1) / C
    return fwd.astype(np.float32), inv.astype(np.float32)


def _attn_fill():
    n = 2 * (SEG + M)
    head = np.array([0] * SEG + [1] * SEG + [0] * M + [1] * M)
    pos = np.concatenate([M + np.arange(SEG), M + np.arange(SEG), np.arange(M), np.arange(M)])
    fill = np.full((n, 128), -np.inf, np.float32)
    for i in range(n):
        for j in range(n):
            if head[i] == head[j]:
                ok = pos[i] < M or pos[i] >= pos[j]
                fill[i, j] = 0.0 if ok else NEG
    return fill


def _dot(a, b):
    return jnp.dot(a, b, preferred_element_type=F32)


def _dot_nt(a, b):
    return jax.lax.dot_general(a, b, (((1,), (1,)), ((), ())), preferred_element_type=F32)


def _pack(a):
    return pltpu.bitcast(a.astype(BF16), U32)


def _unpack(a):
    return pltpu.bitcast(a, BF16)


def _kernel(x_hbm, k_hbm, v_hbm, h_hbm, wq_hbm, wk_hbm, wv_hbm, wo_hbm,
            sk_hbm, dd_hbm, gw_hbm, mem0_hbm, fwd_hbm, inv_hbm, fill_hbm,
            out_hbm,
            x_v, xp, k_v, v_v, h_v, w_even, w_odd, wo_v, y_v, qkv_b, o_b, lo_s, mem_v, oacc, qacc,
            u_s, h_s, yf_s,
            out_v, fwd_ref, inv_ref, fill_ref, sk_ref, dd_ref, gw_ref, zs, sems, qsems):
    scale = E ** (-0.5)
    wbuf = (w_even, w_odd)

    w32 = [w.bitcast(U32) for w in (wq_hbm, wk_hbm, wv_hbm)]
    wo32 = wo_hbm.bitcast(U32)
    x32 = x_hbm.bitcast(U32)

    def lanes(c):
        return pl.ds(pl.multiple_of(c * 128, 128), 128)

    def w_copies(c, e, mat, sem):
        return [pltpu.make_async_copy(w32[mat].at[:, par, 2 * c + e, :], wbuf[e].at[mat, c, par], sem)
                for par in range(2)]

    def wq0_copies(c):
        return w_copies(c, 0, 0, qsems.at[c])

    def block_copies(c):
        sem = sems.at[c % 2]
        return ([[pltpu.make_async_copy(h_hbm.at[lanes(c), :], h_v.at[c], sem)],
                 [pltpu.make_async_copy(k_hbm.at[:, lanes(c)], k_v.at[c], sem)],
                 [pltpu.make_async_copy(v_hbm.at[:, lanes(c)], v_v.at[c], sem)]]
                + [w_copies(c, e, mat, sem) for e in range(2) for mat in range(3) if (e, mat) != (0, 0)])

    def rest_copies(c):
        rows = pl.ds(pl.multiple_of(c * (S // NB), S // NB), S // NB)
        return [pltpu.make_async_copy(wo32.at[:, lanes(c)], wo_v.at[c], sems.at[2]),
                pltpu.make_async_copy(x_hbm.at[rows, :], x_v.at[rows, :], sems.at[2])]

    xp_copy = pltpu.make_async_copy(x32.at[pl.ds(0, PRO // 2), :], xp, sems.at[3])
    small_copies = [pltpu.make_async_copy(src, dst, sems.at[4]) for src, dst in (
        (sk_hbm, sk_ref), (fwd_hbm, fwd_ref), (dd_hbm, dd_ref), (inv_hbm, inv_ref),
        (gw_hbm, gw_ref), (mem0_hbm, mem_v), (fill_hbm, fill_ref))]

    def out_copy(start, n):
        rows = pl.ds(start, n)
        return pltpu.make_async_copy(out_v.at[rows, :], out_hbm.at[rows, :], sems.at[5])

    def row_of(ref, c):
        t = ref[...].astype(F32)
        sel = jax.lax.broadcasted_iota(jnp.int32, (NB, 128), 0) == c
        return jnp.sum(jnp.where(sel, t, 0.0), axis=0, keepdims=True)

    def fwd_dft(c, zw):
        skt = sk_ref[:, lanes(c)].astype(F32)
        tail = jnp.zeros((8, 128), F32)
        for a in range(NCH):
            hf = _dot_nt(fwd_ref[...], h_v[c, :, pl.ds(a * C, C)])
            if a == 0:
                h_s[zw, a, 0:C, :] = hf[0:C] + row_of(dd_ref, c)
                h_s[zw, a, C:, :] = hf[C:]
            else:
                h_s[zw, a] = hf
            kc = k_v[c, pl.ds(a * C, C), :].astype(F32)
            ext = jnp.concatenate([tail, kc], axis=0)
            tail = kc[C - 8:]
            ks_ = kc * skt[0:1, :]
            for j in range(1, KS):
                ks_ = ks_ + pltpu.roll(ext, j, 0)[8:] * skt[j:j + 1, :]
            kv = (ks_ * v_v[c, pl.ds(a * C, C), :].astype(F32)).astype(BF16)
            u_s[zw, a] = _dot(fwd_ref[...], kv)

    def mac(p, zw, zr):
        re = pl.ds(p * 8, 8)
        im = pl.ds(C + p * 8, 8)
        sgn = (1 - 2 * (jax.lax.broadcasted_iota(jnp.int32, (8, 128), 0) % 2)).astype(F32)
        if p >= C // 16:
            sgn = -sgn
        AB = 4
        prev = None
        for a0 in range(0, NCH, AB):
            zre = [None] * AB
            zim = [None] * AB
            for m in range(a0 + AB):
                hr = h_s[zr, m, re, :]
                hi = h_s[zr, m, im, :]
                for i in range(AB):
                    t = a0 + i - m
                    if t < 0:
                        continue
                    ur = u_s[zr, t, re, :]
                    ui = u_s[zr, t, im, :]
                    tr = hr * ur - hi * ui
                    ti = hr * ui + hi * ur
                    zre[i] = tr if zre[i] is None else zre[i] + tr
                    zim[i] = ti if zim[i] is None else zim[i] + ti
            for i in range(AB):
                if prev is None:
                    yf_s[zw, a0 + i, re, :] = zre[i]
                    yf_s[zw, a0 + i, im, :] = zim[i]
                else:
                    yf_s[zw, a0 + i, re, :] = zre[i] - sgn * prev[1]
                    yf_s[zw, a0 + i, im, :] = zim[i] + sgn * prev[0]
                prev = (zre[i], zim[i])

    def inv_dft(c, zr):
        hc = C // 2
        for a in range(NCH):
            yr, yrm = yf_s[zr, a, 0:hc, :], yf_s[zr, a, hc:C, :]
            yi, yim = yf_s[zr, a, C:C + hc, :], yf_s[zr, a, C + hc:, :]
            fe = jnp.concatenate([yr + yrm, yi - yim], axis=0).astype(BF16)
            fo = jnp.concatenate([yr - yrm, yi + yim], axis=0).astype(BF16)
            y_v[c, pl.ds(a * C, hc, stride=2), :] = _dot(inv_ref[0:hc, :], fe)
            y_v[c, pl.ds(a * C + 1, hc, stride=2), :] = _dot(inv_ref[hc:, :], fo)

    def fixup(e, c, mat):
        a = wbuf[e][mat, c, 0]
        b = wbuf[e][mat, c, 1]
        wbuf[e][mat, c, 0] = (a & U32(0xFFFF)) | (b << 16)
        wbuf[e][mat, c, 1] = (a >> 16) | (b & U32(0xFFFF0000))

    RB = 128

    def qkv_tile(e, c, n):
        mat, j = n // 2, n % 2
        for r in range(PRO // RB):
            w = _unpack(wbuf[e][mat, c, j])
            xr = _unpack(xp[pl.ds(r * RB // 2, RB // 2), :])
            qkv_b[mat, 2 * c + e, j, pl.ds((QOFF + r * RB) // 2, RB // 2), :] = _pack(_dot(xr, w))

    xp_copy.start()
    for cp in wq0_copies(0) + wq0_copies(1) + small_copies:
        cp.start()
    zs[0] = 0
    zs[1] = 0
    xp_copy.wait()

    def start_when(cond, copies):
        @pl.when(cond)
        def _():
            for cp in copies:
                cp.start()

    def pro0(c, carry):
        for cp in wq0_copies(c):
            cp.wait()
        fixup(0, c, 0)
        qkv_tile(0, c, 0)
        qkv_tile(0, c, 1)
        start_when(c + 2 < NB, wq0_copies(c + 2))
        for i, piece in enumerate(block_copies(0)):
            start_when(c == min(i, NB - 2), piece)
        return carry

    with jax.named_scope("pro0"):
        jax.lax.fori_loop(0, NB, pro0, 0)
    for piece in block_copies(1):
        for cp in piece:
            cp.start()
    for cp in small_copies:
        cp.wait()

    zw = zs[0]
    zr = zs[1]

    def pro(c, carry):
        for piece in block_copies(c):
            for cp in piece:
                cp.wait()

        tiles = [(0, n) for n in range(2, 6)] + [(1, n) for n in range(6)]

        def tile(i):
            e, n = tiles[i]
            if n % 2 == 0:
                fixup(e, c, n // 2)
            qkv_tile(e, c, n)

        tile(0)
        fwd_dft(c, zw)
        p = 0
        for i in range(1, 8):
            tile(i)
            for _ in range(3 if i < 3 else 2):
                mac(p, zw, zr)
                p += 1
        inv_dft(c, zr)
        tile(8)
        tile(9)
        for piece in block_copies(c + 2):
            start_when(c + 2 < NB, piece)
        start_when(c + 1 < NB, rest_copies(c))
        start_when(c + 2 == NB, rest_copies(NB - 1))
        return carry

    with jax.named_scope("pro"):
        jax.lax.fori_loop(0, NB, pro, 0)
    for c in range(NB):
        for cp in rest_copies(c):
            cp.wait()

    gwt = gw_ref[...].astype(F32)
    gw = jnp.concatenate([gwt[j:j + 1, :] for j in range(NB)], axis=1)

    def finalize(rows, b):
        xr = x_v[rows, :].astype(F32)
        g = jax.nn.sigmoid(jnp.sum(xr * gw, axis=-1, keepdims=True))
        a = xr * jnp.concatenate([y_v[j, rows, :] for j in range(NB)], axis=1)
        out_v[rows, :] = (g * a + (1.0 - g) * b).astype(BF16)

    def step(s, mem, split_first, odd):
        xrows = slice(M, M + RX) if odd else slice(0, RX)
        mrows = slice(0, M) if odd else slice(RX, RX + M)
        sh = 4 if odd else 0
        xo = pl.multiple_of(PRO + RX * s, 8)
        wbase = pl.multiple_of((RX // 2 * s) % (QCAP // 2) - sh, 8)
        rpos = pl.multiple_of((SEG // 2 * s + QOFF // 2) % (QCAP // 2), SEG // 2)
        opos = pl.multiple_of(SEG // 2 * s, SEG // 2)
        fbase = pl.multiple_of(RX // 2 * s - sh, 8)
        xs = x_v[pl.ds(xo, RX), :]
        lhs = jnp.concatenate([mem, xs] if odd else [xs, mem], axis=0)
        zpad = jnp.zeros((128 - 2 * (SEG + M), E), BF16)
        frows = pl.ds(pl.multiple_of(RX * s, 8), RX)
        low = jax.lax.broadcasted_iota(jnp.int32, (8, E), 0) < 4
        NP = H // 2

        mem_qkv = {}
        probs = {}
        cats = {}

        def load(mat, hp):
            parts = [_unpack(qkv_b[mat, hp, 0, pl.ds(rpos, SEG // 2), :]),
                     _unpack(qkv_b[mat, hp, 1, pl.ds(rpos, SEG // 2), :]), mem_qkv[(hp, mat)]]
            if mat > 0:
                parts.append(zpad)
            cats[(mat, hp)] = jnp.concatenate(parts, axis=0)

        def stage_a(hp):
            KH = D // 2
            split = split_first and hp == 0
            if split:
                for mat in range(3):
                    for j in range(2):
                        w = _unpack(wbuf[hp % 2][mat, hp // 2, j, :KH // 2, :])
                        qacc[2 * mat + j] = _dot(lhs[:, :KH], w)
            for mi, mat in enumerate(MAT_ORDER):
                mm = []
                for j in range(2):
                    if split:
                        w = _unpack(wbuf[hp % 2][mat, hp // 2, j, KH // 2:, :])
                        res = qacc[2 * mat + j] + _dot(lhs[:, KH:], w)
                    else:
                        res = _dot(lhs, _unpack(wbuf[hp % 2][mat, hp // 2, j]))
                    pk = _pack(res)
                    if odd:
                        qkv_b[mat, hp, j, pl.ds(wbase + 4, 4), :] = pk[4:8]
                        qkv_b[mat, hp, j, pl.ds(wbase + 8, 8), :] = pk[8:16]
                    else:
                        qkv_b[mat, hp, j, pl.ds(wbase, 8), :] = pk[0:8]
                        qkv_b[mat, hp, j, pl.ds(wbase + 8, 4), :] = pk[8:12]
                    mm.append(res[mrows])
                    if j == 1:
                        mem_qkv[(hp, mat)] = jnp.concatenate(mm, axis=0).astype(BF16)
                    advance(6 * hp + 2 * mi + j + 1)

        def stage_b(hp):
            sc = _dot_nt(cats[(0, hp)], cats[(1, hp)]) * scale
            fill = fill_ref[...]
            sc = jnp.where(fill == 0.0, sc, fill)
            mx = jnp.max(sc, axis=-1, keepdims=True)
            p = jnp.exp(sc - mx)
            l = jnp.sum(p, axis=-1, keepdims=True)
            r = pl.reciprocal(l, approx=True)
            r = r * (2.0 - l * r)
            probs[hp] = (p.astype(BF16), r)

        def stage_c(hp):
            o = _dot(probs[hp][0], cats[(2, hp)]) * probs[hp][1]
            for j in range(2):
                h = 2 * hp + j
                cols = slice(h * E, (h + 1) * E)
                o_b[pl.ds(opos, SEG // 2), cols] = _pack(o[j * SEG:(j + 1) * SEG])
                om = o[2 * SEG + j * M:2 * SEG + (j + 1) * M]
                om = _pack(jnp.concatenate([om, om], axis=0))
                w0 = o_b[pl.ds(fbase, 8), cols]
                w1 = o_b[pl.ds(fbase + 8, 8), cols]
                lo_s[0:8, cols] = jnp.where(low, om, w0) if odd else w0
                lo_s[8:16, cols] = w1 if odd else jnp.where(low, w1, om)

        def oproj(j, late):
            ks = slice(HS * E, H * E) if late else slice(0, HS * E)
            kw = slice(ks.start // 2, ks.stop // 2)
            return _dot(_unpack(lo_s[:, ks]), _unpack(wo_v[j, kw, :]))

        events = []
        for hp in range(NP):
            events.append((6 * hp + OFF_LQK, 0, functools.partial(load, 0, hp)))
            events.append((6 * hp + OFF_LQK, 1, functools.partial(load, 1, hp)))
            events.append((6 * hp + OFF_LV, 2, functools.partial(load, 2, hp)))
            events.append((6 * hp + OFF_PV, 3, functools.partial(stage_c, hp)))
            events.append((6 * hp + OFF_S, 4, functools.partial(stage_b, hp)))
        events.sort(key=lambda ev: ev[:2])

        def advance(slot):
            while events and events[0][0] <= slot:
                events.pop(0)[2]()

        outs = [None] * NB
        for hp in range(NP):
            stage_a(hp)
        for j in range(NB):
            oacc[:, j * 128:(j + 1) * 128] = oproj(j, False)
            advance(6 * NP + (j + 1) * HS // 8)
        assert not events
        for j in range(NB):
            outs[j] = oacc[:, j * 128:(j + 1) * 128] + oproj(j, True)
        res = jnp.concatenate(outs, axis=1)
        finalize(frows, res[xrows])
        return res[mrows].astype(BF16)

    def steps(i, carry):
        mem = mem_v[...]
        for u in range(UNROLL):
            mem = step(i * UNROLL + u, mem, u > 0, u % 2 == 1)
        mem_v[...] = mem
        return carry

    with jax.named_scope("main"):
        jax.lax.fori_loop(0, NSEG // UNROLL, steps, 0)

    def epi_rows(r0, n):
        lo = _unpack(o_b[pl.ds(pl.multiple_of(r0 // 2, 8), n // 2), :])
        outs = [_dot(lo, _unpack(wo_v[j])) for j in range(NB)]
        finalize(pl.ds(r0, n), jnp.concatenate(outs, axis=1))

    EB = 128

    def epi(r, carry):
        r0 = pl.multiple_of(S - PRO + r * EB, EB)

        @pl.when(r == PRO // EB - 1)
        def _():
            out_copy(S - PRO, PRO - EB).start()

        epi_rows(r0, EB)
        return carry

    with jax.named_scope("epi"):
        out_copy(0, S - PRO).start()
        jax.lax.fori_loop(0, PRO // EB, epi, 0)
    out_copy(S - EB, EB).start()
    out_copy(0, S).wait()


@jax.jit
def _run(A_q, A_k, A_v, A_shift_k, A_ssm_k, A_ssm_D, B_mem0, B_Wq, B_Wk, B_Wv, B_Wo, gate_w):
    fwd, inv = _dft_tables()
    any_spec = pl.BlockSpec(memory_space=pl.ANY)
    out = pl.pallas_call(
        _kernel,
        out_shape=jax.ShapeDtypeStruct((S, D), BF16),
        in_specs=[any_spec] * 15,
        out_specs=any_spec,
        scratch_shapes=[
            pltpu.VMEM((S, D), BF16),
            pltpu.VMEM((PRO // 2, D), U32),
            pltpu.VMEM((NB, S, 128), BF16),
            pltpu.VMEM((NB, S, 128), BF16),
            pltpu.VMEM((NB, 128, S), BF16),
            pltpu.VMEM((3, H // 4, 2, D // 2, E), U32),
            pltpu.VMEM((3, H // 4, 2, D // 2, E), U32),
            pltpu.VMEM((NB, H * E // 2, 128), U32),
            pltpu.VMEM((NB, S, 128), F32),
            pltpu.VMEM((3, H // 2, 2, QCAP // 2, E), U32),
            pltpu.VMEM((S // 2, H * E), U32),
            pltpu.VMEM(((M + RX) // 2, H * E), U32),
            pltpu.VMEM((M, D), BF16),
            pltpu.VMEM((M + RX, D), F32),
            pltpu.VMEM((6, M + RX, E), F32),
            pltpu.VMEM((1, NCH, 2 * C, 128), F32),
            pltpu.VMEM((1, NCH, 2 * C, 128), F32),
            pltpu.VMEM((1, NCH, 2 * C, 128), F32),
            pltpu.VMEM((S, D), BF16),
            pltpu.VMEM((2 * C, C), BF16),
            pltpu.VMEM((C, C), BF16),
            pltpu.VMEM((2 * (SEG + M), 128), F32),
            pltpu.VMEM((KS, D), BF16),
            pltpu.VMEM((NB, 128), BF16),
            pltpu.VMEM((NB, 128), BF16),
            pltpu.SMEM((2,), jnp.int32),
            pltpu.SemaphoreType.DMA((6,)),
            pltpu.SemaphoreType.DMA((NB,)),
        ],
        compiler_params=pltpu.CompilerParams(vmem_limit_bytes=120 * 2 ** 20, disable_bounds_checks=True),
    )(
        A_q.reshape(S, D), A_k.reshape(S, D), A_v.reshape(S, D), A_ssm_k,
        B_Wq.reshape(D // 2, 2, H, E), B_Wk.reshape(D // 2, 2, H, E), B_Wv.reshape(D // 2, 2, H, E),
        B_Wo.reshape(H * E, D),
        A_shift_k.T, A_ssm_D.reshape(NB, 128), gate_w.reshape(NB, 128), B_mem0.reshape(M, D),
        jnp.asarray(fwd, BF16), jnp.asarray(inv, BF16), jnp.asarray(_attn_fill()),
    )
    return out.reshape(1, S, D)


def pallas_gated_mix__ssm_conv_h3__memory_aug_recurrent_mem_tr__prompt_kernel(
    A_q, A_k, A_v, A_shift_k, A_ssm_k, A_ssm_D, B_x, B_mem0, B_Wq, B_Wk, B_Wv, B_Wo, B_seg_len, gate_w,
):
    del B_x
    if isinstance(B_seg_len, int):
        assert B_seg_len == SEG
    return _run(A_q, A_k, A_v, A_shift_k, A_ssm_k, A_ssm_D, B_mem0, B_Wq, B_Wk, B_Wv, B_Wo, gate_w)
```

```python
import functools
import math

import jax
import jax.numpy as jnp
import numpy as np
import jax.experimental.pallas as pl
import jax.experimental.pallas.tpu as pltpu

F32 = jnp.float32
BF16 = jnp.bfloat16
U32 = jnp.uint32

S = 2048
D = 1024
H = 32
E = 128
M = 8
SEG = 32
NSEG = S // SEG
RX = 24
PRO = S - RX * NSEG
QCAP = 576
QOFF = QCAP - PRO
HL = 4
HS = H - HL
MAT_ORDER = (0, 1, 2)
OFF_LQK, OFF_S, OFF_LV, OFF_PV = 4, 9, 15, 18
UNROLL = 4
C = 128
NCH = S // C
NB = D // 128
KS = 4
NEG = -1000000000.0


def _dft_tables():
    n = np.arange(C, dtype=np.float64)
    k = np.concatenate([np.arange(C // 2), C - 1 - np.arange(C // 2)]).astype(np.float64)
    th = np.pi * (2.0 * k + 1.0) / (2 * C)
    fwd = np.concatenate([np.cos(th[:, None] * n[None, :]), -np.sin(th[:, None] * n[None, :])], axis=0)
    no = np.concatenate([n[0::2], n[1::2]])
    tl = th[:C // 2]
    inv = np.concatenate([np.cos(no[:, None] * tl[None, :]), -np.sin(no[:, None] * tl[None, :])], axis=1) / C
    return fwd.astype(np.float32), inv.astype(np.float32)


def _attn_fill():
    n = 2 * (SEG + M)
    head = np.array([0] * SEG + [1] * SEG + [0] * M + [1] * M)
    pos = np.concatenate([M + np.arange(SEG), M + np.arange(SEG), np.arange(M), np.arange(M)])
    fill = np.full((n, 128), -np.inf, np.float32)
    for i in range(n):
        for j in range(n):
            if head[i] == head[j]:
                ok = pos[i] < M or pos[i] >= pos[j]
                fill[i, j] = 0.0 if ok else NEG
    return fill


def _dot(a, b):
    return jnp.dot(a, b, preferred_element_type=F32)


def _dot_nt(a, b):
    return jax.lax.dot_general(a, b, (((1,), (1,)), ((), ())), preferred_element_type=F32)


def _pack(a):
    return pltpu.bitcast(a.astype(BF16), U32)


def _unpack(a):
    return pltpu.bitcast(a, BF16)


def _kernel(x_hbm, k_hbm, v_hbm, h_hbm, wq_hbm, wk_hbm, wv_hbm, wo_hbm,
            sk_hbm, dd_hbm, gw_hbm, mem0_hbm, fwd_hbm, inv_hbm, fill_hbm,
            out_hbm,
            x_v, xp, k_v, v_v, h_v, w_even, w_odd, wo_v, y_v, qkv_b, o_b, lo_s, mem_v, oacc, qacc,
            u_s, h_s, yf_s,
            out_v, fwd_ref, inv_ref, fill_ref, sk_ref, dd_ref, gw_ref, zs, sems, qsems):
    scale = E ** (-0.5)
    wbuf = (w_even, w_odd)

    w32 = [w.bitcast(U32) for w in (wq_hbm, wk_hbm, wv_hbm)]
    wo32 = wo_hbm.bitcast(U32)
    x32 = x_hbm.bitcast(U32)

    def lanes(c):
        return pl.ds(pl.multiple_of(c * 128, 128), 128)

    def w_copies(c, e, mat, sem):
        return [pltpu.make_async_copy(w32[mat].at[:, par, 2 * c + e, :], wbuf[e].at[mat, c, par], sem)
                for par in range(2)]

    def wq0_copies(c):
        return w_copies(c, 0, 0, qsems.at[c])

    def block_copies(c):
        sem = sems.at[c % 2]
        return ([[pltpu.make_async_copy(h_hbm.at[lanes(c), :], h_v.at[c], sem)],
                 [pltpu.make_async_copy(k_hbm.at[:, lanes(c)], k_v.at[c], sem)],
                 [pltpu.make_async_copy(v_hbm.at[:, lanes(c)], v_v.at[c], sem)]]
                + [w_copies(c, e, mat, sem) for e in range(2) for mat in range(3) if (e, mat) != (0, 0)])

    def rest_copies(c):
        rows = pl.ds(pl.multiple_of(c * (S // NB), S // NB), S // NB)
        return [pltpu.make_async_copy(wo32.at[:, lanes(c)], wo_v.at[c], sems.at[2]),
                pltpu.make_async_copy(x_hbm.at[rows, :], x_v.at[rows, :], sems.at[2])]

    xp_copy = pltpu.make_async_copy(x32.at[pl.ds(0, PRO // 2), :], xp, sems.at[3])
    small_copies = [pltpu.make_async_copy(src, dst, sems.at[4]) for src, dst in (
        (sk_hbm, sk_ref), (fwd_hbm, fwd_ref), (dd_hbm, dd_ref), (inv_hbm, inv_ref),
        (gw_hbm, gw_ref), (mem0_hbm, mem_v), (fill_hbm, fill_ref))]

    def out_copy(start, n):
        rows = pl.ds(start, n)
        return pltpu.make_async_copy(out_v.at[rows, :], out_hbm.at[rows, :], sems.at[5])

    def row_of(ref, c):
        t = ref[...].astype(F32)
        sel = jax.lax.broadcasted_iota(jnp.int32, (NB, 128), 0) == c
        return jnp.sum(jnp.where(sel, t, 0.0), axis=0, keepdims=True)

    def fwd_dft(c, zw):
        skt = sk_ref[:, lanes(c)].astype(F32)
        tail = jnp.zeros((8, 128), F32)
        for a in range(NCH):
            hf = _dot_nt(fwd_ref[...], h_v[c, :, pl.ds(a * C, C)])
            if a == 0:
                h_s[zw, a, 0:C, :] = hf[0:C] + row_of(dd_ref, c)
                h_s[zw, a, C:, :] = hf[C:]
            else:
                h_s[zw, a] = hf
            kc = k_v[c, pl.ds(a * C, C), :].astype(F32)
            ext = jnp.concatenate([tail, kc], axis=0)
            tail = kc[C - 8:]
            ks_ = kc * skt[0:1, :]
            for j in range(1, KS):
                ks_ = ks_ + pltpu.roll(ext, j, 0)[8:] * skt[j:j + 1, :]
            kv = (ks_ * v_v[c, pl.ds(a * C, C), :].astype(F32)).astype(BF16)
            u_s[zw, a] = _dot(fwd_ref[...], kv)

    def mac(p, zw, zr):
        re = pl.ds(p * 8, 8)
        im = pl.ds(C + p * 8, 8)
        sgn = (1 - 2 * (jax.lax.broadcasted_iota(jnp.int32, (8, 128), 0) % 2)).astype(F32)
        if p >= C // 16:
            sgn = -sgn
        AB = 4
        prev = None
        for a0 in range(0, NCH, AB):
            zre = [None] * AB
            zim = [None] * AB
            for m in range(a0 + AB):
                hr = h_s[zr, m, re, :]
                hi = h_s[zr, m, im, :]
                for i in range(AB):
                    t = a0 + i - m
                    if t < 0:
                        continue
                    ur = u_s[zr, t, re, :]
                    ui = u_s[zr, t, im, :]
                    tr = hr * ur - hi * ui
                    ti = hr * ui + hi * ur
                    zre[i] = tr if zre[i] is None else zre[i] + tr
                    zim[i] = ti if zim[i] is None else zim[i] + ti
            for i in range(AB):
                if prev is None:
                    yf_s[zw, a0 + i, re, :] = zre[i]
                    yf_s[zw, a0 + i, im, :] = zim[i]
                else:
                    yf_s[zw, a0 + i, re, :] = zre[i] - sgn * prev[1]
                    yf_s[zw, a0 + i, im, :] = zim[i] + sgn * prev[0]
                prev = (zre[i], zim[i])

    def inv_dft(c, zr):
        hc = C // 2
        for a in range(NCH):
            yr, yrm = yf_s[zr, a, 0:hc, :], yf_s[zr, a, hc:C, :]
            yi, yim = yf_s[zr, a, C:C + hc, :], yf_s[zr, a, C + hc:, :]
            fe = jnp.concatenate([yr + yrm, yi - yim], axis=0).astype(BF16)
            fo = jnp.concatenate([yr - yrm, yi + yim], axis=0).astype(BF16)
            y_v[c, pl.ds(a * C, hc, stride=2), :] = _dot(inv_ref[0:hc, :], fe)
            y_v[c, pl.ds(a * C + 1, hc, stride=2), :] = _dot(inv_ref[hc:, :], fo)

    def fixup(e, c, mat):
        a = wbuf[e][mat, c, 0]
        b = wbuf[e][mat, c, 1]
        wbuf[e][mat, c, 0] = (a & U32(0xFFFF)) | (b << 16)
        wbuf[e][mat, c, 1] = (a >> 16) | (b & U32(0xFFFF0000))

    RB = 128

    def qkv_tile(e, c, n):
        mat, j = n // 2, n % 2
        for r in range(PRO // RB):
            w = _unpack(wbuf[e][mat, c, j])
            xr = _unpack(xp[pl.ds(r * RB // 2, RB // 2), :])
            qkv_b[mat, 2 * c + e, j, pl.ds((QOFF + r * RB) // 2, RB // 2), :] = _pack(_dot(xr, w))

    for cp in wq0_copies(0) + [xp_copy]:
        cp.start()
    zs[0] = 0
    zs[1] = 0
    xp_copy.wait()
    for cp in wq0_copies(1) + wq0_copies(2) + small_copies + sum(block_copies(0)[:1], []):
        cp.start()

    def start_when(cond, make_copies):
        @pl.when(cond)
        def _():
            for cp in make_copies():
                cp.start()

    def pro0(c, carry):
        for cp in wq0_copies(c):
            cp.wait()
        fixup(0, c, 0)
        qkv_tile(0, c, 0)
        qkv_tile(0, c, 1)
        start_when(c + 3 < NB, lambda: wq0_copies(c + 3))
        for i in range(1, NB):
            start_when(c == min(i - 1, NB - 3), lambda: block_copies(0)[i])
        return carry

    with jax.named_scope("pro0"):
        jax.lax.fori_loop(0, NB, pro0, 0)
    for piece in block_copies(1):
        for cp in piece:
            cp.start()
    for cp in small_copies:
        cp.wait()

    zw = zs[0]
    zr = zs[1]

    def pro(c, carry):
        for piece in block_copies(c):
            for cp in piece:
                cp.wait()

        tiles = [(0, n) for n in range(2, 6)] + [(1, n) for n in range(6)]

        def tile(i):
            e, n = tiles[i]
            if n % 2 == 0:
                fixup(e, c, n // 2)
            qkv_tile(e, c, n)

        tile(0)
        fwd_dft(c, zw)
        p = 0
        for i in range(1, 8):
            tile(i)
            for _ in range(3 if i < 3 else 2):
                mac(p, zw, zr)
                p += 1
        inv_dft(c, zr)
        tile(8)
        tile(9)
        for i in range(NB):
            start_when(c + 2 < NB, lambda: block_copies(c + 2)[i])
        start_when(c + 1 < NB, lambda: rest_copies(c))
        start_when(c + 2 == NB, lambda: rest_copies(NB - 1))
        return carry

    with jax.named_scope("pro"):
        jax.lax.fori_loop(0, NB, pro, 0)
    for c in range(NB):
        for cp in rest_copies(c):
            cp.wait()

    gwt = gw_ref[...].astype(F32)
    gw = jnp.concatenate([gwt[j:j + 1, :] for j in range(NB)], axis=1)

    def finalize(rows, b):
        xr = x_v[rows, :].astype(F32)
        g = jax.nn.sigmoid(jnp.sum(xr * gw, axis=-1, keepdims=True))
        a = xr * jnp.concatenate([y_v[j, rows, :] for j in range(NB)], axis=1)
        out_v[rows, :] = (g * a + (1.0 - g) * b).astype(BF16)

    def step(s, mem, split_first, odd):
        xrows = slice(M, M + RX) if odd else slice(0, RX)
        mrows = slice(0, M) if odd else slice(RX, RX + M)
        sh = 4 if odd else 0
        xo = pl.multiple_of(PRO + RX * s, 8)
        wbase = pl.multiple_of((RX // 2 * s) % (QCAP // 2) - sh, 8)
        rpos = pl.multiple_of((SEG // 2 * s + QOFF // 2) % (QCAP // 2), SEG // 2)
        opos = pl.multiple_of(SEG // 2 * s, SEG // 2)
        fbase = pl.multiple_of(RX // 2 * s - sh, 8)
        xs = x_v[pl.ds(xo, RX), :]
        lhs = jnp.concatenate([mem, xs] if odd else [xs, mem], axis=0)
        zpad = jnp.zeros((128 - 2 * (SEG + M), E), BF16)
        frows = pl.ds(pl.multiple_of(RX * s, 8), RX)
        low = jax.lax.broadcasted_iota(jnp.int32, (8, E), 0) < 4
        NP = H // 2

        mem_qkv = {}
        probs = {}
        cats = {}

        def load(mat, hp):
            parts = [_unpack(qkv_b[mat, hp, 0, pl.ds(rpos, SEG // 2), :]),
                     _unpack(qkv_b[mat, hp, 1, pl.ds(rpos, SEG // 2), :]), mem_qkv[(hp, mat)]]
            if mat > 0:
                parts.append(zpad)
            cats[(mat, hp)] = jnp.concatenate(parts, axis=0)

        def stage_a(hp):
            KH = D // 2
            split = split_first and hp == 0
            if split:
                for mat in range(3):
                    for j in range(2):
                        w = _unpack(wbuf[hp % 2][mat, hp // 2, j, :KH // 2, :])
                        qacc[2 * mat + j] = _dot(lhs[:, :KH], w)
            for mi, mat in enumerate(MAT_ORDER):
                mm = []
                for j in range(2):
                    if split:
                        w = _unpack(wbuf[hp % 2][mat, hp // 2, j, KH // 2:, :])
                        res = qacc[2 * mat + j] + _dot(lhs[:, KH:], w)
                    else:
                        res = _dot(lhs, _unpack(wbuf[hp % 2][mat, hp // 2, j]))
                    pk = _pack(res)
                    if odd:
                        qkv_b[mat, hp, j, pl.ds(wbase + 4, 4), :] = pk[4:8]
                        qkv_b[mat, hp, j, pl.ds(wbase + 8, 8), :] = pk[8:16]
                    else:
                        qkv_b[mat, hp, j, pl.ds(wbase, 8), :] = pk[0:8]
                        qkv_b[mat, hp, j, pl.ds(wbase + 8, 4), :] = pk[8:12]
                    mm.append(res[mrows])
                    if j == 1:
                        mem_qkv[(hp, mat)] = jnp.concatenate(mm, axis=0).astype(BF16)
                    advance(6 * hp + 2 * mi + j + 1)

        def stage_b(hp):
            sc = _dot_nt(cats[(0, hp)], cats[(1, hp)]) * scale
            fill = fill_ref[...]
            sc = jnp.where(fill == 0.0, sc, fill)
            mx = jnp.max(sc, axis=-1, keepdims=True)
            p = jnp.exp(sc - mx)
            l = jnp.sum(p, axis=-1, keepdims=True)
            r = pl.reciprocal(l, approx=True)
            r = r * (2.0 - l * r)
            probs[hp] = (p.astype(BF16), r)

        def stage_c(hp):
            o = _dot(probs[hp][0], cats[(2, hp)]) * probs[hp][1]
            for j in range(2):
                h = 2 * hp + j
                cols = slice(h * E, (h + 1) * E)
                o_b[pl.ds(opos, SEG // 2), cols] = _pack(o[j * SEG:(j + 1) * SEG])
                om = o[2 * SEG + j * M:2 * SEG + (j + 1) * M]
                om = _pack(jnp.concatenate([om, om], axis=0))
                w0 = o_b[pl.ds(fbase, 8), cols]
                w1 = o_b[pl.ds(fbase + 8, 8), cols]
                lo_s[0:8, cols] = jnp.where(low, om, w0) if odd else w0
                lo_s[8:16, cols] = w1 if odd else jnp.where(low, w1, om)

        def oproj(j, late):
            ks = slice(HS * E, H * E) if late else slice(0, HS * E)
            kw = slice(ks.start // 2, ks.stop // 2)
            return _dot(_unpack(lo_s[:, ks]), _unpack(wo_v[j, kw, :]))

        events = []
        for hp in range(NP):
            events.append((6 * hp + OFF_LQK, 0, functools.partial(load, 0, hp)))
            events.append((6 * hp + OFF_LQK, 1, functools.partial(load, 1, hp)))
            events.append((6 * hp + OFF_LV, 2, functools.partial(load, 2, hp)))
            events.append((6 * hp + OFF_PV, 3, functools.partial(stage_c, hp)))
            events.append((6 * hp + OFF_S, 4, functools.partial(stage_b, hp)))
        events.sort(key=lambda ev: ev[:2])

        def advance(slot):
            while events and events[0][0] <= slot:
                events.pop(0)[2]()

        outs = [None] * NB
        for hp in range(NP):
            stage_a(hp)
        for j in range(NB):
            oacc[:, j * 128:(j + 1) * 128] = oproj(j, False)
            advance(6 * NP + (j + 1) * HS // 8)
        assert not events
        for j in range(NB):
            outs[j] = oacc[:, j * 128:(j + 1) * 128] + oproj(j, True)
        res = jnp.concatenate(outs, axis=1)
        finalize(frows, res[xrows])
        return res[mrows].astype(BF16)

    def steps(i, carry):
        mem = mem_v[...]
        for u in range(UNROLL):
            mem = step(i * UNROLL + u, mem, u > 0, u % 2 == 1)
        mem_v[...] = mem
        return carry

    with jax.named_scope("main"):
        jax.lax.fori_loop(0, NSEG // UNROLL, steps, 0)

    def epi_rows(r0, n):
        lo = _unpack(o_b[pl.ds(pl.multiple_of(r0 // 2, 8), n // 2), :])
        outs = [_dot(lo, _unpack(wo_v[j])) for j in range(NB)]
        finalize(pl.ds(r0, n), jnp.concatenate(outs, axis=1))

    EB = 128

    def epi(r, carry):
        r0 = pl.multiple_of(S - PRO + r * EB, EB)

        @pl.when(r == PRO // EB - 1)
        def _():
            out_copy(S - PRO, PRO - EB).start()

        epi_rows(r0, EB)
        return carry

    with jax.named_scope("epi"):
        out_copy(0, S - PRO).start()
        jax.lax.fori_loop(0, PRO // EB, epi, 0)
    out_copy(S - EB, EB).start()
    out_copy(0, S).wait()


@jax.jit
def _run(A_q, A_k, A_v, A_shift_k, A_ssm_k, A_ssm_D, B_mem0, B_Wq, B_Wk, B_Wv, B_Wo, gate_w):
    fwd, inv = _dft_tables()
    any_spec = pl.BlockSpec(memory_space=pl.ANY)
    out = pl.pallas_call(
        _kernel,
        out_shape=jax.ShapeDtypeStruct((S, D), BF16),
        in_specs=[any_spec] * 15,
        out_specs=any_spec,
        scratch_shapes=[
            pltpu.VMEM((S, D), BF16),
            pltpu.VMEM((PRO // 2, D), U32),
            pltpu.VMEM((NB, S, 128), BF16),
            pltpu.VMEM((NB, S, 128), BF16),
            pltpu.VMEM((NB, 128, S), BF16),
            pltpu.VMEM((3, H // 4, 2, D // 2, E), U32),
            pltpu.VMEM((3, H // 4, 2, D // 2, E), U32),
            pltpu.VMEM((NB, H * E // 2, 128), U32),
            pltpu.VMEM((NB, S, 128), F32),
            pltpu.VMEM((3, H // 2, 2, QCAP // 2, E), U32),
            pltpu.VMEM((S // 2, H * E), U32),
            pltpu.VMEM(((M + RX) // 2, H * E), U32),
            pltpu.VMEM((M, D), BF16),
            pltpu.VMEM((M + RX, D), F32),
            pltpu.VMEM((6, M + RX, E), F32),
            pltpu.VMEM((1, NCH, 2 * C, 128), F32),
            pltpu.VMEM((1, NCH, 2 * C, 128), F32),
            pltpu.VMEM((1, NCH, 2 * C, 128), F32),
            pltpu.VMEM((S, D), BF16),
            pltpu.VMEM((2 * C, C), BF16),
            pltpu.VMEM((C, C), BF16),
            pltpu.VMEM((2 * (SEG + M), 128), F32),
            pltpu.VMEM((KS, D), BF16),
            pltpu.VMEM((NB, 128), BF16),
            pltpu.VMEM((NB, 128), BF16),
            pltpu.SMEM((2,), jnp.int32),
            pltpu.SemaphoreType.DMA((6,)),
            pltpu.SemaphoreType.DMA((NB,)),
        ],
        compiler_params=pltpu.CompilerParams(vmem_limit_bytes=120 * 2 ** 20, disable_bounds_checks=True),
    )(
        A_q.reshape(S, D), A_k.reshape(S, D), A_v.reshape(S, D), A_ssm_k,
        B_Wq.reshape(D // 2, 2, H, E), B_Wk.reshape(D // 2, 2, H, E), B_Wv.reshape(D // 2, 2, H, E),
        B_Wo.reshape(H * E, D),
        A_shift_k.T, A_ssm_D.reshape(NB, 128), gate_w.reshape(NB, 128), B_mem0.reshape(M, D),
        jnp.asarray(fwd, BF16), jnp.asarray(inv, BF16), jnp.asarray(_attn_fill()),
    )
    return out.reshape(1, S, D)


def pallas_gated_mix__ssm_conv_h3__memory_aug_recurrent_mem_tr__prompt_kernel(
    A_q, A_k, A_v, A_shift_k, A_ssm_k, A_ssm_D, B_x, B_mem0, B_Wq, B_Wk, B_Wv, B_Wo, B_seg_len, gate_w,
):
    del B_x
    if isinstance(B_seg_len, int):
        assert B_seg_len == SEG
    return _run(A_q, A_k, A_v, A_shift_k, A_ssm_k, A_ssm_D, B_mem0, B_Wq, B_Wk, B_Wv, B_Wo, gate_w)
```

```python
import functools
import math

import jax
import jax.numpy as jnp
import numpy as np
import jax.experimental.pallas as pl
import jax.experimental.pallas.tpu as pltpu

F32 = jnp.float32
BF16 = jnp.bfloat16
U32 = jnp.uint32

S = 2048
D = 1024
H = 32
E = 128
M = 8
SEG = 32
NSEG = S // SEG
RX = 24
PRO = S - RX * NSEG
QCAP = 576
QOFF = QCAP - PRO
HL = 4
HS = H - HL
MAT_ORDER = (0, 1, 2)
OFF_LQK, OFF_S, OFF_LV, OFF_PV = 4, 8, 14, 17
UNROLL = 4
C = 128
NCH = S // C
NB = D // 128
KS = 4
NEG = -1000000000.0


def _dft_tables():
    n = np.arange(C, dtype=np.float64)
    k = np.concatenate([np.arange(C // 2), C - 1 - np.arange(C // 2)]).astype(np.float64)
    th = np.pi * (2.0 * k + 1.0) / (2 * C)
    fwd = np.concatenate([np.cos(th[:, None] * n[None, :]), -np.sin(th[:, None] * n[None, :])], axis=0)
    no = np.concatenate([n[0::2], n[1::2]])
    tl = th[:C // 2]
    inv = np.concatenate([np.cos(no[:, None] * tl[None, :]), -np.sin(no[:, None] * tl[None, :])], axis=1) / C
    return fwd.astype(np.float32), inv.astype(np.float32)


def _attn_fill():
    n = 2 * (SEG + M)
    head = np.array([0] * SEG + [1] * SEG + [0] * M + [1] * M)
    pos = np.concatenate([M + np.arange(SEG), M + np.arange(SEG), np.arange(M), np.arange(M)])
    fill = np.full((n, 128), -np.inf, np.float32)
    for i in range(n):
        for j in range(n):
            if head[i] == head[j]:
                ok = pos[i] < M or pos[i] >= pos[j]
                fill[i, j] = 0.0 if ok else NEG
    return fill


def _dot(a, b):
    return jnp.dot(a, b, preferred_element_type=F32)


def _dot_nt(a, b):
    return jax.lax.dot_general(a, b, (((1,), (1,)), ((), ())), preferred_element_type=F32)


def _pack(a):
    return pltpu.bitcast(a.astype(BF16), U32)


def _unpack(a):
    return pltpu.bitcast(a, BF16)


def _kernel(x_hbm, k_hbm, v_hbm, h_hbm, wq_hbm, wk_hbm, wv_hbm, wo_hbm,
            sk_hbm, dd_hbm, gw_hbm, mem0_hbm, fwd_hbm, inv_hbm, fill_hbm,
            out_hbm,
            x_v, xp, k_v, v_v, h_v, w_even, w_odd, wo_v, y_v, qkv_b, o_b, lo_s, mem_v, oacc, qacc,
            u_s, h_s, yf_s,
            out_v, fwd_ref, inv_ref, fill_ref, sk_ref, dd_ref, gw_ref, zs, sems, qsems):
    scale = E ** (-0.5)
    wbuf = (w_even, w_odd)

    w32 = [w.bitcast(U32) for w in (wq_hbm, wk_hbm, wv_hbm)]
    wo32 = wo_hbm.bitcast(U32)
    x32 = x_hbm.bitcast(U32)

    def lanes(c):
        return pl.ds(pl.multiple_of(c * 128, 128), 128)

    def w_copies(c, e, mat, sem):
        return [pltpu.make_async_copy(w32[mat].at[:, par, 2 * c + e, :], wbuf[e].at[mat, c, par], sem)
                for par in range(2)]

    def wq0_copies(c):
        return w_copies(c, 0, 0, qsems.at[c])

    def block_copies(c):
        sem = sems.at[c % 2]
        return ([[pltpu.make_async_copy(h_hbm.at[lanes(c), :], h_v.at[c], sem)],
                 [pltpu.make_async_copy(k_hbm.at[:, lanes(c)], k_v.at[c], sem)],
                 [pltpu.make_async_copy(v_hbm.at[:, lanes(c)], v_v.at[c], sem)]]
                + [w_copies(c, e, mat, sem) for e in range(2) for mat in range(3) if (e, mat) != (0, 0)])

    def rest_copies(c):
        rows = pl.ds(pl.multiple_of(c * (S // NB), S // NB), S // NB)
        return [pltpu.make_async_copy(wo32.at[:, lanes(c)], wo_v.at[c], sems.at[2]),
                pltpu.make_async_copy(x_hbm.at[rows, :], x_v.at[rows, :], sems.at[2])]

    xp_copy = pltpu.make_async_copy(x32.at[pl.ds(0, PRO // 2), :], xp, sems.at[3])
    small_copies = [pltpu.make_async_copy(src, dst, sems.at[4]) for src, dst in (
        (sk_hbm, sk_ref), (fwd_hbm, fwd_ref), (dd_hbm, dd_ref), (inv_hbm, inv_ref),
        (gw_hbm, gw_ref), (mem0_hbm, mem_v), (fill_hbm, fill_ref))]

    def out_copy(start, n):
        rows = pl.ds(start, n)
        return pltpu.make_async_copy(out_v.at[rows, :], out_hbm.at[rows, :], sems.at[5])

    def row_of(ref, c):
        t = ref[...].astype(F32)
        sel = jax.lax.broadcasted_iota(jnp.int32, (NB, 128), 0) == c
        return jnp.sum(jnp.where(sel, t, 0.0), axis=0, keepdims=True)

    def fwd_dft(c, zw):
        skt = sk_ref[:, lanes(c)].astype(F32)
        tail = jnp.zeros((8, 128), F32)
        for a in range(NCH):
            hf = _dot_nt(fwd_ref[...], h_v[c, :, pl.ds(a * C, C)])
            if a == 0:
                h_s[zw, a, 0:C, :] = hf[0:C] + row_of(dd_ref, c)
                h_s[zw, a, C:, :] = hf[C:]
            else:
                h_s[zw, a] = hf
            kc = k_v[c, pl.ds(a * C, C), :].astype(F32)
            ext = jnp.concatenate([tail, kc], axis=0)
            tail = kc[C - 8:]
            ks_ = kc * skt[0:1, :]
            for j in range(1, KS):
                ks_ = ks_ + pltpu.roll(ext, j, 0)[8:] * skt[j:j + 1, :]
            kv = (ks_ * v_v[c, pl.ds(a * C, C), :].astype(F32)).astype(BF16)
            u_s[zw, a] = _dot(fwd_ref[...], kv)

    def mac(p, zw, zr):
        re = pl.ds(p * 8, 8)
        im = pl.ds(C + p * 8, 8)
        sgn = (1 - 2 * (jax.lax.broadcasted_iota(jnp.int32, (8, 128), 0) % 2)).astype(F32)
        if p >= C // 16:
            sgn = -sgn
        AB = 4
        prev = None
        for a0 in range(0, NCH, AB):
            zre = [None] * AB
            zim = [None] * AB
            for m in range(a0 + AB):
                hr = h_s[zr, m, re, :]
                hi = h_s[zr, m, im, :]
                for i in range(AB):
                    t = a0 + i - m
                    if t < 0:
                        continue
                    ur = u_s[zr, t, re, :]
                    ui = u_s[zr, t, im, :]
                    tr = hr * ur - hi * ui
                    ti = hr * ui + hi * ur
                    zre[i] = tr if zre[i] is None else zre[i] + tr
                    zim[i] = ti if zim[i] is None else zim[i] + ti
            for i in range(AB):
                if prev is None:
                    yf_s[zw, a0 + i, re, :] = zre[i]
                    yf_s[zw, a0 + i, im, :] = zim[i]
                else:
                    yf_s[zw, a0 + i, re, :] = zre[i] - sgn * prev[1]
                    yf_s[zw, a0 + i, im, :] = zim[i] + sgn * prev[0]
                prev = (zre[i], zim[i])

    def inv_dft(c, zr):
        hc = C // 2
        for a in range(NCH):
            yr, yrm = yf_s[zr, a, 0:hc, :], yf_s[zr, a, hc:C, :]
            yi, yim = yf_s[zr, a, C:C + hc, :], yf_s[zr, a, C + hc:, :]
            fe = jnp.concatenate([yr + yrm, yi - yim], axis=0).astype(BF16)
            fo = jnp.concatenate([yr - yrm, yi + yim], axis=0).astype(BF16)
            y_v[c, pl.ds(a * C, hc, stride=2), :] = _dot(inv_ref[0:hc, :], fe)
            y_v[c, pl.ds(a * C + 1, hc, stride=2), :] = _dot(inv_ref[hc:, :], fo)

    def fixup(e, c, mat):
        a = wbuf[e][mat, c, 0]
        b = wbuf[e][mat, c, 1]
        wbuf[e][mat, c, 0] = (a & U32(0xFFFF)) | (b << 16)
        wbuf[e][mat, c, 1] = (a >> 16) | (b & U32(0xFFFF0000))

    RB = 128

    def qkv_tile(e, c, n):
        mat, j = n // 2, n % 2
        for r in range(PRO // RB):
            w = _unpack(wbuf[e][mat, c, j])
            xr = _unpack(xp[pl.ds(r * RB // 2, RB // 2), :])
            qkv_b[mat, 2 * c + e, j, pl.ds((QOFF + r * RB) // 2, RB // 2), :] = _pack(_dot(xr, w))

    for cp in wq0_copies(0) + [xp_copy]:
        cp.start()
    zs[0] = 0
    zs[1] = 0
    xp_copy.wait()
    for cp in wq0_copies(1) + wq0_copies(2) + small_copies + sum(block_copies(0)[:1], []):
        cp.start()

    def start_when(cond, copies):
        @pl.when(cond)
        def _():
            for cp in copies:
                cp.start()

    def pro0(c, carry):
        for cp in wq0_copies(c):
            cp.wait()
        fixup(0, c, 0)
        qkv_tile(0, c, 0)
        qkv_tile(0, c, 1)
        start_when(c + 3 < NB, wq0_copies(jnp.minimum(c + 3, NB - 1)))
        for i in range(1, NB):
            start_when(c == min(i - 1, NB - 3), block_copies(0)[i])
        return carry

    with jax.named_scope("pro0"):
        jax.lax.fori_loop(0, NB, pro0, 0)
    for piece in block_copies(1):
        for cp in piece:
            cp.start()
    for cp in small_copies:
        cp.wait()

    zw = zs[0]
    zr = zs[1]

    def pro(c, carry):
        for piece in block_copies(c):
            for cp in piece:
                cp.wait()

        tiles = [(0, n) for n in range(2, 6)] + [(1, n) for n in range(6)]

        def tile(i):
            e, n = tiles[i]
            if n % 2 == 0:
                fixup(e, c, n // 2)
            qkv_tile(e, c, n)

        tile(0)
        fwd_dft(c, zw)
        p = 0
        for i in range(1, 8):
            tile(i)
            for _ in range(3 if i < 3 else 2):
                mac(p, zw, zr)
                p += 1
        inv_dft(c, zr)
        tile(8)
        tile(9)
        for piece in block_copies(jnp.minimum(c + 2, NB - 1)):
            start_when(c + 2 < NB, piece)
        start_when(c + 1 < NB, rest_copies(c))
        start_when(c + 2 == NB, rest_copies(NB - 1))
        return carry

    with jax.named_scope("pro"):
        jax.lax.fori_loop(0, NB, pro, 0)
    for c in range(NB):
        for cp in rest_copies(c):
            cp.wait()

    gwt = gw_ref[...].astype(F32)
    gw = jnp.concatenate([gwt[j:j + 1, :] for j in range(NB)], axis=1)

    def finalize(rows, b):
        xr = x_v[rows, :].astype(F32)
        g = jax.nn.sigmoid(jnp.sum(xr * gw, axis=-1, keepdims=True))
        a = xr * jnp.concatenate([y_v[j, rows, :] for j in range(NB)], axis=1)
        out_v[rows, :] = (g * a + (1.0 - g) * b).astype(BF16)

    def step(s, mem, split_first, odd):
        xrows = slice(M, M + RX) if odd else slice(0, RX)
        mrows = slice(0, M) if odd else slice(RX, RX + M)
        sh = 4 if odd else 0
        xo = pl.multiple_of(PRO + RX * s, 8)
        wbase = pl.multiple_of((RX // 2 * s) % (QCAP // 2) - sh, 8)
        rpos = pl.multiple_of((SEG // 2 * s + QOFF // 2) % (QCAP // 2), SEG // 2)
        opos = pl.multiple_of(SEG // 2 * s, SEG // 2)
        fbase = pl.multiple_of(RX // 2 * s - sh, 8)
        xs = x_v[pl.ds(xo, RX), :]
        lhs = jnp.concatenate([mem, xs] if odd else [xs, mem], axis=0)
        zpad = jnp.zeros((128 - 2 * (SEG + M), E), BF16)
        frows = pl.ds(pl.multiple_of(RX * s, 8), RX)
        low = jax.lax.broadcasted_iota(jnp.int32, (8, E), 0) < 4
        NP = H // 2

        mem_qkv = {}
        probs = {}
        cats = {}

        def load(mat, hp):
            parts = [_unpack(qkv_b[mat, hp, 0, pl.ds(rpos, SEG // 2), :]),
                     _unpack(qkv_b[mat, hp, 1, pl.ds(rpos, SEG // 2), :]), mem_qkv[(hp, mat)]]
            if mat > 0:
                parts.append(zpad)
            cats[(mat, hp)] = jnp.concatenate(parts, axis=0)

        def stage_a(hp):
            KH = D // 2
            split = split_first and hp == 0
            if split:
                for mat in range(3):
                    for j in range(2):
                        w = _unpack(wbuf[hp % 2][mat, hp // 2, j, :KH // 2, :])
                        qacc[2 * mat + j] = _dot(lhs[:, :KH], w)
            for mi, mat in enumerate(MAT_ORDER):
                mm = []
                for j in range(2):
                    if split:
                        w = _unpack(wbuf[hp % 2][mat, hp // 2, j, KH // 2:, :])
                        res = qacc[2 * mat + j] + _dot(lhs[:, KH:], w)
                    else:
                        res = _dot(lhs, _unpack(wbuf[hp % 2][mat, hp // 2, j]))
                    pk = _pack(res)
                    if odd:
                        qkv_b[mat, hp, j, pl.ds(wbase + 4, 4), :] = pk[4:8]
                        qkv_b[mat, hp, j, pl.ds(wbase + 8, 8), :] = pk[8:16]
                    else:
                        qkv_b[mat, hp, j, pl.ds(wbase, 8), :] = pk[0:8]
                        qkv_b[mat, hp, j, pl.ds(wbase + 8, 4), :] = pk[8:12]
                    mm.append(res[mrows])
                    if j == 1:
                        mem_qkv[(hp, mat)] = jnp.concatenate(mm, axis=0).astype(BF16)
                    advance(6 * hp + 2 * mi + j + 1)

        def stage_b(hp):
            sc = _dot_nt(cats[(0, hp)], cats[(1, hp)]) * scale
            fill = fill_ref[...]
            sc = jnp.where(fill == 0.0, sc, fill)
            mx = jnp.max(sc, axis=-1, keepdims=True)
            p = jnp.exp(sc - mx)
            l = jnp.sum(p, axis=-1, keepdims=True)
            r = pl.reciprocal(l, approx=True)
            r = r * (2.0 - l * r)
            probs[hp] = (p * r).astype(BF16)

        def stage_c(hp):
            o = _dot(probs[hp], cats[(2, hp)])
            for j in range(2):
                h = 2 * hp + j
                cols = slice(h * E, (h + 1) * E)
                o_b[pl.ds(opos, SEG // 2), cols] = _pack(o[j * SEG:(j + 1) * SEG])
                om = o[2 * SEG + j * M:2 * SEG + (j + 1) * M]
                om = _pack(jnp.concatenate([om, om], axis=0))
                w0 = o_b[pl.ds(fbase, 8), cols]
                w1 = o_b[pl.ds(fbase + 8, 8), cols]
                lo_s[0:8, cols] = jnp.where(low, om, w0) if odd else w0
                lo_s[8:16, cols] = w1 if odd else jnp.where(low, w1, om)

        def oproj(j, late):
            ks = slice(HS * E, H * E) if late else slice(0, HS * E)
            kw = slice(ks.start // 2, ks.stop // 2)
            return _dot(_unpack(lo_s[:, ks]), _unpack(wo_v[j, kw, :]))

        events = []
        for hp in range(NP):
            events.append((6 * hp + OFF_LQK, 0, functools.partial(load, 0, hp)))
            events.append((6 * hp + OFF_LQK, 1, functools.partial(load, 1, hp)))
            events.append((6 * hp + OFF_LV, 2, functools.partial(load, 2, hp)))
            events.append((6 * hp + OFF_PV, 3, functools.partial(stage_c, hp)))
            events.append((6 * hp + OFF_S, 4, functools.partial(stage_b, hp)))
        events.sort(key=lambda ev: ev[:2])

        def advance(slot):
            while events and events[0][0] <= slot:
                events.pop(0)[2]()

        outs = [None] * NB
        for hp in range(NP):
            stage_a(hp)
        for j in range(NB):
            oacc[:, j * 128:(j + 1) * 128] = oproj(j, False)
            advance(6 * NP + (j + 1) * HS // 8)
        assert not events
        for j in range(NB):
            outs[j] = oacc[:, j * 128:(j + 1) * 128] + oproj(j, True)
        res = jnp.concatenate(outs, axis=1)
        finalize(frows, res[xrows])
        return res[mrows].astype(BF16)

    def steps(i, carry):
        mem = mem_v[...]
        for u in range(UNROLL):
            mem = step(i * UNROLL + u, mem, u > 0, u % 2 == 1)
        mem_v[...] = mem
        return carry

    with jax.named_scope("main"):
        jax.lax.fori_loop(0, NSEG // UNROLL, steps, 0)

    def epi_rows(r0, n):
        lo = _unpack(o_b[pl.ds(pl.multiple_of(r0 // 2, 8), n // 2), :])
        outs = [_dot(lo, _unpack(wo_v[j])) for j in range(NB)]
        finalize(pl.ds(r0, n), jnp.concatenate(outs, axis=1))

    EB = 128

    def epi(r, carry):
        r0 = pl.multiple_of(S - PRO + r * EB, EB)

        @pl.when(r == PRO // EB - 1)
        def _():
            out_copy(S - PRO, PRO - EB).start()

        epi_rows(r0, EB)
        return carry

    with jax.named_scope("epi"):
        out_copy(0, S - PRO).start()
        jax.lax.fori_loop(0, PRO // EB, epi, 0)
    out_copy(S - EB, EB).start()
    out_copy(0, S).wait()


@jax.jit
def _run(A_q, A_k, A_v, A_shift_k, A_ssm_k, A_ssm_D, B_mem0, B_Wq, B_Wk, B_Wv, B_Wo, gate_w):
    fwd, inv = _dft_tables()
    any_spec = pl.BlockSpec(memory_space=pl.ANY)
    out = pl.pallas_call(
        _kernel,
        out_shape=jax.ShapeDtypeStruct((S, D), BF16),
        in_specs=[any_spec] * 15,
        out_specs=any_spec,
        scratch_shapes=[
            pltpu.VMEM((S, D), BF16),
            pltpu.VMEM((PRO // 2, D), U32),
            pltpu.VMEM((NB, S, 128), BF16),
            pltpu.VMEM((NB, S, 128), BF16),
            pltpu.VMEM((NB, 128, S), BF16),
            pltpu.VMEM((3, H // 4, 2, D // 2, E), U32),
            pltpu.VMEM((3, H // 4, 2, D // 2, E), U32),
            pltpu.VMEM((NB, H * E // 2, 128), U32),
            pltpu.VMEM((NB, S, 128), F32),
            pltpu.VMEM((3, H // 2, 2, QCAP // 2, E), U32),
            pltpu.VMEM((S // 2, H * E), U32),
            pltpu.VMEM(((M + RX) // 2, H * E), U32),
            pltpu.VMEM((M, D), BF16),
            pltpu.VMEM((M + RX, D), F32),
            pltpu.VMEM((6, M + RX, E), F32),
            pltpu.VMEM((1, NCH, 2 * C, 128), F32),
            pltpu.VMEM((1, NCH, 2 * C, 128), F32),
            pltpu.VMEM((1, NCH, 2 * C, 128), F32),
            pltpu.VMEM((S, D), BF16),
            pltpu.VMEM((2 * C, C), BF16),
            pltpu.VMEM((C, C), BF16),
            pltpu.VMEM((2 * (SEG + M), 128), F32),
            pltpu.VMEM((KS, D), BF16),
            pltpu.VMEM((NB, 128), BF16),
            pltpu.VMEM((NB, 128), BF16),
            pltpu.SMEM((2,), jnp.int32),
            pltpu.SemaphoreType.DMA((6,)),
            pltpu.SemaphoreType.DMA((NB,)),
        ],
        compiler_params=pltpu.CompilerParams(vmem_limit_bytes=120 * 2 ** 20, disable_bounds_checks=True),
    )(
        A_q.reshape(S, D), A_k.reshape(S, D), A_v.reshape(S, D), A_ssm_k,
        B_Wq.reshape(D // 2, 2, H, E), B_Wk.reshape(D // 2, 2, H, E), B_Wv.reshape(D // 2, 2, H, E),
        B_Wo.reshape(H * E, D),
        A_shift_k.T, A_ssm_D.reshape(NB, 128), gate_w.reshape(NB, 128), B_mem0.reshape(M, D),
        jnp.asarray(fwd, BF16), jnp.asarray(inv, BF16), jnp.asarray(_attn_fill()),
    )
    return out.reshape(1, S, D)


def pallas_gated_mix__ssm_conv_h3__memory_aug_recurrent_mem_tr__prompt_kernel(
    A_q, A_k, A_v, A_shift_k, A_ssm_k, A_ssm_D, B_x, B_mem0, B_Wq, B_Wk, B_Wv, B_Wo, B_seg_len, gate_w,
):
    del B_x
    if isinstance(B_seg_len, int):
        assert B_seg_len == SEG
    return _run(A_q, A_k, A_v, A_shift_k, A_ssm_k, A_ssm_D, B_mem0, B_Wq, B_Wk, B_Wv, B_Wo, gate_w)
```

```python
import functools
import math

import jax
import jax.numpy as jnp
import numpy as np
import jax.experimental.pallas as pl
import jax.experimental.pallas.tpu as pltpu

F32 = jnp.float32
BF16 = jnp.bfloat16
U32 = jnp.uint32

S = 2048
D = 1024
H = 32
E = 128
M = 8
SEG = 32
NSEG = S // SEG
RX = 24
PRO = S - RX * NSEG
QCAP = 576
QOFF = QCAP - PRO
HL = 4
HS = H - HL
MAT_ORDER = (0, 1, 2)
OFF_LQK, OFF_S, OFF_LV, OFF_PV = 4, 8, 14, 17
UNROLL = 4
C = 128
NCH = S // C
NB = D // 128
KS = 4
NEG = -1000000000.0


def _dft_tables():
    n = np.arange(C, dtype=np.float64)
    th = 2.0 * np.pi * (np.arange(C, dtype=np.float64) + 0.25) / C
    fwd = np.concatenate([np.cos(th[:, None] * n[None, :]), -np.sin(th[:, None] * n[None, :])], axis=0)
    no = np.concatenate([n[0::2], n[1::2]])
    tl = th[:C // 2]
    inv = np.concatenate([np.cos(no[:, None] * tl[None, :]), -np.sin(no[:, None] * tl[None, :])], axis=1) / C
    return fwd.astype(np.float32), inv.astype(np.float32)


def _attn_fill():
    n = 2 * (SEG + M)
    head = np.array([0] * SEG + [1] * SEG + [0] * M + [1] * M)
    pos = np.concatenate([M + np.arange(SEG), M + np.arange(SEG), np.arange(M), np.arange(M)])
    fill = np.full((n, 128), -np.inf, np.float32)
    for i in range(n):
        for j in range(n):
            if head[i] == head[j]:
                ok = pos[i] < M or pos[i] >= pos[j]
                fill[i, j] = 0.0 if ok else NEG
    return fill


def _dot(a, b):
    return jnp.dot(a, b, preferred_element_type=F32)


def _dot_nt(a, b):
    return jax.lax.dot_general(a, b, (((1,), (1,)), ((), ())), preferred_element_type=F32)


def _pack(a):
    return pltpu.bitcast(a.astype(BF16), U32)


def _unpack(a):
    return pltpu.bitcast(a, BF16)


def _kernel(x_hbm, k_hbm, v_hbm, h_hbm, wq_hbm, wk_hbm, wv_hbm, wo_hbm,
            sk_hbm, dd_hbm, gw_hbm, mem0_hbm, fwd_hbm, inv_hbm, fill_hbm,
            out_hbm,
            x_v, xp, k_v, v_v, h_v, w_even, w_odd, wo_v, y_v, qkv_b, o_b, lo_s, mem_v, oacc, qacc,
            u_s, h_s, yf_s,
            out_v, fwd_ref, inv_ref, fill_ref, sk_ref, dd_ref, gw_ref, zs, sems, qsems):
    scale = E ** (-0.5)
    wbuf = (w_even, w_odd)

    w32 = [w.bitcast(U32) for w in (wq_hbm, wk_hbm, wv_hbm)]
    wo32 = wo_hbm.bitcast(U32)
    x32 = x_hbm.bitcast(U32)

    def lanes(c):
        return pl.ds(pl.multiple_of(c * 128, 128), 128)

    def w_copies(c, e, mat, sem):
        return [pltpu.make_async_copy(w32[mat].at[:, par, 2 * c + e, :], wbuf[e].at[mat, c, par], sem)
                for par in range(2)]

    def wq0_copies(c):
        return w_copies(c, 0, 0, qsems.at[c])

    def block_copies(c):
        sem = sems.at[c % 2]
        return ([[pltpu.make_async_copy(h_hbm.at[lanes(c), :], h_v.at[c], sem)],
                 [pltpu.make_async_copy(k_hbm.at[:, lanes(c)], k_v.at[c], sem)],
                 [pltpu.make_async_copy(v_hbm.at[:, lanes(c)], v_v.at[c], sem)]]
                + [w_copies(c, e, mat, sem) for e in range(2) for mat in range(3) if (e, mat) != (0, 0)])

    def rest_copies(c):
        rows = pl.ds(pl.multiple_of(c * (S // NB), S // NB), S // NB)
        return [pltpu.make_async_copy(wo32.at[:, lanes(c)], wo_v.at[c], sems.at[2]),
                pltpu.make_async_copy(x_hbm.at[rows, :], x_v.at[rows, :], sems.at[2])]

    xp_copy = pltpu.make_async_copy(x32.at[pl.ds(0, PRO // 2), :], xp, sems.at[3])
    small_copies = [pltpu.make_async_copy(src, dst, sems.at[4]) for src, dst in (
        (sk_hbm, sk_ref), (fwd_hbm, fwd_ref), (dd_hbm, dd_ref), (inv_hbm, inv_ref),
        (gw_hbm, gw_ref), (mem0_hbm, mem_v), (fill_hbm, fill_ref))]

    def out_copy(start, n):
        rows = pl.ds(start, n)
        return pltpu.make_async_copy(out_v.at[rows, :], out_hbm.at[rows, :], sems.at[5])

    def row_of(ref, c):
        t = ref[...].astype(F32)
        sel = jax.lax.broadcasted_iota(jnp.int32, (NB, 128), 0) == c
        return jnp.sum(jnp.where(sel, t, 0.0), axis=0, keepdims=True)

    def fwd_dft(c, zw):
        skt = sk_ref[:, lanes(c)].astype(F32)
        tail = jnp.zeros((8, 128), F32)
        for a in range(NCH):
            hf = _dot_nt(fwd_ref[...], h_v[c, :, pl.ds(a * C, C)])
            if a == 0:
                h_s[zw, a, 0:C, :] = hf[0:C] + row_of(dd_ref, c)
                h_s[zw, a, C:, :] = hf[C:]
            else:
                h_s[zw, a] = hf
            kc = k_v[c, pl.ds(a * C, C), :].astype(F32)
            ext = jnp.concatenate([tail, kc], axis=0)
            tail = kc[C - 8:]
            ks_ = kc * skt[0:1, :]
            for j in range(1, KS):
                ks_ = ks_ + pltpu.roll(ext, j, 0)[8:] * skt[j:j + 1, :]
            kv = (ks_ * v_v[c, pl.ds(a * C, C), :].astype(F32)).astype(BF16)
            u_s[zw, a] = _dot(fwd_ref[...], kv)

    def mac(p, zw, zr):
        re = pl.ds(p * 8, 8)
        im = pl.ds(C + p * 8, 8)
        AB = 4
        prev = None
        for a0 in range(0, NCH, AB):
            zre = [None] * AB
            zim = [None] * AB
            for m in range(a0 + AB):
                hr = h_s[zr, m, re, :]
                hi = h_s[zr, m, im, :]
                for i in range(AB):
                    t = a0 + i - m
                    if t < 0:
                        continue
                    ur = u_s[zr, t, re, :]
                    ui = u_s[zr, t, im, :]
                    tr = hr * ur - hi * ui
                    ti = hr * ui + hi * ur
                    zre[i] = tr if zre[i] is None else zre[i] + tr
                    zim[i] = ti if zim[i] is None else zim[i] + ti
            for i in range(AB):
                if prev is None:
                    yf_s[zw, a0 + i, re, :] = zre[i]
                    yf_s[zw, a0 + i, im, :] = zim[i]
                else:
                    yf_s[zw, a0 + i, re, :] = zre[i] - prev[1]
                    yf_s[zw, a0 + i, im, :] = zim[i] + prev[0]
                prev = (zre[i], zim[i])

    def inv_dft(c, zr):
        hc = C // 2
        for a in range(NCH):
            yr, yrm = yf_s[zr, a, 0:hc, :], yf_s[zr, a, hc:C, :]
            yi, yim = yf_s[zr, a, C:C + hc, :], yf_s[zr, a, C + hc:, :]
            fe = jnp.concatenate([yr + yrm, yi + yim], axis=0).astype(BF16)
            fo = jnp.concatenate([yr - yrm, yi - yim], axis=0).astype(BF16)
            y_v[c, pl.ds(a * C, hc, stride=2), :] = _dot(inv_ref[0:hc, :], fe)
            y_v[c, pl.ds(a * C + 1, hc, stride=2), :] = _dot(inv_ref[hc:, :], fo)

    def fixup(e, c, mat):
        a = wbuf[e][mat, c, 0]
        b = wbuf[e][mat, c, 1]
        wbuf[e][mat, c, 0] = (a & U32(0xFFFF)) | (b << 16)
        wbuf[e][mat, c, 1] = (a >> 16) | (b & U32(0xFFFF0000))

    RB = 128

    def qkv_tile(e, c, n):
        mat, j = n // 2, n % 2
        for r in range(PRO // RB):
            w = _unpack(wbuf[e][mat, c, j])
            xr = _unpack(xp[pl.ds(r * RB // 2, RB // 2), :])
            qkv_b[mat, 2 * c + e, j, pl.ds((QOFF + r * RB) // 2, RB // 2), :] = _pack(_dot(xr, w))

    for cp in wq0_copies(0) + [xp_copy]:
        cp.start()
    zs[0] = 0
    zs[1] = 0
    xp_copy.wait()
    for cp in wq0_copies(1) + wq0_copies(2) + small_copies + sum(block_copies(0)[:1], []):
        cp.start()

    def start_when(cond, copies):
        @pl.when(cond)
        def _():
            for cp in copies:
                cp.start()

    def pro0(c, carry):
        for cp in wq0_copies(c):
            cp.wait()
        fixup(0, c, 0)
        qkv_tile(0, c, 0)
        qkv_tile(0, c, 1)
        start_when(c + 3 < NB, wq0_copies(jnp.minimum(c + 3, NB - 1)))
        for i in range(1, NB):
            start_when(c == min(i - 1, NB - 3), block_copies(0)[i])
        return carry

    with jax.named_scope("pro0"):
        jax.lax.fori_loop(0, NB, pro0, 0)
    for piece in block_copies(1):
        for cp in piece:
            cp.start()
    for cp in small_copies:
        cp.wait()

    zw = zs[0]
    zr = zs[1]

    def pro(c, carry):
        for piece in block_copies(c):
            for cp in piece:
                cp.wait()

        tiles = [(0, n) for n in range(2, 6)] + [(1, n) for n in range(6)]

        def tile(i):
            e, n = tiles[i]
            if n % 2 == 0:
                fixup(e, c, n // 2)
            qkv_tile(e, c, n)

        tile(0)
        fwd_dft(c, zw)
        p = 0
        for i in range(1, 8):
            tile(i)
            for _ in range(3 if i < 3 else 2):
                mac(p, zw, zr)
                p += 1
        inv_dft(c, zr)
        tile(8)
        tile(9)
        for piece in block_copies(jnp.minimum(c + 2, NB - 1)):
            start_when(c + 2 < NB, piece)
        start_when(c + 1 < NB, rest_copies(c))
        start_when(c + 2 == NB, rest_copies(NB - 1))
        return carry

    with jax.named_scope("pro"):
        jax.lax.fori_loop(0, NB, pro, 0)
    for c in range(NB):
        for cp in rest_copies(c):
            cp.wait()

    gwt = gw_ref[...].astype(F32)
    gw = jnp.concatenate([gwt[j:j + 1, :] for j in range(NB)], axis=1)

    def finalize(rows, b):
        xr = x_v[rows, :].astype(F32)
        g = jax.nn.sigmoid(jnp.sum(xr * gw, axis=-1, keepdims=True))
        a = xr * jnp.concatenate([y_v[j, rows, :] for j in range(NB)], axis=1)
        out_v[rows, :] = (g * a + (1.0 - g) * b).astype(BF16)

    def step(s, mem, split_first, odd):
        xrows = slice(M, M + RX) if odd else slice(0, RX)
        mrows = slice(0, M) if odd else slice(RX, RX + M)
        sh = 4 if odd else 0
        xo = pl.multiple_of(PRO + RX * s, 8)
        wbase = pl.multiple_of((RX // 2 * s) % (QCAP // 2) - sh, 8)
        rpos = pl.multiple_of((SEG // 2 * s + QOFF // 2) % (QCAP // 2), SEG // 2)
        opos = pl.multiple_of(SEG // 2 * s, SEG // 2)
        fbase = pl.multiple_of(RX // 2 * s - sh, 8)
        xs = x_v[pl.ds(xo, RX), :]
        lhs = jnp.concatenate([mem, xs] if odd else [xs, mem], axis=0)
        zpad = jnp.zeros((128 - 2 * (SEG + M), E), BF16)
        frows = pl.ds(pl.multiple_of(RX * s, 8), RX)
        low = jax.lax.broadcasted_iota(jnp.int32, (8, E), 0) < 4
        NP = H // 2

        mem_qkv = {}
        probs = {}
        cats = {}

        def load(mat, hp):
            parts = [_unpack(qkv_b[mat, hp, 0, pl.ds(rpos, SEG // 2), :]),
                     _unpack(qkv_b[mat, hp, 1, pl.ds(rpos, SEG // 2), :]), mem_qkv[(hp, mat)]]
            if mat > 0:
                parts.append(zpad)
            cats[(mat, hp)] = jnp.concatenate(parts, axis=0)

        def stage_a(hp):
            KH = D // 2
            split = split_first and hp == 0
            if split:
                for mat in range(3):
                    for j in range(2):
                        w = _unpack(wbuf[hp % 2][mat, hp // 2, j, :KH // 2, :])
                        qacc[2 * mat + j] = _dot(lhs[:, :KH], w)
            for mi, mat in enumerate(MAT_ORDER):
                mm = []
                for j in range(2):
                    if split:
                        w = _unpack(wbuf[hp % 2][mat, hp // 2, j, KH // 2:, :])
                        res = qacc[2 * mat + j] + _dot(lhs[:, KH:], w)
                    else:
                        res = _dot(lhs, _unpack(wbuf[hp % 2][mat, hp // 2, j]))
                    pk = _pack(res)
                    if odd:
                        qkv_b[mat, hp, j, pl.ds(wbase + 4, 4), :] = pk[4:8]
                        qkv_b[mat, hp, j, pl.ds(wbase + 8, 8), :] = pk[8:16]
                    else:
                        qkv_b[mat, hp, j, pl.ds(wbase, 8), :] = pk[0:8]
                        qkv_b[mat, hp, j, pl.ds(wbase + 8, 4), :] = pk[8:12]
                    mm.append(res[mrows])
                    if j == 1:
                        mem_qkv[(hp, mat)] = jnp.concatenate(mm, axis=0).astype(BF16)
                    advance(6 * hp + 2 * mi + j + 1)

        def stage_b(hp):
            sc = _dot_nt(cats[(0, hp)], cats[(1, hp)]) * scale
            fill = fill_ref[...]
            sc = jnp.where(fill == 0.0, sc, fill)
            mx = jnp.max(sc, axis=-1, keepdims=True)
            p = jnp.exp(sc - mx)
            l = jnp.sum(p, axis=-1, keepdims=True)
            r = pl.reciprocal(l, approx=True)
            r = r * (2.0 - l * r)
            probs[hp] = (p * r).astype(BF16)

        def stage_c(hp):
            o = _dot(probs[hp], cats[(2, hp)])
            for j in range(2):
                h = 2 * hp + j
                cols = slice(h * E, (h + 1) * E)
                o_b[pl.ds(opos, SEG // 2), cols] = _pack(o[j * SEG:(j + 1) * SEG])
                om = o[2 * SEG + j * M:2 * SEG + (j + 1) * M]
                om = _pack(jnp.concatenate([om, om], axis=0))
                w0 = o_b[pl.ds(fbase, 8), cols]
                w1 = o_b[pl.ds(fbase + 8, 8), cols]
                lo_s[0:8, cols] = jnp.where(low, om, w0) if odd else w0
                lo_s[8:16, cols] = w1 if odd else jnp.where(low, w1, om)

        def oproj(j, late):
            ks = slice(HS * E, H * E) if late else slice(0, HS * E)
            kw = slice(ks.start // 2, ks.stop // 2)
            return _dot(_unpack(lo_s[:, ks]), _unpack(wo_v[j, kw, :]))

        events = []
        for hp in range(NP):
            events.append((6 * hp + OFF_LQK, 0, functools.partial(load, 0, hp)))
            events.append((6 * hp + OFF_LQK, 1, functools.partial(load, 1, hp)))
            events.append((6 * hp + OFF_LV, 2, functools.partial(load, 2, hp)))
            events.append((6 * hp + OFF_PV, 3, functools.partial(stage_c, hp)))
            events.append((6 * hp + OFF_S, 4, functools.partial(stage_b, hp)))
        events.sort(key=lambda ev: ev[:2])

        def advance(slot):
            while events and events[0][0] <= slot:
                events.pop(0)[2]()

        outs = [None] * NB
        for hp in range(NP):
            stage_a(hp)
        for j in range(NB):
            oacc[:, j * 128:(j + 1) * 128] = oproj(j, False)
            advance(6 * NP + (j + 1) * HS // 8)
        assert not events
        for j in range(NB):
            outs[j] = oacc[:, j * 128:(j + 1) * 128] + oproj(j, True)
        res = jnp.concatenate(outs, axis=1)
        finalize(frows, res[xrows])
        return res[mrows].astype(BF16)

    def steps(i, carry):
        mem = mem_v[...]
        for u in range(UNROLL):
            mem = step(i * UNROLL + u, mem, u > 0, u % 2 == 1)
        mem_v[...] = mem
        return carry

    with jax.named_scope("main"):
        jax.lax.fori_loop(0, NSEG // UNROLL, steps, 0)

    def epi_rows(r0, n):
        lo = _unpack(o_b[pl.ds(pl.multiple_of(r0 // 2, 8), n // 2), :])
        outs = [_dot(lo, _unpack(wo_v[j])) for j in range(NB)]
        finalize(pl.ds(r0, n), jnp.concatenate(outs, axis=1))

    EB = 128

    def epi(r, carry):
        r0 = pl.multiple_of(S - PRO + r * EB, EB)

        @pl.when(r == PRO // EB - 1)
        def _():
            out_copy(S - PRO, PRO - EB).start()

        epi_rows(r0, EB)
        return carry

    with jax.named_scope("epi"):
        out_copy(0, S - PRO).start()
        jax.lax.fori_loop(0, PRO // EB, epi, 0)
    out_copy(S - EB, EB).start()
    out_copy(0, S).wait()


@jax.jit
def _run(A_q, A_k, A_v, A_shift_k, A_ssm_k, A_ssm_D, B_mem0, B_Wq, B_Wk, B_Wv, B_Wo, gate_w):
    fwd, inv = _dft_tables()
    any_spec = pl.BlockSpec(memory_space=pl.ANY)
    out = pl.pallas_call(
        _kernel,
        out_shape=jax.ShapeDtypeStruct((S, D), BF16),
        in_specs=[any_spec] * 15,
        out_specs=any_spec,
        scratch_shapes=[
            pltpu.VMEM((S, D), BF16),
            pltpu.VMEM((PRO // 2, D), U32),
            pltpu.VMEM((NB, S, 128), BF16),
            pltpu.VMEM((NB, S, 128), BF16),
            pltpu.VMEM((NB, 128, S), BF16),
            pltpu.VMEM((3, H // 4, 2, D // 2, E), U32),
            pltpu.VMEM((3, H // 4, 2, D // 2, E), U32),
            pltpu.VMEM((NB, H * E // 2, 128), U32),
            pltpu.VMEM((NB, S, 128), F32),
            pltpu.VMEM((3, H // 2, 2, QCAP // 2, E), U32),
            pltpu.VMEM((S // 2, H * E), U32),
            pltpu.VMEM(((M + RX) // 2, H * E), U32),
            pltpu.VMEM((M, D), BF16),
            pltpu.VMEM((M + RX, D), F32),
            pltpu.VMEM((6, M + RX, E), F32),
            pltpu.VMEM((1, NCH, 2 * C, 128), F32),
            pltpu.VMEM((1, NCH, 2 * C, 128), F32),
            pltpu.VMEM((1, NCH, 2 * C, 128), F32),
            pltpu.VMEM((S, D), BF16),
            pltpu.VMEM((2 * C, C), BF16),
            pltpu.VMEM((C, C), BF16),
            pltpu.VMEM((2 * (SEG + M), 128), F32),
            pltpu.VMEM((KS, D), BF16),
            pltpu.VMEM((NB, 128), BF16),
            pltpu.VMEM((NB, 128), BF16),
            pltpu.SMEM((2,), jnp.int32),
            pltpu.SemaphoreType.DMA((6,)),
            pltpu.SemaphoreType.DMA((NB,)),
        ],
        compiler_params=pltpu.CompilerParams(vmem_limit_bytes=120 * 2 ** 20, disable_bounds_checks=True),
    )(
        A_q.reshape(S, D), A_k.reshape(S, D), A_v.reshape(S, D), A_ssm_k,
        B_Wq.reshape(D // 2, 2, H, E), B_Wk.reshape(D // 2, 2, H, E), B_Wv.reshape(D // 2, 2, H, E),
        B_Wo.reshape(H * E, D),
        A_shift_k.T, A_ssm_D.reshape(NB, 128), gate_w.reshape(NB, 128), B_mem0.reshape(M, D),
        jnp.asarray(fwd, BF16), jnp.asarray(inv, BF16), jnp.asarray(_attn_fill()),
    )
    return out.reshape(1, S, D)


def pallas_gated_mix__ssm_conv_h3__memory_aug_recurrent_mem_tr__prompt_kernel(
    A_q, A_k, A_v, A_shift_k, A_ssm_k, A_ssm_D, B_x, B_mem0, B_Wq, B_Wk, B_Wv, B_Wo, B_seg_len, gate_w,
):
    del B_x
    if isinstance(B_seg_len, int):
        assert B_seg_len == SEG
    return _run(A_q, A_k, A_v, A_shift_k, A_ssm_k, A_ssm_D, B_mem0, B_Wq, B_Wk, B_Wv, B_Wo, gate_w)
```

```python
import cmath
import functools
import math

import jax
import jax.numpy as jnp
import numpy as np
import jax.experimental.pallas as pl
import jax.experimental.pallas.tpu as pltpu

F32 = jnp.float32
BF16 = jnp.bfloat16
U32 = jnp.uint32

S = 2048
D = 1024
H = 32
E = 128
M = 8
SEG = 32
NSEG = S // SEG
RX = 24
PRO = S - RX * NSEG
QCAP = 576
QOFF = QCAP - PRO
HL = 4
HS = H - HL
MAT_ORDER = (0, 1, 2)
OFF_LQK, OFF_S, OFF_LV, OFF_PV = 4, 8, 14, 17
UNROLL = 4
C = 128
NCH = S // C
NB = D // 128
KS = 4
NEG = -1000000000.0
R1, R2 = 16, 8
PR = 72
SR = 2 * C + 8


def _dft_tables():
    n = np.arange(C, dtype=np.float64)
    th = 2.0 * np.pi * (np.arange(C, dtype=np.float64) + 0.25) / C
    fwd = np.concatenate([np.cos(th[:, None] * n[None, :]), -np.sin(th[:, None] * n[None, :])], axis=0)
    no = np.concatenate([n[0::2], n[1::2]])
    tl = th[:C // 2]
    inv = np.concatenate([np.cos(no[:, None] * tl[None, :]), -np.sin(no[:, None] * tl[None, :])], axis=1) / C
    return fwd.astype(np.float32), inv.astype(np.float32)


def _attn_fill():
    n = 2 * (SEG + M)
    head = np.array([0] * SEG + [1] * SEG + [0] * M + [1] * M)
    pos = np.concatenate([M + np.arange(SEG), M + np.arange(SEG), np.arange(M), np.arange(M)])
    fill = np.full((n, 128), -np.inf, np.float32)
    for i in range(n):
        for j in range(n):
            if head[i] == head[j]:
                ok = pos[i] < M or pos[i] >= pos[j]
                fill[i, j] = 0.0 if ok else NEG
    return fill


def _add(a, b):
    return b if a is None else a if b is None else a + b


def _sub(a, b):
    return a if b is None else -b if a is None else a - b


def _cmul(z, w):
    r, i = z
    wr, wi = w.real, w.imag
    eps = 1e-12
    if abs(wi) < eps and abs(wr - 1.0) < eps:
        return z
    if i is None:
        if abs(abs(wr) - abs(wi)) < eps and wr * wi > 0:
            t = r * wr
            return t, t
        return r * wr, r * wi
    if abs(abs(wr) - abs(wi)) < eps:
        if wr * wi > 0:
            return (r - i) * wr, (r + i) * wr
        return (r + i) * wr, (i - r) * wr
    return r * wr - i * wi, r * wi + i * wr


def _fft(xs):
    n = len(xs)
    if n == 1:
        return xs
    if n == 2:
        (ar, ai), (br, bi) = xs
        return [(_add(ar, br), _add(ai, bi)), (_sub(ar, br), _sub(ai, bi))]
    e = _fft(xs[0::2])
    o1 = _fft(xs[1::4])
    o3 = _fft(xs[3::4])
    out = [None] * n
    for k in range(n // 4):
        ar, ai = _cmul(o1[k], cmath.exp(-2j * math.pi * k / n))
        br, bi = _cmul(o3[k], cmath.exp(-6j * math.pi * k / n))
        sr, si, dr, di = _add(ar, br), _add(ai, bi), _sub(ar, br), _sub(ai, bi)
        er, ei = e[k]
        fr, fi = e[k + n // 4]
        out[k] = (_add(er, sr), _add(ei, si))
        out[k + n // 2] = (_sub(er, sr), _sub(ei, si))
        out[k + n // 4] = (_add(fr, di), _sub(fi, dr))
        out[k + 3 * n // 4] = (_sub(fr, di), _add(fi, dr))
    return out


def _dot(a, b):
    return jnp.dot(a, b, preferred_element_type=F32)


def _dot_nt(a, b):
    return jax.lax.dot_general(a, b, (((1,), (1,)), ((), ())), preferred_element_type=F32)


def _pack(a):
    return pltpu.bitcast(a.astype(BF16), U32)


def _unpack(a):
    return pltpu.bitcast(a, BF16)


def _kernel(x_hbm, k_hbm, v_hbm, h_hbm, wq_hbm, wk_hbm, wv_hbm, wo_hbm,
            sk_hbm, dd_hbm, gw_hbm, mem0_hbm, fwd_hbm, inv_hbm, fill_hbm,
            out_hbm,
            x_v, xp, k_v, v_v, h_v, w_even, w_odd, wo_v, y_v, qkv_b, o_b, lo_s, mem_v, oacc, qacc,
            u_s, h_s, yf_s, t_s, g_s,
            out_v, fwd_ref, inv_ref, fill_ref, sk_ref, dd_ref, gw_ref, zs, sems, qsems):
    scale = E ** (-0.5)
    wbuf = (w_even, w_odd)

    w32 = [w.bitcast(U32) for w in (wq_hbm, wk_hbm, wv_hbm)]
    wo32 = wo_hbm.bitcast(U32)
    x32 = x_hbm.bitcast(U32)
    k32 = k_hbm.bitcast(U32)
    v32 = v_hbm.bitcast(U32)

    def lanes(c):
        return pl.ds(pl.multiple_of(c * 128, 128), 128)

    def w_copies(c, e, mat, sem):
        return [pltpu.make_async_copy(w32[mat].at[:, par, 2 * c + e, :], wbuf[e].at[mat, c, par], sem)
                for par in range(2)]

    def wq0_copies(c):
        return w_copies(c, 0, 0, qsems.at[c])

    W_REST = [(e, mat) for e in range(2) for mat in range(3) if (e, mat) != (0, 0)]
    NPIECE = 3 + len(W_REST)

    def block_piece(c, i):
        sem = sems.at[c % 2]
        if i < 2:
            src, dst = ((k32, k_v), (v32, v_v))[i]
            return [pltpu.make_async_copy(src.at[:, :, lanes(c)], dst.at[c, :, pl.ds(0, C // 2), :], sem)]
        if i == 2:
            return [pltpu.make_async_copy(h_hbm.at[lanes(c), :], h_v.at[c], sem)]
        return w_copies(c, *W_REST[i - 3], sem)

    def rest_copies(c):
        rows = pl.ds(pl.multiple_of(c * (S // NB), S // NB), S // NB)
        return [pltpu.make_async_copy(wo32.at[:, lanes(c)], wo_v.at[c], sems.at[2]),
                pltpu.make_async_copy(x_hbm.at[rows, :], x_v.at[rows, :], sems.at[2])]

    xp_copy = pltpu.make_async_copy(x32.at[pl.ds(0, PRO // 2), :], xp, sems.at[3])
    small_copies = [pltpu.make_async_copy(src, dst, sems.at[4]) for src, dst in (
        (sk_hbm, sk_ref), (fwd_hbm, fwd_ref), (dd_hbm, dd_ref), (inv_hbm, inv_ref),
        (gw_hbm, gw_ref), (mem0_hbm, mem_v), (fill_hbm, fill_ref))]

    def out_copy(start, n):
        rows = pl.ds(start, n)
        return pltpu.make_async_copy(out_v.at[rows, :], out_hbm.at[rows, :], sems.at[5])

    def row_of(ref, c):
        t = ref[...].astype(F32)
        sel = jax.lax.broadcasted_iota(jnp.int32, (NB, 128), 0) == c
        return jnp.sum(jnp.where(sel, t, 0.0), axis=0, keepdims=True)

    k2 = k_v.reshape(NB, NCH * PR, 128)
    v2 = v_v.reshape(NB, NCH * PR, 128)

    def fwd_h(c, zw):
        for a in range(NCH):
            hf = _dot_nt(fwd_ref[...], h_v[c, :, pl.ds(a * C, C)])
            if a == 0:
                h_s[zw, pl.ds(0, C), :] = hf[0:C] + row_of(dd_ref, c)
                h_s[zw, pl.ds(C, C), :] = hf[C:]
                k2[c + zw, pl.ds(C // 2, 8), :] = pltpu.bitcast(hf[0:8], U32)
                v2[c + zw, pl.ds(C // 2, 8), :] = pltpu.bitcast(hf[0:8], U32)
            else:
                h_s[zw, pl.ds(a * SR, 2 * C), :] = hf

    def pair(ref, c, g, pr):
        w = ref[c, pl.ds(8 * g * PR + pr, 8, stride=PR), :]
        return pltpu.bitcast(w << 16, F32), pltpu.bitcast(w & U32(0xFFFF0000), F32)

    def kv_prep(c, zw):
        skt = sk_ref[:, lanes(c)].astype(F32)
        sk = [jnp.broadcast_to(skt[j:j + 1, :], (8, 128)) for j in range(KS)]
        first = jax.lax.broadcasted_iota(jnp.int32, (8, 128), 0) == 0
        carry = [jnp.zeros((8, 128), F32)] * (KS - 1)
        for g in range(NCH // 8):
            tail = list(pair(k2, c, g, C // 2 - 2) + pair(k2, c, g, C // 2 - 1))[1:]
            tail = [pltpu.roll(t, 1, 0) for t in tail]
            win = [jnp.where(first, cr, t) for cr, t in zip(carry, tail)]
            carry = tail
            for pr in range(C // 2):
                ks = pair(k2, c, g, pr)
                vs = pair(v2, c, g, pr)
                for i in range(2):
                    win.append(ks[i])
                    acc = win[-1] * sk[0]
                    for j in range(1, KS):
                        acc = acc + win[-1 - j] * sk[j]
                    win = win[1:]
                    t_s[zw, pl.ds((g * C + 2 * pr + i) * 8, 8), :] = acc * vs[i]

    def fft1(zw, zr):
        for g in range(NCH // 8):
            for b in range(R2):
                z = [_cmul((t_s[zr, pl.ds((g * C + R2 * a + b) * 8, 8), :], None),
                           cmath.exp(-0.5j * math.pi * a / R1)) for a in range(R1)]
                gq = _fft(z)
                for q1 in range(R1):
                    re, im = _cmul(gq[q1], cmath.exp(-2j * math.pi * (q1 + 0.25) * b / C))
                    row = ((g * R1 + q1) * R2 + b) * 16
                    g_s[zw, pl.ds(row, 8), :] = re
                    g_s[zw, pl.ds(row + 8, 8), :] = im

    def fft2(dst, zw, zr):
        for g in range(NCH // 8):
            for q1 in range(R1):
                z = []
                for b in range(R2):
                    row = ((g * R1 + q1) * R2 + b) * 16
                    z.append((g_s[zr, pl.ds(row, 8), :], g_s[zr, pl.ds(row + 8, 8), :]))
                t = _fft(z)
                for q2 in range(R2):
                    q = q1 + R1 * q2
                    dst[zw, pl.ds(8 * g * SR + q, 8, stride=SR), :] = t[q2][0]
                    dst[zw, pl.ds(8 * g * SR + C + q, 8, stride=SR), :] = t[q2][1]

    def mac(p, zw, zr):
        re = pl.ds(p * 8, 8)
        im = pl.ds(C + p * 8, 8)
        AB = 4
        prev = None
        for a0 in range(0, NCH, AB):
            zre = [None] * AB
            zim = [None] * AB
            for m in range(a0 + AB):
                hr = h_s[zr, pl.ds(m * SR + p * 8, 8), :]
                hi = h_s[zr, pl.ds(m * SR + C + p * 8, 8), :]
                for i in range(AB):
                    t = a0 + i - m
                    if t < 0:
                        continue
                    ur = u_s[zr, pl.ds(t * SR + p * 8, 8), :]
                    ui = u_s[zr, pl.ds(t * SR + C + p * 8, 8), :]
                    tr = hr * ur - hi * ui
                    ti = hr * ui + hi * ur
                    zre[i] = tr if zre[i] is None else zre[i] + tr
                    zim[i] = ti if zim[i] is None else zim[i] + ti
            for i in range(AB):
                if prev is None:
                    yf_s[zw, a0 + i, re, :] = zre[i]
                    yf_s[zw, a0 + i, im, :] = zim[i]
                else:
                    yf_s[zw, a0 + i, re, :] = zre[i] - prev[1]
                    yf_s[zw, a0 + i, im, :] = zim[i] + prev[0]
                prev = (zre[i], zim[i])

    def inv_dft(c, zr):
        hc = C // 2
        for a in range(NCH):
            yr, yrm = yf_s[zr, a, 0:hc, :], yf_s[zr, a, hc:C, :]
            yi, yim = yf_s[zr, a, C:C + hc, :], yf_s[zr, a, C + hc:, :]
            fe = jnp.concatenate([yr + yrm, yi + yim], axis=0).astype(BF16)
            fo = jnp.concatenate([yr - yrm, yi - yim], axis=0).astype(BF16)
            y_v[c, pl.ds(a * C, hc, stride=2), :] = _dot(inv_ref[0:hc, :], fe)
            y_v[c, pl.ds(a * C + 1, hc, stride=2), :] = _dot(inv_ref[hc:, :], fo)

    def fixup(e, c, mat):
        a = wbuf[e][mat, c, 0]
        b = wbuf[e][mat, c, 1]
        wbuf[e][mat, c, 0] = (a & U32(0xFFFF)) | (b << 16)
        wbuf[e][mat, c, 1] = (a >> 16) | (b & U32(0xFFFF0000))

    RB = 128

    def qkv_tile(e, c, n, rs=range(PRO // RB)):
        mat, j = n // 2, n % 2
        for r in rs:
            w = _unpack(wbuf[e][mat, c, j])
            xr = _unpack(xp[pl.ds(r * RB // 2, RB // 2), :])
            qkv_b[mat, 2 * c + e, j, pl.ds((QOFF + r * RB) // 2, RB // 2), :] = _pack(_dot(xr, w))

    for cp in wq0_copies(0) + [xp_copy]:
        cp.start()
    zs[0] = 0
    zs[1] = 0
    xp_copy.wait()
    for cp in wq0_copies(1) + wq0_copies(2) + small_copies + block_piece(0, 2):
        cp.start()

    def start_when(cond, copies):
        @pl.when(cond)
        def _():
            for cp in copies:
                cp.start()

    def pro0(c, carry):
        for i in range(2):
            start_when(c == 1 + i, block_piece(0, i))
        for cp in wq0_copies(c):
            cp.wait()
        fixup(0, c, 0)
        qkv_tile(0, c, 0)
        qkv_tile(0, c, 1)
        start_when(c + 3 < NB, wq0_copies(jnp.minimum(c + 3, NB - 1)))
        for i in range(3, NPIECE):
            start_when(c == min(i - 1, NB - 3), block_piece(0, i))
        return carry

    with jax.named_scope("pro0"):
        jax.lax.fori_loop(0, NB, pro0, 0)
    for i in range(2, NPIECE):
        for cp in block_piece(1, i):
            cp.start()
    for cp in small_copies:
        cp.wait()

    zw = zs[0]
    zr = zs[1]

    def pro(c, carry):
        for i in range(2):
            start_when(c + 1 < NB, block_piece(jnp.minimum(c + 1, NB - 1), i))
        for i in range(NPIECE):
            for cp in block_piece(c, i):
                cp.wait()

        tiles = [(0, n) for n in range(2, 6)] + [(1, n) for n in range(6)]

        def tile(i):
            e, n = tiles[i]
            if n % 2 == 0:
                fixup(e, c, n // 2)
            qkv_tile(e, c, n)

        fwd_h(c, zw)
        kv_prep(c, zw)
        tile(0)
        fft1(zw, zr)
        fft2(u_s, zw, zr)
        for i in range(1, 9):
            for p in range(2 * i - 2, 2 * i):
                mac(p, zw, zr)
            tile(i)
        qkv_tile(1, c, 5, range(0, 3))
        inv_dft(c, zr)
        qkv_tile(1, c, 5, range(3, 4))
        for i in range(2, NPIECE):
            start_when(c + 2 < NB, block_piece(jnp.minimum(c + 2, NB - 1), i))
        start_when(c + 1 < NB, rest_copies(c))
        start_when(c + 2 == NB, rest_copies(NB - 1))
        return carry

    with jax.named_scope("pro"):
        jax.lax.fori_loop(0, NB, pro, 0)
    for c in range(NB):
        for cp in rest_copies(c):
            cp.wait()

    gwt = gw_ref[...].astype(F32)
    gw = jnp.concatenate([gwt[j:j + 1, :] for j in range(NB)], axis=1)

    def finalize(rows, b):
        xr = x_v[rows, :].astype(F32)
        g = jax.nn.sigmoid(jnp.sum(xr * gw, axis=-1, keepdims=True))
        a = xr * jnp.concatenate([y_v[j, rows, :] for j in range(NB)], axis=1)
        out_v[rows, :] = (g * a + (1.0 - g) * b).astype(BF16)

    def step(s, mem, split_first, odd):
        xrows = slice(M, M + RX) if odd else slice(0, RX)
        mrows = slice(0, M) if odd else slice(RX, RX + M)
        sh = 4 if odd else 0
        xo = pl.multiple_of(PRO + RX * s, 8)
        wbase = pl.multiple_of((RX // 2 * s) % (QCAP // 2) - sh, 8)
        rpos = pl.multiple_of((SEG // 2 * s + QOFF // 2) % (QCAP // 2), SEG // 2)
        opos = pl.multiple_of(SEG // 2 * s, SEG // 2)
        fbase = pl.multiple_of(RX // 2 * s - sh, 8)
        xs = x_v[pl.ds(xo, RX), :]
        lhs = jnp.concatenate([mem, xs] if odd else [xs, mem], axis=0)
        zpad = jnp.zeros((128 - 2 * (SEG + M), E), BF16)
        frows = pl.ds(pl.multiple_of(RX * s, 8), RX)
        low = jax.lax.broadcasted_iota(jnp.int32, (8, E), 0) < 4
        NP = H // 2

        mem_qkv = {}
        probs = {}
        cats = {}

        def load(mat, hp):
            parts = [_unpack(qkv_b[mat, hp, 0, pl.ds(rpos, SEG // 2), :]),
                     _unpack(qkv_b[mat, hp, 1, pl.ds(rpos, SEG // 2), :]), mem_qkv[(hp, mat)]]
            if mat > 0:
                parts.append(zpad)
            cats[(mat, hp)] = jnp.concatenate(parts, axis=0)

        def stage_a(hp):
            KH = D // 2
            split = split_first and hp == 0
            if split:
                for mat in range(3):
                    for j in range(2):
                        w = _unpack(wbuf[hp % 2][mat, hp // 2, j, :KH // 2, :])
                        qacc[2 * mat + j] = _dot(lhs[:, :KH], w)
            for mi, mat in enumerate(MAT_ORDER):
                mm = []
                for j in range(2):
                    if split:
                        w = _unpack(wbuf[hp % 2][mat, hp // 2, j, KH // 2:, :])
                        res = qacc[2 * mat + j] + _dot(lhs[:, KH:], w)
                    else:
                        res = _dot(lhs, _unpack(wbuf[hp % 2][mat, hp // 2, j]))
                    pk = _pack(res)
                    if odd:
                        qkv_b[mat, hp, j, pl.ds(wbase + 4, 4), :] = pk[4:8]
                        qkv_b[mat, hp, j, pl.ds(wbase + 8, 8), :] = pk[8:16]
                    else:
                        qkv_b[mat, hp, j, pl.ds(wbase, 8), :] = pk[0:8]
                        qkv_b[mat, hp, j, pl.ds(wbase + 8, 4), :] = pk[8:12]
                    mm.append(res[mrows])
                    if j == 1:
                        mem_qkv[(hp, mat)] = jnp.concatenate(mm, axis=0).astype(BF16)
                    advance(6 * hp + 2 * mi + j + 1)

        def stage_b(hp):
            sc = _dot_nt(cats[(0, hp)], cats[(1, hp)]) * scale
            fill = fill_ref[...]
            sc = jnp.where(fill == 0.0, sc, fill)
            mx = jnp.max(sc, axis=-1, keepdims=True)
            p = jnp.exp(sc - mx)
            l = jnp.sum(p, axis=-1, keepdims=True)
            r = pl.reciprocal(l, approx=True)
            r = r * (2.0 - l * r)
            probs[hp] = (p * r).astype(BF16)

        def stage_c(hp):
            o = _dot(probs[hp], cats[(2, hp)])
            for j in range(2):
                h = 2 * hp + j
                cols = slice(h * E, (h + 1) * E)
                o_b[pl.ds(opos, SEG // 2), cols] = _pack(o[j * SEG:(j + 1) * SEG])
                om = o[2 * SEG + j * M:2 * SEG + (j + 1) * M]
                om = _pack(jnp.concatenate([om, om], axis=0))
                w0 = o_b[pl.ds(fbase, 8), cols]
                w1 = o_b[pl.ds(fbase + 8, 8), cols]
                lo_s[0:8, cols] = jnp.where(low, om, w0) if odd else w0
                lo_s[8:16, cols] = w1 if odd else jnp.where(low, w1, om)

        def oproj(j, late):
            ks = slice(HS * E, H * E) if late else slice(0, HS * E)
            kw = slice(ks.start // 2, ks.stop // 2)
            return _dot(_unpack(lo_s[:, ks]), _unpack(wo_v[j, kw, :]))

        events = []
        for hp in range(NP):
            events.append((6 * hp + OFF_LQK, 0, functools.partial(load, 0, hp)))
            events.append((6 * hp + OFF_LQK, 1, functools.partial(load, 1, hp)))
            events.append((6 * hp + OFF_LV, 2, functools.partial(load, 2, hp)))
            events.append((6 * hp + OFF_PV, 3, functools.partial(stage_c, hp)))
            events.append((6 * hp + OFF_S, 4, functools.partial(stage_b, hp)))
        events.sort(key=lambda ev: ev[:2])

        def advance(slot):
            while events and events[0][0] <= slot:
                events.pop(0)[2]()

        outs = [None] * NB
        for hp in range(NP):
            stage_a(hp)
        for j in range(NB):
            oacc[:, j * 128:(j + 1) * 128] = oproj(j, False)
            advance(6 * NP + (j + 1) * HS // 8)
        assert not events
        for j in range(NB):
            outs[j] = oacc[:, j * 128:(j + 1) * 128] + oproj(j, True)
        res = jnp.concatenate(outs, axis=1)
        finalize(frows, res[xrows])
        return res[mrows].astype(BF16)

    def steps(i, carry):
        mem = mem_v[...]
        for u in range(UNROLL):
            mem = step(i * UNROLL + u, mem, u > 0, u % 2 == 1)
        mem_v[...] = mem
        return carry

    with jax.named_scope("main"):
        jax.lax.fori_loop(0, NSEG // UNROLL, steps, 0)

    def epi_rows(r0, n):
        lo = _unpack(o_b[pl.ds(pl.multiple_of(r0 // 2, 8), n // 2), :])
        outs = [_dot(lo, _unpack(wo_v[j])) for j in range(NB)]
        finalize(pl.ds(r0, n), jnp.concatenate(outs, axis=1))

    EB = 128

    def epi(r, carry):
        r0 = pl.multiple_of(S - PRO + r * EB, EB)

        @pl.when(r == PRO // EB - 1)
        def _():
            out_copy(S - PRO, PRO - EB).start()

        epi_rows(r0, EB)
        return carry

    with jax.named_scope("epi"):
        out_copy(0, S - PRO).start()
        jax.lax.fori_loop(0, PRO // EB, epi, 0)
    out_copy(S - EB, EB).start()
    out_copy(0, S).wait()


@jax.jit
def _run(A_q, A_k, A_v, A_shift_k, A_ssm_k, A_ssm_D, B_mem0, B_Wq, B_Wk, B_Wv, B_Wo, gate_w):
    fwd, inv = _dft_tables()
    any_spec = pl.BlockSpec(memory_space=pl.ANY)
    out = pl.pallas_call(
        _kernel,
        out_shape=jax.ShapeDtypeStruct((S, D), BF16),
        in_specs=[any_spec] * 15,
        out_specs=any_spec,
        scratch_shapes=[
            pltpu.VMEM((S, D), BF16),
            pltpu.VMEM((PRO // 2, D), U32),
            pltpu.VMEM((NB, NCH, PR, 128), U32),
            pltpu.VMEM((NB, NCH, PR, 128), U32),
            pltpu.VMEM((NB, 128, S), BF16),
            pltpu.VMEM((3, H // 4, 2, D // 2, E), U32),
            pltpu.VMEM((3, H // 4, 2, D // 2, E), U32),
            pltpu.VMEM((NB, H * E // 2, 128), U32),
            pltpu.VMEM((NB, S, 128), F32),
            pltpu.VMEM((3, H // 2, 2, QCAP // 2, E), U32),
            pltpu.VMEM((S // 2, H * E), U32),
            pltpu.VMEM(((M + RX) // 2, H * E), U32),
            pltpu.VMEM((M, D), BF16),
            pltpu.VMEM((M + RX, D), F32),
            pltpu.VMEM((6, M + RX, E), F32),
            pltpu.VMEM((1, NCH * SR, 128), F32),
            pltpu.VMEM((1, NCH * SR, 128), F32),
            pltpu.VMEM((1, NCH, 2 * C, 128), F32),
            pltpu.VMEM((1, S, 128), F32),
            pltpu.VMEM((1, 2 * S, 128), F32),
            pltpu.VMEM((S, D), BF16),
            pltpu.VMEM((2 * C, C), BF16),
            pltpu.VMEM((C, C), BF16),
            pltpu.VMEM((2 * (SEG + M), 128), F32),
            pltpu.VMEM((KS, D), BF16),
            pltpu.VMEM((NB, 128), BF16),
            pltpu.VMEM((NB, 128), BF16),
            pltpu.SMEM((2,), jnp.int32),
            pltpu.SemaphoreType.DMA((6,)),
            pltpu.SemaphoreType.DMA((NB,)),
        ],
        compiler_params=pltpu.CompilerParams(vmem_limit_bytes=120 * 2 ** 20, disable_bounds_checks=True),
    )(
        A_q.reshape(S, D), A_k.reshape(NCH, C, D), A_v.reshape(NCH, C, D), A_ssm_k,
        B_Wq.reshape(D // 2, 2, H, E), B_Wk.reshape(D // 2, 2, H, E), B_Wv.reshape(D // 2, 2, H, E),
        B_Wo.reshape(H * E, D),
        A_shift_k.T, A_ssm_D.reshape(NB, 128), gate_w.reshape(NB, 128), B_mem0.reshape(M, D),
        jnp.asarray(fwd, BF16), jnp.asarray(inv, BF16), jnp.asarray(_attn_fill()),
    )
    return out.reshape(1, S, D)


def pallas_gated_mix__ssm_conv_h3__memory_aug_recurrent_mem_tr__prompt_kernel(
    A_q, A_k, A_v, A_shift_k, A_ssm_k, A_ssm_D, B_x, B_mem0, B_Wq, B_Wk, B_Wv, B_Wo, B_seg_len, gate_w,
):
    del B_x
    if isinstance(B_seg_len, int):
        assert B_seg_len == SEG
    return _run(A_q, A_k, A_v, A_shift_k, A_ssm_k, A_ssm_D, B_mem0, B_Wq, B_Wk, B_Wv, B_Wo, gate_w)
```

```python
import cmath
import functools
import math

import jax
import jax.numpy as jnp
import numpy as np
import jax.experimental.pallas as pl
import jax.experimental.pallas.tpu as pltpu

F32 = jnp.float32
BF16 = jnp.bfloat16
U32 = jnp.uint32

S = 2048
D = 1024
H = 32
E = 128
M = 8
SEG = 32
NSEG = S // SEG
RX = 24
PRO = S - RX * NSEG
QCAP = 576
QOFF = QCAP - PRO
HL = 4
HS = H - HL
MAT_ORDER = (0, 1, 2)
OFF_LQK, OFF_S, OFF_LV, OFF_PV = 4, 8, 14, 17
UNROLL = 4
XE = 768
C = 256
NCH = S // C
NB = D // 128
KS = 4
NEG = -1000000000.0
R1, R2 = 16, 16
PR = C // 2 + 8
FOLD = 4
SR = 2 * C + 4


def _inv_table():
    n = np.arange(C, dtype=np.float64)
    th = 2.0 * np.pi * (np.arange(C // FOLD, dtype=np.float64) + 0.25) / C
    no = np.concatenate([n[r::FOLD] for r in range(FOLD)])
    inv = np.concatenate([np.cos(no[:, None] * th[None, :]), -np.sin(no[:, None] * th[None, :])], axis=1) / C
    return inv.astype(np.float32)


def _attn_fill():
    n = 2 * (SEG + M)
    head = np.array([0] * SEG + [1] * SEG + [0] * M + [1] * M)
    pos = np.concatenate([M + np.arange(SEG), M + np.arange(SEG), np.arange(M), np.arange(M)])
    fill = np.full((n, 128), -np.inf, np.float32)
    for i in range(n):
        for j in range(n):
            if head[i] == head[j]:
                ok = pos[i] < M or pos[i] >= pos[j]
                fill[i, j] = 0.0 if ok else NEG
    return fill


def _add(a, b):
    return b if a is None else a if b is None else a + b


def _sub(a, b):
    return a if b is None else -b if a is None else a - b


def _cmul(z, w):
    r, i = z
    wr, wi = w.real, w.imag
    eps = 1e-12
    if abs(wi) < eps and abs(wr - 1.0) < eps:
        return z
    if i is None:
        if abs(abs(wr) - abs(wi)) < eps and wr * wi > 0:
            t = r * wr
            return t, t
        return r * wr, r * wi
    if abs(abs(wr) - abs(wi)) < eps:
        if wr * wi > 0:
            return (r - i) * wr, (r + i) * wr
        return (r + i) * wr, (i - r) * wr
    return r * wr - i * wi, r * wi + i * wr


def _fft(xs):
    n = len(xs)
    if n == 1:
        return xs
    if n == 2:
        (ar, ai), (br, bi) = xs
        return [(_add(ar, br), _add(ai, bi)), (_sub(ar, br), _sub(ai, bi))]
    e = _fft(xs[0::2])
    o1 = _fft(xs[1::4])
    o3 = _fft(xs[3::4])
    out = [None] * n
    for k in range(n // 4):
        ar, ai = _cmul(o1[k], cmath.exp(-2j * math.pi * k / n))
        br, bi = _cmul(o3[k], cmath.exp(-6j * math.pi * k / n))
        sr, si, dr, di = _add(ar, br), _add(ai, bi), _sub(ar, br), _sub(ai, bi)
        er, ei = e[k]
        fr, fi = e[k + n // 4]
        out[k] = (_add(er, sr), _add(ei, si))
        out[k + n // 2] = (_sub(er, sr), _sub(ei, si))
        out[k + n // 4] = (_add(fr, di), _sub(fi, dr))
        out[k + 3 * n // 4] = (_sub(fr, di), _add(fi, dr))
    return out


def _dot(a, b):
    return jnp.dot(a, b, preferred_element_type=F32)


def _dot_nt(a, b):
    return jax.lax.dot_general(a, b, (((1,), (1,)), ((), ())), preferred_element_type=F32)


def _pack(a):
    return pltpu.bitcast(a.astype(BF16), U32)


def _unpack(a):
    return pltpu.bitcast(a, BF16)


def _kernel(x_hbm, k_hbm, v_hbm, h_hbm, wq_hbm, wk_hbm, wv_hbm, wo_hbm,
            sk_hbm, dd_hbm, gw_hbm, mem0_hbm, inv_hbm, fill_hbm,
            out_hbm,
            x_v, xp, k_v, v_v, h_v, w_even, w_odd, wo_v, y_v, qkv_b, o_b, lo_s, mem_v, oacc, qacc,
            u_s, h_s, yf_s, t_s, gu_s, gh_s, ht_s,
            out_v, inv_ref, fill_ref, sk_ref, dd_ref, gw_ref, zs, sems, qsems):
    scale = E ** (-0.5)
    wbuf = (w_even, w_odd)

    w32 = [w.bitcast(U32) for w in (wq_hbm, wk_hbm, wv_hbm)]
    wo32 = wo_hbm.bitcast(U32)
    x32 = x_hbm.bitcast(U32)
    k32 = k_hbm.bitcast(U32)
    v32 = v_hbm.bitcast(U32)

    def lanes(c):
        return pl.ds(pl.multiple_of(c * 128, 128), 128)

    def w_copies(c, e, mat, sem):
        return [pltpu.make_async_copy(w32[mat].at[:, par, 2 * c + e, :], wbuf[e].at[mat, c, par], sem)
                for par in range(2)]

    def wq0_copies(c):
        return w_copies(c, 0, 0, qsems.at[c])

    W_REST = [(e, mat) for e in range(2) for mat in range(3) if (e, mat) != (0, 0)]
    NPIECE = 3 + len(W_REST)

    def block_piece(c, i):
        sem = sems.at[c % 2]
        if i < 2:
            src, dst = ((k32, k_v), (v32, v_v))[i]
            return [pltpu.make_async_copy(src.at[:, :, lanes(c)], dst.at[c, :, pl.ds(0, C // 2), :], sem)]
        if i == 2:
            return [pltpu.make_async_copy(h_hbm.at[lanes(c), :], h_v.at[c, pl.ds(0, 128), :], sem)]
        return w_copies(c, *W_REST[i - 3], sem)

    def wo_copy(c):
        return pltpu.make_async_copy(wo32.at[:, lanes(c)], wo_v.at[c], sems.at[2])

    x_early = pltpu.make_async_copy(x_hbm.at[pl.ds(0, XE), :], x_v.at[pl.ds(0, XE), :], sems.at[2])
    x_late = pltpu.make_async_copy(x_hbm.at[pl.ds(XE, S - XE), :], x_v.at[pl.ds(XE, S - XE), :], sems.at[3])

    xp_copy = pltpu.make_async_copy(x32.at[pl.ds(0, PRO // 2), :], xp, sems.at[3])
    small_copies = [pltpu.make_async_copy(src, dst, sems.at[4]) for src, dst in (
        (sk_hbm, sk_ref), (dd_hbm, dd_ref), (inv_hbm, inv_ref),
        (gw_hbm, gw_ref), (mem0_hbm, mem_v), (fill_hbm, fill_ref))]

    def out_copy(start, n):
        rows = pl.ds(start, n)
        return pltpu.make_async_copy(out_v.at[rows, :], out_hbm.at[rows, :], sems.at[5])

    def row_of(ref, c):
        t = ref[...].astype(F32)
        sel = jax.lax.broadcasted_iota(jnp.int32, (NB, 128), 0) == c
        return jnp.sum(jnp.where(sel, t, 0.0), axis=0, keepdims=True)

    k2 = k_v.reshape(NB, NCH * PR, 128)
    v2 = v_v.reshape(NB, NCH * PR, 128)

    def word(ref, c, pr):
        return ref[c, pl.ds(pr, NCH, stride=PR), :]

    def lo16(w):
        return pltpu.bitcast(w << 16, F32)

    def hi16(w):
        return pltpu.bitcast(w & U32(0xFFFF0000), F32)

    def pair(ref, c, pr):
        w = word(ref, c, pr)
        return lo16(w), hi16(w)

    first = jax.lax.broadcasted_iota(jnp.int32, (8, 128), 0) == 0

    def kv_prep(c, zw):
        skt = sk_ref[:, lanes(c)].astype(F32)
        sk = [jnp.broadcast_to(skt[j:j + 1, :], (8, 128)) for j in range(KS)]
        tail = (pair(k2, c, C // 2 - 2) + pair(k2, c, C // 2 - 1))[1:]
        win = [jnp.where(first, 0.0, pltpu.roll(t, 1, 0)) for t in tail]
        for pr in range(C // 2):
            ks = pair(k2, c, pr)
            vs = pair(v2, c, pr)
            for i in range(2):
                win.append(ks[i])
                acc = win[-1] * sk[0]
                for j in range(1, KS):
                    acc = acc + win[-1 - j] * sk[j]
                win = win[1:]
                t_s[zw, pl.ds((2 * pr + i) * 8, 8), :] = acc * vs[i]

    def h_prep(c, zw):
        for t in range(S // 128):
            ht = pltpu.bitcast(h_v[c, 0:128, pl.ds(t * 128, 128)].T, U32)
            ht_s[zw, pl.ds(t * 64 // (C // 2) * PR + t * 64 % (C // 2), 64), :] = ht

    def fft1(sample, mid, zw):
        for b in range(R2):
            z = [_cmul((sample(R2 * a + b), None), cmath.exp(-0.5j * math.pi * a / R1)) for a in range(R1)]
            gq = _fft(z)
            for q1 in range(R1):
                re, im = _cmul(gq[q1], cmath.exp(-2j * math.pi * (q1 + 0.25) * b / C))
                row = (q1 * R2 + b) * 16
                mid[zw, pl.ds(row, 8), :] = re
                mid[zw, pl.ds(row + 8, 8), :] = im

    def fft2(mid, dst, zw, zr):
        for q1 in range(R1):
            z = []
            for b in range(R2):
                row = (q1 * R2 + b) * 16
                z.append((mid[zr, pl.ds(row, 8), :], mid[zr, pl.ds(row + 8, 8), :]))
            t = _fft(z)
            for q2 in range(R2):
                q = q1 + R1 * q2
                dst[zw, pl.ds(q, NCH, stride=SR), :] = t[q2][0]
                dst[zw, pl.ds(C + q, NCH, stride=SR), :] = t[q2][1]

    def mac(p, zw, zr):
        re = pl.ds(p * 8, 8)
        im = pl.ds(C + p * 8, 8)
        AB = 4
        prev = None
        for a0 in range(0, NCH, AB):
            zre = [None] * AB
            zim = [None] * AB
            for m in range(a0 + AB):
                hr = h_s[zr, pl.ds(m * SR + p * 8, 8), :]
                hi = h_s[zr, pl.ds(m * SR + C + p * 8, 8), :]
                for i in range(AB):
                    t = a0 + i - m
                    if t < 0:
                        continue
                    ur = u_s[zr, pl.ds(t * SR + p * 8, 8), :]
                    ui = u_s[zr, pl.ds(t * SR + C + p * 8, 8), :]
                    tr = hr * ur - hi * ui
                    ti = hr * ui + hi * ur
                    zre[i] = tr if zre[i] is None else zre[i] + tr
                    zim[i] = ti if zim[i] is None else zim[i] + ti
            for i in range(AB):
                if prev is None:
                    yf_s[zw, a0 + i, re, :] = zre[i]
                    yf_s[zw, a0 + i, im, :] = zim[i]
                else:
                    yf_s[zw, a0 + i, re, :] = zre[i] - prev[1]
                    yf_s[zw, a0 + i, im, :] = zim[i] + prev[0]
                prev = (zre[i], zim[i])

    def inv_dft(c, zr, chunks, hook=None):
        qc = C // FOLD
        for a in chunks:
            yr = [yf_s[zr, a, j * qc:(j + 1) * qc, :] for j in range(FOLD)]
            yi = [yf_s[zr, a, C + j * qc:C + (j + 1) * qc, :] for j in range(FOLD)]
            sr, si, dr, di = yr[0] + yr[2], yi[0] + yi[2], yr[0] - yr[2], yi[0] - yi[2]
            tr, ti, er, ei = yr[1] + yr[3], yi[1] + yi[3], yr[1] - yr[3], yi[1] - yi[3]
            folded = [(sr + tr, si + ti), (dr - ei, di + er), (sr - tr, si - ti), (dr + ei, di - er)]
            for r in range(FOLD):
                f = jnp.concatenate(folded[r], axis=0).astype(BF16)
                y = _dot(inv_ref[r * qc:(r + 1) * qc, :], f)
                y_v[c, pl.ds(a * C + r, qc, stride=FOLD), :] = y
                if hook is not None and (a, r) == (chunks[0], 0):
                    hook(pltpu.bitcast(y[0:8], U32))

    def fixup(e, c, mat):
        a = wbuf[e][mat, c, 0]
        b = wbuf[e][mat, c, 1]
        wbuf[e][mat, c, 0] = (a & U32(0xFFFF)) | (b << 16)
        wbuf[e][mat, c, 1] = (a >> 16) | (b & U32(0xFFFF0000))

    RB = 128

    def qkv_tile(e, c, n, rs=range(PRO // RB), hook=None):
        mat, j = n // 2, n % 2
        for r in rs:
            w = _unpack(wbuf[e][mat, c, j])
            xr = _unpack(xp[pl.ds(r * RB // 2, RB // 2), :])
            pk = _pack(_dot(xr, w))
            qkv_b[mat, 2 * c + e, j, pl.ds((QOFF + r * RB) // 2, RB // 2), :] = pk
            if hook is not None and r == 0:
                hook(pk[0:8])

    for cp in wq0_copies(0) + [xp_copy]:
        cp.start()
    zs[0] = 0
    zs[1] = 0
    xp_copy.wait()
    for cp in wq0_copies(1) + wq0_copies(2) + small_copies + block_piece(0, 2):
        cp.start()

    def start_when(cond, copies):
        @pl.when(cond)
        def _():
            for cp in copies:
                cp.start()

    def pro0(c, carry):
        for i in range(2):
            start_when(c == 1 + i, block_piece(0, i))
        for cp in wq0_copies(c):
            cp.wait()
        fixup(0, c, 0)
        qkv_tile(0, c, 0)
        qkv_tile(0, c, 1)
        start_when(c + 3 < NB, wq0_copies(jnp.minimum(c + 3, NB - 1)))
        for i in range(3, NPIECE):
            start_when(c == min(i - 1, NB - 3), block_piece(0, i))
        return carry

    with jax.named_scope("pro0"):
        jax.lax.fori_loop(0, NB, pro0, 0)
    for i in range(2, NPIECE):
        for cp in block_piece(1, i):
            cp.start()
    for cp in small_copies:
        cp.wait()

    zw = zs[0]
    zr = zs[1]

    def pro(c, carry):
        for i in range(2):
            start_when(c + 1 < NB, block_piece(jnp.minimum(c + 1, NB - 1), i))
        for i in range(NPIECE):
            for cp in block_piece(c, i):
                cp.wait()

        tiles = [(0, n) for n in range(2, 6)] + [(1, n) for n in range(6)]

        def tile(i, hook=None):
            e, n = tiles[i]
            if n % 2 == 0:
                fixup(e, c, n // 2)
            qkv_tile(e, c, n, hook=hook)

        def trigger(val):
            k2[c + zw, pl.ds(C // 2, 8), :] = val
            v2[c + zw, pl.ds(C // 2, 8), :] = val
            h_v[c + zw, pl.ds(128, 16), 0:128] = _unpack(val)

        def h_sample(n):
            w = word(ht_s, zr, n // 2)
            hv = hi16(w) if n % 2 else lo16(w)
            if n == 0:
                hv = hv + jnp.where(first, row_of(dd_ref, c), 0.0)
            return hv

        tile(0, trigger)
        h_prep(c, zw)
        kv_prep(c, zw)
        fft1(lambda n: t_s[zr, pl.ds(n * 8, 8), :], gu_s, zw)
        fft2(gu_s, u_s, zw, zr)
        fft1(h_sample, gh_s, zw)
        fft2(gh_s, h_s, zw, zr)
        for i in range(1, 9):
            for p in range(4 * i - 4, 4 * i):
                mac(p, zw, zr)
            tile(i)
        tile(9)
        inv_dft(c, zr, range(NCH))
        for i in range(2, NPIECE):
            start_when(c + 2 < NB, block_piece(jnp.minimum(c + 2, NB - 1), i))
        start_when(c + 1 < NB, [wo_copy(c)])
        start_when(c + 2 == NB, [wo_copy(NB - 1), x_early])
        return carry

    with jax.named_scope("pro"):
        jax.lax.fori_loop(0, NB, pro, 0)
    x_late.start()
    x_early.wait()
    for c in range(NB):
        wo_copy(c).wait()

    gwt = gw_ref[...].astype(F32)
    gw = jnp.concatenate([gwt[j:j + 1, :] for j in range(NB)], axis=1)

    def finalize(rows, b):
        xr = x_v[rows, :].astype(F32)
        g = jax.nn.sigmoid(jnp.sum(xr * gw, axis=-1, keepdims=True))
        a = xr * jnp.concatenate([y_v[j, rows, :] for j in range(NB)], axis=1)
        out_v[rows, :] = (g * a + (1.0 - g) * b).astype(BF16)

    def step(s, mem, split_first, odd):
        xrows = slice(M, M + RX) if odd else slice(0, RX)
        mrows = slice(0, M) if odd else slice(RX, RX + M)
        sh = 4 if odd else 0
        xo = pl.multiple_of(PRO + RX * s, 8)
        wbase = pl.multiple_of((RX // 2 * s) % (QCAP // 2) - sh, 8)
        rpos = pl.multiple_of((SEG // 2 * s + QOFF // 2) % (QCAP // 2), SEG // 2)
        opos = pl.multiple_of(SEG // 2 * s, SEG // 2)
        fbase = pl.multiple_of(RX // 2 * s - sh, 8)
        xs = x_v[pl.ds(xo, RX), :]
        lhs = jnp.concatenate([mem, xs] if odd else [xs, mem], axis=0)
        zpad = jnp.zeros((128 - 2 * (SEG + M), E), BF16)
        frows = pl.ds(pl.multiple_of(RX * s, 8), RX)
        low = jax.lax.broadcasted_iota(jnp.int32, (8, E), 0) < 4
        NP = H // 2

        mem_qkv = {}
        probs = {}
        cats = {}

        def load(mat, hp):
            parts = [_unpack(qkv_b[mat, hp, 0, pl.ds(rpos, SEG // 2), :]),
                     _unpack(qkv_b[mat, hp, 1, pl.ds(rpos, SEG // 2), :]), mem_qkv[(hp, mat)]]
            if mat > 0:
                parts.append(zpad)
            cats[(mat, hp)] = jnp.concatenate(parts, axis=0)

        def stage_a(hp):
            KH = D // 2
            split = split_first and hp == 0
            if split:
                for mat in range(3):
                    for j in range(2):
                        w = _unpack(wbuf[hp % 2][mat, hp // 2, j, :KH // 2, :])
                        qacc[2 * mat + j] = _dot(lhs[:, :KH], w)
            for mi, mat in enumerate(MAT_ORDER):
                mm = []
                for j in range(2):
                    if split:
                        w = _unpack(wbuf[hp % 2][mat, hp // 2, j, KH // 2:, :])
                        res = qacc[2 * mat + j] + _dot(lhs[:, KH:], w)
                    else:
                        res = _dot(lhs, _unpack(wbuf[hp % 2][mat, hp // 2, j]))
                    pk = _pack(res)
                    if odd:
                        qkv_b[mat, hp, j, pl.ds(wbase + 4, 4), :] = pk[4:8]
                        qkv_b[mat, hp, j, pl.ds(wbase + 8, 8), :] = pk[8:16]
                    else:
                        qkv_b[mat, hp, j, pl.ds(wbase, 8), :] = pk[0:8]
                        qkv_b[mat, hp, j, pl.ds(wbase + 8, 4), :] = pk[8:12]
                    mm.append(res[mrows])
                    if j == 1:
                        mem_qkv[(hp, mat)] = jnp.concatenate(mm, axis=0).astype(BF16)
                    advance(6 * hp + 2 * mi + j + 1)

        def stage_b(hp):
            sc = _dot_nt(cats[(0, hp)], cats[(1, hp)]) * scale
            fill = fill_ref[...]
            sc = jnp.where(fill == 0.0, sc, fill)
            mx = jnp.max(sc, axis=-1, keepdims=True)
            p = jnp.exp(sc - mx)
            l = jnp.sum(p, axis=-1, keepdims=True)
            r = pl.reciprocal(l, approx=True)
            r = r * (2.0 - l * r)
            probs[hp] = (p * r).astype(BF16)

        def stage_c(hp):
            o = _dot(probs[hp], cats[(2, hp)])
            for j in range(2):
                h = 2 * hp + j
                cols = slice(h * E, (h + 1) * E)
                o_b[pl.ds(opos, SEG // 2), cols] = _pack(o[j * SEG:(j + 1) * SEG])
                om = o[2 * SEG + j * M:2 * SEG + (j + 1) * M]
                om = _pack(jnp.concatenate([om, om], axis=0))
                w0 = o_b[pl.ds(fbase, 8), cols]
                w1 = o_b[pl.ds(fbase + 8, 8), cols]
                lo_s[0:8, cols] = jnp.where(low, om, w0) if odd else w0
                lo_s[8:16, cols] = w1 if odd else jnp.where(low, w1, om)

        def oproj(j, late):
            ks = slice(HS * E, H * E) if late else slice(0, HS * E)
            kw = slice(ks.start // 2, ks.stop // 2)
            return _dot(_unpack(lo_s[:, ks]), _unpack(wo_v[j, kw, :]))

        events = []
        for hp in range(NP):
            events.append((6 * hp + OFF_LQK, 0, functools.partial(load, 0, hp)))
            events.append((6 * hp + OFF_LQK, 1, functools.partial(load, 1, hp)))
            events.append((6 * hp + OFF_LV, 2, functools.partial(load, 2, hp)))
            events.append((6 * hp + OFF_PV, 3, functools.partial(stage_c, hp)))
            events.append((6 * hp + OFF_S, 4, functools.partial(stage_b, hp)))
        events.sort(key=lambda ev: ev[:2])

        def advance(slot):
            while events and events[0][0] <= slot:
                events.pop(0)[2]()

        outs = [None] * NB
        for hp in range(NP):
            stage_a(hp)
        for j in range(NB):
            oacc[:, j * 128:(j + 1) * 128] = oproj(j, False)
            advance(6 * NP + (j + 1) * HS // 8)
        assert not events
        for j in range(NB):
            outs[j] = oacc[:, j * 128:(j + 1) * 128] + oproj(j, True)
        res = jnp.concatenate(outs, axis=1)
        finalize(frows, res[xrows])
        return res[mrows].astype(BF16)

    def steps(i, carry):
        @pl.when(i == (XE - PRO) // (RX * UNROLL))
        def _():
            x_late.wait()

        mem = mem_v[...]
        for u in range(UNROLL):
            mem = step(i * UNROLL + u, mem, u > 0, u % 2 == 1)
        mem_v[...] = mem
        return carry

    with jax.named_scope("main"):
        jax.lax.fori_loop(0, NSEG // UNROLL, steps, 0)

    def epi_rows(r0, n):
        lo = _unpack(o_b[pl.ds(pl.multiple_of(r0 // 2, 8), n // 2), :])
        outs = [_dot(lo, _unpack(wo_v[j])) for j in range(NB)]
        finalize(pl.ds(r0, n), jnp.concatenate(outs, axis=1))

    EB = 128

    def epi(r, carry):
        r0 = pl.multiple_of(S - PRO + r * EB, EB)

        @pl.when(r == PRO // EB - 1)
        def _():
            out_copy(S - PRO, PRO - EB).start()

        epi_rows(r0, EB)
        return carry

    with jax.named_scope("epi"):
        out_copy(0, S - PRO).start()
        jax.lax.fori_loop(0, PRO // EB, epi, 0)
    out_copy(S - EB, EB).start()
    out_copy(0, S).wait()


@jax.jit
def _run(A_q, A_k, A_v, A_shift_k, A_ssm_k, A_ssm_D, B_mem0, B_Wq, B_Wk, B_Wv, B_Wo, gate_w):
    any_spec = pl.BlockSpec(memory_space=pl.ANY)
    out = pl.pallas_call(
        _kernel,
        out_shape=jax.ShapeDtypeStruct((S, D), BF16),
        in_specs=[any_spec] * 14,
        out_specs=any_spec,
        scratch_shapes=[
            pltpu.VMEM((S, D), BF16),
            pltpu.VMEM((PRO // 2, D), U32),
            pltpu.VMEM((NB, NCH, PR, 128), U32),
            pltpu.VMEM((NB, NCH, PR, 128), U32),
            pltpu.VMEM((NB, 128 + 16, S), BF16),
            pltpu.VMEM((3, H // 4, 2, D // 2, E), U32),
            pltpu.VMEM((3, H // 4, 2, D // 2, E), U32),
            pltpu.VMEM((NB, H * E // 2, 128), U32),
            pltpu.VMEM((NB, S, 128), F32),
            pltpu.VMEM((3, H // 2, 2, QCAP // 2, E), U32),
            pltpu.VMEM((S // 2, H * E), U32),
            pltpu.VMEM(((M + RX) // 2, H * E), U32),
            pltpu.VMEM((M, D), BF16),
            pltpu.VMEM((M + RX, D), F32),
            pltpu.VMEM((6, M + RX, E), F32),
            pltpu.VMEM((1, NCH * SR, 128), F32),
            pltpu.VMEM((1, NCH * SR, 128), F32),
            pltpu.VMEM((1, NCH, 2 * C, 128), F32),
            pltpu.VMEM((1, S, 128), F32),
            pltpu.VMEM((1, 2 * S, 128), F32),
            pltpu.VMEM((1, 2 * S, 128), F32),
            pltpu.VMEM((1, NCH * PR, 128), U32),
            pltpu.VMEM((S, D), BF16),
            pltpu.VMEM((C, 2 * C // FOLD), BF16),
            pltpu.VMEM((2 * (SEG + M), 128), F32),
            pltpu.VMEM((KS, D), BF16),
            pltpu.VMEM((NB, 128), BF16),
            pltpu.VMEM((NB, 128), BF16),
            pltpu.SMEM((2,), jnp.int32),
            pltpu.SemaphoreType.DMA((6,)),
            pltpu.SemaphoreType.DMA((NB,)),
        ],
        compiler_params=pltpu.CompilerParams(vmem_limit_bytes=120 * 2 ** 20, disable_bounds_checks=True),
    )(
        A_q.reshape(S, D), A_k.reshape(NCH, C, D), A_v.reshape(NCH, C, D), A_ssm_k,
        B_Wq.reshape(D // 2, 2, H, E), B_Wk.reshape(D // 2, 2, H, E), B_Wv.reshape(D // 2, 2, H, E),
        B_Wo.reshape(H * E, D),
        A_shift_k.T, A_ssm_D.reshape(NB, 128), gate_w.reshape(NB, 128), B_mem0.reshape(M, D),
        jnp.asarray(_inv_table(), BF16), jnp.asarray(_attn_fill()),
    )
    return out.reshape(1, S, D)


def pallas_gated_mix__ssm_conv_h3__memory_aug_recurrent_mem_tr__prompt_kernel(
    A_q, A_k, A_v, A_shift_k, A_ssm_k, A_ssm_D, B_x, B_mem0, B_Wq, B_Wk, B_Wv, B_Wo, B_seg_len, gate_w,
):
    del B_x
    if isinstance(B_seg_len, int):
        assert B_seg_len == SEG
    return _run(A_q, A_k, A_v, A_shift_k, A_ssm_k, A_ssm_D, B_mem0, B_Wq, B_Wk, B_Wv, B_Wo, gate_w)
```

```python
import cmath
import functools
import math

import jax
import jax.numpy as jnp
import numpy as np
import jax.experimental.pallas as pl
import jax.experimental.pallas.tpu as pltpu

F32 = jnp.float32
BF16 = jnp.bfloat16
U32 = jnp.uint32

S = 2048
D = 1024
H = 32
E = 128
M = 8
SEG = 32
NSEG = S // SEG
RX = 24
PRO = S - RX * NSEG
QCAP = 576
QOFF = QCAP - PRO
HL = 4
HS = H - HL
OFF_LQK, OFF_S, OFF_LV, OFF_PV = 4, 8, 14, 17
UNROLL = 4
XE = 768
C = 256
NCH = S // C
NB = D // 128
KS = 4
NEG = -1000000000.0
R1, R2 = 16, 16
PR = C // 2 + 8
NCP = NCH + 4
FOLD = 4
SR = 2 * C + 4


def _inv_table():
    n = np.arange(C, dtype=np.float64)
    th = 2.0 * np.pi * (np.arange(C // FOLD, dtype=np.float64) + 0.25) / C
    no = np.concatenate([n[r::FOLD] for r in range(FOLD)])
    inv = np.concatenate([np.cos(no[:, None] * th[None, :]), -np.sin(no[:, None] * th[None, :])], axis=1) / C
    return inv.astype(np.float32)


def _attn_fill():
    n = 2 * (SEG + M)
    head = np.array([0] * SEG + [1] * SEG + [0] * M + [1] * M)
    pos = np.concatenate([M + np.arange(SEG), M + np.arange(SEG), np.arange(M), np.arange(M)])
    fill = np.full((n, 128), -np.inf, np.float32)
    for i in range(n):
        for j in range(n):
            if head[i] == head[j]:
                ok = pos[i] < M or pos[i] >= pos[j]
                fill[i, j] = 0.0 if ok else NEG
    return fill


def _add(a, b):
    return b if a is None else a if b is None else a + b


def _sub(a, b):
    return a if b is None else -b if a is None else a - b


def _cmul(z, w):
    r, i = z
    wr, wi = w.real, w.imag
    eps = 1e-12
    if abs(wi) < eps and abs(wr - 1.0) < eps:
        return z
    if i is None:
        if abs(abs(wr) - abs(wi)) < eps and wr * wi > 0:
            t = r * wr
            return t, t
        return r * wr, r * wi
    if abs(abs(wr) - abs(wi)) < eps:
        if wr * wi > 0:
            return (r - i) * wr, (r + i) * wr
        return (r + i) * wr, (i - r) * wr
    return r * wr - i * wi, r * wi + i * wr


def _fft(xs):
    n = len(xs)
    if n == 1:
        return xs
    if n == 2:
        (ar, ai), (br, bi) = xs
        return [(_add(ar, br), _add(ai, bi)), (_sub(ar, br), _sub(ai, bi))]
    e = _fft(xs[0::2])
    o1 = _fft(xs[1::4])
    o3 = _fft(xs[3::4])
    out = [None] * n
    for k in range(n // 4):
        ar, ai = _cmul(o1[k], cmath.exp(-2j * math.pi * k / n))
        br, bi = _cmul(o3[k], cmath.exp(-6j * math.pi * k / n))
        sr, si, dr, di = _add(ar, br), _add(ai, bi), _sub(ar, br), _sub(ai, bi)
        er, ei = e[k]
        fr, fi = e[k + n // 4]
        out[k] = (_add(er, sr), _add(ei, si))
        out[k + n // 2] = (_sub(er, sr), _sub(ei, si))
        out[k + n // 4] = (_add(fr, di), _sub(fi, dr))
        out[k + 3 * n // 4] = (_sub(fr, di), _add(fi, dr))
    return out


def _dot(a, b):
    return jnp.dot(a, b, preferred_element_type=F32)


def _dot_nt(a, b):
    return jax.lax.dot_general(a, b, (((1,), (1,)), ((), ())), preferred_element_type=F32)


def _pack(a):
    return pltpu.bitcast(a.astype(BF16), U32)


def _unpack(a):
    return pltpu.bitcast(a, BF16)


def _kernel(x_hbm, k_hbm, v_hbm, h_hbm, wq_hbm, wk_hbm, wv_hbm, wo_hbm,
            sk_hbm, dd_hbm, gw_hbm, mem0_hbm, inv_hbm, fill_hbm,
            out_hbm,
            x_v, xp, k_v, v_v, h_v, w_even, w_odd, wo_v, y_v, qkv_b, o_b, lo_s, mem_v, oacc, qacc,
            u_s, h_s, yf_s, t_s, gu_s, gh_s, ht_s,
            out_v, inv_ref, fill_ref, sk_ref, dd_ref, gw_ref, zs, sems, qsems):
    scale = E ** (-0.5)
    wbuf = (w_even, w_odd)

    w32 = [w.bitcast(U32) for w in (wq_hbm, wk_hbm, wv_hbm)]
    wo32 = wo_hbm.bitcast(U32)
    x32 = x_hbm.bitcast(U32)
    k32 = k_hbm.bitcast(U32)
    v32 = v_hbm.bitcast(U32)

    def lanes(c):
        return pl.ds(pl.multiple_of(c * 128, 128), 128)

    def w_copies(c, e, mat, sem):
        return [pltpu.make_async_copy(w32[mat].at[:, par, 2 * c + e, :], wbuf[e].at[mat, c, par], sem)
                for par in range(2)]

    def wq0_copies(c):
        return w_copies(c, 0, 0, qsems.at[c])

    W_REST = [(e, mat) for e in range(2) for mat in range(3) if (e, mat) != (0, 0)]
    NPIECE = 3 + len(W_REST)

    def block_piece(c, i):
        sem = sems.at[c % 2]
        if i < 2:
            src, dst = ((k32, k_v), (v32, v_v))[i]
            return [pltpu.make_async_copy(src.at[:, :, lanes(c)], dst.at[c, pl.ds(0, NCH), pl.ds(0, C // 2), :], sem)]
        if i == 2:
            return [pltpu.make_async_copy(h_hbm.at[lanes(c), :], h_v.at[c, pl.ds(0, 128), :], sem)]
        return w_copies(c, *W_REST[i - 3], sem)

    def wo_copy(c):
        return pltpu.make_async_copy(wo32.at[:, lanes(c)], wo_v.at[c], sems.at[2])

    x_early = pltpu.make_async_copy(x_hbm.at[pl.ds(0, XE), :], x_v.at[pl.ds(0, XE), :], sems.at[2])
    x_late = pltpu.make_async_copy(x_hbm.at[pl.ds(XE, S - XE), :], x_v.at[pl.ds(XE, S - XE), :], sems.at[3])

    xp_copy = pltpu.make_async_copy(x32.at[pl.ds(0, PRO // 2), :], xp, sems.at[3])
    small_copies = [pltpu.make_async_copy(src, dst, sems.at[4]) for src, dst in (
        (sk_hbm, sk_ref), (dd_hbm, dd_ref), (inv_hbm, inv_ref),
        (gw_hbm, gw_ref), (mem0_hbm, mem_v), (fill_hbm, fill_ref))]

    def out_copy(start, n):
        rows = pl.ds(start, n)
        return pltpu.make_async_copy(out_v.at[rows, :], out_hbm.at[rows, :], sems.at[5])

    def row_of(ref, c):
        t = ref[...].astype(F32)
        sel = jax.lax.broadcasted_iota(jnp.int32, (NB, 128), 0) == c
        return jnp.sum(jnp.where(sel, t, 0.0), axis=0, keepdims=True)

    k2 = k_v.reshape(NB, NCP * PR, 128)
    v2 = v_v.reshape(NB, NCP * PR, 128)

    def word(ref, c, pr):
        return ref[c, pl.ds(pr, NCH, stride=PR), :]

    def lo16(w):
        return pltpu.bitcast(w << 16, F32)

    def hi16(w):
        return pltpu.bitcast(w & U32(0xFFFF0000), F32)

    def pair(ref, c, pr):
        w = word(ref, c, pr)
        return lo16(w), hi16(w)

    first = jax.lax.broadcasted_iota(jnp.int32, (8, 128), 0) == 0

    def kv_prep(c, zw):
        skt = sk_ref[:, lanes(c)].astype(F32)
        sk = [jnp.broadcast_to(skt[j:j + 1, :], (8, 128)) for j in range(KS)]
        tail = (pair(k2, c, C // 2 - 2) + pair(k2, c, C // 2 - 1))[1:]
        win = [jnp.where(first, 0.0, pltpu.roll(t, 1, 0)) for t in tail]
        for pr in range(C // 2):
            ks = pair(k2, c, pr)
            vs = pair(v2, c, pr)
            for i in range(2):
                win.append(ks[i])
                acc = win[-1] * sk[0]
                for j in range(1, KS):
                    acc = acc + win[-1 - j] * sk[j]
                win = win[1:]
                t_s[zw, pl.ds((2 * pr + i) * 8, 8), :] = acc * vs[i]

    def h_prep(c, zw):
        for t in range(S // 128):
            ht = pltpu.bitcast(h_v[c, 0:128, pl.ds(t * 128, 128)].T, U32)
            ht_s[zw, pl.ds(t * 64 // (C // 2) * PR + t * 64 % (C // 2), 64), :] = ht

    def fft1(sample, mid, zw):
        for b in range(R2):
            z = [_cmul((sample(R2 * a + b), None), cmath.exp(-0.5j * math.pi * a / R1)) for a in range(R1)]
            gq = _fft(z)
            for q1 in range(R1):
                re, im = _cmul(gq[q1], cmath.exp(-2j * math.pi * (q1 + 0.25) * b / C))
                row = (q1 * R2 + b) * 16
                mid[zw, pl.ds(row, 8), :] = re
                mid[zw, pl.ds(row + 8, 8), :] = im

    def fft2(mid, dst, zw, zr):
        for q1 in range(R1):
            z = []
            for b in range(R2):
                row = (q1 * R2 + b) * 16
                z.append((mid[zr, pl.ds(row, 8), :], mid[zr, pl.ds(row + 8, 8), :]))
            t = _fft(z)
            for q2 in range(R2):
                q = q1 + R1 * q2
                dst[zw, pl.ds(q, NCH, stride=SR), :] = t[q2][0]
                dst[zw, pl.ds(C + q, NCH, stride=SR), :] = t[q2][1]

    def mac(p, zw, zr):
        re = pl.ds(p * 8, 8)
        im = pl.ds(C + p * 8, 8)
        AB = 4
        prev = None
        for a0 in range(0, NCH, AB):
            zre = [None] * AB
            zim = [None] * AB
            for m in range(a0 + AB):
                hr = h_s[zr, pl.ds(m * SR + p * 8, 8), :]
                hi = h_s[zr, pl.ds(m * SR + C + p * 8, 8), :]
                for i in range(AB):
                    t = a0 + i - m
                    if t < 0:
                        continue
                    ur = u_s[zr, pl.ds(t * SR + p * 8, 8), :]
                    ui = u_s[zr, pl.ds(t * SR + C + p * 8, 8), :]
                    tr = hr * ur - hi * ui
                    ti = hr * ui + hi * ur
                    zre[i] = tr if zre[i] is None else zre[i] + tr
                    zim[i] = ti if zim[i] is None else zim[i] + ti
            for i in range(AB):
                if prev is None:
                    yf_s[zw, a0 + i, re, :] = zre[i]
                    yf_s[zw, a0 + i, im, :] = zim[i]
                else:
                    yf_s[zw, a0 + i, re, :] = zre[i] - prev[1]
                    yf_s[zw, a0 + i, im, :] = zim[i] + prev[0]
                prev = (zre[i], zim[i])

    def inv_dft(c, zr):
        qc = C // FOLD
        for a in range(NCH):
            yr = [yf_s[zr, a, j * qc:(j + 1) * qc, :] for j in range(FOLD)]
            yi = [yf_s[zr, a, C + j * qc:C + (j + 1) * qc, :] for j in range(FOLD)]
            sr, si, dr, di = yr[0] + yr[2], yi[0] + yi[2], yr[0] - yr[2], yi[0] - yi[2]
            tr, ti, er, ei = yr[1] + yr[3], yi[1] + yi[3], yr[1] - yr[3], yi[1] - yi[3]
            folded = [(sr + tr, si + ti), (dr - ei, di + er), (sr - tr, si - ti), (dr + ei, di - er)]
            for r in range(FOLD):
                f = jnp.concatenate(folded[r], axis=0).astype(BF16)
                y_v[c, pl.ds(a * C + r, qc, stride=FOLD), :] = _dot(inv_ref[r * qc:(r + 1) * qc, :], f)

    def fixup(e, c, mat):
        a = wbuf[e][mat, c, 0]
        b = wbuf[e][mat, c, 1]
        wbuf[e][mat, c, 0] = (a & U32(0xFFFF)) | (b << 16)
        wbuf[e][mat, c, 1] = (a >> 16) | (b & U32(0xFFFF0000))

    RB = 128

    def qkv_tile(e, c, n, hook=None):
        mat, j = n // 2, n % 2
        for r in range(PRO // RB):
            w = _unpack(wbuf[e][mat, c, j])
            xr = _unpack(xp[pl.ds(r * RB // 2, RB // 2), :])
            pk = _pack(_dot(xr, w))
            qkv_b[mat, 2 * c + e, j, pl.ds((QOFF + r * RB) // 2, RB // 2), :] = pk
            if hook is not None and r == 0:
                hook(pk[0:8])

    for cp in wq0_copies(0) + [xp_copy]:
        cp.start()
    zs[0] = 0
    zs[1] = 0
    xp_copy.wait()
    for cp in wq0_copies(1) + wq0_copies(2) + small_copies + block_piece(0, 2):
        cp.start()

    def start_when(cond, copies):
        @pl.when(cond)
        def _():
            for cp in copies:
                cp.start()

    def pro0(c, carry):
        for i in range(2):
            start_when(c == 1 + i, block_piece(0, i))
        for cp in wq0_copies(c):
            cp.wait()
        fixup(0, c, 0)
        qkv_tile(0, c, 0)
        qkv_tile(0, c, 1)
        start_when(c + 3 < NB, wq0_copies(jnp.minimum(c + 3, NB - 1)))
        for i in range(3, NPIECE):
            start_when(c == min(i - 1, NB - 3), block_piece(0, i))
        return carry

    with jax.named_scope("pro0"):
        jax.lax.fori_loop(0, NB, pro0, 0)
    for i in range(2, NPIECE):
        for cp in block_piece(1, i):
            cp.start()
    for cp in small_copies:
        cp.wait()

    zw = zs[0]
    zr = zs[1]

    def pro(c, carry):
        for i in range(2):
            start_when(c + 1 < NB, block_piece(jnp.minimum(c + 1, NB - 1), i))
        for i in range(NPIECE):
            for cp in block_piece(c, i):
                cp.wait()

        tiles = [(0, n) for n in range(2, 6)] + [(1, n) for n in range(6)]

        def tile(i, hook=None):
            e, n = tiles[i]
            if n % 2 == 0:
                fixup(e, c, n // 2)
            qkv_tile(e, c, n, hook=hook)

        def trigger(val):
            k2[c + zw, pl.ds(C // 2, 8), :] = val
            v2[c + zw, pl.ds(C // 2, 8), :] = val
            h_v[c + zw, pl.ds(128, 16), 0:128] = _unpack(val)

        def h_sample(n):
            w = word(ht_s, zr, n // 2)
            hv = hi16(w) if n % 2 else lo16(w)
            if n == 0:
                hv = hv + jnp.where(first, row_of(dd_ref, c), 0.0)
            return hv

        tile(0, trigger)
        h_prep(c, zw)
        kv_prep(c, zw)
        fft1(lambda n: t_s[zr, pl.ds(n * 8, 8), :], gu_s, zw)
        fft2(gu_s, u_s, zw, zr)
        fft1(h_sample, gh_s, zw)
        fft2(gh_s, h_s, zw, zr)
        for i in range(1, 9):
            for p in range(4 * i - 4, 4 * i):
                mac(p, zw, zr)
            tile(i)
        tile(9)
        inv_dft(c, zr)
        for i in range(2, NPIECE):
            start_when(c + 2 < NB, block_piece(jnp.minimum(c + 2, NB - 1), i))
        start_when(c + 1 < NB, [wo_copy(c)])
        start_when(c + 2 == NB, [wo_copy(NB - 1), x_early])
        return carry

    with jax.named_scope("pro"):
        jax.lax.fori_loop(0, NB, pro, 0)
    x_late.start()
    x_early.wait()
    for c in range(NB):
        wo_copy(c).wait()

    gwt = gw_ref[...].astype(F32)
    gw = jnp.concatenate([gwt[j:j + 1, :] for j in range(NB)], axis=1)

    def finalize(rows, b):
        xr = x_v[rows, :].astype(F32)
        g = jax.nn.sigmoid(jnp.sum(xr * gw, axis=-1, keepdims=True))
        a = xr * jnp.concatenate([y_v[j, rows, :] for j in range(NB)], axis=1)
        out_v[rows, :] = (g * a + (1.0 - g) * b).astype(BF16)

    def step(s, mem, split_first, odd):
        xrows = slice(M, M + RX) if odd else slice(0, RX)
        mrows = slice(0, M) if odd else slice(RX, RX + M)
        sh = 4 if odd else 0
        xo = pl.multiple_of(PRO + RX * s, 8)
        wbase = pl.multiple_of((RX // 2 * s) % (QCAP // 2) - sh, 8)
        rpos = pl.multiple_of((SEG // 2 * s + QOFF // 2) % (QCAP // 2), SEG // 2)
        opos = pl.multiple_of(SEG // 2 * s, SEG // 2)
        fbase = pl.multiple_of(RX // 2 * s - sh, 8)
        xs = x_v[pl.ds(xo, RX), :]
        lhs = jnp.concatenate([mem, xs] if odd else [xs, mem], axis=0)
        zpad = jnp.zeros((128 - 2 * (SEG + M), E), BF16)
        frows = pl.ds(pl.multiple_of(RX * s, 8), RX)
        low = jax.lax.broadcasted_iota(jnp.int32, (8, E), 0) < 4
        NP = H // 2

        mem_qkv = {}
        probs = {}
        cats = {}

        def load(mat, hp):
            parts = [_unpack(qkv_b[mat, hp, 0, pl.ds(rpos, SEG // 2), :]),
                     _unpack(qkv_b[mat, hp, 1, pl.ds(rpos, SEG // 2), :]), mem_qkv[(hp, mat)]]
            if mat > 0:
                parts.append(zpad)
            cats[(mat, hp)] = jnp.concatenate(parts, axis=0)

        def stage_a(hp):
            KH = D // 2
            split = split_first and hp == 0
            if split:
                for mat in range(3):
                    for j in range(2):
                        w = _unpack(wbuf[hp % 2][mat, hp // 2, j, :KH // 2, :])
                        qacc[2 * mat + j] = _dot(lhs[:, :KH], w)
            for mat in range(3):
                mm = []
                for j in range(2):
                    if split:
                        w = _unpack(wbuf[hp % 2][mat, hp // 2, j, KH // 2:, :])
                        res = qacc[2 * mat + j] + _dot(lhs[:, KH:], w)
                    else:
                        res = _dot(lhs, _unpack(wbuf[hp % 2][mat, hp // 2, j]))
                    pk = _pack(res)
                    if odd:
                        qkv_b[mat, hp, j, pl.ds(wbase + 4, 4), :] = pk[4:8]
                        qkv_b[mat, hp, j, pl.ds(wbase + 8, 8), :] = pk[8:16]
                    else:
                        qkv_b[mat, hp, j, pl.ds(wbase, 8), :] = pk[0:8]
                        qkv_b[mat, hp, j, pl.ds(wbase + 8, 4), :] = pk[8:12]
                    mm.append(res[mrows])
                    if j == 1:
                        mem_qkv[(hp, mat)] = jnp.concatenate(mm, axis=0).astype(BF16)
                    advance(6 * hp + 2 * mat + j + 1)

        def stage_b(hp):
            sc = _dot_nt(cats[(0, hp)], cats[(1, hp)]) * scale
            fill = fill_ref[...]
            sc = jnp.where(fill == 0.0, sc, fill)
            mx = jnp.max(sc, axis=-1, keepdims=True)
            p = jnp.exp(sc - mx)
            l = jnp.sum(p, axis=-1, keepdims=True)
            r = pl.reciprocal(l, approx=True)
            r = r * (2.0 - l * r)
            probs[hp] = (p * r).astype(BF16)

        def stage_c(hp):
            o = _dot(probs[hp], cats[(2, hp)])
            for j in range(2):
                h = 2 * hp + j
                cols = slice(h * E, (h + 1) * E)
                o_b[pl.ds(opos, SEG // 2), cols] = _pack(o[j * SEG:(j + 1) * SEG])
                om = o[2 * SEG + j * M:2 * SEG + (j + 1) * M]
                om = _pack(jnp.concatenate([om, om], axis=0))
                w0 = o_b[pl.ds(fbase, 8), cols]
                w1 = o_b[pl.ds(fbase + 8, 8), cols]
                lo_s[0:8, cols] = jnp.where(low, om, w0) if odd else w0
                lo_s[8:16, cols] = w1 if odd else jnp.where(low, w1, om)

        def oproj(j, late):
            ks = slice(HS * E, H * E) if late else slice(0, HS * E)
            kw = slice(ks.start // 2, ks.stop // 2)
            return _dot(_unpack(lo_s[:, ks]), _unpack(wo_v[j, kw, :]))

        events = []
        for hp in range(NP):
            events.append((6 * hp + OFF_LQK, 0, functools.partial(load, 0, hp)))
            events.append((6 * hp + OFF_LQK, 1, functools.partial(load, 1, hp)))
            events.append((6 * hp + OFF_LV, 2, functools.partial(load, 2, hp)))
            events.append((6 * hp + OFF_PV, 3, functools.partial(stage_c, hp)))
            events.append((6 * hp + OFF_S, 4, functools.partial(stage_b, hp)))
        events.sort(key=lambda ev: ev[:2])

        def advance(slot):
            while events and events[0][0] <= slot:
                events.pop(0)[2]()

        outs = [None] * NB
        for hp in range(NP):
            stage_a(hp)
        for j in range(NB):
            oacc[:, j * 128:(j + 1) * 128] = oproj(j, False)
            advance(6 * NP + (j + 1) * HS // 8)
        assert not events
        for j in range(NB):
            outs[j] = oacc[:, j * 128:(j + 1) * 128] + oproj(j, True)
        res = jnp.concatenate(outs, axis=1)
        finalize(frows, res[xrows])
        return res[mrows].astype(BF16)

    def steps(i, carry):
        @pl.when(i == (XE - PRO) // (RX * UNROLL))
        def _():
            x_late.wait()

        mem = mem_v[...]
        for u in range(UNROLL):
            mem = step(i * UNROLL + u, mem, u > 0, u % 2 == 1)
        mem_v[...] = mem
        return carry

    with jax.named_scope("main"):
        jax.lax.fori_loop(0, NSEG // UNROLL, steps, 0)

    def epi_rows(r0, n):
        lo = _unpack(o_b[pl.ds(pl.multiple_of(r0 // 2, 8), n // 2), :])
        outs = [_dot(lo, _unpack(wo_v[j])) for j in range(NB)]
        finalize(pl.ds(r0, n), jnp.concatenate(outs, axis=1))

    EB = 128

    def epi(r, carry):
        r0 = pl.multiple_of(S - PRO + r * EB, EB)

        @pl.when(r == PRO // EB - 1)
        def _():
            out_copy(S - PRO, PRO - EB).start()

        epi_rows(r0, EB)
        return carry

    with jax.named_scope("epi"):
        out_copy(0, S - PRO).start()
        jax.lax.fori_loop(0, PRO // EB, epi, 0)
    out_copy(S - EB, EB).start()
    out_copy(0, S).wait()


@jax.jit
def _run(A_q, A_k, A_v, A_shift_k, A_ssm_k, A_ssm_D, B_mem0, B_Wq, B_Wk, B_Wv, B_Wo, gate_w):
    any_spec = pl.BlockSpec(memory_space=pl.ANY)
    out = pl.pallas_call(
        _kernel,
        out_shape=jax.ShapeDtypeStruct((S, D), BF16),
        in_specs=[any_spec] * 14,
        out_specs=any_spec,
        scratch_shapes=[
            pltpu.VMEM((S, D), BF16),
            pltpu.VMEM((PRO // 2, D), U32),
            pltpu.VMEM((NB, NCP, PR, 128), U32),
            pltpu.VMEM((NB, NCP, PR, 128), U32),
            pltpu.VMEM((NB, 128 + 16, S), BF16),
            pltpu.VMEM((3, H // 4, 2, D // 2, E), U32),
            pltpu.VMEM((3, H // 4, 2, D // 2, E), U32),
            pltpu.VMEM((NB, H * E // 2, 128), U32),
            pltpu.VMEM((NB, S + 32, 128), F32),
            pltpu.VMEM((3, H // 2, 2, QCAP // 2, E), U32),
            pltpu.VMEM((S // 2, H * E), U32),
            pltpu.VMEM(((M + RX) // 2, H * E), U32),
            pltpu.VMEM((M, D), BF16),
            pltpu.VMEM((M + RX, D), F32),
            pltpu.VMEM((6, M + RX, E), F32),
            pltpu.VMEM((1, NCH * SR + 2 * C, 128), F32),
            pltpu.VMEM((1, NCH * SR + 2 * C, 128), F32),
            pltpu.VMEM((1, NCH, 2 * C, 128), F32),
            pltpu.VMEM((1, S, 128), F32),
            pltpu.VMEM((1, 2 * S, 128), F32),
            pltpu.VMEM((1, 2 * S, 128), F32),
            pltpu.VMEM((1, NCP * PR, 128), U32),
            pltpu.VMEM((S, D), BF16),
            pltpu.VMEM((C, 2 * C // FOLD), BF16),
            pltpu.VMEM((2 * (SEG + M), 128), F32),
            pltpu.VMEM((KS, D), BF16),
            pltpu.VMEM((NB, 128), BF16),
            pltpu.VMEM((NB, 128), BF16),
            pltpu.SMEM((2,), jnp.int32),
            pltpu.SemaphoreType.DMA((6,)),
            pltpu.SemaphoreType.DMA((NB,)),
        ],
        compiler_params=pltpu.CompilerParams(vmem_limit_bytes=120 * 2 ** 20, disable_bounds_checks=True),
    )(
        A_q.reshape(S, D), A_k.reshape(NCH, C, D), A_v.reshape(NCH, C, D), A_ssm_k,
        B_Wq.reshape(D // 2, 2, H, E), B_Wk.reshape(D // 2, 2, H, E), B_Wv.reshape(D // 2, 2, H, E),
        B_Wo.reshape(H * E, D),
        A_shift_k.T, A_ssm_D.reshape(NB, 128), gate_w.reshape(NB, 128), B_mem0.reshape(M, D),
        jnp.asarray(_inv_table(), BF16), jnp.asarray(_attn_fill()),
    )
    return out.reshape(1, S, D)


def pallas_gated_mix__ssm_conv_h3__memory_aug_recurrent_mem_tr__prompt_kernel(
    A_q, A_k, A_v, A_shift_k, A_ssm_k, A_ssm_D, B_x, B_mem0, B_Wq, B_Wk, B_Wv, B_Wo, B_seg_len, gate_w,
):
    del B_x
    if isinstance(B_seg_len, int):
        assert B_seg_len == SEG
    return _run(A_q, A_k, A_v, A_shift_k, A_ssm_k, A_ssm_D, B_mem0, B_Wq, B_Wk, B_Wv, B_Wo, gate_w)
```

```python
import cmath
import functools
import math

import jax
import jax.numpy as jnp
import numpy as np
import jax.experimental.pallas as pl
import jax.experimental.pallas.tpu as pltpu

F32 = jnp.float32
BF16 = jnp.bfloat16
U32 = jnp.uint32

S = 2048
D = 1024
H = 32
E = 128
M = 8
SEG = 32
NSEG = S // SEG
RX = 24
PRO = S - RX * NSEG
QCAP = 576
QOFF = QCAP - PRO
HL = 4
HS = H - HL
OFF_LQK, OFF_S, OFF_LV, OFF_PV = 4, 8, 14, 17
UNROLL = 4
XE = 768
C = 256
NCH = S // C
NB = D // 128
KS = 4
NEG = -1000000000.0
R1, R2 = 16, 16
PR = C // 2 + 8
NCP = NCH + 4
FOLD = 4
SR = 2 * C + 4


def _inv_table():
    n = np.arange(C, dtype=np.float64)
    th = 2.0 * np.pi * (np.arange(C // FOLD, dtype=np.float64) + 0.25) / C
    no = np.concatenate([n[r::FOLD] for r in range(FOLD)])
    inv = np.concatenate([np.cos(no[:, None] * th[None, :]), -np.sin(no[:, None] * th[None, :])], axis=1) / C
    return inv.astype(np.float32)


def _attn_fill():
    n = 2 * (SEG + M)
    head = np.array([0] * SEG + [1] * SEG + [0] * M + [1] * M)
    pos = np.concatenate([M + np.arange(SEG), M + np.arange(SEG), np.arange(M), np.arange(M)])
    fill = np.full((n, 128), -np.inf, np.float32)
    for i in range(n):
        for j in range(n):
            if head[i] == head[j]:
                ok = pos[i] < M or pos[i] >= pos[j]
                fill[i, j] = 0.0 if ok else NEG
    return fill


def _add(a, b):
    return b if a is None else a if b is None else a + b


def _sub(a, b):
    return a if b is None else -b if a is None else a - b


def _cmul(z, w):
    r, i = z
    wr, wi = w.real, w.imag
    eps = 1e-12
    if abs(wi) < eps and abs(wr - 1.0) < eps:
        return z
    if i is None:
        if abs(abs(wr) - abs(wi)) < eps and wr * wi > 0:
            t = r * wr
            return t, t
        return r * wr, r * wi
    if abs(abs(wr) - abs(wi)) < eps:
        if wr * wi > 0:
            return (r - i) * wr, (r + i) * wr
        return (r + i) * wr, (i - r) * wr
    return r * wr - i * wi, r * wi + i * wr


def _fft(xs):
    n = len(xs)
    if n == 1:
        return xs
    if n == 2:
        (ar, ai), (br, bi) = xs
        return [(_add(ar, br), _add(ai, bi)), (_sub(ar, br), _sub(ai, bi))]
    e = _fft(xs[0::2])
    o1 = _fft(xs[1::4])
    o3 = _fft(xs[3::4])
    out = [None] * n
    for k in range(n // 4):
        ar, ai = _cmul(o1[k], cmath.exp(-2j * math.pi * k / n))
        br, bi = _cmul(o3[k], cmath.exp(-6j * math.pi * k / n))
        sr, si, dr, di = _add(ar, br), _add(ai, bi), _sub(ar, br), _sub(ai, bi)
        er, ei = e[k]
        fr, fi = e[k + n // 4]
        out[k] = (_add(er, sr), _add(ei, si))
        out[k + n // 2] = (_sub(er, sr), _sub(ei, si))
        out[k + n // 4] = (_add(fr, di), _sub(fi, dr))
        out[k + 3 * n // 4] = (_sub(fr, di), _add(fi, dr))
    return out


def _dot(a, b):
    return jnp.dot(a, b, preferred_element_type=F32)


def _dot_nt(a, b):
    return jax.lax.dot_general(a, b, (((1,), (1,)), ((), ())), preferred_element_type=F32)


def _pack(a):
    return pltpu.bitcast(a.astype(BF16), U32)


def _unpack(a):
    return pltpu.bitcast(a, BF16)


def _kernel(x_hbm, k_hbm, v_hbm, h_hbm, wq_hbm, wk_hbm, wv_hbm, wo_hbm,
            sk_hbm, dd_hbm, gw_hbm, mem0_hbm, inv_hbm, fill_hbm,
            out_hbm,
            x_v, xp, k_v, v_v, h_v, w_even, w_odd, wo_v, y_v, qkv_b, o_b, lo_s, mem_v, oacc, qacc,
            u_s, h_s, yf_s, t_s, gu_s, gh_s, ht_s,
            out_v, inv_ref, fill_ref, sk_ref, dd_ref, gw_ref, zs, sems, qsems):
    scale = E ** (-0.5)
    wbuf = (w_even, w_odd)

    w32 = [w.bitcast(U32) for w in (wq_hbm, wk_hbm, wv_hbm)]
    wo32 = wo_hbm.bitcast(U32)
    x32 = x_hbm.bitcast(U32)
    k32 = k_hbm.bitcast(U32)
    v32 = v_hbm.bitcast(U32)

    def lanes(c):
        return pl.ds(pl.multiple_of(c * 128, 128), 128)

    def w_copies(c, e, mat, sem):
        return [pltpu.make_async_copy(w32[mat].at[:, par, 2 * c + e, :], wbuf[e].at[mat, c, par], sem)
                for par in range(2)]

    def wq0_copies(c):
        return w_copies(c, 0, 0, qsems.at[c])

    W_REST = [(e, mat) for e in range(2) for mat in range(3) if (e, mat) != (0, 0)]
    NPIECE = 3 + len(W_REST)

    def block_piece(c, i):
        sem = sems.at[c % 2]
        if i < 2:
            src, dst = ((k32, k_v), (v32, v_v))[i]
            return [pltpu.make_async_copy(src.at[:, :, lanes(c)], dst.at[c, pl.ds(0, NCH), pl.ds(0, C // 2), :], sem)]
        if i == 2:
            return [pltpu.make_async_copy(h_hbm.at[lanes(c), :], h_v.at[c, pl.ds(0, 128), :], sem)]
        return w_copies(c, *W_REST[i - 3], sem)

    def wo_copy(c):
        return pltpu.make_async_copy(wo32.at[:, lanes(c)], wo_v.at[c], sems.at[2])

    x_early = pltpu.make_async_copy(x_hbm.at[pl.ds(0, XE), :], x_v.at[pl.ds(0, XE), :], sems.at[2])
    x_late = pltpu.make_async_copy(x_hbm.at[pl.ds(XE, S - XE), :], x_v.at[pl.ds(XE, S - XE), :], sems.at[3])

    xp_copies = [pltpu.make_async_copy(x32.at[pl.ds(i * PRO // 4, PRO // 4), :], xp.at[pl.ds(i * PRO // 4, PRO // 4), :],
                                       sems.at[3 + 3 * i]) for i in range(2)]
    small_copies = [pltpu.make_async_copy(src, dst, sems.at[4]) for src, dst in (
        (sk_hbm, sk_ref), (dd_hbm, dd_ref), (inv_hbm, inv_ref),
        (gw_hbm, gw_ref), (mem0_hbm, mem_v), (fill_hbm, fill_ref))]

    def out_copy(start, n):
        rows = pl.ds(start, n)
        return pltpu.make_async_copy(out_v.at[rows, :], out_hbm.at[rows, :], sems.at[5])

    def row_of(ref, c):
        t = ref[...].astype(F32)
        sel = jax.lax.broadcasted_iota(jnp.int32, (NB, 128), 0) == c
        return jnp.sum(jnp.where(sel, t, 0.0), axis=0, keepdims=True)

    k2 = k_v.reshape(NB, NCP * PR, 128)
    v2 = v_v.reshape(NB, NCP * PR, 128)

    def word(ref, c, pr):
        return ref[c, pl.ds(pr, NCH, stride=PR), :]

    def lo16(w):
        return pltpu.bitcast(w << 16, F32)

    def hi16(w):
        return pltpu.bitcast(w & U32(0xFFFF0000), F32)

    def pair(ref, c, pr):
        w = word(ref, c, pr)
        return lo16(w), hi16(w)

    first = jax.lax.broadcasted_iota(jnp.int32, (8, 128), 0) == 0

    def kv_prep(c, zw):
        skt = sk_ref[:, lanes(c)].astype(F32)
        sk = [jnp.broadcast_to(skt[j:j + 1, :], (8, 128)) for j in range(KS)]
        tail = (pair(k2, c, C // 2 - 2) + pair(k2, c, C // 2 - 1))[1:]
        win = [jnp.where(first, 0.0, pltpu.roll(t, 1, 0)) for t in tail]
        for pr in range(C // 2):
            ks = pair(k2, c, pr)
            vs = pair(v2, c, pr)
            for i in range(2):
                win.append(ks[i])
                acc = win[-1] * sk[0]
                for j in range(1, KS):
                    acc = acc + win[-1 - j] * sk[j]
                win = win[1:]
                t_s[zw, pl.ds((2 * pr + i) * 8, 8), :] = acc * vs[i]

    def h_prep(c, zw):
        for t in range(S // 128):
            ht = pltpu.bitcast(h_v[c, 0:128, pl.ds(t * 128, 128)].T, U32)
            ht_s[zw, pl.ds(t * 64 // (C // 2) * PR + t * 64 % (C // 2), 64), :] = ht

    def fft1(sample, mid, zw):
        for b in range(R2):
            z = [_cmul((sample(R2 * a + b), None), cmath.exp(-0.5j * math.pi * a / R1)) for a in range(R1)]
            gq = _fft(z)
            for q1 in range(R1):
                re, im = _cmul(gq[q1], cmath.exp(-2j * math.pi * (q1 + 0.25) * b / C))
                row = (q1 * R2 + b) * 16
                mid[zw, pl.ds(row, 8), :] = re
                mid[zw, pl.ds(row + 8, 8), :] = im

    def fft2(mid, dst, zw, zr):
        for q1 in range(R1):
            z = []
            for b in range(R2):
                row = (q1 * R2 + b) * 16
                z.append((mid[zr, pl.ds(row, 8), :], mid[zr, pl.ds(row + 8, 8), :]))
            t = _fft(z)
            for q2 in range(R2):
                q = q1 + R1 * q2
                dst[zw, pl.ds(q, NCH, stride=SR), :] = t[q2][0]
                dst[zw, pl.ds(C + q, NCH, stride=SR), :] = t[q2][1]

    def mac(p, zw, zr):
        re = pl.ds(p * 8, 8)
        im = pl.ds(C + p * 8, 8)
        AB = 4
        prev = None
        for a0 in range(0, NCH, AB):
            zre = [None] * AB
            zim = [None] * AB
            for m in range(a0 + AB):
                hr = h_s[zr, pl.ds(m * SR + p * 8, 8), :]
                hi = h_s[zr, pl.ds(m * SR + C + p * 8, 8), :]
                for i in range(AB):
                    t = a0 + i - m
                    if t < 0:
                        continue
                    ur = u_s[zr, pl.ds(t * SR + p * 8, 8), :]
                    ui = u_s[zr, pl.ds(t * SR + C + p * 8, 8), :]
                    tr = hr * ur - hi * ui
                    ti = hr * ui + hi * ur
                    zre[i] = tr if zre[i] is None else zre[i] + tr
                    zim[i] = ti if zim[i] is None else zim[i] + ti
            for i in range(AB):
                if prev is None:
                    yf_s[zw, a0 + i, re, :] = zre[i]
                    yf_s[zw, a0 + i, im, :] = zim[i]
                else:
                    yf_s[zw, a0 + i, re, :] = zre[i] - prev[1]
                    yf_s[zw, a0 + i, im, :] = zim[i] + prev[0]
                prev = (zre[i], zim[i])

    def inv_dft(c, zr):
        qc = C // FOLD
        for a in range(NCH):
            yr = [yf_s[zr, a, j * qc:(j + 1) * qc, :] for j in range(FOLD)]
            yi = [yf_s[zr, a, C + j * qc:C + (j + 1) * qc, :] for j in range(FOLD)]
            sr, si, dr, di = yr[0] + yr[2], yi[0] + yi[2], yr[0] - yr[2], yi[0] - yi[2]
            tr, ti, er, ei = yr[1] + yr[3], yi[1] + yi[3], yr[1] - yr[3], yi[1] - yi[3]
            folded = [(sr + tr, si + ti), (dr - ei, di + er), (sr - tr, si - ti), (dr + ei, di - er)]
            for r in range(FOLD):
                f = jnp.concatenate(folded[r], axis=0).astype(BF16)
                y_v[c, pl.ds(a * C + r, qc, stride=FOLD), :] = _dot(inv_ref[r * qc:(r + 1) * qc, :], f)

    def fixup(e, c, mat):
        a = wbuf[e][mat, c, 0]
        b = wbuf[e][mat, c, 1]
        wbuf[e][mat, c, 0] = (a & U32(0xFFFF)) | (b << 16)
        wbuf[e][mat, c, 1] = (a >> 16) | (b & U32(0xFFFF0000))

    RB = 128

    def qkv_tile(e, c, n, hook=None, rs=range(PRO // RB)):
        mat, j = n // 2, n % 2
        for r in rs:
            w = _unpack(wbuf[e][mat, c, j])
            xr = _unpack(xp[pl.ds(r * RB // 2, RB // 2), :])
            pk = _pack(_dot(xr, w))
            qkv_b[mat, 2 * c + e, j, pl.ds((QOFF + r * RB) // 2, RB // 2), :] = pk
            if hook is not None and r == 0:
                hook(pk[0:8])

    def start_when(cond, copies):
        @pl.when(cond)
        def _():
            for cp in copies:
                cp.start()

    def wq0_tiles(c, rs=range(PRO // RB)):
        qkv_tile(0, c, 0, rs=rs)
        qkv_tile(0, c, 1, rs=rs)

    for cp in wq0_copies(0) + xp_copies + wq0_copies(1):
        cp.start()
    zs[0] = 0
    zs[1] = 0
    for cp in wq0_copies(0) + xp_copies[:1]:
        cp.wait()
    fixup(0, 0, 0)
    wq0_tiles(0, range(2))
    for cp in wq0_copies(2) + wq0_copies(3):
        cp.start()
    xp_copies[1].wait()
    wq0_tiles(0, range(2, 4))
    for cp in small_copies + block_piece(0, 0):
        cp.start()
    for cp in wq0_copies(1):
        cp.wait()
    fixup(0, 1, 0)
    wq0_tiles(1)
    for cp in wq0_copies(4) + wq0_copies(5) + block_piece(0, 2) + block_piece(0, 1):
        cp.start()

    def pro0(i, carry):
        for u in range(2):
            for cp in wq0_copies(2 * i + u):
                cp.wait()
        for u in range(2):
            fixup(0, 2 * i + u, 0)
            wq0_tiles(2 * i + u)
        start_when(i == 1, wq0_copies(6) + wq0_copies(7))
        for j in range(3, NPIECE):
            start_when(i == (1 if j < 5 else 2), block_piece(0, j))
        return carry

    with jax.named_scope("pro0"):
        jax.lax.fori_loop(1, NB // 2, pro0, 0)
    for i in range(2, NPIECE):
        for cp in block_piece(1, i):
            cp.start()
    for cp in small_copies:
        cp.wait()

    zw = zs[0]
    zr = zs[1]

    def pro(c, carry):
        for i in range(2):
            start_when(c + 1 < NB, block_piece(jnp.minimum(c + 1, NB - 1), i))
        for i in range(NPIECE):
            for cp in block_piece(c, i):
                cp.wait()

        tiles = [(0, n) for n in range(2, 6)] + [(1, n) for n in range(6)]

        def tile(i, hook=None):
            e, n = tiles[i]
            if n % 2 == 0:
                fixup(e, c, n // 2)
            qkv_tile(e, c, n, hook=hook)

        def trigger(val):
            k2[c + zw, pl.ds(C // 2, 8), :] = val
            v2[c + zw, pl.ds(C // 2, 8), :] = val
            h_v[c + zw, pl.ds(128, 16), 0:128] = _unpack(val)

        def h_sample(n):
            w = word(ht_s, zr, n // 2)
            hv = hi16(w) if n % 2 else lo16(w)
            if n == 0:
                hv = hv + jnp.where(first, row_of(dd_ref, c), 0.0)
            return hv

        tile(0, trigger)
        h_prep(c, zw)
        kv_prep(c, zw)
        fft1(lambda n: t_s[zr, pl.ds(n * 8, 8), :], gu_s, zw)
        fft2(gu_s, u_s, zw, zr)
        fft1(h_sample, gh_s, zw)
        fft2(gh_s, h_s, zw, zr)
        for i in range(1, 9):
            for p in range(4 * i - 4, 4 * i):
                mac(p, zw, zr)
            tile(i)
        tile(9)
        inv_dft(c, zr)
        for i in range(2, NPIECE):
            start_when(c + 2 < NB, block_piece(jnp.minimum(c + 2, NB - 1), i))
        start_when(c + 1 < NB, [wo_copy(c)])
        start_when(c + 2 == NB, [wo_copy(NB - 1), x_early])
        return carry

    with jax.named_scope("pro"):
        jax.lax.fori_loop(0, NB, pro, 0)
    x_late.start()
    x_early.wait()
    for c in range(NB):
        wo_copy(c).wait()

    gwt = gw_ref[...].astype(F32)
    gw = jnp.concatenate([gwt[j:j + 1, :] for j in range(NB)], axis=1)

    def finalize(rows, b):
        xr = x_v[rows, :].astype(F32)
        g = jax.nn.sigmoid(jnp.sum(xr * gw, axis=-1, keepdims=True))
        a = xr * jnp.concatenate([y_v[j, rows, :] for j in range(NB)], axis=1)
        out_v[rows, :] = (g * a + (1.0 - g) * b).astype(BF16)

    def step(s, mem, split_first, odd):
        xrows = slice(M, M + RX) if odd else slice(0, RX)
        mrows = slice(0, M) if odd else slice(RX, RX + M)
        sh = 4 if odd else 0
        xo = pl.multiple_of(PRO + RX * s, 8)
        wbase = pl.multiple_of((RX // 2 * s) % (QCAP // 2) - sh, 8)
        rpos = pl.multiple_of((SEG // 2 * s + QOFF // 2) % (QCAP // 2), SEG // 2)
        opos = pl.multiple_of(SEG // 2 * s, SEG // 2)
        fbase = pl.multiple_of(RX // 2 * s - sh, 8)
        xs = x_v[pl.ds(xo, RX), :]
        lhs = jnp.concatenate([mem, xs] if odd else [xs, mem], axis=0)
        zpad = jnp.zeros((128 - 2 * (SEG + M), E), BF16)
        frows = pl.ds(pl.multiple_of(RX * s, 8), RX)
        low = jax.lax.broadcasted_iota(jnp.int32, (8, E), 0) < 4
        NP = H // 2

        mem_qkv = {}
        probs = {}
        cats = {}

        def load(mat, hp):
            parts = [_unpack(qkv_b[mat, hp, 0, pl.ds(rpos, SEG // 2), :]),
                     _unpack(qkv_b[mat, hp, 1, pl.ds(rpos, SEG // 2), :]), mem_qkv[(hp, mat)]]
            if mat > 0:
                parts.append(zpad)
            cats[(mat, hp)] = jnp.concatenate(parts, axis=0)

        def stage_a(hp):
            KH = D // 2
            split = split_first and hp == 0
            if split:
                for mat in range(3):
                    for j in range(2):
                        w = _unpack(wbuf[hp % 2][mat, hp // 2, j, :KH // 2, :])
                        qacc[2 * mat + j] = _dot(lhs[:, :KH], w)
            for mat in range(3):
                mm = []
                for j in range(2):
                    if split:
                        w = _unpack(wbuf[hp % 2][mat, hp // 2, j, KH // 2:, :])
                        res = qacc[2 * mat + j] + _dot(lhs[:, KH:], w)
                    else:
                        res = _dot(lhs, _unpack(wbuf[hp % 2][mat, hp // 2, j]))
                    pk = _pack(res)
                    if odd:
                        qkv_b[mat, hp, j, pl.ds(wbase + 4, 4), :] = pk[4:8]
                        qkv_b[mat, hp, j, pl.ds(wbase + 8, 8), :] = pk[8:16]
                    else:
                        qkv_b[mat, hp, j, pl.ds(wbase, 8), :] = pk[0:8]
                        qkv_b[mat, hp, j, pl.ds(wbase + 8, 4), :] = pk[8:12]
                    mm.append(res[mrows])
                    if j == 1:
                        mem_qkv[(hp, mat)] = jnp.concatenate(mm, axis=0).astype(BF16)
                    advance(6 * hp + 2 * mat + j + 1)

        def stage_b(hp):
            sc = _dot_nt(cats[(0, hp)], cats[(1, hp)]) * scale
            fill = fill_ref[...]
            sc = jnp.where(fill == 0.0, sc, fill)
            mx = jnp.max(sc, axis=-1, keepdims=True)
            p = jnp.exp(sc - mx)
            l = jnp.sum(p, axis=-1, keepdims=True)
            r = pl.reciprocal(l, approx=True)
            r = r * (2.0 - l * r)
            probs[hp] = (p * r).astype(BF16)

        def stage_c(hp):
            o = _dot(probs[hp], cats[(2, hp)])
            for j in range(2):
                h = 2 * hp + j
                cols = slice(h * E, (h + 1) * E)
                o_b[pl.ds(opos, SEG // 2), cols] = _pack(o[j * SEG:(j + 1) * SEG])
                om = o[2 * SEG + j * M:2 * SEG + (j + 1) * M]
                om = _pack(jnp.concatenate([om, om], axis=0))
                w0 = o_b[pl.ds(fbase, 8), cols]
                w1 = o_b[pl.ds(fbase + 8, 8), cols]
                lo_s[0:8, cols] = jnp.where(low, om, w0) if odd else w0
                lo_s[8:16, cols] = w1 if odd else jnp.where(low, w1, om)

        def oproj(j, late):
            ks = slice(HS * E, H * E) if late else slice(0, HS * E)
            kw = slice(ks.start // 2, ks.stop // 2)
            return _dot(_unpack(lo_s[:, ks]), _unpack(wo_v[j, kw, :]))

        events = []
        for hp in range(NP):
            events.append((6 * hp + OFF_LQK, 0, functools.partial(load, 0, hp)))
            events.append((6 * hp + OFF_LQK, 1, functools.partial(load, 1, hp)))
            events.append((6 * hp + OFF_LV, 2, functools.partial(load, 2, hp)))
            events.append((6 * hp + OFF_PV, 3, functools.partial(stage_c, hp)))
            events.append((6 * hp + OFF_S, 4, functools.partial(stage_b, hp)))
        events.sort(key=lambda ev: ev[:2])

        def advance(slot):
            while events and events[0][0] <= slot:
                events.pop(0)[2]()

        outs = [None] * NB
        for hp in range(NP):
            stage_a(hp)
        for j in range(NB):
            oacc[:, j * 128:(j + 1) * 128] = oproj(j, False)
            advance(6 * NP + (j + 1) * HS // 8)
        assert not events
        for j in range(NB):
            outs[j] = oacc[:, j * 128:(j + 1) * 128] + oproj(j, True)
        res = jnp.concatenate(outs, axis=1)
        finalize(frows, res[xrows])
        return res[mrows].astype(BF16)

    def steps(i, carry):
        @pl.when(i == (XE - PRO) // (RX * UNROLL))
        def _():
            x_late.wait()

        mem = mem_v[...]
        for u in range(UNROLL):
            mem = step(i * UNROLL + u, mem, u > 0, u % 2 == 1)
        mem_v[...] = mem
        return carry

    with jax.named_scope("main"):
        jax.lax.fori_loop(0, NSEG // UNROLL, steps, 0)

    def epi_rows(r0, n):
        lo = _unpack(o_b[pl.ds(pl.multiple_of(r0 // 2, 8), n // 2), :])
        outs = [_dot(lo, _unpack(wo_v[j])) for j in range(NB)]
        finalize(pl.ds(r0, n), jnp.concatenate(outs, axis=1))

    EB = 128

    def epi(r, carry):
        r0 = pl.multiple_of(S - PRO + r * EB, EB)

        @pl.when(r == PRO // EB - 1)
        def _():
            out_copy(S - PRO, PRO - EB).start()

        epi_rows(r0, EB)
        return carry

    with jax.named_scope("epi"):
        out_copy(0, S - PRO).start()
        jax.lax.fori_loop(0, PRO // EB, epi, 0)
    out_copy(S - EB, EB).start()
    out_copy(0, S).wait()


@jax.jit
def _run(A_q, A_k, A_v, A_shift_k, A_ssm_k, A_ssm_D, B_mem0, B_Wq, B_Wk, B_Wv, B_Wo, gate_w):
    any_spec = pl.BlockSpec(memory_space=pl.ANY)
    out = pl.pallas_call(
        _kernel,
        out_shape=jax.ShapeDtypeStruct((S, D), BF16),
        in_specs=[any_spec] * 14,
        out_specs=any_spec,
        scratch_shapes=[
            pltpu.VMEM((S, D), BF16),
            pltpu.VMEM((PRO // 2, D), U32),
            pltpu.VMEM((NB, NCP, PR, 128), U32),
            pltpu.VMEM((NB, NCP, PR, 128), U32),
            pltpu.VMEM((NB, 128 + 16, S), BF16),
            pltpu.VMEM((3, H // 4, 2, D // 2, E), U32),
            pltpu.VMEM((3, H // 4, 2, D // 2, E), U32),
            pltpu.VMEM((NB, H * E // 2, 128), U32),
            pltpu.VMEM((NB, S + 32, 128), F32),
            pltpu.VMEM((3, H // 2, 2, QCAP // 2, E), U32),
            pltpu.VMEM((S // 2, H * E), U32),
            pltpu.VMEM(((M + RX) // 2, H * E), U32),
            pltpu.VMEM((M, D), BF16),
            pltpu.VMEM((M + RX, D), F32),
            pltpu.VMEM((6, M + RX, E), F32),
            pltpu.VMEM((1, NCH * SR + 2 * C, 128), F32),
            pltpu.VMEM((1, NCH * SR + 2 * C, 128), F32),
            pltpu.VMEM((1, NCH, 2 * C, 128), F32),
            pltpu.VMEM((1, S, 128), F32),
            pltpu.VMEM((1, 2 * S, 128), F32),
            pltpu.VMEM((1, 2 * S, 128), F32),
            pltpu.VMEM((1, NCP * PR, 128), U32),
            pltpu.VMEM((S, D), BF16),
            pltpu.VMEM((C, 2 * C // FOLD), BF16),
            pltpu.VMEM((2 * (SEG + M), 128), F32),
            pltpu.VMEM((KS, D), BF16),
            pltpu.VMEM((NB, 128), BF16),
            pltpu.VMEM((NB, 128), BF16),
            pltpu.SMEM((2,), jnp.int32),
            pltpu.SemaphoreType.DMA((7,)),
            pltpu.SemaphoreType.DMA((NB,)),
        ],
        compiler_params=pltpu.CompilerParams(vmem_limit_bytes=120 * 2 ** 20, disable_bounds_checks=True),
    )(
        A_q.reshape(S, D), A_k.reshape(NCH, C, D), A_v.reshape(NCH, C, D), A_ssm_k,
        B_Wq.reshape(D // 2, 2, H, E), B_Wk.reshape(D // 2, 2, H, E), B_Wv.reshape(D // 2, 2, H, E),
        B_Wo.reshape(H * E, D),
        A_shift_k.T, A_ssm_D.reshape(NB, 128), gate_w.reshape(NB, 128), B_mem0.reshape(M, D),
        jnp.asarray(_inv_table(), BF16), jnp.asarray(_attn_fill()),
    )
    return out.reshape(1, S, D)


def pallas_gated_mix__ssm_conv_h3__memory_aug_recurrent_mem_tr__prompt_kernel(
    A_q, A_k, A_v, A_shift_k, A_ssm_k, A_ssm_D, B_x, B_mem0, B_Wq, B_Wk, B_Wv, B_Wo, B_seg_len, gate_w,
):
    del B_x
    if isinstance(B_seg_len, int):
        assert B_seg_len == SEG
    return _run(A_q, A_k, A_v, A_shift_k, A_ssm_k, A_ssm_D, B_mem0, B_Wq, B_Wk, B_Wv, B_Wo, gate_w)
```

```python
import cmath
import functools
import math

import jax
import jax.numpy as jnp
import numpy as np
import jax.experimental.pallas as pl
import jax.experimental.pallas.tpu as pltpu

F32 = jnp.float32
BF16 = jnp.bfloat16
U32 = jnp.uint32

S = 2048
D = 1024
H = 32
E = 128
M = 8
SEG = 32
NSEG = S // SEG
RX = 24
PRO = S - RX * NSEG
QCAP = 576
QOFF = QCAP - PRO
HL = 4
HS = H - HL
OFF_LQK, OFF_S, OFF_LV, OFF_PV = 4, 8, 14, 17
UNROLL = 4
XE = 768
C = 256
NCH = S // C
NB = D // 128
KS = 4
NEG = -1000000000.0
R1, R2 = 16, 16
PR = C // 2 + 8
NCP = NCH + 4
FOLD = 4
SR = 2 * C + 4


def _inv_table():
    n = np.arange(C, dtype=np.float64)
    th = 2.0 * np.pi * (np.arange(C // FOLD, dtype=np.float64) + 0.25) / C
    no = np.concatenate([n[r::FOLD] for r in range(FOLD)])
    inv = np.concatenate([np.cos(no[:, None] * th[None, :]), -np.sin(no[:, None] * th[None, :])], axis=1) / C
    return inv.astype(np.float32)


def _attn_fill():
    n = 2 * (SEG + M)
    head = np.array([0] * SEG + [1] * SEG + [0] * M + [1] * M)
    pos = np.concatenate([M + np.arange(SEG), M + np.arange(SEG), np.arange(M), np.arange(M)])
    fill = np.full((n, 128), -np.inf, np.float32)
    for i in range(n):
        for j in range(n):
            if head[i] == head[j]:
                ok = pos[i] < M or pos[i] >= pos[j]
                fill[i, j] = 0.0 if ok else NEG
    return fill


def _add(a, b):
    return b if a is None else a if b is None else a + b


def _sub(a, b):
    return a if b is None else -b if a is None else a - b


def _cmul(z, w):
    r, i = z
    wr, wi = w.real, w.imag
    eps = 1e-12
    if abs(wi) < eps and abs(wr - 1.0) < eps:
        return z
    if i is None:
        if abs(abs(wr) - abs(wi)) < eps and wr * wi > 0:
            t = r * wr
            return t, t
        return r * wr, r * wi
    if abs(abs(wr) - abs(wi)) < eps:
        if wr * wi > 0:
            return (r - i) * wr, (r + i) * wr
        return (r + i) * wr, (i - r) * wr
    return r * wr - i * wi, r * wi + i * wr


def _fft(xs):
    n = len(xs)
    if n == 1:
        return xs
    if n == 2:
        (ar, ai), (br, bi) = xs
        return [(_add(ar, br), _add(ai, bi)), (_sub(ar, br), _sub(ai, bi))]
    e = _fft(xs[0::2])
    o1 = _fft(xs[1::4])
    o3 = _fft(xs[3::4])
    out = [None] * n
    for k in range(n // 4):
        ar, ai = _cmul(o1[k], cmath.exp(-2j * math.pi * k / n))
        br, bi = _cmul(o3[k], cmath.exp(-6j * math.pi * k / n))
        sr, si, dr, di = _add(ar, br), _add(ai, bi), _sub(ar, br), _sub(ai, bi)
        er, ei = e[k]
        fr, fi = e[k + n // 4]
        out[k] = (_add(er, sr), _add(ei, si))
        out[k + n // 2] = (_sub(er, sr), _sub(ei, si))
        out[k + n // 4] = (_add(fr, di), _sub(fi, dr))
        out[k + 3 * n // 4] = (_sub(fr, di), _add(fi, dr))
    return out


def _dot(a, b):
    return jnp.dot(a, b, preferred_element_type=F32)


def _dot_nt(a, b):
    return jax.lax.dot_general(a, b, (((1,), (1,)), ((), ())), preferred_element_type=F32)


def _pack(a):
    return pltpu.bitcast(a.astype(BF16), U32)


def _unpack(a):
    return pltpu.bitcast(a, BF16)


def _kernel(x_hbm, k_hbm, v_hbm, h_hbm, wq_hbm, wk_hbm, wv_hbm, wo_hbm,
            sk_hbm, dd_hbm, gw_hbm, mem0_hbm, inv_hbm, fill_hbm,
            out_hbm,
            x_v, xp, k_v, v_v, h_v, w_even, w_odd, wo_v, y_v, qkv_b, o_b, lo_s, mem_v, oacc, qacc,
            u_s, h_s, yf_s, t_s, gu_s, gh_s, ht_s,
            out_v, inv_ref, fill_ref, sk_ref, dd_ref, gw_ref, sems, qsems):
    scale = E ** (-0.5)
    wbuf = (w_even, w_odd)

    w32 = [w.bitcast(U32) for w in (wq_hbm, wk_hbm, wv_hbm)]
    wo32 = wo_hbm.bitcast(U32)
    x32 = x_hbm.bitcast(U32)
    k32 = k_hbm.bitcast(U32)
    v32 = v_hbm.bitcast(U32)

    def lanes(c):
        return pl.ds(pl.multiple_of(c * 128, 128), 128)

    def w_copies(c, e, mat, sem):
        return [pltpu.make_async_copy(w32[mat].at[:, par, 2 * c + e, :], wbuf[e].at[mat, c, par], sem)
                for par in range(2)]

    def wq0_copies(c):
        return w_copies(c, 0, 0, qsems.at[c])

    W_REST = [(e, mat) for e in range(2) for mat in range(3) if (e, mat) != (0, 0)]
    NPIECE = 3 + len(W_REST)

    def block_piece(c, i):
        sem = sems.at[c % 2]
        if i < 2:
            src, dst = ((k32, k_v), (v32, v_v))[i]
            return [pltpu.make_async_copy(src.at[:, :, lanes(c)], dst.at[c, pl.ds(0, NCH), pl.ds(0, C // 2), :], sem)]
        if i == 2:
            return [pltpu.make_async_copy(h_hbm.at[lanes(c), :], h_v.at[c, pl.ds(0, 128), :], sem)]
        return w_copies(c, *W_REST[i - 3], sem)

    def wo_copy(c):
        return pltpu.make_async_copy(wo32.at[:, lanes(c)], wo_v.at[c], sems.at[2])

    x_early = pltpu.make_async_copy(x_hbm.at[pl.ds(0, XE), :], x_v.at[pl.ds(0, XE), :], sems.at[2])
    x_late = pltpu.make_async_copy(x_hbm.at[pl.ds(XE, S - XE), :], x_v.at[pl.ds(XE, S - XE), :], sems.at[3])

    xp_copies = [pltpu.make_async_copy(x32.at[pl.ds(i * PRO // 4, PRO // 4), :], xp.at[pl.ds(i * PRO // 4, PRO // 4), :],
                                       sems.at[3 + 3 * i]) for i in range(2)]
    small_copies = [pltpu.make_async_copy(src, dst, sems.at[4]) for src, dst in (
        (sk_hbm, sk_ref), (dd_hbm, dd_ref), (inv_hbm, inv_ref),
        (gw_hbm, gw_ref), (mem0_hbm, mem_v), (fill_hbm, fill_ref))]

    def out_copy(start, n):
        rows = pl.ds(start, n)
        return pltpu.make_async_copy(out_v.at[rows, :], out_hbm.at[rows, :], sems.at[5])

    def row_of(ref, c):
        t = ref[...].astype(F32)
        sel = jax.lax.broadcasted_iota(jnp.int32, (NB, 128), 0) == c
        return jnp.sum(jnp.where(sel, t, 0.0), axis=0, keepdims=True)

    k2 = k_v.reshape(NB, NCP * PR, 128)
    v2 = v_v.reshape(NB, NCP * PR, 128)

    def word(ref, c, pr):
        return ref[c, pl.ds(pr, NCH, stride=PR), :]

    def lo16(w):
        return pltpu.bitcast(w << 16, F32)

    def hi16(w):
        return pltpu.bitcast(w & U32(0xFFFF0000), F32)

    def pair(ref, c, pr):
        w = word(ref, c, pr)
        return lo16(w), hi16(w)

    first = jax.lax.broadcasted_iota(jnp.int32, (8, 128), 0) == 0

    def kv_prep(c, zw):
        skt = sk_ref[:, lanes(c)].astype(F32)
        sk = [jnp.broadcast_to(skt[j:j + 1, :], (8, 128)) for j in range(KS)]
        tail = (pair(k2, c, C // 2 - 2) + pair(k2, c, C // 2 - 1))[1:]
        win = [jnp.where(first, 0.0, pltpu.roll(t, 1, 0)) for t in tail]
        for pr in range(C // 2):
            ks = pair(k2, c, pr)
            vs = pair(v2, c, pr)
            for i in range(2):
                win.append(ks[i])
                acc = win[-1] * sk[0]
                for j in range(1, KS):
                    acc = acc + win[-1 - j] * sk[j]
                win = win[1:]
                t_s[zw, pl.ds((2 * pr + i) * 8, 8), :] = acc * vs[i]

    def h_prep(c, zw):
        for t in range(S // 128):
            ht = pltpu.bitcast(h_v[c, 0:128, pl.ds(t * 128, 128)].T, U32)
            ht_s[zw, pl.ds(t * 64 // (C // 2) * PR + t * 64 % (C // 2), 64), :] = ht

    def fft1(sample, mid, zw):
        for b in range(R2):
            z = [_cmul((sample(R2 * a + b), None), cmath.exp(-0.5j * math.pi * a / R1)) for a in range(R1)]
            gq = _fft(z)
            for q1 in range(R1):
                re, im = _cmul(gq[q1], cmath.exp(-2j * math.pi * (q1 + 0.25) * b / C))
                row = (q1 * R2 + b) * 16
                mid[zw, pl.ds(row, 8), :] = re
                mid[zw, pl.ds(row + 8, 8), :] = im

    def fft2(mid, dst, zw, zr):
        for q1 in range(R1):
            z = []
            for b in range(R2):
                row = (q1 * R2 + b) * 16
                z.append((mid[zr, pl.ds(row, 8), :], mid[zr, pl.ds(row + 8, 8), :]))
            t = _fft(z)
            for q2 in range(R2):
                q = q1 + R1 * q2
                dst[zw, pl.ds(q, NCH, stride=SR), :] = t[q2][0]
                dst[zw, pl.ds(C + q, NCH, stride=SR), :] = t[q2][1]

    def mac(p, zw, zr):
        re = pl.ds(p * 8, 8)
        im = pl.ds(C + p * 8, 8)
        AB = 4
        prev = None
        for a0 in range(0, NCH, AB):
            zre = [None] * AB
            zim = [None] * AB
            for m in range(a0 + AB):
                hr = h_s[zr, pl.ds(m * SR + p * 8, 8), :]
                hi = h_s[zr, pl.ds(m * SR + C + p * 8, 8), :]
                for i in range(AB):
                    t = a0 + i - m
                    if t < 0:
                        continue
                    ur = u_s[zr, pl.ds(t * SR + p * 8, 8), :]
                    ui = u_s[zr, pl.ds(t * SR + C + p * 8, 8), :]
                    tr = hr * ur - hi * ui
                    ti = hr * ui + hi * ur
                    zre[i] = tr if zre[i] is None else zre[i] + tr
                    zim[i] = ti if zim[i] is None else zim[i] + ti
            for i in range(AB):
                if prev is None:
                    yf_s[zw, a0 + i, re, :] = zre[i]
                    yf_s[zw, a0 + i, im, :] = zim[i]
                else:
                    yf_s[zw, a0 + i, re, :] = zre[i] - prev[1]
                    yf_s[zw, a0 + i, im, :] = zim[i] + prev[0]
                prev = (zre[i], zim[i])

    def inv_dft(c, zr):
        qc = C // FOLD
        for a in range(NCH):
            yr = [yf_s[zr, a, j * qc:(j + 1) * qc, :] for j in range(FOLD)]
            yi = [yf_s[zr, a, C + j * qc:C + (j + 1) * qc, :] for j in range(FOLD)]
            sr, si, dr, di = yr[0] + yr[2], yi[0] + yi[2], yr[0] - yr[2], yi[0] - yi[2]
            tr, ti, er, ei = yr[1] + yr[3], yi[1] + yi[3], yr[1] - yr[3], yi[1] - yi[3]
            folded = [(sr + tr, si + ti), (dr - ei, di + er), (sr - tr, si - ti), (dr + ei, di - er)]
            for r in range(FOLD):
                f = jnp.concatenate(folded[r], axis=0).astype(BF16)
                y_v[c, pl.ds(a * C + r, qc, stride=FOLD), :] = _dot(inv_ref[r * qc:(r + 1) * qc, :], f)

    def fixup(e, c, mat):
        a = wbuf[e][mat, c, 0]
        b = wbuf[e][mat, c, 1]
        wbuf[e][mat, c, 0] = (a & U32(0xFFFF)) | (b << 16)
        wbuf[e][mat, c, 1] = (a >> 16) | (b & U32(0xFFFF0000))

    RB = 128

    def qkv_tile(e, c, n, hook=None, rs=range(PRO // RB)):
        mat, j = n // 2, n % 2
        for r in rs:
            w = _unpack(wbuf[e][mat, c, j])
            xr = _unpack(xp[pl.ds(r * RB // 2, RB // 2), :])
            pk = _pack(_dot(xr, w))
            qkv_b[mat, 2 * c + e, j, pl.ds((QOFF + r * RB) // 2, RB // 2), :] = pk
            if hook is not None and r == 0:
                hook(pk[0:8])

    def start_when(cond, copies):
        @pl.when(cond)
        def _():
            for cp in copies:
                cp.start()

    def wq0_tiles(c, rs=range(PRO // RB)):
        qkv_tile(0, c, 0, rs=rs)
        qkv_tile(0, c, 1, rs=rs)

    for cp in wq0_copies(0) + xp_copies + wq0_copies(1):
        cp.start()
    for cp in wq0_copies(0) + xp_copies[:1]:
        cp.wait()
    fixup(0, 0, 0)
    wq0_tiles(0, range(2))
    for cp in wq0_copies(2) + wq0_copies(3):
        cp.start()
    xp_copies[1].wait()
    wq0_tiles(0, range(2, 4))
    for cp in small_copies + block_piece(0, 0):
        cp.start()
    for cp in wq0_copies(1):
        cp.wait()
    fixup(0, 1, 0)
    wq0_tiles(1)
    for cp in wq0_copies(4) + wq0_copies(5) + block_piece(0, 2) + block_piece(0, 1):
        cp.start()

    def pro0(i, carry):
        for u in range(2):
            for cp in wq0_copies(2 * i + u):
                cp.wait()
        for u in range(2):
            fixup(0, 2 * i + u, 0)
            wq0_tiles(2 * i + u)
        start_when(i == 1, wq0_copies(6) + wq0_copies(7))
        for j in range(3, NPIECE):
            start_when(i == (1 if j < 5 else 2), block_piece(0, j))
        return carry

    with jax.named_scope("pro0"):
        jax.lax.fori_loop(1, NB // 2, pro0, 0)
    for i in range(2, NPIECE):
        for cp in block_piece(1, i):
            cp.start()
    for cp in small_copies:
        cp.wait()

    def pro(c, carry):
        zw = c >> 3
        zr = c >> 4
        for i in range(2):
            start_when(c + 1 < NB, block_piece(jnp.minimum(c + 1, NB - 1), i))
        for i in range(NPIECE):
            for cp in block_piece(c, i):
                cp.wait()

        tiles = [(0, n) for n in range(2, 6)] + [(1, n) for n in range(6)]

        def tile(i, hook=None):
            e, n = tiles[i]
            if n % 2 == 0:
                fixup(e, c, n // 2)
            qkv_tile(e, c, n, hook=hook)

        def trigger(val):
            k2[c + zw, pl.ds(C // 2, 8), :] = val
            v2[c + zw, pl.ds(C // 2, 8), :] = val
            h_v[c + zw, pl.ds(128, 16), 0:128] = _unpack(val)

        def h_sample(n):
            w = word(ht_s, zr, n // 2)
            hv = hi16(w) if n % 2 else lo16(w)
            if n == 0:
                hv = hv + jnp.where(first, row_of(dd_ref, c), 0.0)
            return hv

        tile(0, trigger)
        h_prep(c, zw)
        kv_prep(c, zw)
        fft1(lambda n: t_s[zr, pl.ds(n * 8, 8), :], gu_s, zw)
        fft2(gu_s, u_s, zw, zr)
        fft1(h_sample, gh_s, zw)
        fft2(gh_s, h_s, zw, zr)
        for i in range(1, 9):
            for p in range(4 * i - 4, 4 * i):
                mac(p, zw, zr)
            tile(i)
        tile(9)
        inv_dft(c, zr)
        for i in range(2, NPIECE):
            start_when(c + 2 < NB, block_piece(jnp.minimum(c + 2, NB - 1), i))
        start_when(c + 1 < NB, [wo_copy(c)])
        start_when(c + 2 == NB, [wo_copy(NB - 1), x_early])
        return carry

    with jax.named_scope("pro"):
        jax.lax.fori_loop(0, NB, pro, 0)
    x_late.start()
    x_early.wait()
    for c in range(NB):
        wo_copy(c).wait()

    gwt = gw_ref[...].astype(F32)
    gw = jnp.concatenate([gwt[j:j + 1, :] for j in range(NB)], axis=1)

    def finalize(rows, b):
        xr = x_v[rows, :].astype(F32)
        g = jax.nn.sigmoid(jnp.sum(xr * gw, axis=-1, keepdims=True))
        a = xr * jnp.concatenate([y_v[j, rows, :] for j in range(NB)], axis=1)
        out_v[rows, :] = (g * a + (1.0 - g) * b).astype(BF16)

    def step(s, mem, split_first, odd):
        xrows = slice(M, M + RX) if odd else slice(0, RX)
        mrows = slice(0, M) if odd else slice(RX, RX + M)
        sh = 4 if odd else 0
        xo = pl.multiple_of(PRO + RX * s, 8)
        wbase = pl.multiple_of((RX // 2 * s) % (QCAP // 2) - sh, 8)
        rpos = pl.multiple_of((SEG // 2 * s + QOFF // 2) % (QCAP // 2), SEG // 2)
        opos = pl.multiple_of(SEG // 2 * s, SEG // 2)
        fbase = pl.multiple_of(RX // 2 * s - sh, 8)
        xs = x_v[pl.ds(xo, RX), :]
        lhs = jnp.concatenate([mem, xs] if odd else [xs, mem], axis=0)
        zpad = jnp.zeros((128 - 2 * (SEG + M), E), BF16)
        frows = pl.ds(pl.multiple_of(RX * s, 8), RX)
        low = jax.lax.broadcasted_iota(jnp.int32, (8, E), 0) < 4
        NP = H // 2

        mem_qkv = {}
        probs = {}
        cats = {}

        def load(mat, hp):
            parts = [_unpack(qkv_b[mat, hp, 0, pl.ds(rpos, SEG // 2), :]),
                     _unpack(qkv_b[mat, hp, 1, pl.ds(rpos, SEG // 2), :]), mem_qkv[(hp, mat)]]
            if mat > 0:
                parts.append(zpad)
            cats[(mat, hp)] = jnp.concatenate(parts, axis=0)

        def stage_a(hp):
            KH = D // 2
            split = split_first and hp == 0
            if split:
                for mat in range(3):
                    for j in range(2):
                        w = _unpack(wbuf[hp % 2][mat, hp // 2, j, :KH // 2, :])
                        qacc[2 * mat + j] = _dot(lhs[:, :KH], w)
            for mat in range(3):
                mm = []
                for j in range(2):
                    if split:
                        w = _unpack(wbuf[hp % 2][mat, hp // 2, j, KH // 2:, :])
                        res = qacc[2 * mat + j] + _dot(lhs[:, KH:], w)
                    else:
                        res = _dot(lhs, _unpack(wbuf[hp % 2][mat, hp // 2, j]))
                    pk = _pack(res)
                    if odd:
                        qkv_b[mat, hp, j, pl.ds(wbase + 4, 4), :] = pk[4:8]
                        qkv_b[mat, hp, j, pl.ds(wbase + 8, 8), :] = pk[8:16]
                    else:
                        qkv_b[mat, hp, j, pl.ds(wbase, 8), :] = pk[0:8]
                        qkv_b[mat, hp, j, pl.ds(wbase + 8, 4), :] = pk[8:12]
                    mm.append(res[mrows])
                    if j == 1:
                        mem_qkv[(hp, mat)] = jnp.concatenate(mm, axis=0).astype(BF16)
                    advance(6 * hp + 2 * mat + j + 1)

        def stage_b(hp):
            sc = _dot_nt(cats[(0, hp)], cats[(1, hp)]) * scale
            fill = fill_ref[...]
            sc = jnp.where(fill == 0.0, sc, fill)
            mx = jnp.max(sc, axis=-1, keepdims=True)
            p = jnp.exp(sc - mx)
            l = jnp.sum(p, axis=-1, keepdims=True)
            r = pl.reciprocal(l, approx=True)
            r = r * (2.0 - l * r)
            probs[hp] = (p * r).astype(BF16)

        def stage_c(hp):
            o = _dot(probs[hp], cats[(2, hp)])
            for j in range(2):
                h = 2 * hp + j
                cols = slice(h * E, (h + 1) * E)
                o_b[pl.ds(opos, SEG // 2), cols] = _pack(o[j * SEG:(j + 1) * SEG])
                om = o[2 * SEG + j * M:2 * SEG + (j + 1) * M]
                om = _pack(jnp.concatenate([om, om], axis=0))
                w0 = o_b[pl.ds(fbase, 8), cols]
                w1 = o_b[pl.ds(fbase + 8, 8), cols]
                lo_s[0:8, cols] = jnp.where(low, om, w0) if odd else w0
                lo_s[8:16, cols] = w1 if odd else jnp.where(low, w1, om)

        def oproj(j, late):
            ks = slice(HS * E, H * E) if late else slice(0, HS * E)
            kw = slice(ks.start // 2, ks.stop // 2)
            return _dot(_unpack(lo_s[:, ks]), _unpack(wo_v[j, kw, :]))

        events = []
        for hp in range(NP):
            events.append((6 * hp + OFF_LQK, 0, functools.partial(load, 0, hp)))
            events.append((6 * hp + OFF_LQK, 1, functools.partial(load, 1, hp)))
            events.append((6 * hp + OFF_LV, 2, functools.partial(load, 2, hp)))
            events.append((6 * hp + OFF_PV, 3, functools.partial(stage_c, hp)))
            events.append((6 * hp + OFF_S, 4, functools.partial(stage_b, hp)))
        events.sort(key=lambda ev: ev[:2])

        def advance(slot):
            while events and events[0][0] <= slot:
                events.pop(0)[2]()

        outs = [None] * NB
        for hp in range(NP):
            stage_a(hp)
        for j in range(NB):
            oacc[:, j * 128:(j + 1) * 128] = oproj(j, False)
            advance(6 * NP + (j + 1) * HS // 8)
        assert not events
        for j in range(NB):
            outs[j] = oacc[:, j * 128:(j + 1) * 128] + oproj(j, True)
        res = jnp.concatenate(outs, axis=1)
        finalize(frows, res[xrows])
        return res[mrows].astype(BF16)

    def steps(i, carry):
        @pl.when(i == (XE - PRO) // (RX * UNROLL))
        def _():
            x_late.wait()

        mem = mem_v[...]
        for u in range(UNROLL):
            mem = step(i * UNROLL + u, mem, u > 0, u % 2 == 1)
        mem_v[...] = mem
        return carry

    with jax.named_scope("main"):
        jax.lax.fori_loop(0, NSEG // UNROLL, steps, 0)

    def epi_rows(r0, n):
        lo = _unpack(o_b[pl.ds(pl.multiple_of(r0 // 2, 8), n // 2), :])
        outs = [_dot(lo, _unpack(wo_v[j])) for j in range(NB)]
        finalize(pl.ds(r0, n), jnp.concatenate(outs, axis=1))

    EB = 128

    def epi(r, carry):
        r0 = pl.multiple_of(S - PRO + r * EB, EB)

        @pl.when(r == PRO // EB - 1)
        def _():
            out_copy(S - PRO, PRO - EB).start()

        epi_rows(r0, EB)
        return carry

    with jax.named_scope("epi"):
        out_copy(0, S - PRO).start()
        jax.lax.fori_loop(0, PRO // EB, epi, 0)
    out_copy(S - EB, EB).start()
    out_copy(0, S).wait()


@jax.jit
def _run(A_q, A_k, A_v, A_shift_k, A_ssm_k, A_ssm_D, B_mem0, B_Wq, B_Wk, B_Wv, B_Wo, gate_w):
    any_spec = pl.BlockSpec(memory_space=pl.ANY)
    out = pl.pallas_call(
        _kernel,
        out_shape=jax.ShapeDtypeStruct((S, D), BF16),
        in_specs=[any_spec] * 14,
        out_specs=any_spec,
        scratch_shapes=[
            pltpu.VMEM((S, D), BF16),
            pltpu.VMEM((PRO // 2, D), U32),
            pltpu.VMEM((NB, NCP, PR, 128), U32),
            pltpu.VMEM((NB, NCP, PR, 128), U32),
            pltpu.VMEM((NB, 128 + 16, S), BF16),
            pltpu.VMEM((3, H // 4, 2, D // 2, E), U32),
            pltpu.VMEM((3, H // 4, 2, D // 2, E), U32),
            pltpu.VMEM((NB, H * E // 2, 128), U32),
            pltpu.VMEM((NB, S + 32, 128), F32),
            pltpu.VMEM((3, H // 2, 2, QCAP // 2, E), U32),
            pltpu.VMEM((S // 2, H * E), U32),
            pltpu.VMEM(((M + RX) // 2, H * E), U32),
            pltpu.VMEM((M, D), BF16),
            pltpu.VMEM((M + RX, D), F32),
            pltpu.VMEM((6, M + RX, E), F32),
            pltpu.VMEM((1, NCH * SR + 2 * C, 128), F32),
            pltpu.VMEM((1, NCH * SR + 2 * C, 128), F32),
            pltpu.VMEM((1, NCH, 2 * C, 128), F32),
            pltpu.VMEM((1, S, 128), F32),
            pltpu.VMEM((1, 2 * S, 128), F32),
            pltpu.VMEM((1, 2 * S, 128), F32),
            pltpu.VMEM((1, NCP * PR, 128), U32),
            pltpu.VMEM((S, D), BF16),
            pltpu.VMEM((C, 2 * C // FOLD), BF16),
            pltpu.VMEM((2 * (SEG + M), 128), F32),
            pltpu.VMEM((KS, D), BF16),
            pltpu.VMEM((NB, 128), BF16),
            pltpu.VMEM((NB, 128), BF16),
            pltpu.SemaphoreType.DMA((7,)),
            pltpu.SemaphoreType.DMA((NB,)),
        ],
        compiler_params=pltpu.CompilerParams(vmem_limit_bytes=120 * 2 ** 20, disable_bounds_checks=True),
    )(
        A_q.reshape(S, D), A_k.reshape(NCH, C, D), A_v.reshape(NCH, C, D), A_ssm_k,
        B_Wq.reshape(D // 2, 2, H, E), B_Wk.reshape(D // 2, 2, H, E), B_Wv.reshape(D // 2, 2, H, E),
        B_Wo.reshape(H * E, D),
        A_shift_k.T, A_ssm_D.reshape(NB, 128), gate_w.reshape(NB, 128), B_mem0.reshape(M, D),
        jnp.asarray(_inv_table(), BF16), jnp.asarray(_attn_fill()),
    )
    return out.reshape(1, S, D)


def pallas_gated_mix__ssm_conv_h3__memory_aug_recurrent_mem_tr__prompt_kernel(
    A_q, A_k, A_v, A_shift_k, A_ssm_k, A_ssm_D, B_x, B_mem0, B_Wq, B_Wk, B_Wv, B_Wo, B_seg_len, gate_w,
):
    del B_x
    if isinstance(B_seg_len, int):
        assert B_seg_len == SEG
    return _run(A_q, A_k, A_v, A_shift_k, A_ssm_k, A_ssm_D, B_mem0, B_Wq, B_Wk, B_Wv, B_Wo, gate_w)
```

```python
import cmath
import functools
import math

import jax
import jax.numpy as jnp
import numpy as np
import jax.experimental.pallas as pl
import jax.experimental.pallas.tpu as pltpu

F32 = jnp.float32
BF16 = jnp.bfloat16
U32 = jnp.uint32

S = 2048
D = 1024
H = 32
E = 128
M = 8
SEG = 32
NSEG = S // SEG
RX = 24
PRO = S - RX * NSEG
QCAP = 576
QOFF = QCAP - PRO
HL = 4
HS = H - HL
OFF_LQK, OFF_S, OFF_LV, OFF_PV = 4, 8, 14, 17
UNROLL = 4
XE = 768
C = 256
NCH = S // C
NB = D // 128
KS = 4
NEG = -1000000000.0
R1, R2 = 16, 16
PR = C // 2 + 8
NCP = NCH + 4
FOLD = 4
SR = 2 * C + 4


def _inv_table():
    n = np.arange(C, dtype=np.float64)
    th = 2.0 * np.pi * (np.arange(C // FOLD, dtype=np.float64) + 0.25) / C
    no = np.concatenate([n[r::FOLD] for r in range(FOLD)])
    inv = np.concatenate([np.cos(no[:, None] * th[None, :]), -np.sin(no[:, None] * th[None, :])], axis=1) / C
    return inv.astype(np.float32)


def _attn_fill():
    n = 2 * (SEG + M)
    head = np.array([0] * SEG + [1] * SEG + [0] * M + [1] * M)
    pos = np.concatenate([M + np.arange(SEG), M + np.arange(SEG), np.arange(M), np.arange(M)])
    fill = np.full((n, 128), -np.inf, np.float32)
    for i in range(n):
        for j in range(n):
            if head[i] == head[j]:
                ok = pos[i] < M or pos[i] >= pos[j]
                fill[i, j] = 0.0 if ok else NEG
    return fill


def _add(a, b):
    return b if a is None else a if b is None else a + b


def _sub(a, b):
    return a if b is None else -b if a is None else a - b


def _cmul(z, w):
    r, i = z
    wr, wi = w.real, w.imag
    eps = 1e-12
    if abs(wi) < eps and abs(wr - 1.0) < eps:
        return z
    if i is None:
        if abs(abs(wr) - abs(wi)) < eps and wr * wi > 0:
            t = r * wr
            return t, t
        return r * wr, r * wi
    if abs(abs(wr) - abs(wi)) < eps:
        if wr * wi > 0:
            return (r - i) * wr, (r + i) * wr
        return (r + i) * wr, (i - r) * wr
    return r * wr - i * wi, r * wi + i * wr


def _fft(xs):
    n = len(xs)
    if n == 1:
        return xs
    if n == 2:
        (ar, ai), (br, bi) = xs
        return [(_add(ar, br), _add(ai, bi)), (_sub(ar, br), _sub(ai, bi))]
    e = _fft(xs[0::2])
    o1 = _fft(xs[1::4])
    o3 = _fft(xs[3::4])
    out = [None] * n
    for k in range(n // 4):
        ar, ai = _cmul(o1[k], cmath.exp(-2j * math.pi * k / n))
        br, bi = _cmul(o3[k], cmath.exp(-6j * math.pi * k / n))
        sr, si, dr, di = _add(ar, br), _add(ai, bi), _sub(ar, br), _sub(ai, bi)
        er, ei = e[k]
        fr, fi = e[k + n // 4]
        out[k] = (_add(er, sr), _add(ei, si))
        out[k + n // 2] = (_sub(er, sr), _sub(ei, si))
        out[k + n // 4] = (_add(fr, di), _sub(fi, dr))
        out[k + 3 * n // 4] = (_sub(fr, di), _add(fi, dr))
    return out


def _dot(a, b):
    return jnp.dot(a, b, preferred_element_type=F32)


def _dot_nt(a, b):
    return jax.lax.dot_general(a, b, (((1,), (1,)), ((), ())), preferred_element_type=F32)


def _pack(a):
    return pltpu.bitcast(a.astype(BF16), U32)


def _unpack(a):
    return pltpu.bitcast(a, BF16)


def _kernel(x_hbm, k_hbm, v_hbm, h_hbm, wq_hbm, wk_hbm, wv_hbm, wo_hbm,
            sk_hbm, dd_hbm, gw_hbm, mem0_hbm, inv_hbm, fill_hbm,
            out_hbm,
            x_v, xp, k_v, v_v, h_v, w_even, w_odd, wo_v, y_v, qkv_b, left, lo_s, mem_v, oacc, qacc,
            u_s, h_s, yf_s, t_s, gu_s, gh_s, ht_s,
            out_v, inv_ref, fill_ref, sk_ref, dd_ref, gw_ref, sems, qsems):
    scale = E ** (-0.5)
    wbuf = (w_even, w_odd)

    w32 = [w.bitcast(U32) for w in (wq_hbm, wk_hbm, wv_hbm)]
    wo32 = wo_hbm.bitcast(U32)
    x32 = x_hbm.bitcast(U32)
    k32 = k_hbm.bitcast(U32)
    v32 = v_hbm.bitcast(U32)

    def lanes(c):
        return pl.ds(pl.multiple_of(c * 128, 128), 128)

    def w_copies(c, e, mat, sem):
        return [pltpu.make_async_copy(w32[mat].at[:, par, 2 * c + e, :], wbuf[e].at[mat, c, par], sem)
                for par in range(2)]

    def wq0_copies(c):
        return w_copies(c, 0, 0, qsems.at[c])

    W_REST = [(e, mat) for e in range(2) for mat in range(3) if (e, mat) != (0, 0)]
    NPIECE = 3 + len(W_REST)

    def block_piece(c, i):
        sem = sems.at[c % 2]
        if i < 2:
            src, dst = ((k32, k_v), (v32, v_v))[i]
            return [pltpu.make_async_copy(src.at[:, :, lanes(c)], dst.at[c, pl.ds(0, NCH), pl.ds(0, C // 2), :], sem)]
        if i == 2:
            return [pltpu.make_async_copy(h_hbm.at[lanes(c), :], h_v.at[c, pl.ds(0, 128), :], sem)]
        return w_copies(c, *W_REST[i - 3], sem)

    def wo_copy(c):
        return pltpu.make_async_copy(wo32.at[:, lanes(c)], wo_v.at[c], sems.at[2])

    x_early = pltpu.make_async_copy(x_hbm.at[pl.ds(0, XE), :], x_v.at[pl.ds(0, XE), :], sems.at[2])
    x_late = pltpu.make_async_copy(x_hbm.at[pl.ds(XE, S - XE), :], x_v.at[pl.ds(XE, S - XE), :], sems.at[3])

    xp_copies = [pltpu.make_async_copy(x32.at[pl.ds(i * PRO // 4, PRO // 4), :], xp.at[pl.ds(i * PRO // 4, PRO // 4), :],
                                       sems.at[3 + 3 * i]) for i in range(2)]
    small_copies = [pltpu.make_async_copy(src, dst, sems.at[4]) for src, dst in (
        (sk_hbm, sk_ref), (dd_hbm, dd_ref), (inv_hbm, inv_ref),
        (gw_hbm, gw_ref), (mem0_hbm, mem_v), (fill_hbm, fill_ref))]

    def out_copy(start, n):
        rows = pl.ds(start, n)
        return pltpu.make_async_copy(out_v.at[rows, :], out_hbm.at[rows, :], sems.at[5])

    def row_of(ref, c):
        t = ref[...].astype(F32)
        sel = jax.lax.broadcasted_iota(jnp.int32, (NB, 128), 0) == c
        return jnp.sum(jnp.where(sel, t, 0.0), axis=0, keepdims=True)

    k2 = k_v.reshape(NB, NCP * PR, 128)
    v2 = v_v.reshape(NB, NCP * PR, 128)

    def word(ref, c, pr):
        return ref[c, pl.ds(pr, NCH, stride=PR), :]

    def lo16(w):
        return pltpu.bitcast(w << 16, F32)

    def hi16(w):
        return pltpu.bitcast(w & U32(0xFFFF0000), F32)

    def pair(ref, c, pr):
        w = word(ref, c, pr)
        return lo16(w), hi16(w)

    first = jax.lax.broadcasted_iota(jnp.int32, (8, 128), 0) == 0

    def kv_prep(c, zw):
        skt = sk_ref[:, lanes(c)].astype(F32)
        sk = [jnp.broadcast_to(skt[j:j + 1, :], (8, 128)) for j in range(KS)]
        tail = (pair(k2, c, C // 2 - 2) + pair(k2, c, C // 2 - 1))[1:]
        win = [jnp.where(first, 0.0, pltpu.roll(t, 1, 0)) for t in tail]
        for pr in range(C // 2):
            ks = pair(k2, c, pr)
            vs = pair(v2, c, pr)
            for i in range(2):
                win.append(ks[i])
                acc = win[-1] * sk[0]
                for j in range(1, KS):
                    acc = acc + win[-1 - j] * sk[j]
                win = win[1:]
                t_s[zw, pl.ds((2 * pr + i) * 8, 8), :] = acc * vs[i]

    def h_prep(c, zw):
        for t in range(S // 128):
            ht = pltpu.bitcast(h_v[c, 0:128, pl.ds(t * 128, 128)].T, U32)
            ht_s[zw, pl.ds(t * 64 // (C // 2) * PR + t * 64 % (C // 2), 64), :] = ht

    def fft1(sample, mid, zw):
        for b in range(R2):
            z = [_cmul((sample(R2 * a + b), None), cmath.exp(-0.5j * math.pi * a / R1)) for a in range(R1)]
            gq = _fft(z)
            for q1 in range(R1):
                re, im = _cmul(gq[q1], cmath.exp(-2j * math.pi * (q1 + 0.25) * b / C))
                row = (q1 * R2 + b) * 16
                mid[zw, pl.ds(row, 8), :] = re
                mid[zw, pl.ds(row + 8, 8), :] = im

    def fft2(mid, dst, zw, zr):
        for q1 in range(R1):
            z = []
            for b in range(R2):
                row = (q1 * R2 + b) * 16
                z.append((mid[zr, pl.ds(row, 8), :], mid[zr, pl.ds(row + 8, 8), :]))
            t = _fft(z)
            for q2 in range(R2):
                q = q1 + R1 * q2
                dst[zw, pl.ds(q, NCH, stride=SR), :] = t[q2][0]
                dst[zw, pl.ds(C + q, NCH, stride=SR), :] = t[q2][1]

    def mac(p, zw, zr):
        re = pl.ds(p * 8, 8)
        im = pl.ds(C + p * 8, 8)
        AB = 4
        prev = None
        for a0 in range(0, NCH, AB):
            zre = [None] * AB
            zim = [None] * AB
            for m in range(a0 + AB):
                hr = h_s[zr, pl.ds(m * SR + p * 8, 8), :]
                hi = h_s[zr, pl.ds(m * SR + C + p * 8, 8), :]
                for i in range(AB):
                    t = a0 + i - m
                    if t < 0:
                        continue
                    ur = u_s[zr, pl.ds(t * SR + p * 8, 8), :]
                    ui = u_s[zr, pl.ds(t * SR + C + p * 8, 8), :]
                    tr = hr * ur - hi * ui
                    ti = hr * ui + hi * ur
                    zre[i] = tr if zre[i] is None else zre[i] + tr
                    zim[i] = ti if zim[i] is None else zim[i] + ti
            for i in range(AB):
                if prev is None:
                    yf_s[zw, a0 + i, re, :] = zre[i]
                    yf_s[zw, a0 + i, im, :] = zim[i]
                else:
                    yf_s[zw, a0 + i, re, :] = zre[i] - prev[1]
                    yf_s[zw, a0 + i, im, :] = zim[i] + prev[0]
                prev = (zre[i], zim[i])

    def inv_dft(c, zr):
        qc = C // FOLD
        for a in range(NCH):
            yr = [yf_s[zr, a, j * qc:(j + 1) * qc, :] for j in range(FOLD)]
            yi = [yf_s[zr, a, C + j * qc:C + (j + 1) * qc, :] for j in range(FOLD)]
            sr, si, dr, di = yr[0] + yr[2], yi[0] + yi[2], yr[0] - yr[2], yi[0] - yi[2]
            tr, ti, er, ei = yr[1] + yr[3], yi[1] + yi[3], yr[1] - yr[3], yi[1] - yi[3]
            folded = [(sr + tr, si + ti), (dr - ei, di + er), (sr - tr, si - ti), (dr + ei, di - er)]
            for r in range(FOLD):
                f = jnp.concatenate(folded[r], axis=0).astype(BF16)
                y_v[c, pl.ds(a * C + r, qc, stride=FOLD), :] = _dot(inv_ref[r * qc:(r + 1) * qc, :], f)

    def fixup(e, c, mat):
        a = wbuf[e][mat, c, 0]
        b = wbuf[e][mat, c, 1]
        wbuf[e][mat, c, 0] = (a & U32(0xFFFF)) | (b << 16)
        wbuf[e][mat, c, 1] = (a >> 16) | (b & U32(0xFFFF0000))

    RB = 128

    def qkv_tile(e, c, n, hook=None, rs=range(PRO // RB)):
        mat, j = n // 2, n % 2
        for r in rs:
            w = _unpack(wbuf[e][mat, c, j])
            xr = _unpack(xp[pl.ds(r * RB // 2, RB // 2), :])
            pk = _pack(_dot(xr, w))
            qkv_b[mat, 2 * c + e, j, pl.ds((QOFF + r * RB) // 2, RB // 2), :] = pk
            if hook is not None and r == 0:
                hook(pk[0:8])

    def start_when(cond, copies):
        @pl.when(cond)
        def _():
            for cp in copies:
                cp.start()

    def wq0_tiles(c, rs=range(PRO // RB)):
        qkv_tile(0, c, 0, rs=rs)
        qkv_tile(0, c, 1, rs=rs)

    for cp in wq0_copies(0) + xp_copies + wq0_copies(1):
        cp.start()
    for cp in wq0_copies(0) + xp_copies[:1]:
        cp.wait()
    fixup(0, 0, 0)
    wq0_tiles(0, range(2))
    for cp in wq0_copies(2) + wq0_copies(3):
        cp.start()
    xp_copies[1].wait()
    wq0_tiles(0, range(2, 4))
    for cp in small_copies + block_piece(0, 0):
        cp.start()
    for cp in wq0_copies(1):
        cp.wait()
    fixup(0, 1, 0)
    wq0_tiles(1)
    for cp in wq0_copies(4) + wq0_copies(5) + block_piece(0, 2) + block_piece(0, 1):
        cp.start()

    def pro0(i, carry):
        for u in range(2):
            for cp in wq0_copies(2 * i + u):
                cp.wait()
        for u in range(2):
            fixup(0, 2 * i + u, 0)
            wq0_tiles(2 * i + u)
        start_when(i == 1, wq0_copies(6) + wq0_copies(7))
        for j in range(3, NPIECE):
            start_when(i == (1 if j < 5 else 2), block_piece(0, j))
        return carry

    with jax.named_scope("pro0"):
        jax.lax.fori_loop(1, NB // 2, pro0, 0)
    for i in range(2, NPIECE):
        for cp in block_piece(1, i):
            cp.start()
    for cp in small_copies:
        cp.wait()

    def pro(c, carry):
        zw = c >> 3
        zr = c >> 4
        for i in range(2):
            start_when(c + 1 < NB, block_piece(jnp.minimum(c + 1, NB - 1), i))
        for i in range(NPIECE):
            for cp in block_piece(c, i):
                cp.wait()

        tiles = [(0, n) for n in range(2, 6)] + [(1, n) for n in range(6)]

        def tile(i, hook=None):
            e, n = tiles[i]
            if n % 2 == 0:
                fixup(e, c, n // 2)
            qkv_tile(e, c, n, hook=hook)

        def trigger(val):
            k2[c + zw, pl.ds(C // 2, 8), :] = val
            v2[c + zw, pl.ds(C // 2, 8), :] = val
            h_v[c + zw, pl.ds(128, 16), 0:128] = _unpack(val)

        def h_sample(n):
            w = word(ht_s, zr, n // 2)
            hv = hi16(w) if n % 2 else lo16(w)
            if n == 0:
                hv = hv + jnp.where(first, row_of(dd_ref, c), 0.0)
            return hv

        tile(0, trigger)
        h_prep(c, zw)
        kv_prep(c, zw)
        fft1(lambda n: t_s[zr, pl.ds(n * 8, 8), :], gu_s, zw)
        fft2(gu_s, u_s, zw, zr)
        fft1(h_sample, gh_s, zw)
        fft2(gh_s, h_s, zw, zr)
        for i in range(1, 9):
            for p in range(4 * i - 4, 4 * i):
                mac(p, zw, zr)
            tile(i)
        tile(9)
        inv_dft(c, zr)
        for i in range(2, NPIECE):
            start_when(c + 2 < NB, block_piece(jnp.minimum(c + 2, NB - 1), i))
        start_when(c + 1 < NB, [wo_copy(c)])
        start_when(c + 2 == NB, [wo_copy(NB - 1), x_early])
        return carry

    with jax.named_scope("pro"):
        jax.lax.fori_loop(0, NB, pro, 0)
    x_late.start()
    x_early.wait()
    for c in range(NB):
        wo_copy(c).wait()

    gwt = gw_ref[...].astype(F32)
    gw = jnp.concatenate([gwt[j:j + 1, :] for j in range(NB)], axis=1)

    def finalize(rows, b):
        xr = x_v[rows, :].astype(F32)
        g = jax.nn.sigmoid(jnp.sum(xr * gw, axis=-1, keepdims=True))
        a = xr * jnp.concatenate([y_v[j, rows, :] for j in range(NB)], axis=1)
        out_v[rows, :] = (g * a + (1.0 - g) * b).astype(BF16)

    def step(s, mem, split_first, odd):
        mrows = slice(0, M) if odd else slice(RX, RX + M)
        sh = 4 if odd else 0
        xo = pl.multiple_of(PRO + RX * s, 8)
        wbase = pl.multiple_of((RX // 2 * s) % (QCAP // 2) - sh, 8)
        rpos = pl.multiple_of((SEG // 2 * s + QOFF // 2) % (QCAP // 2), SEG // 2)
        xs = x_v[pl.ds(xo, RX), :]
        lhs = jnp.concatenate([mem, xs] if odd else [xs, mem], axis=0)
        zpad = jnp.zeros((128 - 2 * (SEG + M), E), BF16)
        no = SEG + M if odd else RX
        frows = pl.ds(pl.multiple_of(SEG * s - (M if odd else 0), 8), no)
        orows = slice(M, M + no) if odd else slice(0, no)
        omrows = slice(0, M) if odd else slice(no, no + M)
        low = jax.lax.broadcasted_iota(jnp.int32, (8, E), 0) < 4
        NP = H // 2

        mem_qkv = {}
        probs = {}
        cats = {}

        def load(mat, hp):
            parts = [_unpack(qkv_b[mat, hp, 0, pl.ds(rpos, SEG // 2), :]),
                     _unpack(qkv_b[mat, hp, 1, pl.ds(rpos, SEG // 2), :]), mem_qkv[(hp, mat)]]
            if mat > 0:
                parts.append(zpad)
            cats[(mat, hp)] = jnp.concatenate(parts, axis=0)

        def stage_a(hp):
            KH = D // 2
            split = split_first and hp == 0
            if split:
                for mat in range(3):
                    for j in range(2):
                        w = _unpack(wbuf[hp % 2][mat, hp // 2, j, :KH // 2, :])
                        qacc[2 * mat + j] = _dot(lhs[:, :KH], w)
            for mat in range(3):
                mm = []
                for j in range(2):
                    if split:
                        w = _unpack(wbuf[hp % 2][mat, hp // 2, j, KH // 2:, :])
                        res = qacc[2 * mat + j] + _dot(lhs[:, KH:], w)
                    else:
                        res = _dot(lhs, _unpack(wbuf[hp % 2][mat, hp // 2, j]))
                    pk = _pack(res)
                    if odd:
                        qkv_b[mat, hp, j, pl.ds(wbase + 4, 4), :] = pk[4:8]
                        qkv_b[mat, hp, j, pl.ds(wbase + 8, 8), :] = pk[8:16]
                    else:
                        qkv_b[mat, hp, j, pl.ds(wbase, 8), :] = pk[0:8]
                        qkv_b[mat, hp, j, pl.ds(wbase + 8, 4), :] = pk[8:12]
                    mm.append(res[mrows])
                    if j == 1:
                        mem_qkv[(hp, mat)] = jnp.concatenate(mm, axis=0).astype(BF16)
                    advance(6 * hp + 2 * mat + j + 1)

        def stage_b(hp):
            sc = _dot_nt(cats[(0, hp)], cats[(1, hp)]) * scale
            fill = fill_ref[...]
            sc = jnp.where(fill == 0.0, sc, fill)
            mx = jnp.max(sc, axis=-1, keepdims=True)
            p = jnp.exp(sc - mx)
            l = jnp.sum(p, axis=-1, keepdims=True)
            r = pl.reciprocal(l, approx=True)
            r = r * (2.0 - l * r)
            probs[hp] = (p * r).astype(BF16)

        def stage_c(hp):
            o = _dot(probs[hp], cats[(2, hp)])
            for j in range(2):
                h = 2 * hp + j
                cols = slice(h * E, (h + 1) * E)
                ox = _pack(o[j * SEG:(j + 1) * SEG])
                om = o[2 * SEG + j * M:2 * SEG + (j + 1) * M]
                om = _pack(jnp.concatenate([om, om], axis=0))
                if odd:
                    lo_s[0:8, cols] = jnp.where(low, om, left[:, cols])
                    lo_s[8:24, cols] = ox
                else:
                    lo_s[0:8, cols] = ox[0:8]
                    lo_s[8:16, cols] = jnp.where(low, ox[8:16], om)
                    left[:, cols] = ox[8:16]

        def oproj(j, late):
            ks = slice(HS * E, H * E) if late else slice(0, HS * E)
            kw = slice(ks.start // 2, ks.stop // 2)
            return _dot(_unpack(lo_s[0:(no + M) // 2, ks]), _unpack(wo_v[j, kw, :]))

        events = []
        for hp in range(NP):
            events.append((6 * hp + OFF_LQK, 0, functools.partial(load, 0, hp)))
            events.append((6 * hp + OFF_LQK, 1, functools.partial(load, 1, hp)))
            events.append((6 * hp + OFF_LV, 2, functools.partial(load, 2, hp)))
            events.append((6 * hp + OFF_PV, 3, functools.partial(stage_c, hp)))
            events.append((6 * hp + OFF_S, 4, functools.partial(stage_b, hp)))
        events.sort(key=lambda ev: ev[:2])

        def advance(slot):
            while events and events[0][0] <= slot:
                events.pop(0)[2]()

        outs = [None] * NB
        for hp in range(NP):
            stage_a(hp)
        for j in range(NB):
            oacc[0:no + M, j * 128:(j + 1) * 128] = oproj(j, False)
            advance(6 * NP + (j + 1) * HS // 8)
        assert not events
        for j in range(NB):
            outs[j] = oacc[0:no + M, j * 128:(j + 1) * 128] + oproj(j, True)
        res = jnp.concatenate(outs, axis=1)
        finalize(frows, res[orows])
        return res[omrows].astype(BF16)

    def steps(i, carry):
        @pl.when(i == (XE - PRO) // (RX * UNROLL))
        def _():
            x_late.wait()

        OB = SEG * UNROLL
        start_when(i > 0, [out_copy(pl.multiple_of(jnp.maximum(i - 1, 0) * OB, OB), OB)])
        mem = mem_v[...]
        for u in range(UNROLL):
            mem = step(i * UNROLL + u, mem, u > 0, u % 2 == 1)
        mem_v[...] = mem
        return carry

    with jax.named_scope("main"):
        jax.lax.fori_loop(0, NSEG // UNROLL, steps, 0)

    out_copy(S - SEG * UNROLL, SEG * UNROLL).start()
    out_copy(0, S).wait()


@jax.jit
def _run(A_q, A_k, A_v, A_shift_k, A_ssm_k, A_ssm_D, B_mem0, B_Wq, B_Wk, B_Wv, B_Wo, gate_w):
    any_spec = pl.BlockSpec(memory_space=pl.ANY)
    out = pl.pallas_call(
        _kernel,
        out_shape=jax.ShapeDtypeStruct((S, D), BF16),
        in_specs=[any_spec] * 14,
        out_specs=any_spec,
        scratch_shapes=[
            pltpu.VMEM((S, D), BF16),
            pltpu.VMEM((PRO // 2, D), U32),
            pltpu.VMEM((NB, NCP, PR, 128), U32),
            pltpu.VMEM((NB, NCP, PR, 128), U32),
            pltpu.VMEM((NB, 128 + 16, S), BF16),
            pltpu.VMEM((3, H // 4, 2, D // 2, E), U32),
            pltpu.VMEM((3, H // 4, 2, D // 2, E), U32),
            pltpu.VMEM((NB, H * E // 2, 128), U32),
            pltpu.VMEM((NB, S + 32, 128), F32),
            pltpu.VMEM((3, H // 2, 2, QCAP // 2, E), U32),
            pltpu.VMEM((8, H * E), U32),
            pltpu.VMEM((24, H * E), U32),
            pltpu.VMEM((M, D), BF16),
            pltpu.VMEM((48, D), F32),
            pltpu.VMEM((6, M + RX, E), F32),
            pltpu.VMEM((1, NCH * SR + 2 * C, 128), F32),
            pltpu.VMEM((1, NCH * SR + 2 * C, 128), F32),
            pltpu.VMEM((1, NCH, 2 * C, 128), F32),
            pltpu.VMEM((1, S, 128), F32),
            pltpu.VMEM((1, 2 * S, 128), F32),
            pltpu.VMEM((1, 2 * S, 128), F32),
            pltpu.VMEM((1, NCP * PR, 128), U32),
            pltpu.VMEM((S, D), BF16),
            pltpu.VMEM((C, 2 * C // FOLD), BF16),
            pltpu.VMEM((2 * (SEG + M), 128), F32),
            pltpu.VMEM((KS, D), BF16),
            pltpu.VMEM((NB, 128), BF16),
            pltpu.VMEM((NB, 128), BF16),
            pltpu.SemaphoreType.DMA((7,)),
            pltpu.SemaphoreType.DMA((NB,)),
        ],
        compiler_params=pltpu.CompilerParams(vmem_limit_bytes=120 * 2 ** 20, disable_bounds_checks=True),
    )(
        A_q.reshape(S, D), A_k.reshape(NCH, C, D), A_v.reshape(NCH, C, D), A_ssm_k,
        B_Wq.reshape(D // 2, 2, H, E), B_Wk.reshape(D // 2, 2, H, E), B_Wv.reshape(D // 2, 2, H, E),
        B_Wo.reshape(H * E, D),
        A_shift_k.T, A_ssm_D.reshape(NB, 128), gate_w.reshape(NB, 128), B_mem0.reshape(M, D),
        jnp.asarray(_inv_table(), BF16), jnp.asarray(_attn_fill()),
    )
    return out.reshape(1, S, D)


def pallas_gated_mix__ssm_conv_h3__memory_aug_recurrent_mem_tr__prompt_kernel(
    A_q, A_k, A_v, A_shift_k, A_ssm_k, A_ssm_D, B_x, B_mem0, B_Wq, B_Wk, B_Wv, B_Wo, B_seg_len, gate_w,
):
    del B_x
    if isinstance(B_seg_len, int):
        assert B_seg_len == SEG
    return _run(A_q, A_k, A_v, A_shift_k, A_ssm_k, A_ssm_D, B_mem0, B_Wq, B_Wk, B_Wv, B_Wo, gate_w)
```

```python
import cmath
import functools
import math

import jax
import jax.numpy as jnp
import numpy as np
import jax.experimental.pallas as pl
import jax.experimental.pallas.tpu as pltpu

F32 = jnp.float32
BF16 = jnp.bfloat16
U32 = jnp.uint32

S = 2048
D = 1024
H = 32
E = 128
M = 8
SEG = 32
NSEG = S // SEG
RX = 24
PRO = S - RX * NSEG
QCAP = 576
QOFF = QCAP - PRO
HL = 4
HS = H - HL
OFF_LQK, OFF_S, OFF_LV, OFF_PV = 4, 8, 14, 17
UNROLL = 4
LASTR = SEG + M
XE = 768
C = 256
NCH = S // C
NB = D // 128
KS = 4
NEG = -1000000000.0
R1, R2 = 16, 16
PR = C // 2 + 8
NCP = NCH + 4
FOLD = 4
SR = 2 * C + 4


def _inv_table():
    n = np.arange(C, dtype=np.float64)
    th = 2.0 * np.pi * (np.arange(C // FOLD, dtype=np.float64) + 0.25) / C
    no = np.concatenate([n[r::FOLD] for r in range(FOLD)])
    inv = np.concatenate([np.cos(no[:, None] * th[None, :]), -np.sin(no[:, None] * th[None, :])], axis=1) / C
    return inv.astype(np.float32)


def _attn_fill():
    n = 2 * (SEG + M)
    head = np.array([0] * SEG + [1] * SEG + [0] * M + [1] * M)
    pos = np.concatenate([M + np.arange(SEG), M + np.arange(SEG), np.arange(M), np.arange(M)])
    fill = np.full((n, 128), -np.inf, np.float32)
    for i in range(n):
        for j in range(n):
            if head[i] == head[j]:
                ok = pos[i] < M or pos[i] >= pos[j]
                fill[i, j] = 0.0 if ok else NEG
    return fill


def _add(a, b):
    return b if a is None else a if b is None else a + b


def _sub(a, b):
    return a if b is None else -b if a is None else a - b


def _cmul(z, w):
    r, i = z
    wr, wi = w.real, w.imag
    eps = 1e-12
    if abs(wi) < eps and abs(wr - 1.0) < eps:
        return z
    if i is None:
        if abs(abs(wr) - abs(wi)) < eps and wr * wi > 0:
            t = r * wr
            return t, t
        return r * wr, r * wi
    if abs(abs(wr) - abs(wi)) < eps:
        if wr * wi > 0:
            return (r - i) * wr, (r + i) * wr
        return (r + i) * wr, (i - r) * wr
    return r * wr - i * wi, r * wi + i * wr


def _fft(xs):
    n = len(xs)
    if n == 1:
        return xs
    if n == 2:
        (ar, ai), (br, bi) = xs
        return [(_add(ar, br), _add(ai, bi)), (_sub(ar, br), _sub(ai, bi))]
    e = _fft(xs[0::2])
    o1 = _fft(xs[1::4])
    o3 = _fft(xs[3::4])
    out = [None] * n
    for k in range(n // 4):
        ar, ai = _cmul(o1[k], cmath.exp(-2j * math.pi * k / n))
        br, bi = _cmul(o3[k], cmath.exp(-6j * math.pi * k / n))
        sr, si, dr, di = _add(ar, br), _add(ai, bi), _sub(ar, br), _sub(ai, bi)
        er, ei = e[k]
        fr, fi = e[k + n // 4]
        out[k] = (_add(er, sr), _add(ei, si))
        out[k + n // 2] = (_sub(er, sr), _sub(ei, si))
        out[k + n // 4] = (_add(fr, di), _sub(fi, dr))
        out[k + 3 * n // 4] = (_sub(fr, di), _add(fi, dr))
    return out


def _dot(a, b):
    return jnp.dot(a, b, preferred_element_type=F32)


def _dot_nt(a, b):
    return jax.lax.dot_general(a, b, (((1,), (1,)), ((), ())), preferred_element_type=F32)


def _pack(a):
    return pltpu.bitcast(a.astype(BF16), U32)


def _unpack(a):
    return pltpu.bitcast(a, BF16)


def _kernel(x_hbm, k_hbm, v_hbm, h_hbm, wq_hbm, wk_hbm, wv_hbm, wo_hbm,
            sk_hbm, dd_hbm, gw_hbm, mem0_hbm, inv_hbm, fill_hbm,
            out_hbm,
            x_v, xp, k_v, v_v, h_v, w_even, w_odd, wo_v, y_v, qkv_b, left, lo_s, mem_v, oacc, qacc,
            u_s, h_s, yf_s, t_s, gu_s, gh_s, ht_s,
            out_v, inv_ref, fill_ref, sk_ref, dd_ref, gw_ref, sems, qsems):
    scale = E ** (-0.5)
    wbuf = (w_even, w_odd)

    w32 = [w.bitcast(U32) for w in (wq_hbm, wk_hbm, wv_hbm)]
    wo32 = wo_hbm.bitcast(U32)
    x32 = x_hbm.bitcast(U32)
    k32 = k_hbm.bitcast(U32)
    v32 = v_hbm.bitcast(U32)

    def lanes(c):
        return pl.ds(pl.multiple_of(c * 128, 128), 128)

    def w_copies(c, e, mat, sem):
        return [pltpu.make_async_copy(w32[mat].at[:, par, 2 * c + e, :], wbuf[e].at[mat, c, par], sem)
                for par in range(2)]

    def wq0_copies(c):
        return w_copies(c, 0, 0, qsems.at[c])

    W_REST = [(e, mat) for e in range(2) for mat in range(3) if (e, mat) != (0, 0)]
    NPIECE = 3 + len(W_REST)

    def block_piece(c, i):
        sem = sems.at[c % 2]
        if i < 2:
            src, dst = ((k32, k_v), (v32, v_v))[i]
            return [pltpu.make_async_copy(src.at[:, :, lanes(c)], dst.at[c, pl.ds(0, NCH), pl.ds(0, C // 2), :], sem)]
        if i == 2:
            return [pltpu.make_async_copy(h_hbm.at[lanes(c), :], h_v.at[c, pl.ds(0, 128), :], sem)]
        return w_copies(c, *W_REST[i - 3], sem)

    def wo_copy(c):
        return pltpu.make_async_copy(wo32.at[:, lanes(c)], wo_v.at[c], sems.at[2])

    x_early = pltpu.make_async_copy(x_hbm.at[pl.ds(0, XE), :], x_v.at[pl.ds(0, XE), :], sems.at[2])
    x_late = pltpu.make_async_copy(x_hbm.at[pl.ds(XE, S - XE), :], x_v.at[pl.ds(XE, S - XE), :], sems.at[3])

    xp_copies = [pltpu.make_async_copy(x32.at[pl.ds(i * PRO // 4, PRO // 4), :], xp.at[pl.ds(i * PRO // 4, PRO // 4), :],
                                       sems.at[3 + 3 * i]) for i in range(2)]
    small_copies = [pltpu.make_async_copy(src, dst, sems.at[4]) for src, dst in (
        (sk_hbm, sk_ref), (dd_hbm, dd_ref), (inv_hbm, inv_ref),
        (gw_hbm, gw_ref), (mem0_hbm, mem_v), (fill_hbm, fill_ref))]

    def out_copy(start, n):
        rows = pl.ds(start, n)
        return pltpu.make_async_copy(out_v.at[rows, :], out_hbm.at[rows, :], sems.at[5])

    def row_of(ref, c):
        t = ref[...].astype(F32)
        sel = jax.lax.broadcasted_iota(jnp.int32, (NB, 128), 0) == c
        return jnp.sum(jnp.where(sel, t, 0.0), axis=0, keepdims=True)

    k2 = k_v.reshape(NB, NCP * PR, 128)
    v2 = v_v.reshape(NB, NCP * PR, 128)

    def word(ref, c, pr):
        return ref[c, pl.ds(pr, NCH, stride=PR), :]

    def lo16(w):
        return pltpu.bitcast(w << 16, F32)

    def hi16(w):
        return pltpu.bitcast(w & U32(0xFFFF0000), F32)

    def pair(ref, c, pr):
        w = word(ref, c, pr)
        return lo16(w), hi16(w)

    first = jax.lax.broadcasted_iota(jnp.int32, (8, 128), 0) == 0

    def kv_prep(c, zw):
        skt = sk_ref[:, lanes(c)].astype(F32)
        sk = [jnp.broadcast_to(skt[j:j + 1, :], (8, 128)) for j in range(KS)]
        tail = (pair(k2, c, C // 2 - 2) + pair(k2, c, C // 2 - 1))[1:]
        win = [jnp.where(first, 0.0, pltpu.roll(t, 1, 0)) for t in tail]
        for pr in range(C // 2):
            ks = pair(k2, c, pr)
            vs = pair(v2, c, pr)
            for i in range(2):
                win.append(ks[i])
                acc = win[-1] * sk[0]
                for j in range(1, KS):
                    acc = acc + win[-1 - j] * sk[j]
                win = win[1:]
                t_s[zw, pl.ds((2 * pr + i) * 8, 8), :] = acc * vs[i]

    def h_prep(c, zw):
        for t in range(S // 128):
            ht = pltpu.bitcast(h_v[c, 0:128, pl.ds(t * 128, 128)].T, U32)
            ht_s[zw, pl.ds(t * 64 // (C // 2) * PR + t * 64 % (C // 2), 64), :] = ht

    def fft1(sample, mid, zw):
        for b in range(R2):
            z = [_cmul((sample(R2 * a + b), None), cmath.exp(-0.5j * math.pi * a / R1)) for a in range(R1)]
            gq = _fft(z)
            for q1 in range(R1):
                re, im = _cmul(gq[q1], cmath.exp(-2j * math.pi * (q1 + 0.25) * b / C))
                row = (q1 * R2 + b) * 16
                mid[zw, pl.ds(row, 8), :] = re
                mid[zw, pl.ds(row + 8, 8), :] = im

    def fft2(mid, dst, zw, zr):
        for q1 in range(R1):
            z = []
            for b in range(R2):
                row = (q1 * R2 + b) * 16
                z.append((mid[zr, pl.ds(row, 8), :], mid[zr, pl.ds(row + 8, 8), :]))
            t = _fft(z)
            for q2 in range(R2):
                q = q1 + R1 * q2
                dst[zw, pl.ds(q, NCH, stride=SR), :] = t[q2][0]
                dst[zw, pl.ds(C + q, NCH, stride=SR), :] = t[q2][1]

    def mac(p, zw, zr):
        re = pl.ds(p * 8, 8)
        im = pl.ds(C + p * 8, 8)
        AB = 4
        prev = None
        for a0 in range(0, NCH, AB):
            zre = [None] * AB
            zim = [None] * AB
            for m in range(a0 + AB):
                hr = h_s[zr, pl.ds(m * SR + p * 8, 8), :]
                hi = h_s[zr, pl.ds(m * SR + C + p * 8, 8), :]
                for i in range(AB):
                    t = a0 + i - m
                    if t < 0:
                        continue
                    ur = u_s[zr, pl.ds(t * SR + p * 8, 8), :]
                    ui = u_s[zr, pl.ds(t * SR + C + p * 8, 8), :]
                    tr = hr * ur - hi * ui
                    ti = hr * ui + hi * ur
                    zre[i] = tr if zre[i] is None else zre[i] + tr
                    zim[i] = ti if zim[i] is None else zim[i] + ti
            for i in range(AB):
                if prev is None:
                    yf_s[zw, a0 + i, re, :] = zre[i]
                    yf_s[zw, a0 + i, im, :] = zim[i]
                else:
                    yf_s[zw, a0 + i, re, :] = zre[i] - prev[1]
                    yf_s[zw, a0 + i, im, :] = zim[i] + prev[0]
                prev = (zre[i], zim[i])

    def inv_dft(c, zr):
        qc = C // FOLD
        for a in range(NCH):
            yr = [yf_s[zr, a, j * qc:(j + 1) * qc, :] for j in range(FOLD)]
            yi = [yf_s[zr, a, C + j * qc:C + (j + 1) * qc, :] for j in range(FOLD)]
            sr, si, dr, di = yr[0] + yr[2], yi[0] + yi[2], yr[0] - yr[2], yi[0] - yi[2]
            tr, ti, er, ei = yr[1] + yr[3], yi[1] + yi[3], yr[1] - yr[3], yi[1] - yi[3]
            folded = [(sr + tr, si + ti), (dr - ei, di + er), (sr - tr, si - ti), (dr + ei, di - er)]
            for r in range(FOLD):
                f = jnp.concatenate(folded[r], axis=0).astype(BF16)
                y_v[c, pl.ds(a * C + r, qc, stride=FOLD), :] = _dot(inv_ref[r * qc:(r + 1) * qc, :], f)

    def fixup(e, c, mat):
        a = wbuf[e][mat, c, 0]
        b = wbuf[e][mat, c, 1]
        wbuf[e][mat, c, 0] = (a & U32(0xFFFF)) | (b << 16)
        wbuf[e][mat, c, 1] = (a >> 16) | (b & U32(0xFFFF0000))

    RB = 128

    def qkv_tile(e, c, n, hook=None, rs=range(PRO // RB)):
        mat, j = n // 2, n % 2
        for r in rs:
            w = _unpack(wbuf[e][mat, c, j])
            xr = _unpack(xp[pl.ds(r * RB // 2, RB // 2), :])
            pk = _pack(_dot(xr, w))
            qkv_b[mat, 2 * c + e, j, pl.ds((QOFF + r * RB) // 2, RB // 2), :] = pk
            if hook is not None and r == 0:
                hook(pk[0:8])

    def start_when(cond, copies):
        @pl.when(cond)
        def _():
            for cp in copies:
                cp.start()

    def wq0_tiles(c, rs=range(PRO // RB)):
        qkv_tile(0, c, 0, rs=rs)
        qkv_tile(0, c, 1, rs=rs)

    for cp in wq0_copies(0) + xp_copies + wq0_copies(1):
        cp.start()
    for cp in wq0_copies(0) + xp_copies[:1]:
        cp.wait()
    fixup(0, 0, 0)
    wq0_tiles(0, range(2))
    for cp in wq0_copies(2) + wq0_copies(3):
        cp.start()
    xp_copies[1].wait()
    wq0_tiles(0, range(2, 4))
    for cp in small_copies + block_piece(0, 0):
        cp.start()
    for cp in wq0_copies(1):
        cp.wait()
    fixup(0, 1, 0)
    wq0_tiles(1)
    for cp in wq0_copies(4) + wq0_copies(5) + block_piece(0, 2) + block_piece(0, 1):
        cp.start()

    def pro0(i, carry):
        for u in range(2):
            for cp in wq0_copies(2 * i + u):
                cp.wait()
        for u in range(2):
            fixup(0, 2 * i + u, 0)
            wq0_tiles(2 * i + u)
        start_when(i == 1, wq0_copies(6) + wq0_copies(7))
        for j in range(3, NPIECE):
            start_when(i == (1 if j < 5 else 2), block_piece(0, j))
        return carry

    with jax.named_scope("pro0"):
        jax.lax.fori_loop(1, NB // 2, pro0, 0)
    for i in range(2, NPIECE):
        for cp in block_piece(1, i):
            cp.start()
    for cp in small_copies:
        cp.wait()

    def pro(c, carry):
        zw = c >> 3
        zr = c >> 4
        for i in range(2):
            start_when(c + 1 < NB, block_piece(jnp.minimum(c + 1, NB - 1), i))
        for i in range(NPIECE):
            for cp in block_piece(c, i):
                cp.wait()

        tiles = [(0, n) for n in range(2, 6)] + [(1, n) for n in range(6)]

        def tile(i, hook=None):
            e, n = tiles[i]
            if n % 2 == 0:
                fixup(e, c, n // 2)
            qkv_tile(e, c, n, hook=hook)

        def trigger(val):
            k2[c + zw, pl.ds(C // 2, 8), :] = val
            v2[c + zw, pl.ds(C // 2, 8), :] = val
            h_v[c + zw, pl.ds(128, 16), 0:128] = _unpack(val)

        def h_sample(n):
            w = word(ht_s, zr, n // 2)
            hv = hi16(w) if n % 2 else lo16(w)
            if n == 0:
                hv = hv + jnp.where(first, row_of(dd_ref, c), 0.0)
            return hv

        tile(0, trigger)
        h_prep(c, zw)
        kv_prep(c, zw)
        fft1(lambda n: t_s[zr, pl.ds(n * 8, 8), :], gu_s, zw)
        fft2(gu_s, u_s, zw, zr)
        fft1(h_sample, gh_s, zw)
        fft2(gh_s, h_s, zw, zr)
        for i in range(1, 9):
            for p in range(4 * i - 4, 4 * i):
                mac(p, zw, zr)
            tile(i)
        tile(9)
        inv_dft(c, zr)
        for i in range(2, NPIECE):
            start_when(c + 2 < NB, block_piece(jnp.minimum(c + 2, NB - 1), i))
        start_when(c + 1 < NB, [wo_copy(c)])
        start_when(c + 2 == NB, [wo_copy(NB - 1), x_early])
        return carry

    with jax.named_scope("pro"):
        jax.lax.fori_loop(0, NB, pro, 0)
    x_late.start()
    x_early.wait()
    for c in range(NB):
        wo_copy(c).wait()

    gwt = gw_ref[...].astype(F32)
    gw = jnp.concatenate([gwt[j:j + 1, :] for j in range(NB)], axis=1)

    def finalize(rows, b):
        xr = x_v[rows, :].astype(F32)
        g = jax.nn.sigmoid(jnp.sum(xr * gw, axis=-1, keepdims=True))
        a = xr * jnp.concatenate([y_v[j, rows, :] for j in range(NB)], axis=1)
        out_v[rows, :] = (g * a + (1.0 - g) * b).astype(BF16)

    def step(s, mem, split_first, odd):
        mrows = slice(0, M) if odd else slice(RX, RX + M)
        sh = 4 if odd else 0
        xo = pl.multiple_of(PRO + RX * s, 8)
        wbase = pl.multiple_of((RX // 2 * s) % (QCAP // 2) - sh, 8)
        rpos = pl.multiple_of((SEG // 2 * s + QOFF // 2) % (QCAP // 2), SEG // 2)
        xs = x_v[pl.ds(xo, RX), :]
        lhs = jnp.concatenate([mem, xs] if odd else [xs, mem], axis=0)
        zpad = jnp.zeros((128 - 2 * (SEG + M), E), BF16)
        no = SEG + M if odd else RX
        frows = pl.ds(pl.multiple_of(SEG * s - (M if odd else 0), 8), no)
        orows = slice(M, M + no) if odd else slice(0, no)
        omrows = slice(0, M) if odd else slice(no, no + M)
        low = jax.lax.broadcasted_iota(jnp.int32, (8, E), 0) < 4
        NP = H // 2

        mem_qkv = {}
        probs = {}
        cats = {}

        def load(mat, hp):
            parts = [_unpack(qkv_b[mat, hp, 0, pl.ds(rpos, SEG // 2), :]),
                     _unpack(qkv_b[mat, hp, 1, pl.ds(rpos, SEG // 2), :]), mem_qkv[(hp, mat)]]
            if mat > 0:
                parts.append(zpad)
            cats[(mat, hp)] = jnp.concatenate(parts, axis=0)

        def stage_a(hp):
            KH = D // 2
            split = split_first and hp == 0
            if split:
                for mat in range(3):
                    for j in range(2):
                        w = _unpack(wbuf[hp % 2][mat, hp // 2, j, :KH // 2, :])
                        qacc[2 * mat + j] = _dot(lhs[:, :KH], w)
            for mat in range(3):
                mm = []
                for j in range(2):
                    if split:
                        w = _unpack(wbuf[hp % 2][mat, hp // 2, j, KH // 2:, :])
                        res = qacc[2 * mat + j] + _dot(lhs[:, KH:], w)
                    else:
                        res = _dot(lhs, _unpack(wbuf[hp % 2][mat, hp // 2, j]))
                    pk = _pack(res)
                    if odd:
                        qkv_b[mat, hp, j, pl.ds(wbase + 4, 4), :] = pk[4:8]
                        qkv_b[mat, hp, j, pl.ds(wbase + 8, 8), :] = pk[8:16]
                    else:
                        qkv_b[mat, hp, j, pl.ds(wbase, 8), :] = pk[0:8]
                        qkv_b[mat, hp, j, pl.ds(wbase + 8, 4), :] = pk[8:12]
                    mm.append(res[mrows])
                    if j == 1:
                        mem_qkv[(hp, mat)] = jnp.concatenate(mm, axis=0).astype(BF16)
                    advance(6 * hp + 2 * mat + j + 1)

        def stage_b(hp):
            sc = _dot_nt(cats[(0, hp)], cats[(1, hp)]) * scale
            fill = fill_ref[...]
            sc = jnp.where(fill == 0.0, sc, fill)
            mx = jnp.max(sc, axis=-1, keepdims=True)
            p = jnp.exp(sc - mx)
            l = jnp.sum(p, axis=-1, keepdims=True)
            r = pl.reciprocal(l, approx=True)
            r = r * (2.0 - l * r)
            probs[hp] = (p * r).astype(BF16)

        def stage_c(hp):
            o = _dot(probs[hp], cats[(2, hp)])
            for j in range(2):
                h = 2 * hp + j
                cols = slice(h * E, (h + 1) * E)
                ox = _pack(o[j * SEG:(j + 1) * SEG])
                om = o[2 * SEG + j * M:2 * SEG + (j + 1) * M]
                om = _pack(jnp.concatenate([om, om], axis=0))
                if odd:
                    lo_s[0:8, cols] = jnp.where(low, om, left[:, cols])
                    lo_s[8:24, cols] = ox
                else:
                    lo_s[0:8, cols] = ox[0:8]
                    lo_s[8:16, cols] = jnp.where(low, ox[8:16], om)
                    left[:, cols] = ox[8:16]

        def oproj(j, late):
            ks = slice(HS * E, H * E) if late else slice(0, HS * E)
            kw = slice(ks.start // 2, ks.stop // 2)
            return _dot(_unpack(lo_s[0:(no + M) // 2, ks]), _unpack(wo_v[j, kw, :]))

        events = []
        for hp in range(NP):
            events.append((6 * hp + OFF_LQK, 0, functools.partial(load, 0, hp)))
            events.append((6 * hp + OFF_LQK, 1, functools.partial(load, 1, hp)))
            events.append((6 * hp + OFF_LV, 2, functools.partial(load, 2, hp)))
            events.append((6 * hp + OFF_PV, 3, functools.partial(stage_c, hp)))
            events.append((6 * hp + OFF_S, 4, functools.partial(stage_b, hp)))
        events.sort(key=lambda ev: ev[:2])

        def advance(slot):
            while events and events[0][0] <= slot:
                events.pop(0)[2]()

        outs = [None] * NB
        for hp in range(NP):
            stage_a(hp)
        for j in range(NB):
            oacc[0:no + M, j * 128:(j + 1) * 128] = oproj(j, False)
            advance(6 * NP + (j + 1) * HS // 8)
        assert not events
        for j in range(NB):
            outs[j] = oacc[0:no + M, j * 128:(j + 1) * 128] + oproj(j, True)
        res = jnp.concatenate(outs, axis=1)
        finalize(frows, res[orows])
        return res[omrows].astype(BF16)

    def steps(i, carry):
        @pl.when(i == (XE - PRO) // (RX * UNROLL))
        def _():
            x_late.wait()

        OB = SEG * UNROLL
        start_when(i > 0, [out_copy(pl.multiple_of(jnp.maximum(i * OB - LASTR, 0), 8), LASTR)])
        mem = mem_v[...]
        for u in range(UNROLL):
            if u == UNROLL - 1:
                out_copy(pl.multiple_of(i * OB, OB), OB - LASTR).start()
            mem = step(i * UNROLL + u, mem, u > 0, u % 2 == 1)
        mem_v[...] = mem
        return carry

    with jax.named_scope("main"):
        jax.lax.fori_loop(0, NSEG // UNROLL, steps, 0)

    out_copy(S - LASTR, LASTR).start()
    out_copy(0, S).wait()


@jax.jit
def _run(A_q, A_k, A_v, A_shift_k, A_ssm_k, A_ssm_D, B_mem0, B_Wq, B_Wk, B_Wv, B_Wo, gate_w):
    any_spec = pl.BlockSpec(memory_space=pl.ANY)
    out = pl.pallas_call(
        _kernel,
        out_shape=jax.ShapeDtypeStruct((S, D), BF16),
        in_specs=[any_spec] * 14,
        out_specs=any_spec,
        scratch_shapes=[
            pltpu.VMEM((S, D), BF16),
            pltpu.VMEM((PRO // 2, D), U32),
            pltpu.VMEM((NB, NCP, PR, 128), U32),
            pltpu.VMEM((NB, NCP, PR, 128), U32),
            pltpu.VMEM((NB, 128 + 16, S), BF16),
            pltpu.VMEM((3, H // 4, 2, D // 2, E), U32),
            pltpu.VMEM((3, H // 4, 2, D // 2, E), U32),
            pltpu.VMEM((NB, H * E // 2, 128), U32),
            pltpu.VMEM((NB, S + 32, 128), F32),
            pltpu.VMEM((3, H // 2, 2, QCAP // 2, E), U32),
            pltpu.VMEM((8, H * E), U32),
            pltpu.VMEM((24, H * E), U32),
            pltpu.VMEM((M, D), BF16),
            pltpu.VMEM((48, D), F32),
            pltpu.VMEM((6, M + RX, E), F32),
            pltpu.VMEM((1, NCH * SR + 2 * C, 128), F32),
            pltpu.VMEM((1, NCH * SR + 2 * C, 128), F32),
            pltpu.VMEM((1, NCH, 2 * C, 128), F32),
            pltpu.VMEM((1, S, 128), F32),
            pltpu.VMEM((1, 2 * S, 128), F32),
            pltpu.VMEM((1, 2 * S, 128), F32),
            pltpu.VMEM((1, NCP * PR, 128), U32),
            pltpu.VMEM((S, D), BF16),
            pltpu.VMEM((C, 2 * C // FOLD), BF16),
            pltpu.VMEM((2 * (SEG + M), 128), F32),
            pltpu.VMEM((KS, D), BF16),
            pltpu.VMEM((NB, 128), BF16),
            pltpu.VMEM((NB, 128), BF16),
            pltpu.SemaphoreType.DMA((7,)),
            pltpu.SemaphoreType.DMA((NB,)),
        ],
        compiler_params=pltpu.CompilerParams(vmem_limit_bytes=120 * 2 ** 20, disable_bounds_checks=True),
    )(
        A_q.reshape(S, D), A_k.reshape(NCH, C, D), A_v.reshape(NCH, C, D), A_ssm_k,
        B_Wq.reshape(D // 2, 2, H, E), B_Wk.reshape(D // 2, 2, H, E), B_Wv.reshape(D // 2, 2, H, E),
        B_Wo.reshape(H * E, D),
        A_shift_k.T, A_ssm_D.reshape(NB, 128), gate_w.reshape(NB, 128), B_mem0.reshape(M, D),
        jnp.asarray(_inv_table(), BF16), jnp.asarray(_attn_fill()),
    )
    return out.reshape(1, S, D)


def pallas_gated_mix__ssm_conv_h3__memory_aug_recurrent_mem_tr__prompt_kernel(
    A_q, A_k, A_v, A_shift_k, A_ssm_k, A_ssm_D, B_x, B_mem0, B_Wq, B_Wk, B_Wv, B_Wo, B_seg_len, gate_w,
):
    del B_x
    if isinstance(B_seg_len, int):
        assert B_seg_len == SEG
    return _run(A_q, A_k, A_v, A_shift_k, A_ssm_k, A_ssm_D, B_mem0, B_Wq, B_Wk, B_Wv, B_Wo, gate_w)
```

```python
import cmath
import functools
import math

import jax
import jax.numpy as jnp
import numpy as np
import jax.experimental.pallas as pl
import jax.experimental.pallas.tpu as pltpu

F32 = jnp.float32
BF16 = jnp.bfloat16
U32 = jnp.uint32

S = 2048
D = 1024
H = 32
E = 128
M = 8
SEG = 32
NSEG = S // SEG
RX = 24
PRO = S - RX * NSEG
QCAP = 576
QOFF = QCAP - PRO
HL = 4
HS = H - HL
OFF_LQK, OFF_S, OFF_LV, OFF_PV = 4, 8, 14, 17
UNROLL = 4
LASTR = SEG + M
XE = 768
C = 256
NCH = S // C
NB = D // 128
KS = 4
NEG = -1000000000.0
R1, R2 = 16, 16
PR = C // 2 + 8
NCP = NCH + 4
HR = C // 2 + 4
FOLD = 4
SR = 2 * C + 4


def _inv_table():
    n = np.arange(C, dtype=np.float64)
    th = 2.0 * np.pi * (np.arange(C // FOLD, dtype=np.float64) + 0.25) / C
    no = np.concatenate([n[r::FOLD] for r in range(FOLD)])
    inv = np.concatenate([np.cos(no[:, None] * th[None, :]), -np.sin(no[:, None] * th[None, :])], axis=1) / C
    return inv.astype(np.float32)


def _attn_fill():
    n = 2 * (SEG + M)
    head = np.array([0] * SEG + [1] * SEG + [0] * M + [1] * M)
    pos = np.concatenate([M + np.arange(SEG), M + np.arange(SEG), np.arange(M), np.arange(M)])
    fill = np.full((n, 128), -np.inf, np.float32)
    for i in range(n):
        for j in range(n):
            if head[i] == head[j]:
                ok = pos[i] < M or pos[i] >= pos[j]
                fill[i, j] = 0.0 if ok else NEG
    return fill


def _add(a, b):
    return b if a is None else a if b is None else a + b


def _sub(a, b):
    return a if b is None else -b if a is None else a - b


def _cmul(z, w):
    r, i = z
    wr, wi = w.real, w.imag
    eps = 1e-12
    if abs(wi) < eps and abs(wr - 1.0) < eps:
        return z
    if i is None:
        if abs(abs(wr) - abs(wi)) < eps and wr * wi > 0:
            t = r * wr
            return t, t
        return r * wr, r * wi
    if abs(abs(wr) - abs(wi)) < eps:
        if wr * wi > 0:
            return (r - i) * wr, (r + i) * wr
        return (r + i) * wr, (i - r) * wr
    return r * wr - i * wi, r * wi + i * wr


def _fft(xs):
    n = len(xs)
    if n == 1:
        return xs
    if n == 2:
        (ar, ai), (br, bi) = xs
        return [(_add(ar, br), _add(ai, bi)), (_sub(ar, br), _sub(ai, bi))]
    e = _fft(xs[0::2])
    o1 = _fft(xs[1::4])
    o3 = _fft(xs[3::4])
    out = [None] * n
    for k in range(n // 4):
        ar, ai = _cmul(o1[k], cmath.exp(-2j * math.pi * k / n))
        br, bi = _cmul(o3[k], cmath.exp(-6j * math.pi * k / n))
        sr, si, dr, di = _add(ar, br), _add(ai, bi), _sub(ar, br), _sub(ai, bi)
        er, ei = e[k]
        fr, fi = e[k + n // 4]
        out[k] = (_add(er, sr), _add(ei, si))
        out[k + n // 2] = (_sub(er, sr), _sub(ei, si))
        out[k + n // 4] = (_add(fr, di), _sub(fi, dr))
        out[k + 3 * n // 4] = (_sub(fr, di), _add(fi, dr))
    return out


def _dot(a, b):
    return jnp.dot(a, b, preferred_element_type=F32)


def _dot_nt(a, b):
    return jax.lax.dot_general(a, b, (((1,), (1,)), ((), ())), preferred_element_type=F32)


def _pack(a):
    return pltpu.bitcast(a.astype(BF16), U32)


def _unpack(a):
    return pltpu.bitcast(a, BF16)


def _kernel(x_hbm, k_hbm, v_hbm, h_hbm, wq_hbm, wk_hbm, wv_hbm, wo_hbm,
            sk_hbm, dd_hbm, gw_hbm, mem0_hbm, inv_hbm, fill_hbm,
            out_hbm,
            x_v, xp, k_v, v_v, h_v, w_even, w_odd, wo_v, y_v, qkv_b, left, lo_s, mem_v, oacc, qacc,
            u_s, h_s, yf_s, t_s, gu_s, gh_s, ht_s,
            out_v, inv_ref, fill_ref, sk_ref, dd_ref, gw_ref, sems, qsems):
    scale = E ** (-0.5)
    wbuf = (w_even, w_odd)

    w32 = [w.bitcast(U32) for w in (wq_hbm, wk_hbm, wv_hbm)]
    wo32 = wo_hbm.bitcast(U32)
    x32 = x_hbm.bitcast(U32)
    k32 = k_hbm.bitcast(U32)
    v32 = v_hbm.bitcast(U32)

    def lanes(c):
        return pl.ds(pl.multiple_of(c * 128, 128), 128)

    def w_copies(c, e, mat, sem):
        return [pltpu.make_async_copy(w32[mat].at[:, par, 2 * c + e, :], wbuf[e].at[mat, c, par], sem)
                for par in range(2)]

    def wq0_copies(c):
        return w_copies(c, 0, 0, qsems.at[c])

    W_REST = [(e, mat) for e in range(2) for mat in range(3) if (e, mat) != (0, 0)]
    NPIECE = 3 + len(W_REST)

    def block_piece(c, i):
        sem = sems.at[c % 2]
        if i < 2:
            src, dst = ((k32, k_v), (v32, v_v))[i]
            return [pltpu.make_async_copy(src.at[:, :, lanes(c)], dst.at[c, pl.ds(0, NCH), pl.ds(0, C // 2), :], sem)]
        if i == 2:
            return [pltpu.make_async_copy(h_hbm.at[lanes(c), :], h_v.at[c, pl.ds(0, 128), :], sem)]
        return w_copies(c, *W_REST[i - 3], sem)

    def wo_copy(c):
        return pltpu.make_async_copy(wo32.at[:, lanes(c)], wo_v.at[c], sems.at[2])

    x_early = pltpu.make_async_copy(x_hbm.at[pl.ds(0, XE), :], x_v.at[pl.ds(0, XE), :], sems.at[2])
    x_late = pltpu.make_async_copy(x_hbm.at[pl.ds(XE, S - XE), :], x_v.at[pl.ds(XE, S - XE), :], sems.at[3])

    xp_copies = [pltpu.make_async_copy(x32.at[pl.ds(i * PRO // 4, PRO // 4), :], xp.at[pl.ds(i * PRO // 4, PRO // 4), :],
                                       sems.at[3 + 3 * i]) for i in range(2)]
    small_copies = [pltpu.make_async_copy(src, dst, sems.at[4]) for src, dst in (
        (sk_hbm, sk_ref), (dd_hbm, dd_ref), (inv_hbm, inv_ref),
        (gw_hbm, gw_ref), (mem0_hbm, mem_v), (fill_hbm, fill_ref))]

    def out_copy(start, n):
        rows = pl.ds(start, n)
        return pltpu.make_async_copy(out_v.at[rows, :], out_hbm.at[rows, :], sems.at[5])

    def row_of(ref, c):
        t = ref[...].astype(F32)
        sel = jax.lax.broadcasted_iota(jnp.int32, (NB, 128), 0) == c
        return jnp.sum(jnp.where(sel, t, 0.0), axis=0, keepdims=True)

    k2 = k_v.reshape(NB, NCP * PR, 128)
    v2 = v_v.reshape(NB, NCP * PR, 128)

    def lo16(w):
        return pltpu.bitcast(w << 16, F32)

    def hi16(w):
        return pltpu.bitcast(w & U32(0xFFFF0000), F32)

    def pair(ref, c, pr):
        w = ref[c, pl.ds(pr, NCH, stride=PR), :]
        return lo16(w), hi16(w)

    first = jax.lax.broadcasted_iota(jnp.int32, (8, 128), 0) == 0

    def kv_prep(c, zw):
        skt = sk_ref[:, lanes(c)].astype(F32)
        sk = [jnp.broadcast_to(skt[j:j + 1, :], (8, 128)) for j in range(KS)]
        tail = (pair(k2, c, C // 2 - 2) + pair(k2, c, C // 2 - 1))[1:]
        win = [jnp.where(first, 0.0, pltpu.roll(t, 1, 0)) for t in tail]
        for pr in range(C // 2):
            ks = pair(k2, c, pr)
            vs = pair(v2, c, pr)
            for i in range(2):
                win.append(ks[i])
                acc = win[-1] * sk[0]
                for j in range(1, KS):
                    acc = acc + win[-1 - j] * sk[j]
                win = win[1:]
                t_s[zw, pl.ds((2 * pr + i) * 8, 8), :] = acc * vs[i]

    def h_prep(c, zw):
        for t in range(S // 128):
            ht = pltpu.bitcast(h_v[c, 0:128, pl.ds(t * 128, 128)].T, U32)
            ht_s[zw, pl.ds(t * 64 // (C // 2) * HR + t * 64 % (C // 2), 64), :] = ht

    def fft1(sample, mid, zw):
        for b in range(R2):
            z = [_cmul((sample(R2 * a + b), None), cmath.exp(-0.5j * math.pi * a / R1)) for a in range(R1)]
            gq = _fft(z)
            for q1 in range(R1):
                re, im = _cmul(gq[q1], cmath.exp(-2j * math.pi * (q1 + 0.25) * b / C))
                row = (q1 * R2 + b) * 16
                mid[zw, pl.ds(row, 8), :] = re
                mid[zw, pl.ds(row + 8, 8), :] = im

    def fft2(mid, dst, zw, zr):
        for q1 in range(R1):
            z = []
            for b in range(R2):
                row = (q1 * R2 + b) * 16
                z.append((mid[zr, pl.ds(row, 8), :], mid[zr, pl.ds(row + 8, 8), :]))
            t = _fft(z)
            for q2 in range(R2):
                q = q1 + R1 * q2
                dst[zw, pl.ds(q, NCH, stride=SR), :] = t[q2][0]
                dst[zw, pl.ds(C + q, NCH, stride=SR), :] = t[q2][1]

    def mac(p, zw, zr):
        re = pl.ds(p * 8, 8)
        im = pl.ds(C + p * 8, 8)
        AB = 4
        prev = None
        for a0 in range(0, NCH, AB):
            zre = [None] * AB
            zim = [None] * AB
            for m in range(a0 + AB):
                hr = h_s[zr, pl.ds(m * SR + p * 8, 8), :]
                hi = h_s[zr, pl.ds(m * SR + C + p * 8, 8), :]
                for i in range(AB):
                    t = a0 + i - m
                    if t < 0:
                        continue
                    ur = u_s[zr, pl.ds(t * SR + p * 8, 8), :]
                    ui = u_s[zr, pl.ds(t * SR + C + p * 8, 8), :]
                    tr = hr * ur - hi * ui
                    ti = hr * ui + hi * ur
                    zre[i] = tr if zre[i] is None else zre[i] + tr
                    zim[i] = ti if zim[i] is None else zim[i] + ti
            for i in range(AB):
                if prev is None:
                    yf_s[zw, a0 + i, re, :] = zre[i]
                    yf_s[zw, a0 + i, im, :] = zim[i]
                else:
                    yf_s[zw, a0 + i, re, :] = zre[i] - prev[1]
                    yf_s[zw, a0 + i, im, :] = zim[i] + prev[0]
                prev = (zre[i], zim[i])

    def inv_dft(c, zr):
        qc = C // FOLD
        for a in range(NCH):
            yr = [yf_s[zr, a, j * qc:(j + 1) * qc, :] for j in range(FOLD)]
            yi = [yf_s[zr, a, C + j * qc:C + (j + 1) * qc, :] for j in range(FOLD)]
            sr, si, dr, di = yr[0] + yr[2], yi[0] + yi[2], yr[0] - yr[2], yi[0] - yi[2]
            tr, ti, er, ei = yr[1] + yr[3], yi[1] + yi[3], yr[1] - yr[3], yi[1] - yi[3]
            folded = [(sr + tr, si + ti), (dr - ei, di + er), (sr - tr, si - ti), (dr + ei, di - er)]
            for r in range(FOLD):
                f = jnp.concatenate(folded[r], axis=0).astype(BF16)
                y_v[c, pl.ds(a * C + r, qc, stride=FOLD), :] = _dot(inv_ref[r * qc:(r + 1) * qc, :], f)

    def fixup(e, c, mat):
        a = wbuf[e][mat, c, 0]
        b = wbuf[e][mat, c, 1]
        wbuf[e][mat, c, 0] = (a & U32(0xFFFF)) | (b << 16)
        wbuf[e][mat, c, 1] = (a >> 16) | (b & U32(0xFFFF0000))

    RB = 128

    def qkv_tile(e, c, n, hook=None, rs=range(PRO // RB)):
        mat, j = n // 2, n % 2
        for r in rs:
            w = _unpack(wbuf[e][mat, c, j])
            xr = _unpack(xp[pl.ds(r * RB // 2, RB // 2), :])
            pk = _pack(_dot(xr, w))
            qkv_b[mat, 2 * c + e, j, pl.ds((QOFF + r * RB) // 2, RB // 2), :] = pk
            if hook is not None and r == 0:
                hook(pk[0:8])

    def start_when(cond, copies):
        @pl.when(cond)
        def _():
            for cp in copies:
                cp.start()

    def wq0_tiles(c, rs=range(PRO // RB)):
        qkv_tile(0, c, 0, rs=rs)
        qkv_tile(0, c, 1, rs=rs)

    for cp in wq0_copies(0) + xp_copies + wq0_copies(1):
        cp.start()
    for cp in wq0_copies(0) + xp_copies[:1]:
        cp.wait()
    fixup(0, 0, 0)
    wq0_tiles(0, range(2))
    for cp in wq0_copies(2) + wq0_copies(3):
        cp.start()
    xp_copies[1].wait()
    wq0_tiles(0, range(2, 4))
    for cp in small_copies + block_piece(0, 0):
        cp.start()
    for cp in wq0_copies(1):
        cp.wait()
    fixup(0, 1, 0)
    wq0_tiles(1)
    for cp in wq0_copies(4) + wq0_copies(5) + block_piece(0, 2) + block_piece(0, 1):
        cp.start()

    def pro0(i, carry):
        for u in range(2):
            for cp in wq0_copies(2 * i + u):
                cp.wait()
        for u in range(2):
            fixup(0, 2 * i + u, 0)
            wq0_tiles(2 * i + u)
        start_when(i == 1, wq0_copies(6) + wq0_copies(7))
        for j in range(3, NPIECE):
            start_when(i == (1 if j < 5 else 2), block_piece(0, j))
        return carry

    with jax.named_scope("pro0"):
        jax.lax.fori_loop(1, NB // 2, pro0, 0)
    for i in range(2, NPIECE):
        for cp in block_piece(1, i):
            cp.start()
    for cp in small_copies:
        cp.wait()

    def pro(c, carry):
        zw = c >> 3
        zr = c >> 4
        for i in range(2):
            start_when(c + 1 < NB, block_piece(jnp.minimum(c + 1, NB - 1), i))
        for i in range(NPIECE):
            for cp in block_piece(c, i):
                cp.wait()

        tiles = [(0, n) for n in range(2, 6)] + [(1, n) for n in range(6)]

        def tile(i, hook=None):
            e, n = tiles[i]
            if n % 2 == 0:
                fixup(e, c, n // 2)
            qkv_tile(e, c, n, hook=hook)

        def trigger(val):
            k2[c + zw, pl.ds(C // 2, 8), :] = val
            v2[c + zw, pl.ds(C // 2, 8), :] = val
            h_v[c + zw, pl.ds(128, 16), 0:128] = _unpack(val)

        def h_sample(n):
            w = ht_s[zr, pl.ds(n // 2, NCH, stride=HR), :]
            hv = hi16(w) if n % 2 else lo16(w)
            if n == 0:
                hv = hv + jnp.where(first, row_of(dd_ref, c), 0.0)
            return hv

        tile(0, trigger)
        h_prep(c, zw)
        kv_prep(c, zw)
        fft1(lambda n: t_s[zr, pl.ds(n * 8, 8), :], gu_s, zw)
        fft2(gu_s, u_s, zw, zr)
        fft1(h_sample, gh_s, zw)
        fft2(gh_s, h_s, zw, zr)
        for i in range(1, 9):
            for p in range(4 * i - 4, 4 * i):
                mac(p, zw, zr)
            tile(i)
        tile(9)
        inv_dft(c, zr)
        for i in range(2, NPIECE):
            start_when(c + 2 < NB, block_piece(jnp.minimum(c + 2, NB - 1), i))
        start_when(c + 1 < NB, [wo_copy(c)])
        start_when(c + 2 == NB, [wo_copy(NB - 1), x_early])
        return carry

    with jax.named_scope("pro"):
        jax.lax.fori_loop(0, NB, pro, 0)
    x_late.start()
    x_early.wait()
    for c in range(NB):
        wo_copy(c).wait()

    gwt = gw_ref[...].astype(F32)
    gw = jnp.concatenate([gwt[j:j + 1, :] for j in range(NB)], axis=1)

    def finalize(rows, b):
        xr = x_v[rows, :].astype(F32)
        g = jax.nn.sigmoid(jnp.sum(xr * gw, axis=-1, keepdims=True))
        a = xr * jnp.concatenate([y_v[j, rows, :] for j in range(NB)], axis=1)
        out_v[rows, :] = (g * a + (1.0 - g) * b).astype(BF16)

    def step(s, mem, split_first, odd):
        mrows = slice(0, M) if odd else slice(RX, RX + M)
        sh = 4 if odd else 0
        xo = pl.multiple_of(PRO + RX * s, 8)
        wbase = pl.multiple_of((RX // 2 * s) % (QCAP // 2) - sh, 8)
        rpos = pl.multiple_of((SEG // 2 * s + QOFF // 2) % (QCAP // 2), SEG // 2)
        xs = x_v[pl.ds(xo, RX), :]
        lhs = jnp.concatenate([mem, xs] if odd else [xs, mem], axis=0)
        zpad = jnp.zeros((128 - 2 * (SEG + M), E), BF16)
        no = SEG + M if odd else RX
        frows = pl.ds(pl.multiple_of(SEG * s - (M if odd else 0), 8), no)
        orows = slice(M, M + no) if odd else slice(0, no)
        omrows = slice(0, M) if odd else slice(no, no + M)
        low = jax.lax.broadcasted_iota(jnp.int32, (8, E), 0) < 4
        NP = H // 2

        mem_qkv = {}
        probs = {}
        cats = {}

        def load(mat, hp):
            parts = [_unpack(qkv_b[mat, hp, 0, pl.ds(rpos, SEG // 2), :]),
                     _unpack(qkv_b[mat, hp, 1, pl.ds(rpos, SEG // 2), :]), mem_qkv[(hp, mat)]]
            if mat > 0:
                parts.append(zpad)
            cats[(mat, hp)] = jnp.concatenate(parts, axis=0)

        def stage_a(hp):
            KH = D // 2
            split = split_first and hp == 0
            if split:
                for mat in range(3):
                    for j in range(2):
                        w = _unpack(wbuf[hp % 2][mat, hp // 2, j, :KH // 2, :])
                        qacc[2 * mat + j] = _dot(lhs[:, :KH], w)
            for mat in range(3):
                mm = []
                for j in range(2):
                    if split:
                        w = _unpack(wbuf[hp % 2][mat, hp // 2, j, KH // 2:, :])
                        res = qacc[2 * mat + j] + _dot(lhs[:, KH:], w)
                    else:
                        res = _dot(lhs, _unpack(wbuf[hp % 2][mat, hp // 2, j]))
                    pk = _pack(res)
                    if odd:
                        qkv_b[mat, hp, j, pl.ds(wbase + 4, 4), :] = pk[4:8]
                        qkv_b[mat, hp, j, pl.ds(wbase + 8, 8), :] = pk[8:16]
                    else:
                        qkv_b[mat, hp, j, pl.ds(wbase, 8), :] = pk[0:8]
                        qkv_b[mat, hp, j, pl.ds(wbase + 8, 4), :] = pk[8:12]
                    mm.append(res[mrows])
                    if j == 1:
                        mem_qkv[(hp, mat)] = jnp.concatenate(mm, axis=0).astype(BF16)
                    advance(6 * hp + 2 * mat + j + 1)

        def stage_b(hp):
            sc = _dot_nt(cats[(0, hp)], cats[(1, hp)]) * scale
            fill = fill_ref[...]
            sc = jnp.where(fill == 0.0, sc, fill)
            mx = jnp.max(sc, axis=-1, keepdims=True)
            p = jnp.exp(sc - mx)
            l = jnp.sum(p, axis=-1, keepdims=True)
            r = pl.reciprocal(l, approx=True)
            r = r * (2.0 - l * r)
            probs[hp] = (p * r).astype(BF16)

        def stage_c(hp):
            o = _dot(probs[hp], cats[(2, hp)])
            for j in range(2):
                h = 2 * hp + j
                cols = slice(h * E, (h + 1) * E)
                ox = _pack(o[j * SEG:(j + 1) * SEG])
                om = o[2 * SEG + j * M:2 * SEG + (j + 1) * M]
                om = _pack(jnp.concatenate([om, om], axis=0))
                if odd:
                    lo_s[0:8, cols] = jnp.where(low, om, left[:, cols])
                    lo_s[8:24, cols] = ox
                else:
                    lo_s[0:8, cols] = ox[0:8]
                    lo_s[8:16, cols] = jnp.where(low, ox[8:16], om)
                    left[:, cols] = ox[8:16]

        def oproj(j, late):
            ks = slice(HS * E, H * E) if late else slice(0, HS * E)
            kw = slice(ks.start // 2, ks.stop // 2)
            return _dot(_unpack(lo_s[0:(no + M) // 2, ks]), _unpack(wo_v[j, kw, :]))

        events = []
        for hp in range(NP):
            events.append((6 * hp + OFF_LQK, 0, functools.partial(load, 0, hp)))
            events.append((6 * hp + OFF_LQK, 1, functools.partial(load, 1, hp)))
            events.append((6 * hp + OFF_LV, 2, functools.partial(load, 2, hp)))
            events.append((6 * hp + OFF_PV, 3, functools.partial(stage_c, hp)))
            events.append((6 * hp + OFF_S, 4, functools.partial(stage_b, hp)))
        events.sort(key=lambda ev: ev[:2])

        def advance(slot):
            while events and events[0][0] <= slot:
                events.pop(0)[2]()

        outs = [None] * NB
        for hp in range(NP):
            stage_a(hp)
        for j in range(NB):
            oacc[0:no + M, j * 128:(j + 1) * 128] = oproj(j, False)
            advance(6 * NP + (j + 1) * HS // 8)
        assert not events
        for j in range(NB):
            outs[j] = oacc[0:no + M, j * 128:(j + 1) * 128] + oproj(j, True)
        res = jnp.concatenate(outs, axis=1)
        finalize(frows, res[orows])
        return res[omrows].astype(BF16)

    def steps(i, carry):
        @pl.when(i == (XE - PRO) // (RX * UNROLL))
        def _():
            x_late.wait()

        OB = SEG * UNROLL
        start_when(i > 0, [out_copy(pl.multiple_of(jnp.maximum(i * OB - LASTR, 0), 8), LASTR)])
        mem = mem_v[...]
        for u in range(UNROLL):
            if u == UNROLL - 1:
                out_copy(pl.multiple_of(i * OB, OB), OB - LASTR).start()
            mem = step(i * UNROLL + u, mem, u > 0, u % 2 == 1)
        mem_v[...] = mem
        return carry

    with jax.named_scope("main"):
        jax.lax.fori_loop(0, NSEG // UNROLL, steps, 0)

    out_copy(S - LASTR, LASTR).start()
    out_copy(0, S).wait()


@jax.jit
def _run(A_q, A_k, A_v, A_shift_k, A_ssm_k, A_ssm_D, B_mem0, B_Wq, B_Wk, B_Wv, B_Wo, gate_w):
    any_spec = pl.BlockSpec(memory_space=pl.ANY)
    out = pl.pallas_call(
        _kernel,
        out_shape=jax.ShapeDtypeStruct((S, D), BF16),
        in_specs=[any_spec] * 14,
        out_specs=any_spec,
        scratch_shapes=[
            pltpu.VMEM((S, D), BF16),
            pltpu.VMEM((PRO // 2, D), U32),
            pltpu.VMEM((NB, NCP, PR, 128), U32),
            pltpu.VMEM((NB, NCP, PR, 128), U32),
            pltpu.VMEM((NB, 128 + 16, S), BF16),
            pltpu.VMEM((3, H // 4, 2, D // 2, E), U32),
            pltpu.VMEM((3, H // 4, 2, D // 2, E), U32),
            pltpu.VMEM((NB, H * E // 2, 128), U32),
            pltpu.VMEM((NB, S + 32, 128), F32),
            pltpu.VMEM((3, H // 2, 2, QCAP // 2, E), U32),
            pltpu.VMEM((8, H * E), U32),
            pltpu.VMEM((24, H * E), U32),
            pltpu.VMEM((M, D), BF16),
            pltpu.VMEM((48, D), F32),
            pltpu.VMEM((6, M + RX, E), F32),
            pltpu.VMEM((1, NCH * SR + 2 * C, 128), F32),
            pltpu.VMEM((1, NCH * SR + 2 * C, 128), F32),
            pltpu.VMEM((1, NCH, 2 * C, 128), F32),
            pltpu.VMEM((1, S, 128), F32),
            pltpu.VMEM((1, 2 * S, 128), F32),
            pltpu.VMEM((1, 2 * S, 128), F32),
            pltpu.VMEM((1, NCP * PR, 128), U32),
            pltpu.VMEM((S, D), BF16),
            pltpu.VMEM((C, 2 * C // FOLD), BF16),
            pltpu.VMEM((2 * (SEG + M), 128), F32),
            pltpu.VMEM((KS, D), BF16),
            pltpu.VMEM((NB, 128), BF16),
            pltpu.VMEM((NB, 128), BF16),
            pltpu.SemaphoreType.DMA((7,)),
            pltpu.SemaphoreType.DMA((NB,)),
        ],
        compiler_params=pltpu.CompilerParams(vmem_limit_bytes=120 * 2 ** 20, disable_bounds_checks=True),
    )(
        A_q.reshape(S, D), A_k.reshape(NCH, C, D), A_v.reshape(NCH, C, D), A_ssm_k,
        B_Wq.reshape(D // 2, 2, H, E), B_Wk.reshape(D // 2, 2, H, E), B_Wv.reshape(D // 2, 2, H, E),
        B_Wo.reshape(H * E, D),
        A_shift_k.T, A_ssm_D.reshape(NB, 128), gate_w.reshape(NB, 128), B_mem0.reshape(M, D),
        jnp.asarray(_inv_table(), BF16), jnp.asarray(_attn_fill()),
    )
    return out.reshape(1, S, D)


def pallas_gated_mix__ssm_conv_h3__memory_aug_recurrent_mem_tr__prompt_kernel(
    A_q, A_k, A_v, A_shift_k, A_ssm_k, A_ssm_D, B_x, B_mem0, B_Wq, B_Wk, B_Wv, B_Wo, B_seg_len, gate_w,
):
    del B_x
    if isinstance(B_seg_len, int):
        assert B_seg_len == SEG
    return _run(A_q, A_k, A_v, A_shift_k, A_ssm_k, A_ssm_D, B_mem0, B_Wq, B_Wk, B_Wv, B_Wo, gate_w)
```

```python
import cmath
import functools
import math

import jax
import jax.numpy as jnp
import numpy as np
import jax.experimental.pallas as pl
import jax.experimental.pallas.tpu as pltpu

F32 = jnp.float32
BF16 = jnp.bfloat16
U32 = jnp.uint32

S = 2048
D = 1024
H = 32
E = 128
M = 8
SEG = 32
NSEG = S // SEG
RX = 24
PRO = S - RX * NSEG
QCAP = 576
QOFF = QCAP - PRO
HL = 4
HS = H - HL
OFF_LQK, OFF_S, OFF_LV, OFF_PV = 4, 8, 14, 17
UNROLL = 4
LASTR = SEG + M
XE = 768
C = 256
NCH = S // C
NB = D // 128
KS = 4
NEG = -1000000000.0
R1, R2 = 16, 16
PR = C // 2 + 4
PT = 1216
FOLD = 4
SR = 2 * C + 4


def _inv_table():
    n = np.arange(C, dtype=np.float64)
    th = 2.0 * np.pi * (np.arange(C // FOLD, dtype=np.float64) + 0.25) / C
    no = np.concatenate([n[r::FOLD] for r in range(FOLD)])
    inv = np.concatenate([np.cos(no[:, None] * th[None, :]), -np.sin(no[:, None] * th[None, :])], axis=1) / C
    return inv.astype(np.float32)


def _attn_fill():
    n = 2 * (SEG + M)
    head = np.array([0] * SEG + [1] * SEG + [0] * M + [1] * M)
    pos = np.concatenate([M + np.arange(SEG), M + np.arange(SEG), np.arange(M), np.arange(M)])
    fill = np.full((n, 128), -np.inf, np.float32)
    for i in range(n):
        for j in range(n):
            if head[i] == head[j]:
                ok = pos[i] < M or pos[i] >= pos[j]
                fill[i, j] = 0.0 if ok else NEG
    return fill


def _add(a, b):
    return b if a is None else a if b is None else a + b


def _sub(a, b):
    return a if b is None else -b if a is None else a - b


def _cmul(z, w):
    r, i = z
    wr, wi = w.real, w.imag
    eps = 1e-12
    if abs(wi) < eps and abs(wr - 1.0) < eps:
        return z
    if i is None:
        if abs(abs(wr) - abs(wi)) < eps and wr * wi > 0:
            t = r * wr
            return t, t
        return r * wr, r * wi
    if abs(abs(wr) - abs(wi)) < eps:
        if wr * wi > 0:
            return (r - i) * wr, (r + i) * wr
        return (r + i) * wr, (i - r) * wr
    return r * wr - i * wi, r * wi + i * wr


def _fft(xs):
    n = len(xs)
    if n == 1:
        return xs
    if n == 2:
        (ar, ai), (br, bi) = xs
        return [(_add(ar, br), _add(ai, bi)), (_sub(ar, br), _sub(ai, bi))]
    e = _fft(xs[0::2])
    o1 = _fft(xs[1::4])
    o3 = _fft(xs[3::4])
    out = [None] * n
    for k in range(n // 4):
        ar, ai = _cmul(o1[k], cmath.exp(-2j * math.pi * k / n))
        br, bi = _cmul(o3[k], cmath.exp(-6j * math.pi * k / n))
        sr, si, dr, di = _add(ar, br), _add(ai, bi), _sub(ar, br), _sub(ai, bi)
        er, ei = e[k]
        fr, fi = e[k + n // 4]
        out[k] = (_add(er, sr), _add(ei, si))
        out[k + n // 2] = (_sub(er, sr), _sub(ei, si))
        out[k + n // 4] = (_add(fr, di), _sub(fi, dr))
        out[k + 3 * n // 4] = (_sub(fr, di), _add(fi, dr))
    return out


def _dot(a, b):
    return jnp.dot(a, b, preferred_element_type=F32)


def _dot_nt(a, b):
    return jax.lax.dot_general(a, b, (((1,), (1,)), ((), ())), preferred_element_type=F32)


def _pack(a):
    return pltpu.bitcast(a.astype(BF16), U32)


def _unpack(a):
    return pltpu.bitcast(a, BF16)


def _kernel(x_hbm, k_hbm, v_hbm, h_hbm, wq_hbm, wk_hbm, wv_hbm, wo_hbm,
            sk_hbm, dd_hbm, gw_hbm, mem0_hbm, inv_hbm, fill_hbm,
            out_hbm,
            x_v, xp, k_v, v_v, h_v, w_even, w_odd, wo_v, y_v, qkv_b, left, lo_s, mem_v, oacc, qacc,
            u_s, h_s, yf_s, t_s, gu_s, gh_s, ht_s,
            out_v, inv_ref, fill_ref, sk_ref, dd_ref, gw_ref, sems, qsems):
    scale = E ** (-0.5)
    wbuf = (w_even, w_odd)

    w32 = [w.bitcast(U32) for w in (wq_hbm, wk_hbm, wv_hbm)]
    wo32 = wo_hbm.bitcast(U32)
    x32 = x_hbm.bitcast(U32)
    k32 = k_hbm.bitcast(U32)
    v32 = v_hbm.bitcast(U32)

    def lanes(c):
        return pl.ds(pl.multiple_of(c * 128, 128), 128)

    def w_copies(c, e, mat, sem):
        return [pltpu.make_async_copy(w32[mat].at[:, par, 2 * c + e, :], wbuf[e].at[mat, c, par], sem)
                for par in range(2)]

    def wq0_copies(c):
        return w_copies(c, 0, 0, qsems.at[c])

    W_REST = [(e, mat) for e in range(2) for mat in range(3) if (e, mat) != (0, 0)]
    NPIECE = 3 + len(W_REST)

    def block_piece(c, i):
        sem = sems.at[c % 2]
        if i < 2:
            src, dst = ((k32, k_v), (v32, v_v))[i]
            return [pltpu.make_async_copy(src.at[a, :, lanes(c)], dst.at[c, pl.ds(a * PR, C // 2), :], sem)
                    for a in range(NCH)]
        if i == 2:
            return [pltpu.make_async_copy(h_hbm.at[lanes(c), :], h_v.at[c, pl.ds(0, 128), :], sem)]
        return w_copies(c, *W_REST[i - 3], sem)

    def wo_copy(c):
        return pltpu.make_async_copy(wo32.at[:, lanes(c)], wo_v.at[c], sems.at[2])

    x_early = pltpu.make_async_copy(x_hbm.at[pl.ds(0, XE), :], x_v.at[pl.ds(0, XE), :], sems.at[2])
    x_late = pltpu.make_async_copy(x_hbm.at[pl.ds(XE, S - XE), :], x_v.at[pl.ds(XE, S - XE), :], sems.at[3])

    xp_copies = [pltpu.make_async_copy(x32.at[pl.ds(i * PRO // 4, PRO // 4), :], xp.at[pl.ds(i * PRO // 4, PRO // 4), :],
                                       sems.at[3 + 3 * i]) for i in range(2)]
    small_copies = [pltpu.make_async_copy(src, dst, sems.at[4]) for src, dst in (
        (sk_hbm, sk_ref), (dd_hbm, dd_ref), (inv_hbm, inv_ref),
        (gw_hbm, gw_ref), (mem0_hbm, mem_v), (fill_hbm, fill_ref))]

    def out_copy(start, n):
        rows = pl.ds(start, n)
        return pltpu.make_async_copy(out_v.at[rows, :], out_hbm.at[rows, :], sems.at[5])

    def row_of(ref, c):
        t = ref[...].astype(F32)
        sel = jax.lax.broadcasted_iota(jnp.int32, (NB, 128), 0) == c
        return jnp.sum(jnp.where(sel, t, 0.0), axis=0, keepdims=True)

    def word(ref, c, pr):
        return ref[c, pl.ds(pr, NCH, stride=PR), :]

    def lo16(w):
        return pltpu.bitcast(w << 16, F32)

    def hi16(w):
        return pltpu.bitcast(w & U32(0xFFFF0000), F32)

    def pair(ref, c, pr):
        w = word(ref, c, pr)
        return lo16(w), hi16(w)

    first = jax.lax.broadcasted_iota(jnp.int32, (8, 128), 0) == 0

    def kv_prep(c, zw):
        skt = sk_ref[:, lanes(c)].astype(F32)
        sk = [jnp.broadcast_to(skt[j:j + 1, :], (8, 128)) for j in range(KS)]
        tail = (pair(k_v, c, C // 2 - 2) + pair(k_v, c, C // 2 - 1))[1:]
        win = [jnp.where(first, 0.0, pltpu.roll(t, 1, 0)) for t in tail]
        for pr in range(C // 2):
            ks = pair(k_v, c, pr)
            vs = pair(v_v, c, pr)
            for i in range(2):
                win.append(ks[i])
                acc = win[-1] * sk[0]
                for j in range(1, KS):
                    acc = acc + win[-1 - j] * sk[j]
                win = win[1:]
                t_s[zw, pl.ds((2 * pr + i) * 8, 8), :] = acc * vs[i]

    def h_prep(c, zw):
        for t in range(S // 128):
            ht = pltpu.bitcast(h_v[c, 0:128, pl.ds(t * 128, 128)].T, U32)
            ht_s[zw, pl.ds(t * 64 // (C // 2) * PR + t * 64 % (C // 2), 64), :] = ht

    def fft1(sample, mid, zw):
        for b in range(R2):
            z = [_cmul((sample(R2 * a + b), None), cmath.exp(-0.5j * math.pi * a / R1)) for a in range(R1)]
            gq = _fft(z)
            for q1 in range(R1):
                re, im = _cmul(gq[q1], cmath.exp(-2j * math.pi * (q1 + 0.25) * b / C))
                row = (q1 * R2 + b) * 16
                mid[zw, pl.ds(row, 8), :] = re
                mid[zw, pl.ds(row + 8, 8), :] = im

    def fft2(mid, dst, zw, zr):
        for q1 in range(R1):
            z = []
            for b in range(R2):
                row = (q1 * R2 + b) * 16
                z.append((mid[zr, pl.ds(row, 8), :], mid[zr, pl.ds(row + 8, 8), :]))
            t = _fft(z)
            for q2 in range(R2):
                q = q1 + R1 * q2
                dst[zw, pl.ds(q, NCH, stride=SR), :] = t[q2][0]
                dst[zw, pl.ds(C + q, NCH, stride=SR), :] = t[q2][1]

    def mac(p, zw, zr):
        re = pl.ds(p * 8, 8)
        im = pl.ds(C + p * 8, 8)
        AB = 4
        prev = None
        for a0 in range(0, NCH, AB):
            zre = [None] * AB
            zim = [None] * AB
            for m in range(a0 + AB):
                hr = h_s[zr, pl.ds(m * SR + p * 8, 8), :]
                hi = h_s[zr, pl.ds(m * SR + C + p * 8, 8), :]
                for i in range(AB):
                    t = a0 + i - m
                    if t < 0:
                        continue
                    ur = u_s[zr, pl.ds(t * SR + p * 8, 8), :]
                    ui = u_s[zr, pl.ds(t * SR + C + p * 8, 8), :]
                    tr = hr * ur - hi * ui
                    ti = hr * ui + hi * ur
                    zre[i] = tr if zre[i] is None else zre[i] + tr
                    zim[i] = ti if zim[i] is None else zim[i] + ti
            for i in range(AB):
                if prev is None:
                    yf_s[zw, a0 + i, re, :] = zre[i]
                    yf_s[zw, a0 + i, im, :] = zim[i]
                else:
                    yf_s[zw, a0 + i, re, :] = zre[i] - prev[1]
                    yf_s[zw, a0 + i, im, :] = zim[i] + prev[0]
                prev = (zre[i], zim[i])

    def inv_dft(c, zr):
        qc = C // FOLD
        for a in range(NCH):
            yr = [yf_s[zr, a, j * qc:(j + 1) * qc, :] for j in range(FOLD)]
            yi = [yf_s[zr, a, C + j * qc:C + (j + 1) * qc, :] for j in range(FOLD)]
            sr, si, dr, di = yr[0] + yr[2], yi[0] + yi[2], yr[0] - yr[2], yi[0] - yi[2]
            tr, ti, er, ei = yr[1] + yr[3], yi[1] + yi[3], yr[1] - yr[3], yi[1] - yi[3]
            folded = [(sr + tr, si + ti), (dr - ei, di + er), (sr - tr, si - ti), (dr + ei, di - er)]
            for r in range(FOLD):
                f = jnp.concatenate(folded[r], axis=0).astype(BF16)
                y_v[c, pl.ds(a * C + r, qc, stride=FOLD), :] = _dot(inv_ref[r * qc:(r + 1) * qc, :], f)

    def fixup(e, c, mat):
        a = wbuf[e][mat, c, 0]
        b = wbuf[e][mat, c, 1]
        wbuf[e][mat, c, 0] = (a & U32(0xFFFF)) | (b << 16)
        wbuf[e][mat, c, 1] = (a >> 16) | (b & U32(0xFFFF0000))

    RB = 128

    def qkv_tile(e, c, n, hook=None, rs=range(PRO // RB)):
        mat, j = n // 2, n % 2
        for r in rs:
            w = _unpack(wbuf[e][mat, c, j])
            xr = _unpack(xp[pl.ds(r * RB // 2, RB // 2), :])
            pk = _pack(_dot(xr, w))
            qkv_b[mat, 2 * c + e, j, pl.ds((QOFF + r * RB) // 2, RB // 2), :] = pk
            if hook is not None and r == 0:
                hook(pk[0:8])

    def start_when(cond, copies):
        @pl.when(cond)
        def _():
            for cp in copies:
                cp.start()

    def wq0_tiles(c, rs=range(PRO // RB)):
        qkv_tile(0, c, 0, rs=rs)
        qkv_tile(0, c, 1, rs=rs)

    for cp in wq0_copies(0) + xp_copies + wq0_copies(1):
        cp.start()
    for cp in wq0_copies(0) + xp_copies[:1]:
        cp.wait()
    fixup(0, 0, 0)
    wq0_tiles(0, range(2))
    for cp in wq0_copies(2) + wq0_copies(3):
        cp.start()
    xp_copies[1].wait()
    wq0_tiles(0, range(2, 4))
    for cp in wq0_copies(4) + wq0_copies(5) + small_copies:
        cp.start()
    for cp in wq0_copies(1):
        cp.wait()
    fixup(0, 1, 0)
    wq0_tiles(1)
    for cp in wq0_copies(6) + wq0_copies(7) + block_piece(0, 2) + block_piece(0, 3):
        cp.start()

    def pro0(i, carry):
        for u in range(2):
            for cp in wq0_copies(2 * i + u):
                cp.wait()
        for u in range(2):
            fixup(0, 2 * i + u, 0)
            wq0_tiles(2 * i + u)
        for j in range(4, NPIECE):
            start_when(i == 1, block_piece(0, j))
        start_when(i == 2, block_piece(0, 0))
        start_when(i + 1 == 3, block_piece(0, 1))
        last = [i == 3, i >= 3] + [i > 2] * (NPIECE - 2)
        for j in range(NPIECE):
            start_when(last[j], block_piece(1, j))
        return carry

    with jax.named_scope("pro0"):
        jax.lax.fori_loop(1, NB // 2, pro0, 0)
    for cp in small_copies:
        cp.wait()

    def pro(c, carry):
        zw = c >> 3
        zr = c >> 4
        for i in range(NPIECE):
            for cp in block_piece(c, i):
                cp.wait()

        tiles = [(0, n) for n in range(2, 6)] + [(1, n) for n in range(6)]

        def tile(i, hook=None):
            e, n = tiles[i]
            if n % 2 == 0:
                fixup(e, c, n // 2)
            qkv_tile(e, c, n, hook=hook)

        def trigger(val):
            k_v[c + zw, pl.ds(PT - 8, 8), :] = val
            v_v[c + zw, pl.ds(PT - 8, 8), :] = val
            h_v[c + zw, pl.ds(128, 16), 0:128] = _unpack(val)

        def h_sample(n):
            w = word(ht_s, zr, n // 2)
            hv = hi16(w) if n % 2 else lo16(w)
            if n == 0:
                hv = hv + jnp.where(first, row_of(dd_ref, c), 0.0)
            return hv

        tile(0, trigger)
        h_prep(c, zw)
        kv_prep(c, zw)
        fft1(lambda n: t_s[zr, pl.ds(n * 8, 8), :], gu_s, zw)
        fft2(gu_s, u_s, zw, zr)
        fft1(h_sample, gh_s, zw)
        fft2(gh_s, h_s, zw, zr)
        for i in range(1, 9):
            for p in range(4 * i - 4, 4 * i):
                mac(p, zw, zr)
            tile(i)
        tile(9)
        inv_dft(c, zr)
        more = [c < NB - 2, c <= NB - 3] + [c + 2 < NB] * (NPIECE - 2)
        for i in range(NPIECE):
            start_when(more[i], block_piece(jnp.minimum(c + 2, NB - 1), i))
        start_when(c + 1 < NB, [wo_copy(c)])
        start_when(c + 2 == NB, [wo_copy(NB - 1), x_early])
        return carry

    with jax.named_scope("pro"):
        jax.lax.fori_loop(0, NB, pro, 0)
    x_late.start()
    x_early.wait()
    for c in range(NB):
        wo_copy(c).wait()

    gwt = gw_ref[...].astype(F32)
    gw = jnp.concatenate([gwt[j:j + 1, :] for j in range(NB)], axis=1)

    def finalize(rows, b):
        xr = x_v[rows, :].astype(F32)
        g = jax.nn.sigmoid(jnp.sum(xr * gw, axis=-1, keepdims=True))
        a = xr * jnp.concatenate([y_v[j, rows, :] for j in range(NB)], axis=1)
        out_v[rows, :] = (g * a + (1.0 - g) * b).astype(BF16)

    def step(s, mem, split_first, odd):
        mrows = slice(0, M) if odd else slice(RX, RX + M)
        sh = 4 if odd else 0
        xo = pl.multiple_of(PRO + RX * s, 8)
        wbase = pl.multiple_of((RX // 2 * s) % (QCAP // 2) - sh, 8)
        rpos = pl.multiple_of((SEG // 2 * s + QOFF // 2) % (QCAP // 2), SEG // 2)
        xs = x_v[pl.ds(xo, RX), :]
        lhs = jnp.concatenate([mem, xs] if odd else [xs, mem], axis=0)
        zpad = jnp.zeros((128 - 2 * (SEG + M), E), BF16)
        no = SEG + M if odd else RX
        frows = pl.ds(pl.multiple_of(SEG * s - (M if odd else 0), 8), no)
        orows = slice(M, M + no) if odd else slice(0, no)
        omrows = slice(0, M) if odd else slice(no, no + M)
        low = jax.lax.broadcasted_iota(jnp.int32, (8, E), 0) < 4
        NP = H // 2

        mem_qkv = {}
        probs = {}
        cats = {}

        def load(mat, hp):
            parts = [_unpack(qkv_b[mat, hp, 0, pl.ds(rpos, SEG // 2), :]),
                     _unpack(qkv_b[mat, hp, 1, pl.ds(rpos, SEG // 2), :]), mem_qkv[(hp, mat)]]
            if mat > 0:
                parts.append(zpad)
            cats[(mat, hp)] = jnp.concatenate(parts, axis=0)

        def stage_a(hp):
            KH = D // 2
            split = split_first and hp == 0
            if split:
                for mat in range(3):
                    for j in range(2):
                        w = _unpack(wbuf[hp % 2][mat, hp // 2, j, :KH // 2, :])
                        qacc[2 * mat + j] = _dot(lhs[:, :KH], w)
            for mat in range(3):
                mm = []
                for j in range(2):
                    if split:
                        w = _unpack(wbuf[hp % 2][mat, hp // 2, j, KH // 2:, :])
                        res = qacc[2 * mat + j] + _dot(lhs[:, KH:], w)
                    else:
                        res = _dot(lhs, _unpack(wbuf[hp % 2][mat, hp // 2, j]))
                    pk = _pack(res)
                    if odd:
                        qkv_b[mat, hp, j, pl.ds(wbase + 4, 4), :] = pk[4:8]
                        qkv_b[mat, hp, j, pl.ds(wbase + 8, 8), :] = pk[8:16]
                    else:
                        qkv_b[mat, hp, j, pl.ds(wbase, 8), :] = pk[0:8]
                        qkv_b[mat, hp, j, pl.ds(wbase + 8, 4), :] = pk[8:12]
                    mm.append(res[mrows])
                    if j == 1:
                        mem_qkv[(hp, mat)] = jnp.concatenate(mm, axis=0).astype(BF16)
                    advance(6 * hp + 2 * mat + j + 1)

        def stage_b(hp):
            sc = _dot_nt(cats[(0, hp)], cats[(1, hp)]) * scale
            fill = fill_ref[...]
            sc = jnp.where(fill == 0.0, sc, fill)
            mx = jnp.max(sc, axis=-1, keepdims=True)
            p = jnp.exp(sc - mx)
            l = jnp.sum(p, axis=-1, keepdims=True)
            r = pl.reciprocal(l, approx=True)
            r = r * (2.0 - l * r)
            probs[hp] = (p * r).astype(BF16)

        def stage_c(hp):
            o = _dot(probs[hp], cats[(2, hp)])
            for j in range(2):
                h = 2 * hp + j
                cols = slice(h * E, (h + 1) * E)
                ox = _pack(o[j * SEG:(j + 1) * SEG])
                om = o[2 * SEG + j * M:2 * SEG + (j + 1) * M]
                om = _pack(jnp.concatenate([om, om], axis=0))
                if odd:
                    lo_s[0:8, cols] = jnp.where(low, om, left[:, cols])
                    lo_s[8:24, cols] = ox
                else:
                    lo_s[0:8, cols] = ox[0:8]
                    lo_s[8:16, cols] = jnp.where(low, ox[8:16], om)
                    left[:, cols] = ox[8:16]

        def oproj(j, late):
            ks = slice(HS * E, H * E) if late else slice(0, HS * E)
            kw = slice(ks.start // 2, ks.stop // 2)
            return _dot(_unpack(lo_s[0:(no + M) // 2, ks]), _unpack(wo_v[j, kw, :]))

        events = []
        for hp in range(NP):
            events.append((6 * hp + OFF_LQK, 0, functools.partial(load, 0, hp)))
            events.append((6 * hp + OFF_LQK, 1, functools.partial(load, 1, hp)))
            events.append((6 * hp + OFF_LV, 2, functools.partial(load, 2, hp)))
            events.append((6 * hp + OFF_PV, 3, functools.partial(stage_c, hp)))
            events.append((6 * hp + OFF_S, 4, functools.partial(stage_b, hp)))
        events.sort(key=lambda ev: ev[:2])

        def advance(slot):
            while events and events[0][0] <= slot:
                events.pop(0)[2]()

        outs = [None] * NB
        for hp in range(NP):
            stage_a(hp)
        for j in range(NB):
            oacc[0:no + M, j * 128:(j + 1) * 128] = oproj(j, False)
            advance(6 * NP + (j + 1) * HS // 8)
        assert not events
        for j in range(NB):
            outs[j] = oacc[0:no + M, j * 128:(j + 1) * 128] + oproj(j, True)
        res = jnp.concatenate(outs, axis=1)
        finalize(frows, res[orows])
        return res[omrows].astype(BF16)

    def steps(i, carry):
        @pl.when(i == (XE - PRO) // (RX * UNROLL))
        def _():
            x_late.wait()

        OB = SEG * UNROLL
        start_when(i > 0, [out_copy(pl.multiple_of(jnp.maximum(i * OB - LASTR, 0), 8), LASTR)])
        mem = mem_v[...]
        for u in range(UNROLL):
            if u == UNROLL - 1:
                out_copy(pl.multiple_of(i * OB, OB), OB - LASTR).start()
            mem = step(i * UNROLL + u, mem, u > 0, u % 2 == 1)
        mem_v[...] = mem
        return carry

    with jax.named_scope("main"):
        jax.lax.fori_loop(0, NSEG // UNROLL, steps, 0)

    out_copy(S - LASTR, LASTR).start()
    out_copy(0, S).wait()


@jax.jit
def _run(A_q, A_k, A_v, A_shift_k, A_ssm_k, A_ssm_D, B_mem0, B_Wq, B_Wk, B_Wv, B_Wo, gate_w):
    any_spec = pl.BlockSpec(memory_space=pl.ANY)
    out = pl.pallas_call(
        _kernel,
        out_shape=jax.ShapeDtypeStruct((S, D), BF16),
        in_specs=[any_spec] * 14,
        out_specs=any_spec,
        scratch_shapes=[
            pltpu.VMEM((S, D), BF16),
            pltpu.VMEM((PRO // 2, D), U32),
            pltpu.VMEM((NB, PT, 128), U32),
            pltpu.VMEM((NB, PT, 128), U32),
            pltpu.VMEM((NB, 128 + 16, S), BF16),
            pltpu.VMEM((3, H // 4, 2, D // 2, E), U32),
            pltpu.VMEM((3, H // 4, 2, D // 2, E), U32),
            pltpu.VMEM((NB, H * E // 2, 128), U32),
            pltpu.VMEM((NB, S + 32, 128), F32),
            pltpu.VMEM((3, H // 2, 2, QCAP // 2, E), U32),
            pltpu.VMEM((8, H * E), U32),
            pltpu.VMEM((24, H * E), U32),
            pltpu.VMEM((M, D), BF16),
            pltpu.VMEM((48, D), F32),
            pltpu.VMEM((6, M + RX, E), F32),
            pltpu.VMEM((1, NCH * SR + 2 * C, 128), F32),
            pltpu.VMEM((1, NCH * SR + 2 * C, 128), F32),
            pltpu.VMEM((1, NCH, 2 * C, 128), F32),
            pltpu.VMEM((1, S, 128), F32),
            pltpu.VMEM((1, 2 * S, 128), F32),
            pltpu.VMEM((1, 2 * S, 128), F32),
            pltpu.VMEM((1, PT, 128), U32),
            pltpu.VMEM((S, D), BF16),
            pltpu.VMEM((C, 2 * C // FOLD), BF16),
            pltpu.VMEM((2 * (SEG + M), 128), F32),
            pltpu.VMEM((KS, D), BF16),
            pltpu.VMEM((NB, 128), BF16),
            pltpu.VMEM((NB, 128), BF16),
            pltpu.SemaphoreType.DMA((7,)),
            pltpu.SemaphoreType.DMA((NB,)),
        ],
        compiler_params=pltpu.CompilerParams(vmem_limit_bytes=100 * 2 ** 20, disable_bounds_checks=True),
    )(
        A_q.reshape(S, D), A_k.reshape(NCH, C, D), A_v.reshape(NCH, C, D), A_ssm_k,
        B_Wq.reshape(D // 2, 2, H, E), B_Wk.reshape(D // 2, 2, H, E), B_Wv.reshape(D // 2, 2, H, E),
        B_Wo.reshape(H * E, D),
        A_shift_k.T, A_ssm_D.reshape(NB, 128), gate_w.reshape(NB, 128), B_mem0.reshape(M, D),
        jnp.asarray(_inv_table(), BF16), jnp.asarray(_attn_fill()),
    )
    return out.reshape(1, S, D)


def pallas_gated_mix__ssm_conv_h3__memory_aug_recurrent_mem_tr__prompt_kernel(
    A_q, A_k, A_v, A_shift_k, A_ssm_k, A_ssm_D, B_x, B_mem0, B_Wq, B_Wk, B_Wv, B_Wo, B_seg_len, gate_w,
):
    del B_x
    if isinstance(B_seg_len, int):
        assert B_seg_len == SEG
    return _run(A_q, A_k, A_v, A_shift_k, A_ssm_k, A_ssm_D, B_mem0, B_Wq, B_Wk, B_Wv, B_Wo, gate_w)
```
